```python
import jax
import jax.numpy as jnp

def _softmax(x, axis=-1):
    return jax.nn.softmax(x, axis=axis)
def _gelu(x):
    return jax.nn.gelu(x, approximate=True)
def _silu(x):
    return jax.nn.silu(x)
def _sigmoid(x):
    return jax.nn.sigmoid(x)
def _layernorm(x, axis=-1, eps=1e-5):
    m = jnp.mean(x, axis=axis, keepdims=True)
    v = jnp.var(x, axis=axis, keepdims=True)
    return (x - m) / jnp.sqrt(v + eps)
def _scatter_add(tgt, idx, src, axis=0):
    return tgt.at[idx].add(src)
def _segment_sum(src, seg, n):
    return jax.ops.segment_sum(src, seg, n)
class _Rng:
    def __init__(self, key):
        self._k = key
    def _next(self):
        self._k, sub = jax.random.split(self._k)
        return sub
    def normal(self, shape):
        return jax.random.normal(self._next(), shape, dtype=jnp.bfloat16)
    def randint(self, lo, hi, shape):
        return jax.random.randint(self._next(), shape, lo, hi, dtype=jnp.int32)
    def uniform(self, shape, lo=0.0, hi=1.0):
        return jax.random.uniform(self._next(), shape, jnp.bfloat16, lo, hi)
    def permutation(self, n):
        return jax.random.permutation(self._next(), n)


kernel_name = 'interleave_layers__sliding_local_dilated__glu_gated_bilinear__prompt'

def setup_inputs():
    _rng = _Rng(jax.random.key(int.from_bytes(__import__("os").urandom(4), "little")))
    _w = (lambda a: (lambda t: t.astype(jnp.bfloat16) if jnp.issubdtype(t.dtype, jnp.floating) else t)(jnp.asarray(a)))
    def _A_setup():
        B, S, D = 1, 2048, 576
        return {
            "x": _w((lambda *s: _rng.normal(s) * 0.05)(B, S, D)),
            "wqkv": _w((lambda *s: _rng.normal(s) * 0.05)(D, 3 * D)),
            "wo": _w((lambda *s: _rng.normal(s) * 0.05)(D, D)),
        }
    _A_in = _A_setup()

    def _B_setup():
        B, S, D, F = 1, 2048, 576, 4608
        return {
            "x": _w((lambda *s: _rng.normal(s) * 0.05)(B, S, D)),
            "w_gate": _w((lambda *s: _rng.normal(s) * 0.05)(D, F) * (D ** -0.5)),
            "w_up": _w((lambda *s: _rng.normal(s) * 0.05)(D, F) * (D ** -0.5)),
            "w_down": _w((lambda *s: _rng.normal(s) * 0.05)(F, D) * (F ** -0.5)),
        }
    _B_in = _B_setup()

    return {
        "A_x": _A_in["x"],
        "A_wqkv": _A_in["wqkv"],
        "A_wo": _A_in["wo"],
        "B_x": _B_in["x"],
        "B_w_gate": _B_in["w_gate"],
        "B_w_up": _B_in["w_up"],
        "B_w_down": _B_in["w_down"],
    }

def reference(A_x, A_wqkv, A_wo, B_x, B_w_gate, B_w_up, B_w_down):
    def _A_ref(x, wqkv, wo):
        B, S, D = x.shape
        H = 32; Dh = D // H
        W, dil = 8, 2
        qkv = (lambda x, *d: x.transpose(*d))((x @ wqkv).reshape(B, S, 3, H, Dh), 2, 0, 3, 1, 4)
        q, k, v = qkv[0], qkv[1], qkv[2]
        scale = Dh ** -0.5
        pos = jnp.arange(S)
        off = jnp.arange(W) * dil
        idx = pos[:, None] - off[None, :]
        mask = idx >= 0
        idx_c = jnp.where(mask, idx, 0).reshape(-1)
        kg = k[:, :, idx_c, :].reshape(B, H, S, W, Dh)
        vg = v[:, :, idx_c, :].reshape(B, H, S, W, Dh)
        logits = jnp.einsum("bhsd,bhswd->bhsw", q, kg) * scale
        logits = jnp.where(mask[None, None, :, :], logits, -1e9)
        attn = _softmax(logits, axis=-1)
        o = jnp.einsum("bhsw,bhswd->bhsd", attn, vg)
        return (lambda x, *d: x.transpose(*d))(o, 0, 2, 1, 3).reshape(B, S, D) @ wo

    def _B_ref(x, w_gate, w_up, w_down):
        g = jnp.einsum("bsd,df->bsf", x, w_gate)
        u = jnp.einsum("bsd,df->bsf", x, w_up)
        h = g * u
        return jnp.einsum("bsf,fd->bsd", h, w_down)

    x = A_x
    x = x + _A_ref(_layernorm(x, axis=-1), A_wqkv, A_wo)
    x = x + _B_ref(_layernorm(x, axis=-1), B_w_gate, B_w_up, B_w_down)
    x = x + _A_ref(_layernorm(x, axis=-1), A_wqkv, A_wo)
    x = x + _B_ref(_layernorm(x, axis=-1), B_w_gate, B_w_up, B_w_down)
    return x
```

```python
import math

import jax
import jax.numpy as jnp
from jax import lax
import jax.experimental.pallas as pl
import jax.experimental.pallas.tpu as pltpu

f32 = jnp.float32
bf16 = jnp.bfloat16
u32 = jnp.uint32

S, D, F = 2048, 576, 4608
H, DH, WIN, DIL = 32, 18, 8, 2
EPS = 1e-5
LOG2E = math.log2(math.e)
NSLAB = S // 128
TILE = 512
NTILE = S // TILE
FC = 512
NCHUNK = F // FC
MB = D // 4
HALO = 16
WC_ROWS = 800 * 16
WD_ROWS = 448 * 16
NT = (((1,), (1,)), ((), ()))
AUG = (0, 1, 2, 5)

DN_PLAN = dict(u1=(0, 0, 0, 0, 4, 4, 6), g2=(4, 0, 0, 0, 0, 0, 0), u2=(0, 0, 0, 0, 4, 4, 4))


def _up(v):
    return pltpu.bitcast(v, bf16)


def _quad(x):
    n = len(x) // 2
    return ([r[:n] for r in x[:n]], [r[n:] for r in x[:n]],
            [r[:n] for r in x[n:]], [r[n:] for r in x[n:]])


def _badd(x, y):
    return [[a + b for a, b in zip(r, s)] for r, s in zip(x, y)]


def _bsub(x, y):
    return [[a - b for a, b in zip(r, s)] for r, s in zip(x, y)]


def _lhs_terms(a):
    a11, a12, a21, a22 = _quad(a)
    return [lambda: _badd(a11, a22), lambda: _badd(a21, a22), lambda: a11, lambda: a22,
            lambda: _badd(a11, a12), lambda: _bsub(a21, a11), lambda: _bsub(a12, a22)]


def _rhs_terms(b):
    b11, b12, b21, b22 = _quad(b)
    return [lambda: _badd(b11, b22), lambda: b11, lambda: _bsub(b12, b22), lambda: _bsub(b21, b11),
            lambda: b22, lambda: _badd(b11, b12), lambda: _badd(b21, b22)]


def _combos(x, terms, emit):
    for o, fo in enumerate(terms(x)):
        y = fo()
        for i, fi in enumerate(terms(y)):
            emit(o * 7 + i, fi()[0][0])


def _lhs_ext(e):
    n = len(e) // 2
    return {0: e[:n], 1: e[n:], 2: e[:n], 5: [y - x for x, y in zip(e[:n], e[n:])]}


def _rhs_ext(e):
    n = len(e) // 2
    return {0: e[:n], 1: e[:n], 2: e[n:], 5: [x + y for x, y in zip(e[:n], e[n:])]}


def _ext_combos(e, fn, emit):
    for oi, o in enumerate(AUG):
        d = fn(fn(e)[o])
        for ii, i in enumerate(AUG):
            emit(oi * 4 + ii, d[i][0])


def _adv(gen, n):
    for _ in range(n):
        try:
            next(gen)
        except StopIteration:
            return


def _ld(ref, idx):
    n = ref.shape[-2] // 2
    return jnp.concatenate([ref[idx, :n, :], ref[idx, n:, :]], axis=0)


class _Temps:
    def __init__(self, ref):
        self.ref = ref
        self.n = 0

    def put(self, v):
        i = self.n % self.ref.shape[0]
        self.n += 1
        self.ref[i] = v
        return i

    def get(self, i):
        return _ld(self.ref, i)


def _recombine(prod, fin, ti, to):
    def inner(o, sink):
        a = ti.put(prod(o, 0))
        b = ti.put(prod(o, 1))
        c = ti.put(prod(o, 2))
        sink(1, 1, ti.get(a) - ti.get(b) + ti.get(c) + prod(o, 5))
        m3 = prod(o, 3)
        m4 = prod(o, 4)
        m6 = prod(o, 6)
        sink(1, 0, ti.get(b) + m3)
        sink(0, 1, ti.get(c) + m4)
        sink(0, 0, ti.get(a) + m3 - m4 + m6)

    m = {}
    for o in (0, 1, 2):
        def keep(y, z, v, o=o):
            m[o, y, z] = to.put(v)
        inner(o, keep)
        yield

    def s5(y, z, v):
        fin(2 + y, 2 + z, to.get(m[0, y, z]) - to.get(m[1, y, z]) + to.get(m[2, y, z]) + v)
    inner(5, s5)
    yield

    def s3(y, z, v):
        fin(2 + y, z, to.get(m[1, y, z]) + v)
        m[3, y, z] = to.put(to.get(m[0, y, z]) + v)
    inner(3, s3)
    yield

    def s4(y, z, v):
        fin(y, 2 + z, to.get(m[2, y, z]) + v)
        m[3, y, z] = to.put(to.get(m[3, y, z]) - v)
    inner(4, s4)
    yield

    def s6(y, z, v):
        fin(y, z, to.get(m[3, y, z]) + v)
    inner(6, s6)
    yield


def _layernorm_t(x):
    mu = jnp.sum(x, axis=0, keepdims=True) * (1.0 / D)
    xc = x - mu
    var = jnp.sum(xc * xc, axis=0, keepdims=True) * (1.0 / D)
    return xc * lax.rsqrt(var + EPS)


def _kernel(xt_hbm, wqkv_hbm, wo_hbm, wg_hbm, wu_hbm, wdt_hbm, out_hbm,
            xin, xs, ost, wq_raw, wo_raw, wtmp, wqb, wob, raw, wcb, web, wdcb,
            xnb, qkv, ob, xn2, acb, aeb, gs, hs, hcb, acc, tin, tout, tin2, tout2,
            sem_x, sem_w, sem_c, sem_o):
    wq, wo, wc, we, wdc, xn, o32, ac, ae, hc = [
        r.bitcast(u32) for r in (wqb, wob, wcb, web, wdcb, xnb, ob, acb, aeb, hcb)]

    def x_copy(t):
        return pltpu.make_async_copy(
            xt_hbm.at[:, pl.ds(t * TILE, TILE)], xin.at[:, pl.ds(t * TILE, TILE)], sem_x.at[t])

    def chunk_copies(j):
        cols = pl.ds(pl.multiple_of(j * FC, FC), FC)
        return [pltpu.make_async_copy(src.at[:, cols], raw.at[j, m], sem_c.at[j, m])
                for m, src in enumerate((wg_hbm, wu_hbm, wdt_hbm))]

    def out_copy(p):
        return pltpu.make_async_copy(
            ost.at[p], out_hbm.at[:, pl.ds(pl.multiple_of(p * 128, 128), 128)], sem_o.at[p])

    wq_copy = pltpu.make_async_copy(wqkv_hbm, wq_raw, sem_w.at[0])
    wo_copy = pltpu.make_async_copy(wo_hbm, wo_raw, sem_w.at[1])
    wq_copy.start()
    x_copy(0).start()
    wo_copy.start()
    wq_copy.wait()
    for cp in chunk_copies(0):
        cp.start()

    def wq_transpose(n, carry):
        c0 = pl.multiple_of(n * 128, 128)
        t = wq_raw[:, pl.ds(c0, 128)].astype(f32).T
        for k in range(4):
            wtmp[k, pl.ds(c0, 128), :] = t[:, k * 128:(k + 1) * 128]
        wtmp[4, pl.ds(c0, 128), 0:64] = t[:, 512:576]
        return carry
    lax.fori_loop(0, 13, wq_transpose, 0, unroll=True)
    t = wq_raw[:, 1664:1728].astype(f32).T
    for k in range(4):
        wtmp[k, 1664:1728, :] = t[:, k * 128:(k + 1) * 128]
    wtmp[4, 1664:1728, 0:64] = t[:, 512:576]
    for k in range(5):
        lanes = slice(0, 128) if k < 4 else slice(0, 64)
        for part in range(3):
            for d in range(DH):
                if d < 16:
                    row = part * 512 + d * 32
                else:
                    row = (1536, 1664, 1600)[part] + (d - 16) * 32
                wqb[k, row:row + 32, lanes] = wtmp[
                    k, pl.ds(part * D + d, H, stride=DH), lanes].astype(bf16)
        wqb[k, 1728:1792, lanes] = jnp.zeros((64, lanes.stop), bf16)

    for j in range(1, 3):
        for cp in chunk_copies(j):
            cp.start()
    x_copy(1).start()

    wo_copy.wait()
    for n in range(5):
        w = 128 if n < 4 else 64
        wtmp[n, 0:D, 0:w] = wo_raw[:, n * 128:n * 128 + w].astype(f32)
    for n in range(5):
        w = 128 if n < 4 else 64
        for c in range(5):
            if c < 4:
                rows = [wtmp[n, pl.ds(4 * c + g, H, stride=DH), 0:w] for g in range(4)]
            else:
                rows = [jnp.zeros((64, w), f32)] + [
                    wtmp[n, pl.ds(16 + g, H, stride=DH), 0:w] for g in range(2)]
            wob[c, n * 128:n * 128 + w, :] = jnp.concatenate(rows, axis=0).T.astype(bf16)

    for j in range(3, NCHUNK):
        for cp in chunk_copies(j):
            cp.start()
        if j in (4, 6):
            x_copy(j // 2).start()

    def prep_chunk(j):
        for m in range(2):
            for s in range(8):
                b = [[raw[j, m, k * 128 + s * 16:k * 128 + s * 16 + 16,
                          c * 128:(c + 1) * 128].astype(f32) for c in range(4)] for k in range(4)]

                def emit(i, v, m=m, s=s):
                    r = (m * 49 + i) * 128 + s * 16
                    wcb[j, r:r + 16, :] = v.astype(bf16)
                _combos(b, _rhs_terms, emit)
            e = [raw[j, m, 512:576, c * 128:(c + 1) * 128].astype(f32) for c in range(4)]

            def emit_e(i, v, m=m):
                web[j, m * 16 + i] = v.astype(bf16)
            _ext_combos(e, _rhs_ext, emit_e)
        for s in range(9):
            a = [[raw[j, 2, r * MB + s * 16:r * MB + s * 16 + 16,
                      k * 128:(k + 1) * 128].astype(f32) for k in range(4)] for r in range(4)]

            def emit_d(i, v, s=s):
                r = i * MB + s * 16
                wdcb[j, r:r + 16, :] = v.astype(bf16)
            _combos(a, _lhs_terms, emit_d)

    def layer(li, carry):
        first = li == 0

        def load_x(p):
            x0 = xin[:, pl.ds(pl.multiple_of(p * 128, 128), 128)].astype(f32)
            return jnp.where(first, x0, xs[p, 0:D, :])

        def ln1(p, b):
            y = _layernorm_t(load_x(p)).T.astype(bf16)
            for k in range(4):
                xnb[b, k] = y[:, k * 128:(k + 1) * 128]
            xnb[b, 4, :, 0:64] = y[:, 512:576]

        def qkv_proj(b):
            lhs = jnp.concatenate(
                [_up(xn[b, k]) for k in range(4)] + [_up(xn[b, 4, :, 0:64])], axis=1)
            for n in (4, 5, 6, 7, 13, 0, 1, 2, 3, 12, 8, 9, 10, 11):
                rows = slice(n * 64, (n + 1) * 64)
                rhs = jnp.concatenate(
                    [_up(wq[k, rows, :]) for k in range(4)] + [_up(wq[4, rows, 0:64])], axis=1)
                r = lax.dot_general(lhs, rhs, NT, preferred_element_type=f32)
                if n in (4, 5, 6, 7, 13):
                    r = r * (DH ** -0.5 * LOG2E)
                qkv[b, n, HALO:HALO + 128, :] = r

        def halo(b):
            for n in range(4, 14):
                qkv[b, n, 0:HALO, :] = qkv[1 - b, n, 128:128 + HALO, :]

        def attend(b, row0):
            qs, ks, vs = (0, 1, 2, 3, 12), (4, 5, 6, 7, 13), (8, 9, 10, 11, 12)
            for s in range(8):
                r = HALO + s * 16
                q = [qkv[b, n, r:r + 16, :] for n in qs]
                logit = []
                for w in range(WIN):
                    rw = r - DIL * w
                    part = q[0] * qkv[b, ks[0], rw:rw + 16, :]
                    for c in range(1, 5):
                        part = part + q[c] * qkv[b, ks[c], rw:rw + 16, :]
                    part = part + pltpu.roll(part, 64, 1)
                    part = part + pltpu.roll(part, 32, 1)
                    if row0 is not None and s == 0 and w > 0:
                        pos = row0 + lax.broadcasted_iota(jnp.int32, (16, 128), 0)
                        part = jnp.where(pos >= DIL * w, part, -1e9 * LOG2E)
                    logit.append(part)
                mx = logit[0]
                for w in range(1, WIN):
                    mx = jnp.maximum(mx, logit[w])
                e = [jnp.exp2(l - mx) for l in logit]
                den = e[0]
                for w in range(1, WIN):
                    den = den + e[w]
                inv = 1.0 / den
                for c in range(5):
                    o = e[0] * qkv[b, vs[c], r:r + 16, :]
                    for w in range(1, WIN):
                        rw = r - DIL * w
                        o = o + e[w] * qkv[b, vs[c], rw:rw + 16, :]
                    ob[b, c, s * 16:(s + 1) * 16, :] = (o * inv).astype(bf16)

        def out_proj(p, b):
            lhs = jnp.concatenate([_up(wo[c]) for c in range(5)], axis=1)
            rhs = jnp.concatenate([_up(o32[b, c]) for c in range(5)], axis=1)
            xs[p, 0:D, :] = load_x(p) + lax.dot_general(lhs, rhs, NT, preferred_element_type=f32)

        def ffn_lhs(t):
            for r in range(4):
                y = _layernorm_t(xs[t * 4 + r, 0:D, :]).T
                for k in range(4):
                    xn2[r * 5 + k] = y[:, k * 128:(k + 1) * 128]
                xn2[r * 5 + 4, :, 0:64] = y[:, 512:576]
            for s in range(8):
                rows = slice(s * 16, (s + 1) * 16)
                a = [[xn2[r * 5 + k, rows, :] for k in range(4)] for r in range(4)]

                def emit(i, v, rows=rows):
                    acb[i, rows, :] = v.astype(bf16)
                _combos(a, _lhs_terms, emit)
                e = [xn2[r * 5 + 4, rows, 0:64] for r in range(4)]

                def emit_e(i, v, rows=rows):
                    aeb[i, rows, 0:64] = v.astype(bf16)
                _ext_combos(e, _lhs_ext, emit_e)

        @pl.when(first)
        def _():
            x_copy(0).wait()
            for cp in chunk_copies(0):
                cp.wait()

        for n in range(4, 14):
            qkv[0, n, 0:HALO, :] = jnp.zeros((HALO, 128), f32)
        ln1(0, 0)
        qkv_proj(0)
        ln1(1, 1)
        prep_chunk(0)

        def attn_step(i, c):
            @pl.when(first)
            def _():
                for cp in chunk_copies(i + 1):
                    cp.wait()

            @pl.when(jnp.logical_and(first, jnp.logical_and(i % 2 == 1, i < 7)))
            def _():
                x_copy((i + 1) // 2).wait()

            halo(1)
            qkv_proj(1)
            ln1(jnp.minimum(2 * i + 2, NSLAB - 1), 0)
            attend(0, i * 256)
            out_proj(2 * i, 0)
            halo(0)
            qkv_proj(0)
            ln1(jnp.minimum(2 * i + 3, NSLAB - 1), 1)
            attend(1, None)
            out_proj(2 * i + 1, 1)
            prep_chunk(i + 1)
            return c
        lax.fori_loop(0, NSLAB // 2, attn_step, 0)

        ffn_lhs(0)

        def ffn_group(t, g, last):
            ti = _Temps(tin)
            to = _Temps(tout)

            def proj(c, m):
                j = g * 3 + c

                def prod(o, i):
                    r = (m * 49 + o * 7 + i) * 64
                    p = jnp.dot(_up(ac[o * 7 + i]), _up(wc[j, r:r + 64, :]),
                                preferred_element_type=f32)
                    if o in AUG and i in AUG:
                        q = AUG.index(o) * 4 + AUG.index(i)
                        p = p + jnp.dot(_up(ae[q, :, 0:64]), _up(we[j, m * 16 + q]),
                                        preferred_element_type=f32)
                    return p
                return prod

            def gate(c):
                def fin(r, cc, v):
                    gs[(c % 2) * 16 + r * 4 + cc] = v
                return _recombine(proj(c, 0), fin, ti, to)

            def upgate(c):
                def fin(r, cc, v):
                    hs[c, r * 4 + cc] = _ld(gs, (c % 2) * 16 + r * 4 + cc) * v
                yield from _recombine(proj(c, 1), fin, ti, to)
                for s in range(8):
                    rows = slice(s * 16, (s + 1) * 16)
                    b = [[hs[c, r * 4 + cc, rows, :] for r in range(4)] for cc in range(4)]

                    def emit(i, v, rows=rows):
                        hcb[c, i, rows, :] = v.astype(bf16)
                    _combos(b, _rhs_terms, emit)

            def dprod(cs, i):
                p = None
                for c in cs:
                    r = i * (MB // 2)
                    q = lax.dot_general(_up(wdc[g * 3 + c, r:r + MB // 2, :]), _up(hc[c, i]), NT,
                                        preferred_element_type=f32)
                    p = q if p is None else p + q
                return p

            def down(cs, reset):
                for i in range(49):
                    a = _ld(acc, i)
                    if reset:
                        a = jnp.where(g == 0, 0.0, a)
                    acc[i] = a + dprod(cs, i)
                    yield

            def down_final(cs):
                def fin(mb, r, v):
                    rows = slice(mb * MB, (mb + 1) * MB)
                    y = xs[t * 4 + r, rows, :] + v
                    xs[t * 4 + r, rows, :] = y
                    ost[t * 4 + r, rows, :] = y.astype(bf16)
                return _recombine(lambda o, i: _ld(acc, o * 7 + i) + dprod(cs, o * 7 + i),
                                  fin, _Temps(tin2), _Temps(tout2))

            for gen in (gate(0), upgate(0), gate(1)):
                _adv(gen, 100)
            d0 = down((0,), not last)
            for gen, plan in ((upgate(1), DN_PLAN["u1"]), (gate(2), DN_PLAN["g2"]),
                              (upgate(2), DN_PLAN["u2"])):
                for n in plan:
                    _adv(gen, 1)
                    _adv(d0, n)
                _adv(gen, 100)
            if last:
                ffn_lhs((t + 1) % NTILE)
            _adv(d0, 100)
            _adv(down_final((1, 2)) if last else down((1, 2), False), 100)

        def ffn_tile(t, c):
            def grp(g, c2):
                ffn_group(t, g, False)
                return c2
            lax.fori_loop(0, 2, grp, 0)
            ffn_group(t, 2, True)

            @pl.when(li == 1)
            def _():
                for r in range(4):
                    out_copy(t * 4 + r).start()
            return c
        lax.fori_loop(0, NTILE, ffn_tile, 0)
        return carry

    lax.fori_loop(0, 2, layer, 0)
    for p in range(NSLAB):
        out_copy(p).wait()


@jax.jit
def pallas_interleave_layers__sliding_local_dilated__glu_gated_bilinear__prompt_kernel(
    A_x: jax.Array,
    A_wqkv: jax.Array,
    A_wo: jax.Array,
    B_x: jax.Array,
    B_w_gate: jax.Array,
    B_w_up: jax.Array,
    B_w_down: jax.Array,
):
    del B_x
    vm = pltpu.VMEM
    hbm = pl.BlockSpec(memory_space=pl.ANY)
    out_t = pl.pallas_call(
        _kernel,
        in_specs=[hbm] * 6,
        out_specs=hbm,
        out_shape=jax.ShapeDtypeStruct((D, S), bf16),
        scratch_shapes=[
            vm((D, S), bf16),
            vm((NSLAB, 640, 128), f32),
            vm((NSLAB, D, 128), bf16),
            vm((D, 3 * D), bf16),
            vm((D, D), bf16),
            vm((5, 3 * D, 128), f32),
            vm((5, 1792, 128), bf16),
            vm((5, D, 128), bf16),
            vm((NCHUNK, 3, D, FC), bf16),
            vm((NCHUNK, WC_ROWS, 128), bf16),
            vm((NCHUNK, 32, 64, 128), bf16),
            vm((NCHUNK, WD_ROWS, 128), bf16),
            vm((2, 5, 128, 128), bf16),
            vm((2, 14, HALO + 128, 128), f32),
            vm((2, 5, 128, 128), bf16),
            vm((20, 128, 128), f32),
            vm((49, 128, 128), bf16),
            vm((16, 128, 128), bf16),
            vm((32, 128, 128), f32),
            vm((3, 16, 128, 128), f32),
            vm((3, 49, 128, 128), bf16),
            vm((49, MB, 128), f32),
            vm((12, 128, 128), f32),
            vm((40, 128, 128), f32),
            vm((12, MB, 128), f32),
            vm((20, MB, 128), f32),
            pltpu.SemaphoreType.DMA((NTILE,)),
            pltpu.SemaphoreType.DMA((2,)),
            pltpu.SemaphoreType.DMA((NCHUNK, 3)),
            pltpu.SemaphoreType.DMA((NSLAB,)),
        ],
        compiler_params=pltpu.CompilerParams(vmem_limit_bytes=120 * 1024 * 1024),
    )(A_x[0].T, A_wqkv, A_wo, B_w_gate, B_w_up, B_w_down.T)
    return out_t.T[None]
```

```python
import math

import jax
import jax.numpy as jnp
from jax import lax
import jax.experimental.pallas as pl
import jax.experimental.pallas.tpu as pltpu

f32 = jnp.float32
bf16 = jnp.bfloat16
u32 = jnp.uint32

S, D, F = 2048, 576, 4608
H, DH, WIN, DIL = 32, 18, 8, 2
EPS = 1e-5
LOG2E = math.log2(math.e)
NSLAB = S // 128
TILE = 512
NTILE = S // TILE
FC = 512
NCHUNK = F // FC
MB = D // 4
HALO = 16
WC_ROWS = 800 * 16
WD_ROWS = 448 * 16
NT = (((1,), (1,)), ((), ()))
AUG = (0, 1, 2, 5)

OPT = dict(att=1, skip_ffn=False, skip_attn=False, prep=1, a0=0, aper=6, alat=35, ldue=32, hdue=40)
DN_PLAN = dict(u1=(0, 0, 0, 0, 4, 4, 6), g2=(4, 0, 0, 0, 0, 0, 0), u2=(0, 0, 0, 0, 4, 4, 4))


def _up(v):
    return pltpu.bitcast(v, bf16)


def _quad(x):
    n = len(x) // 2
    return ([r[:n] for r in x[:n]], [r[n:] for r in x[:n]],
            [r[:n] for r in x[n:]], [r[n:] for r in x[n:]])


def _badd(x, y):
    return [[a + b for a, b in zip(r, s)] for r, s in zip(x, y)]


def _bsub(x, y):
    return [[a - b for a, b in zip(r, s)] for r, s in zip(x, y)]


def _lhs_terms(a):
    a11, a12, a21, a22 = _quad(a)
    return [lambda: _badd(a11, a22), lambda: _badd(a21, a22), lambda: a11, lambda: a22,
            lambda: _badd(a11, a12), lambda: _bsub(a21, a11), lambda: _bsub(a12, a22)]


def _rhs_terms(b):
    b11, b12, b21, b22 = _quad(b)
    return [lambda: _badd(b11, b22), lambda: b11, lambda: _bsub(b12, b22), lambda: _bsub(b21, b11),
            lambda: b22, lambda: _badd(b11, b12), lambda: _badd(b21, b22)]


def _combos(x, terms, emit):
    for o, fo in enumerate(terms(x)):
        y = fo()
        for i, fi in enumerate(terms(y)):
            emit(o * 7 + i, fi()[0][0])


_LHS_SPEC = (((0, 0), (1, 1), 1), ((1, 0), (1, 1), 1), ((0, 0), None, 0), ((1, 1), None, 0),
             ((0, 0), (0, 1), 1), ((1, 0), (0, 0), -1), ((0, 1), (1, 1), -1))
_RHS_SPEC = (((0, 0), (1, 1), 1), ((0, 0), None, 0), ((0, 1), (1, 1), -1), ((1, 0), (0, 0), -1),
             ((1, 1), None, 0), ((0, 0), (0, 1), 1), ((1, 0), (1, 1), 1))


def _outer_term(load, spec, o):
    p, q, sign = spec[o]
    out = []
    for y in range(2):
        row = []
        for z in range(2):
            v = load(2 * p[0] + y, 2 * p[1] + z)
            if sign:
                w = load(2 * q[0] + y, 2 * q[1] + z)
                v = v + w if sign > 0 else v - w
            row.append(v)
        out.append(row)
    return out


def _inner_terms(y, terms, o, emit):
    for i, fi in enumerate(terms(y)):
        emit(o * 7 + i, fi()[0][0])


def _lhs_ext(e):
    n = len(e) // 2
    return {0: e[:n], 1: e[n:], 2: e[:n], 5: [y - x for x, y in zip(e[:n], e[n:])]}


def _rhs_ext(e):
    n = len(e) // 2
    return {0: e[:n], 1: e[:n], 2: e[n:], 5: [x + y for x, y in zip(e[:n], e[n:])]}


def _ext_combos(e, fn, emit):
    for oi, o in enumerate(AUG):
        d = fn(fn(e)[o])
        for ii, i in enumerate(AUG):
            emit(oi * 4 + ii, d[i][0])


def _adv(gen, n):
    for _ in range(n):
        try:
            next(gen)
        except StopIteration:
            return


def _ld(ref, idx):
    n = ref.shape[-2] // 2
    return jnp.concatenate([ref[idx, :n, :], ref[idx, n:, :]], axis=0)


class _Temps:
    def __init__(self, ref):
        self.ref = ref
        self.n = 0

    def put(self, v):
        i = self.n % self.ref.shape[0]
        self.n += 1
        self.ref[i] = v
        return i

    def get(self, i):
        return _ld(self.ref, i)


def _recombine(prod, fin, ti, to):
    def inner(o, sink):
        a = ti.put(prod(o, 0))
        b = ti.put(prod(o, 1))
        c = ti.put(prod(o, 2))
        sink(1, 1, ti.get(a) - ti.get(b) + ti.get(c) + prod(o, 5))
        m3 = prod(o, 3)
        m4 = prod(o, 4)
        m6 = prod(o, 6)
        sink(1, 0, ti.get(b) + m3)
        sink(0, 1, ti.get(c) + m4)
        sink(0, 0, ti.get(a) + m3 - m4 + m6)

    m = {}
    for o in (0, 1, 2):
        def keep(y, z, v, o=o):
            m[o, y, z] = to.put(v)
        inner(o, keep)
        yield

    def s5(y, z, v):
        fin(2 + y, 2 + z, to.get(m[0, y, z]) - to.get(m[1, y, z]) + to.get(m[2, y, z]) + v)
    inner(5, s5)
    yield

    def s3(y, z, v):
        fin(2 + y, z, to.get(m[1, y, z]) + v)
        m[3, y, z] = to.put(to.get(m[0, y, z]) + v)
    inner(3, s3)
    yield

    def s4(y, z, v):
        fin(y, 2 + z, to.get(m[2, y, z]) + v)
        m[3, y, z] = to.put(to.get(m[3, y, z]) - v)
    inner(4, s4)
    yield

    def s6(y, z, v):
        fin(y, z, to.get(m[3, y, z]) + v)
    inner(6, s6)
    yield


def _kernel(xt_hbm, wqkv_hbm, wo_hbm, wg_hbm, wu_hbm, wdt_hbm, out_hbm,
            xin, xa, xb, ost, wq_raw, wo_raw, wtmp, wqb, wob, raw, wcb, web, wdcb,
            xnb, qkv, ob, xn2, acb, aeb, gs, hs, hcb, acc, tin, tout, tin2, tout2, zero,
            sem_x, sem_w, sem_c, sem_o):
    wq, wo, wc, we, wdc, xn, o32, ac, ae, hc = [
        r.bitcast(u32) for r in (wqb, wob, wcb, web, wdcb, xnb, ob, acb, aeb, hcb)]

    def x_copy(t):
        return pltpu.make_async_copy(
            xt_hbm.at[:, pl.ds(t * TILE, TILE)], xin.at[:, pl.ds(t * TILE, TILE)], sem_x.at[t])

    def chunk_copies(j):
        cols = pl.ds(pl.multiple_of(j * FC, FC), FC)
        return [pltpu.make_async_copy(src.at[:, cols], raw.at[j, m], sem_c.at[j, m])
                for m, src in enumerate((wg_hbm, wu_hbm, wdt_hbm))]

    def out_copy(p):
        return pltpu.make_async_copy(
            ost.at[p], out_hbm.at[:, pl.ds(pl.multiple_of(p * 128, 128), 128)], sem_o.at[p])

    wq_copy = pltpu.make_async_copy(wqkv_hbm, wq_raw, sem_w.at[0])
    wo_copy = pltpu.make_async_copy(wo_hbm, wo_raw, sem_w.at[1])
    zero[0] = 0
    wq_copy.start()
    x_copy(0).start()
    wo_copy.start()
    wq_copy.wait()
    for cp in chunk_copies(0):
        cp.start()

    def wq_transpose(n, carry):
        c0 = pl.multiple_of(n * 128, 128)
        t = wq_raw[:, pl.ds(c0, 128)].astype(f32).T
        for k in range(4):
            wtmp[k, pl.ds(c0, 128), :] = t[:, k * 128:(k + 1) * 128]
        wtmp[4, pl.ds(c0, 128), 0:64] = t[:, 512:576]
        return carry
    lax.fori_loop(0, 13, wq_transpose, 0, unroll=True)
    t = wq_raw[:, 1664:1728].astype(f32).T
    for k in range(4):
        wtmp[k, 1664:1728, :] = t[:, k * 128:(k + 1) * 128]
    wtmp[4, 1664:1728, 0:64] = t[:, 512:576]
    for k in range(5):
        lanes = slice(0, 128) if k < 4 else slice(0, 64)
        for part in range(3):
            for d in range(DH):
                if d < 16:
                    row = part * 512 + d * 32
                else:
                    row = (1536, 1664, 1600)[part] + (d - 16) * 32
                wqb[k, row:row + 32, lanes] = wtmp[
                    k, pl.ds(part * D + d, H, stride=DH), lanes].astype(bf16)
        wqb[k, 1728:1792, lanes] = jnp.zeros((64, lanes.stop), bf16)
    wqb[4, :, 64:128] = jnp.zeros((1792, 64), bf16)
    xnb[:, 4, :, 64:128] = jnp.zeros((2, 128, 64), bf16)
    ob[1] = jnp.zeros((5, 128, 128), bf16)

    for j in range(1, 3):
        for cp in chunk_copies(j):
            cp.start()
    x_copy(1).start()

    wo_copy.wait()
    for n in range(5):
        w = 128 if n < 4 else 64
        wtmp[n, 0:D, 0:w] = wo_raw[:, n * 128:n * 128 + w].astype(f32)
    for n in range(5):
        w = 128 if n < 4 else 64
        for c in range(5):
            if c < 4:
                rows = [wtmp[n, pl.ds(4 * c + g, H, stride=DH), 0:w] for g in range(4)]
            else:
                rows = [jnp.zeros((64, w), f32)] + [
                    wtmp[n, pl.ds(16 + g, H, stride=DH), 0:w] for g in range(2)]
            wob[c, n * 128:n * 128 + w, :] = jnp.concatenate(rows, axis=0).T.astype(bf16)

    for j in range(3, NCHUNK):
        for cp in chunk_copies(j):
            cp.start()
        if j in (4, 6):
            x_copy(j // 2).start()

    def after(v, row=0):
        return lax.bitcast_convert_type(v[row:row + 1, 0:1], jnp.int32)[0, 0] & zero[0]

    def prep_chunk(j0):
        def idx(z):
            return jnp.clip(j0 + z, 0, NCHUNK - 1)
        for m in range(2):
            for s in range(8):
                def emit(i, v, m=m, s=s):
                    r = (m * 49 + i) * 128 + s * 16
                    wcb[j0, r:r + 16, :] = v.astype(bf16)
                for o in range(7):
                    j = idx((yield))
                    y = _outer_term(lambda k, c: raw[
                        j, m, k * 128 + s * 16:k * 128 + s * 16 + 16,
                        c * 128:(c + 1) * 128].astype(f32), _RHS_SPEC, o)
                    _inner_terms(y, _rhs_terms, o, emit)
            for s in range(4):
                j = idx((yield))
                rows = slice(512 + s * 16, 528 + s * 16)
                e = [raw[j, m, rows, c * 128:(c + 1) * 128].astype(f32) for c in range(4)]

                def emit_e(i, v, m=m, s=s):
                    web[j0, m * 16 + i, s * 16:(s + 1) * 16, :] = v.astype(bf16)
                _ext_combos(e, _rhs_ext, emit_e)
        for s in range(9):
            def emit_d(i, v, s=s):
                r = i * MB + s * 16
                wdcb[j0, r:r + 16, :] = v.astype(bf16)
            for o in range(7):
                j = idx((yield))
                y = _outer_term(lambda r, k: raw[
                    j, 2, r * MB + s * 16:r * MB + s * 16 + 16,
                    k * 128:(k + 1) * 128].astype(f32), _LHS_SPEC, o)
                _inner_terms(y, _lhs_terms, o, emit_d)

    def feed(gen, z, n):
        for _ in range(n):
            try:
                gen.send(z)
            except StopIteration:
                return

    def layer(li, carry):
        first = li == 0

        never = zero[0] != 0

        class Pace:
            def __init__(self):
                self.tok = 0
                self.plan = []
                self.due = []

            def add(self, gen, t0, period, count=1, lat=None):
                next(gen)
                self.plan.append((gen, t0, period, count, lat))

            def step(self, z):
                for gen, t0, period, count, lat in self.plan:
                    if self.tok >= t0 and (self.tok - t0) % period == 0:
                        for _ in range(count):
                            try:
                                v = gen.send(z())
                            except StopIteration:
                                break
                            if v is not None and lat is not None:
                                self.due.append((self.tok + lat, v))
                self.tok += 1

            def tokens(self, r, n):
                for k in range(n):
                    cache = []

                    def z(k=k, cache=cache):
                        if not cache:
                            cache.append(after(r, k * 16))
                        return cache[0]
                    self.step(z)

            def gate(self, v):
                now = [x for t, x in self.due if t <= self.tok]
                self.due = [(t, x) for t, x in self.due if t > self.tok]
                if not now:
                    return v
                head = jnp.where(never, pltpu.bitcast(tree(now), u32), v[0:8])
                return jnp.concatenate([head, v[8:]], axis=0)

            def drain(self):
                for gen, *_ in self.plan:
                    feed(gen, 0, 1000)

        def tree(vals):
            while len(vals) > 1:
                vals = [a + b for a, b in zip(vals[::2], vals[1::2])] + vals[len(vals) & ~1:]
            return vals[0]

        def norm_slab(src, p0, emit):
            def total(x):
                return tree([x[k * 8:(k + 1) * 8] for k in range(D // 8)])
            t = total(src[p0, 0:D, :])
            mu = jnp.sum(t, axis=0, keepdims=True) * (1.0 / D)
            xc = src[jnp.clip(p0 + after(t), 0, NSLAB - 1), 0:D, :] - mu
            t = total(xc * xc)
            rs = lax.rsqrt(jnp.sum(t, axis=0, keepdims=True) * (1.0 / D) + EPS)
            p = jnp.clip(p0 + after(t), 0, NSLAB - 1)
            ends = []
            for k in (4, 0, 1, 2, 3):
                y = ((src[p, k * 128:min((k + 1) * 128, D), :] - mu) * rs).T
                emit(k, y)
                ends.append(y[120:128] if k < 4 else jnp.concatenate([y[120:128]] * 2, axis=1))
            return tree(ends)

        def ln1(p, b):
            def emit(k, y):
                xnb[b, k, :, 0:y.shape[1]] = y.astype(bf16)
            return norm_slab(xa, p, emit)

        def widen(t):
            for r in range(4):
                c0 = pl.multiple_of(t * TILE + r * 128, 128)
                xa[t * 4 + r, 0:D, :] = xin[:, pl.ds(c0, 128)].astype(f32)

        def qkv_proj(b, pace):
            for grp in ((4, 5, 6, 7), (13, 0, 1, 2), (3, 12, 8, 9), (10, 11)):
                for n in grp:
                    qkv[b, n, HALO:HALO + 128, :] = lax.dot_general(
                        _up(xn[b, 4]), _up(wq[4, n * 64:(n + 1) * 64, :]), NT,
                        preferred_element_type=f32)
                for n in grp:
                    rows = slice(n * 64, (n + 1) * 64)
                    lhs = jnp.concatenate(
                        [_up(pace.gate(xn[b, 0]))] + [_up(xn[b, k]) for k in range(1, 4)], axis=1)
                    rhs = jnp.concatenate([_up(wq[k, rows, :]) for k in range(4)], axis=1)
                    r = lax.dot_general(lhs, rhs, NT, preferred_element_type=f32)
                    r = r + jnp.concatenate([qkv[b, n, HALO:HALO + 64, :],
                                             qkv[b, n, HALO + 64:HALO + 128, :]], axis=0)
                    if n in (4, 5, 6, 7, 13):
                        r = r * (DH ** -0.5 * LOG2E)
                    qkv[b, n, HALO:HALO + 128, :] = r
                    pace.tokens(r, 7)

        def halo(b):
            for n in range(4, 14):
                qkv[b, n, 0:HALO, :] = qkv[1 - b, n, 128:128 + HALO, :]

        def attend(b, row0):
            qs, ks, vs = (0, 1, 2, 3, 12), (4, 5, 6, 7, 13), (8, 9, 10, 11, 12)
            v = None
            for s in range(16 * OPT["att"]):
                z = yield v
                r = HALO + s * 8
                rq = pl.multiple_of(jnp.clip(r + z, HALO, 120 + HALO), 8)
                q = [qkv[b, n, pl.ds(rq, 8), :] for n in qs]
                logit = []
                for w in range(WIN):
                    rw = r - DIL * w
                    part = tree([q[c] * qkv[b, ks[c], rw:rw + 8, :] for c in range(5)])
                    part = part + pltpu.roll(part, 64, 1)
                    part = part + pltpu.roll(part, 32, 1)
                    if row0 is not None and s * 8 < DIL * w:
                        pos = row0 + s * 8 + lax.broadcasted_iota(jnp.int32, (8, 128), 0)
                        part = jnp.where(pos >= DIL * w, part, -1e9 * LOG2E)
                    logit.append(part)
                mx = logit
                while len(mx) > 1:
                    mx = [jnp.maximum(a, c) for a, c in zip(mx[::2], mx[1::2])]
                e = [jnp.exp2(l - mx[0]) for l in logit]
                inv = 1.0 / tree(e)
                outs = []
                for c in range(5):
                    o = e[0] * qkv[b, vs[c], r:r + 8, :]
                    for w in range(1, WIN):
                        rw = r - DIL * w
                        o = o + e[w] * qkv[b, vs[c], rw:rw + 8, :]
                    o = o * inv
                    outs.append(o)
                    ob[b, c, s * 8:(s + 1) * 8, :] = o.astype(bf16)
                v = tree(outs)
            yield v

        def out_proj(p, b, pace):
            h = MB // 2
            for m in range(4):
                xb[p, m * MB:(m + 1) * MB, :] = xa[p, m * MB:(m + 1) * MB, :] + lax.dot_general(
                    _up(wo[4, m * h:(m + 1) * h, :]), _up(o32[b, 4]), NT, preferred_element_type=f32)
            rhs = jnp.concatenate([_up(o32[b, c]) for c in range(4)], axis=1)
            for m in range(4):
                rows = slice(m * h, (m + 1) * h)
                lhs = jnp.concatenate(
                    [_up(pace.gate(wo[0, rows, :]))] + [_up(wo[c, rows, :]) for c in range(1, 4)],
                    axis=1)
                r = lax.dot_general(lhs, rhs, NT, preferred_element_type=f32)
                r = r + jnp.concatenate([xb[p, m * MB:m * MB + h, :],
                                         xb[p, m * MB + h:(m + 1) * MB, :]], axis=0)
                xb[p, m * MB:(m + 1) * MB, :] = r
                pace.tokens(r, 8)

        def ffn_lhs(t):
            for r in range(4):
                def emit_n(k, y, r=r):
                    xn2[r * 5 + k, :, 0:y.shape[1]] = y
                norm_slab(xb, t * 4 + r, emit_n)
            for s in range(8):
                rows = slice(s * 16, (s + 1) * 16)
                a = [[xn2[r * 5 + k, rows, :] for k in range(4)] for r in range(4)]

                def emit(i, v, rows=rows):
                    acb[i, rows, :] = v.astype(bf16)
                _combos(a, _lhs_terms, emit)
                e = [xn2[r * 5 + 4, rows, 0:64] for r in range(4)]

                def emit_e(i, v, rows=rows):
                    aeb[i, rows, 0:64] = v.astype(bf16)
                _ext_combos(e, _lhs_ext, emit_e)

        @pl.when(first)
        def _():
            x_copy(0).wait()
            widen(0)
            for cp in chunk_copies(0):
                cp.wait()

        for n in range(4, 14):
            qkv[0, n, 0:HALO, :] = jnp.zeros((HALO, 128), f32)
        ln1(0, 0)
        pace = Pace()
        pace.add(prep_chunk(0), 0, 1, 2 * OPT["prep"])
        pace.due.append((OPT["hdue"], ln1(1, 1)))
        qkv_proj(0, pace)

        def attn_step(i, c):
            @pl.when(first)
            def _():
                for cp in chunk_copies(i + 1):
                    cp.wait()

            @pl.when(jnp.logical_and(first, jnp.logical_and(i % 2 == 1, i < 7)))
            def _():
                x_copy((i + 1) // 2).wait()
                widen((i + 1) // 2)

            side = prep_chunk(i + 1)
            next(side)
            for b in (1, 0):
                pace = Pace()
                if OPT["prep"]:
                    for t0 in (0, 1, 2):
                        pace.plan.append((side, t0, 4, 1, None))
                pace.due.append((OPT["ldue"], ln1(jnp.minimum(2 * i + 3 - b, NSLAB - 1), 1 - b)))
                pace.add(attend(1 - b, i * 256 if b == 1 else None),
                         OPT["a0"], OPT["aper"], 1, OPT["alat"])
                out_proj(jnp.maximum(2 * i - 1, 0) if b == 1 else 2 * i, b, pace)
                halo(b)
                qkv_proj(b, pace)
                pace.plan = pace.plan[-1:]
                pace.drain()
            if OPT["prep"]:
                feed(side, 0, 1000)
            return c
        if not OPT["skip_attn"]:
            lax.fori_loop(0, NSLAB // 2, attn_step, 0)

        out_proj(NSLAB - 1, 1, Pace())
        ffn_lhs(0)

        def ffn_group(t, g, last):
            ti = _Temps(tin)
            to = _Temps(tout)

            def proj(c, m):
                j = g * 3 + c

                def prod(o, i):
                    r = (m * 49 + o * 7 + i) * 64
                    p = jnp.dot(_up(ac[o * 7 + i]), _up(wc[j, r:r + 64, :]),
                                preferred_element_type=f32)
                    if o in AUG and i in AUG:
                        q = AUG.index(o) * 4 + AUG.index(i)
                        p = p + jnp.dot(_up(ae[q, :, 0:64]), _up(we[j, m * 16 + q]),
                                        preferred_element_type=f32)
                    return p
                return prod

            def gate(c):
                def fin(r, cc, v):
                    gs[(c % 2) * 16 + r * 4 + cc] = v
                return _recombine(proj(c, 0), fin, ti, to)

            def upgate(c):
                def fin(r, cc, v):
                    hs[c, r * 4 + cc] = _ld(gs, (c % 2) * 16 + r * 4 + cc) * v
                yield from _recombine(proj(c, 1), fin, ti, to)
                for s in range(8):
                    rows = slice(s * 16, (s + 1) * 16)
                    b = [[hs[c, r * 4 + cc, rows, :] for r in range(4)] for cc in range(4)]

                    def emit(i, v, rows=rows):
                        hcb[c, i, rows, :] = v.astype(bf16)
                    _combos(b, _rhs_terms, emit)

            def dprod(cs, i):
                p = None
                for c in cs:
                    r = i * (MB // 2)
                    q = lax.dot_general(_up(wdc[g * 3 + c, r:r + MB // 2, :]), _up(hc[c, i]), NT,
                                        preferred_element_type=f32)
                    p = q if p is None else p + q
                return p

            def down(cs, reset):
                for i in range(49):
                    a = _ld(acc, i)
                    if reset:
                        a = jnp.where(g == 0, 0.0, a)
                    acc[i] = a + dprod(cs, i)
                    yield

            def down_final(cs):
                def fin(mb, r, v):
                    rows = slice(mb * MB, (mb + 1) * MB)
                    y = xb[t * 4 + r, rows, :] + v
                    xa[t * 4 + r, rows, :] = y
                    ost[t * 4 + r, rows, :] = y.astype(bf16)
                return _recombine(lambda o, i: _ld(acc, o * 7 + i) + dprod(cs, o * 7 + i),
                                  fin, _Temps(tin2), _Temps(tout2))

            for gen in (gate(0), upgate(0), gate(1)):
                _adv(gen, 100)
            d0 = down((0,), not last)
            for gen, plan in ((upgate(1), DN_PLAN["u1"]), (gate(2), DN_PLAN["g2"]),
                              (upgate(2), DN_PLAN["u2"])):
                for n in plan:
                    _adv(gen, 1)
                    _adv(d0, n)
                _adv(gen, 100)
            if last:
                ffn_lhs((t + 1) % NTILE)
            _adv(d0, 100)
            _adv(down_final((1, 2)) if last else down((1, 2), False), 100)

        def ffn_tile(t, c):
            def grp(g, c2):
                ffn_group(t, g, False)
                return c2
            lax.fori_loop(0, 2, grp, 0)
            ffn_group(t, 2, True)

            @pl.when(li == 1)
            def _():
                for r in range(4):
                    out_copy(t * 4 + r).start()
            return c
        if not OPT["skip_ffn"]:
            lax.fori_loop(0, NTILE, ffn_tile, 0)
        else:
            r0 = pl.multiple_of(zero[0] * 16, 16)
            ost[0, 0:16, :] = wcb[li, pl.ds(r0, 16), :] + wdcb[li, pl.ds(r0, 16), :] + web[li, li, 0:16, :]
            ost[1, 0:16, :] = acb[li, 0:16, :] + aeb[li, 0:16, :] + qkv[li, li, 0:16, :].astype(bf16)
            ost[2] = xb[li, 0:D, :].astype(bf16)
            for r in range(8):
                out_copy(li * 8 + r).start()
        return carry

    lax.fori_loop(0, 2, layer, 0)
    for p in range(NSLAB):
        out_copy(p).wait()


@jax.jit
def pallas_interleave_layers__sliding_local_dilated__glu_gated_bilinear__prompt_kernel(
    A_x: jax.Array,
    A_wqkv: jax.Array,
    A_wo: jax.Array,
    B_x: jax.Array,
    B_w_gate: jax.Array,
    B_w_up: jax.Array,
    B_w_down: jax.Array,
):
    del B_x
    vm = pltpu.VMEM
    hbm = pl.BlockSpec(memory_space=pl.ANY)
    out_t = pl.pallas_call(
        _kernel,
        in_specs=[hbm] * 6,
        out_specs=hbm,
        out_shape=jax.ShapeDtypeStruct((D, S), bf16),
        scratch_shapes=[
            vm((D, S), bf16),
            vm((NSLAB, 768, 128), f32),
            vm((NSLAB, 768, 128), f32),
            vm((NSLAB, D, 128), bf16),
            vm((D, 3 * D), bf16),
            vm((D, D), bf16),
            vm((5, 3 * D, 128), f32),
            vm((5, 1792, 128), bf16),
            vm((5, D, 128), bf16),
            vm((NCHUNK, 3, D, FC), bf16),
            vm((NCHUNK, WC_ROWS, 128), bf16),
            vm((NCHUNK, 32, 64, 128), bf16),
            vm((NCHUNK, WD_ROWS, 128), bf16),
            vm((2, 5, 128, 128), bf16),
            vm((2, 14, HALO + 128, 128), f32),
            vm((2, 5, 128, 128), bf16),
            vm((20, 128, 128), f32),
            vm((49, 128, 128), bf16),
            vm((16, 128, 128), bf16),
            vm((32, 128, 128), f32),
            vm((3, 16, 128, 128), f32),
            vm((3, 49, 128, 128), bf16),
            vm((49, MB, 128), f32),
            vm((12, 128, 128), f32),
            vm((40, 128, 128), f32),
            vm((12, MB, 128), f32),
            vm((20, MB, 128), f32),
            pltpu.SMEM((1,), jnp.int32),
            pltpu.SemaphoreType.DMA((NTILE,)),
            pltpu.SemaphoreType.DMA((2,)),
            pltpu.SemaphoreType.DMA((NCHUNK, 3)),
            pltpu.SemaphoreType.DMA((NSLAB,)),
        ],
        compiler_params=pltpu.CompilerParams(vmem_limit_bytes=120 * 1024 * 1024),
    )(A_x[0].T, A_wqkv, A_wo, B_w_gate, B_w_up, B_w_down.T)
    return out_t.T[None]
```

```python
import math

import jax
import jax.numpy as jnp
from jax import lax
import jax.experimental.pallas as pl
import jax.experimental.pallas.tpu as pltpu

f32 = jnp.float32
bf16 = jnp.bfloat16
u32 = jnp.uint32

S, D, F = 2048, 576, 4608
H, DH, WIN, DIL = 32, 18, 8, 2
EPS = 1e-5
LOG2E = math.log2(math.e)
NSLAB = S // 128
TILE = 512
NTILE = S // TILE
FC = 512
NCHUNK = F // FC
MB = D // 4
HALO = 16
WC_ROWS = 800 * 16
WD_ROWS = 448 * 16
NT = (((1,), (1,)), ((), ()))
AUG = (0, 1, 2, 5)

OPT = dict(qtok=1, att=1, skip_ffn=False, skip_attn=False, prep=1, a0=0, aper=6, alat=35, ldue=32, hdue=40)
DN_PLAN = dict(u1=(0, 0, 0, 0, 4, 4, 6), g2=(4, 0, 0, 0, 0, 0, 0), u2=(0, 0, 0, 0, 4, 4, 4))


def _up(v):
    return pltpu.bitcast(v, bf16)


def _quad(x):
    n = len(x) // 2
    return ([r[:n] for r in x[:n]], [r[n:] for r in x[:n]],
            [r[:n] for r in x[n:]], [r[n:] for r in x[n:]])


def _badd(x, y):
    return [[a + b for a, b in zip(r, s)] for r, s in zip(x, y)]


def _bsub(x, y):
    return [[a - b for a, b in zip(r, s)] for r, s in zip(x, y)]


def _lhs_terms(a):
    a11, a12, a21, a22 = _quad(a)
    return [lambda: _badd(a11, a22), lambda: _badd(a21, a22), lambda: a11, lambda: a22,
            lambda: _badd(a11, a12), lambda: _bsub(a21, a11), lambda: _bsub(a12, a22)]


def _rhs_terms(b):
    b11, b12, b21, b22 = _quad(b)
    return [lambda: _badd(b11, b22), lambda: b11, lambda: _bsub(b12, b22), lambda: _bsub(b21, b11),
            lambda: b22, lambda: _badd(b11, b12), lambda: _badd(b21, b22)]


def _combos(x, terms, emit):
    for o, fo in enumerate(terms(x)):
        y = fo()
        for i, fi in enumerate(terms(y)):
            emit(o * 7 + i, fi()[0][0])


_LHS_SPEC = (((0, 0), (1, 1), 1), ((1, 0), (1, 1), 1), ((0, 0), None, 0), ((1, 1), None, 0),
             ((0, 0), (0, 1), 1), ((1, 0), (0, 0), -1), ((0, 1), (1, 1), -1))
_RHS_SPEC = (((0, 0), (1, 1), 1), ((0, 0), None, 0), ((0, 1), (1, 1), -1), ((1, 0), (0, 0), -1),
             ((1, 1), None, 0), ((0, 0), (0, 1), 1), ((1, 0), (1, 1), 1))


def _outer_term(load, spec, o):
    p, q, sign = spec[o]
    out = []
    for y in range(2):
        row = []
        for z in range(2):
            v = load(2 * p[0] + y, 2 * p[1] + z)
            if sign:
                w = load(2 * q[0] + y, 2 * q[1] + z)
                v = v + w if sign > 0 else v - w
            row.append(v)
        out.append(row)
    return out


def _inner_terms(y, terms, o, emit):
    for i, fi in enumerate(terms(y)):
        emit(o * 7 + i, fi()[0][0])


def _lhs_ext(e):
    n = len(e) // 2
    return {0: e[:n], 1: e[n:], 2: e[:n], 5: [y - x for x, y in zip(e[:n], e[n:])]}


def _rhs_ext(e):
    n = len(e) // 2
    return {0: e[:n], 1: e[:n], 2: e[n:], 5: [x + y for x, y in zip(e[:n], e[n:])]}


def _ext_combos(e, fn, emit):
    for oi, o in enumerate(AUG):
        d = fn(fn(e)[o])
        for ii, i in enumerate(AUG):
            emit(oi * 4 + ii, d[i][0])


def _adv(gen, n):
    for _ in range(n):
        try:
            next(gen)
        except StopIteration:
            return


def _ld(ref, idx):
    n = ref.shape[-2] // 2
    return jnp.concatenate([ref[idx, :n, :], ref[idx, n:, :]], axis=0)


class _Temps:
    def __init__(self, ref):
        self.ref = ref
        self.n = 0

    def put(self, v):
        i = self.n % self.ref.shape[0]
        self.n += 1
        self.ref[i] = v
        return i

    def get(self, i):
        return _ld(self.ref, i)


def _recombine(prod, fin, ti, to):
    def inner(o, sink):
        a = ti.put(prod(o, 0))
        b = ti.put(prod(o, 1))
        c = ti.put(prod(o, 2))
        sink(1, 1, ti.get(a) - ti.get(b) + ti.get(c) + prod(o, 5))
        m3 = prod(o, 3)
        m4 = prod(o, 4)
        m6 = prod(o, 6)
        sink(1, 0, ti.get(b) + m3)
        sink(0, 1, ti.get(c) + m4)
        sink(0, 0, ti.get(a) + m3 - m4 + m6)

    m = {}
    for o in (0, 1, 2):
        def keep(y, z, v, o=o):
            m[o, y, z] = to.put(v)
        inner(o, keep)
        yield

    def s5(y, z, v):
        fin(2 + y, 2 + z, to.get(m[0, y, z]) - to.get(m[1, y, z]) + to.get(m[2, y, z]) + v)
    inner(5, s5)
    yield

    def s3(y, z, v):
        fin(2 + y, z, to.get(m[1, y, z]) + v)
        m[3, y, z] = to.put(to.get(m[0, y, z]) + v)
    inner(3, s3)
    yield

    def s4(y, z, v):
        fin(y, 2 + z, to.get(m[2, y, z]) + v)
        m[3, y, z] = to.put(to.get(m[3, y, z]) - v)
    inner(4, s4)
    yield

    def s6(y, z, v):
        fin(y, z, to.get(m[3, y, z]) + v)
    inner(6, s6)
    yield


def _kernel(xt_hbm, wqkv_hbm, wo_hbm, wg_hbm, wu_hbm, wdt_hbm, out_hbm,
            xin, xa, xb, ost, wq_raw, wo_raw, wtmp, wqb, wob, raw, wcb, web, wdcb,
            xnb, qkv, ob, xn2, acb, aeb, gs, hs, hcb, acc, tin, tout, tin2, tout2, zero,
            sem_x, sem_w, sem_c, sem_o):
    wq, wo, wc, we, wdc, xn, o32, ac, ae, hc, raw32 = [
        r.bitcast(u32) for r in (wqb, wob, wcb, web, wdcb, xnb, ob, acb, aeb, hcb, raw)]

    def x_copy(t):
        return pltpu.make_async_copy(
            xt_hbm.at[:, pl.ds(t * TILE, TILE)], xin.at[:, pl.ds(t * TILE, TILE)], sem_x.at[t])

    def chunk_copies(j):
        return [pltpu.make_async_copy(
            src.at[:, pl.ds(pl.multiple_of(j * FC + c * 128, 128), 128)],
            raw.at[j, pl.ds((m * 4 + c) * D, D)], sem_c.at[j, m * 4 + c])
            for m, src in enumerate((wg_hbm, wu_hbm, wdt_hbm)) for c in range(4)]

    def out_copy(p):
        return pltpu.make_async_copy(
            ost.at[p], out_hbm.at[:, pl.ds(pl.multiple_of(p * 128, 128), 128)], sem_o.at[p])

    wq_copy = pltpu.make_async_copy(wqkv_hbm, wq_raw, sem_w.at[0])
    wo_copy = pltpu.make_async_copy(wo_hbm, wo_raw, sem_w.at[1])
    zero[0] = 0
    wq_copy.start()
    x_copy(0).start()
    wo_copy.start()
    wq_copy.wait()
    for cp in chunk_copies(0):
        cp.start()

    def wq_transpose(n, carry):
        c0 = pl.multiple_of(n * 128, 128)
        t = wq_raw[:, pl.ds(c0, 128)].astype(f32).T
        for k in range(4):
            wtmp[k, pl.ds(c0, 128), :] = t[:, k * 128:(k + 1) * 128]
        wtmp[4, pl.ds(c0, 128), 0:64] = t[:, 512:576]
        return carry
    lax.fori_loop(0, 13, wq_transpose, 0, unroll=True)
    t = wq_raw[:, 1664:1728].astype(f32).T
    for k in range(4):
        wtmp[k, 1664:1728, :] = t[:, k * 128:(k + 1) * 128]
    wtmp[4, 1664:1728, 0:64] = t[:, 512:576]
    for k in range(5):
        lanes = slice(0, 128) if k < 4 else slice(0, 64)
        for part in range(3):
            for d in range(DH):
                if d < 16:
                    row = part * 512 + d * 32
                else:
                    row = (1536, 1664, 1600)[part] + (d - 16) * 32
                wqb[k, row:row + 32, lanes] = wtmp[
                    k, pl.ds(part * D + d, H, stride=DH), lanes].astype(bf16)
        wqb[k, 1728:1792, lanes] = jnp.zeros((64, lanes.stop), bf16)
    wqb[4, :, 64:128] = jnp.zeros((1792, 64), bf16)
    xnb[:, 4, :, 64:128] = jnp.zeros((2, 128, 64), bf16)
    ob[1] = jnp.zeros((5, 128, 128), bf16)

    for j in range(1, 3):
        for cp in chunk_copies(j):
            cp.start()
    x_copy(1).start()

    wo_copy.wait()
    for n in range(5):
        w = 128 if n < 4 else 64
        wtmp[n, 0:D, 0:w] = wo_raw[:, n * 128:n * 128 + w].astype(f32)
    for n in range(5):
        w = 128 if n < 4 else 64
        for c in range(5):
            if c < 4:
                rows = [wtmp[n, pl.ds(4 * c + g, H, stride=DH), 0:w] for g in range(4)]
            else:
                rows = [jnp.zeros((64, w), f32)] + [
                    wtmp[n, pl.ds(16 + g, H, stride=DH), 0:w] for g in range(2)]
            wob[c, n * 128:n * 128 + w, :] = jnp.concatenate(rows, axis=0).T.astype(bf16)

    for j in range(3, NCHUNK):
        for cp in chunk_copies(j):
            cp.start()
        if j in (4, 6):
            x_copy(j // 2).start()

    def after(v, row=0):
        return lax.bitcast_convert_type(v[row:row + 1, 0:1], jnp.int32)[0, 0] & zero[0]

    never = zero[0] != 0

    def held(v, z):
        if z is None:
            return v
        return jnp.where(never, pltpu.bitcast(z, v.dtype), v)

    def prep_chunk(j):
        def load(m, row, c, z):
            r = ((m * 4 + c) * D + row) // 2
            v = raw32[j, r:r + 8, :]
            return _up(held(v, z)).astype(f32)
        for m in range(2):
            for s in range(8):
                def emit(i, v, m=m, s=s):
                    r = (m * 49 + i) * 128 + s * 16
                    wcb[j, r:r + 16, :] = v.astype(bf16)
                for o in range(7):
                    z = yield
                    y = _outer_term(lambda k, c: load(m, k * 128 + s * 16, c, z), _RHS_SPEC, o)
                    _inner_terms(y, _rhs_terms, o, emit)
            for s in range(4):
                z = yield
                e = [load(m, 512 + s * 16, c, z) for c in range(4)]

                def emit_e(i, v, m=m, s=s):
                    web[j, m * 16 + i, s * 16:(s + 1) * 16, :] = v.astype(bf16)
                _ext_combos(e, _rhs_ext, emit_e)
        for s in range(9):
            def emit_d(i, v, s=s):
                r = i * MB + s * 16
                wdcb[j, r:r + 16, :] = v.astype(bf16)
            for o in range(7):
                z = yield
                y = _outer_term(lambda r, k: load(2, r * MB + s * 16, k, z), _LHS_SPEC, o)
                _inner_terms(y, _lhs_terms, o, emit_d)

    def feed(gen, z, n):
        for _ in range(n):
            try:
                gen.send(z)
            except StopIteration:
                return

    def layer(li, carry):
        first = li == 0

        class Pace:
            def __init__(self):
                self.tok = 0
                self.plan = []
                self.due = []

            def add(self, gen, t0, period, count=1, lat=None):
                next(gen)
                self.plan.append((gen, t0, period, count, lat))

            def step(self, z):
                for gen, t0, period, count, lat in self.plan:
                    if self.tok >= t0 and (self.tok - t0) % period == 0:
                        for _ in range(count):
                            try:
                                v = gen.send(z)
                            except StopIteration:
                                break
                            if v is not None and lat is not None:
                                self.due.append((self.tok + lat, v))
                self.tok += 1

            def tokens(self, r, n):
                for k in range(n):
                    self.step(r[k * 16:k * 16 + 8])

            def gate(self, v):
                now = [x for t, x in self.due if t <= self.tok]
                self.due = [(t, x) for t, x in self.due if t > self.tok]
                if not now:
                    return v
                head = jnp.where(never, pltpu.bitcast(tree(now), u32), v[0:8])
                return jnp.concatenate([head, v[8:]], axis=0)

            def drain(self):
                for gen, *_ in self.plan:
                    feed(gen, None, 1000)

        def tree(vals):
            while len(vals) > 1:
                vals = [a + b for a, b in zip(vals[::2], vals[1::2])] + vals[len(vals) & ~1:]
            return vals[0]

        def norm_slab(src, p0, emit):
            def total(x):
                return tree([x[k * 8:(k + 1) * 8] for k in range(D // 8)])
            t = total(src[p0, 0:D, :])
            mu = jnp.sum(t, axis=0, keepdims=True) * (1.0 / D)
            xc = src[jnp.clip(p0 + after(t), 0, NSLAB - 1), 0:D, :] - mu
            t = total(xc * xc)
            rs = lax.rsqrt(jnp.sum(t, axis=0, keepdims=True) * (1.0 / D) + EPS)
            p = jnp.clip(p0 + after(t), 0, NSLAB - 1)
            ends = []
            for k in (4, 0, 1, 2, 3):
                y = ((src[p, k * 128:min((k + 1) * 128, D), :] - mu) * rs).T
                emit(k, y)
                ends.append(y[120:128] if k < 4 else jnp.concatenate([y[120:128]] * 2, axis=1))
            return tree(ends)

        def ln1(p, b):
            def emit(k, y):
                xnb[b, k, :, 0:y.shape[1]] = y.astype(bf16)
            return norm_slab(xa, p, emit)

        def widen(t):
            for r in range(4):
                c0 = pl.multiple_of(t * TILE + r * 128, 128)
                xa[t * 4 + r, 0:D, :] = xin[:, pl.ds(c0, 128)].astype(f32)

        def qkv_proj(b, pace):
            for grp in ((4, 5, 6, 7), (13, 0, 1, 2), (3, 12, 8, 9), (10, 11)):
                for n in grp:
                    qkv[b, n, HALO:HALO + 128, :] = lax.dot_general(
                        _up(xn[b, 4]), _up(wq[4, n * 64:(n + 1) * 64, :]), NT,
                        preferred_element_type=f32)
                for n in grp:
                    rows = slice(n * 64, (n + 1) * 64)
                    lhs = jnp.concatenate(
                        [_up(pace.gate(xn[b, 0]))] + [_up(xn[b, k]) for k in range(1, 4)], axis=1)
                    rhs = jnp.concatenate([_up(wq[k, rows, :]) for k in range(4)], axis=1)
                    r = lax.dot_general(lhs, rhs, NT, preferred_element_type=f32)
                    r = r + jnp.concatenate([qkv[b, n, HALO:HALO + 64, :],
                                             qkv[b, n, HALO + 64:HALO + 128, :]], axis=0)
                    if n in (4, 5, 6, 7, 13):
                        r = r * (DH ** -0.5 * LOG2E)
                    qkv[b, n, HALO:HALO + 128, :] = r
                    pace.tokens(r, 7)

        def halo(b):
            for n in range(4, 14):
                qkv[b, n, 0:HALO, :] = qkv[1 - b, n, 128:128 + HALO, :]

        def attend(b, row0):
            qs, ks, vs = (0, 1, 2, 3, 12), (4, 5, 6, 7, 13), (8, 9, 10, 11, 12)
            v = None
            for s in range(16 * OPT["att"]):
                z = yield v
                r = HALO + s * 8
                q = [held(qkv[b, n, r:r + 8, :], z if OPT["qtok"] else None) for n in qs]
                logit = []
                for w in range(WIN):
                    rw = r - DIL * w
                    part = tree([q[c] * qkv[b, ks[c], rw:rw + 8, :] for c in range(5)])
                    part = part + pltpu.roll(part, 64, 1)
                    part = part + pltpu.roll(part, 32, 1)
                    if row0 is not None and s * 8 < DIL * w:
                        pos = row0 + s * 8 + lax.broadcasted_iota(jnp.int32, (8, 128), 0)
                        part = jnp.where(pos >= DIL * w, part, -1e9 * LOG2E)
                    logit.append(part)
                mx = logit
                while len(mx) > 1:
                    mx = [jnp.maximum(a, c) for a, c in zip(mx[::2], mx[1::2])]
                e = [jnp.exp2(l - mx[0]) for l in logit]
                inv = 1.0 / tree(e)
                outs = []
                for c in range(5):
                    o = e[0] * qkv[b, vs[c], r:r + 8, :]
                    for w in range(1, WIN):
                        rw = r - DIL * w
                        o = o + e[w] * qkv[b, vs[c], rw:rw + 8, :]
                    o = o * inv
                    outs.append(o)
                    ob[b, c, s * 8:(s + 1) * 8, :] = o.astype(bf16)
                v = tree(outs)
            yield v

        def out_proj(p, b, pace):
            h = MB // 2
            for m in range(4):
                xb[p, m * MB:(m + 1) * MB, :] = xa[p, m * MB:(m + 1) * MB, :] + lax.dot_general(
                    _up(wo[4, m * h:(m + 1) * h, :]), _up(o32[b, 4]), NT, preferred_element_type=f32)
            rhs = jnp.concatenate([_up(o32[b, c]) for c in range(4)], axis=1)
            for m in range(4):
                rows = slice(m * h, (m + 1) * h)
                lhs = jnp.concatenate(
                    [_up(pace.gate(wo[0, rows, :]))] + [_up(wo[c, rows, :]) for c in range(1, 4)],
                    axis=1)
                r = lax.dot_general(lhs, rhs, NT, preferred_element_type=f32)
                r = r + jnp.concatenate([xb[p, m * MB:m * MB + h, :],
                                         xb[p, m * MB + h:(m + 1) * MB, :]], axis=0)
                xb[p, m * MB:(m + 1) * MB, :] = r
                pace.tokens(r, 8)

        def ffn_lhs(t):
            for r in range(4):
                def emit_n(k, y, r=r):
                    xn2[r * 5 + k, :, 0:y.shape[1]] = y
                norm_slab(xb, t * 4 + r, emit_n)
            for s in range(8):
                rows = slice(s * 16, (s + 1) * 16)
                a = [[xn2[r * 5 + k, rows, :] for k in range(4)] for r in range(4)]

                def emit(i, v, rows=rows):
                    acb[i, rows, :] = v.astype(bf16)
                _combos(a, _lhs_terms, emit)
                e = [xn2[r * 5 + 4, rows, 0:64] for r in range(4)]

                def emit_e(i, v, rows=rows):
                    aeb[i, rows, 0:64] = v.astype(bf16)
                _ext_combos(e, _lhs_ext, emit_e)

        @pl.when(first)
        def _():
            x_copy(0).wait()
            widen(0)
            for cp in chunk_copies(0):
                cp.wait()

        for n in range(4, 14):
            qkv[0, n, 0:HALO, :] = jnp.zeros((HALO, 128), f32)
        ln1(0, 0)
        pace = Pace()
        pace.add(prep_chunk(0), 0, 1, 2 * OPT["prep"])
        pace.due.append((OPT["hdue"], ln1(1, 1)))
        qkv_proj(0, pace)

        def attn_step(i, c):
            @pl.when(first)
            def _():
                for cp in chunk_copies(i + 1):
                    cp.wait()

            @pl.when(jnp.logical_and(first, jnp.logical_and(i % 2 == 1, i < 7)))
            def _():
                x_copy((i + 1) // 2).wait()
                widen((i + 1) // 2)

            side = prep_chunk(i + 1)
            next(side)
            for b in (1, 0):
                pace = Pace()
                if OPT["prep"]:
                    for t0 in (0, 1, 2):
                        pace.plan.append((side, t0, 4, 1, None))
                pace.due.append((OPT["ldue"], ln1(jnp.minimum(2 * i + 3 - b, NSLAB - 1), 1 - b)))
                pace.add(attend(1 - b, i * 256 if b == 1 else None),
                         OPT["a0"], OPT["aper"], 1, OPT["alat"])
                out_proj(jnp.maximum(2 * i - 1, 0) if b == 1 else 2 * i, b, pace)
                halo(b)
                qkv_proj(b, pace)
                pace.plan = pace.plan[-1:]
                pace.drain()
            if OPT["prep"]:
                feed(side, None, 1000)
            return c
        if not OPT["skip_attn"]:
            lax.fori_loop(0, NSLAB // 2, attn_step, 0)

        out_proj(NSLAB - 1, 1, Pace())
        ffn_lhs(0)

        def ffn_group(t, g, last):
            ti = _Temps(tin)
            to = _Temps(tout)

            def proj(c, m):
                j = g * 3 + c

                def prod(o, i):
                    r = (m * 49 + o * 7 + i) * 64
                    p = jnp.dot(_up(ac[o * 7 + i]), _up(wc[j, r:r + 64, :]),
                                preferred_element_type=f32)
                    if o in AUG and i in AUG:
                        q = AUG.index(o) * 4 + AUG.index(i)
                        p = p + jnp.dot(_up(ae[q, :, 0:64]), _up(we[j, m * 16 + q]),
                                        preferred_element_type=f32)
                    return p
                return prod

            def gate(c):
                def fin(r, cc, v):
                    gs[(c % 2) * 16 + r * 4 + cc] = v
                return _recombine(proj(c, 0), fin, ti, to)

            def upgate(c):
                def fin(r, cc, v):
                    hs[c, r * 4 + cc] = _ld(gs, (c % 2) * 16 + r * 4 + cc) * v
                yield from _recombine(proj(c, 1), fin, ti, to)
                for s in range(8):
                    rows = slice(s * 16, (s + 1) * 16)
                    b = [[hs[c, r * 4 + cc, rows, :] for r in range(4)] for cc in range(4)]

                    def emit(i, v, rows=rows):
                        hcb[c, i, rows, :] = v.astype(bf16)
                    _combos(b, _rhs_terms, emit)

            def dprod(cs, i):
                p = None
                for c in cs:
                    r = i * (MB // 2)
                    q = lax.dot_general(_up(wdc[g * 3 + c, r:r + MB // 2, :]), _up(hc[c, i]), NT,
                                        preferred_element_type=f32)
                    p = q if p is None else p + q
                return p

            def down(cs, reset):
                for i in range(49):
                    a = _ld(acc, i)
                    if reset:
                        a = jnp.where(g == 0, 0.0, a)
                    acc[i] = a + dprod(cs, i)
                    yield

            def down_final(cs):
                def fin(mb, r, v):
                    rows = slice(mb * MB, (mb + 1) * MB)
                    y = xb[t * 4 + r, rows, :] + v
                    xa[t * 4 + r, rows, :] = y
                    ost[t * 4 + r, rows, :] = y.astype(bf16)
                return _recombine(lambda o, i: _ld(acc, o * 7 + i) + dprod(cs, o * 7 + i),
                                  fin, _Temps(tin2), _Temps(tout2))

            for gen in (gate(0), upgate(0), gate(1)):
                _adv(gen, 100)
            d0 = down((0,), not last)
            for gen, plan in ((upgate(1), DN_PLAN["u1"]), (gate(2), DN_PLAN["g2"]),
                              (upgate(2), DN_PLAN["u2"])):
                for n in plan:
                    _adv(gen, 1)
                    _adv(d0, n)
                _adv(gen, 100)
            if last:
                ffn_lhs((t + 1) % NTILE)
            _adv(d0, 100)
            _adv(down_final((1, 2)) if last else down((1, 2), False), 100)

        def ffn_tile(t, c):
            def grp(g, c2):
                ffn_group(t, g, False)
                return c2
            lax.fori_loop(0, 2, grp, 0)
            ffn_group(t, 2, True)

            @pl.when(li == 1)
            def _():
                for r in range(4):
                    out_copy(t * 4 + r).start()
            return c
        if not OPT["skip_ffn"]:
            lax.fori_loop(0, NTILE, ffn_tile, 0)
        else:
            r0 = pl.multiple_of(zero[0] * 16, 16)
            ost[0, 0:16, :] = wcb[li, pl.ds(r0, 16), :] + wdcb[li, pl.ds(r0, 16), :] + web[li, li, 0:16, :]
            ost[1, 0:16, :] = acb[li, 0:16, :] + aeb[li, 0:16, :] + qkv[li, li, 0:16, :].astype(bf16)
            ost[2] = xb[li, 0:D, :].astype(bf16)
            for r in range(8):
                out_copy(li * 8 + r).start()
        return carry

    lax.fori_loop(0, 2, layer, 0)
    for p in range(NSLAB):
        out_copy(p).wait()


@jax.jit
def pallas_interleave_layers__sliding_local_dilated__glu_gated_bilinear__prompt_kernel(
    A_x: jax.Array,
    A_wqkv: jax.Array,
    A_wo: jax.Array,
    B_x: jax.Array,
    B_w_gate: jax.Array,
    B_w_up: jax.Array,
    B_w_down: jax.Array,
):
    del B_x
    vm = pltpu.VMEM
    hbm = pl.BlockSpec(memory_space=pl.ANY)
    out_t = pl.pallas_call(
        _kernel,
        in_specs=[hbm] * 6,
        out_specs=hbm,
        out_shape=jax.ShapeDtypeStruct((D, S), bf16),
        scratch_shapes=[
            vm((D, S), bf16),
            vm((NSLAB, 768, 128), f32),
            vm((NSLAB, 768, 128), f32),
            vm((NSLAB, D, 128), bf16),
            vm((D, 3 * D), bf16),
            vm((D, D), bf16),
            vm((5, 3 * D, 128), f32),
            vm((5, 1792, 128), bf16),
            vm((5, D, 128), bf16),
            vm((NCHUNK, WD_ROWS, 128), bf16),
            vm((NCHUNK, WC_ROWS, 128), bf16),
            vm((NCHUNK, 32, 64, 128), bf16),
            vm((NCHUNK, WD_ROWS, 128), bf16),
            vm((2, 5, 128, 128), bf16),
            vm((2, 14, HALO + 128, 128), f32),
            vm((2, 5, 128, 128), bf16),
            vm((20, 128, 128), f32),
            vm((49, 128, 128), bf16),
            vm((16, 128, 128), bf16),
            vm((32, 128, 128), f32),
            vm((3, 16, 128, 128), f32),
            vm((3, 49, 128, 128), bf16),
            vm((49, MB, 128), f32),
            vm((12, 128, 128), f32),
            vm((40, 128, 128), f32),
            vm((12, MB, 128), f32),
            vm((20, MB, 128), f32),
            pltpu.SMEM((1,), jnp.int32),
            pltpu.SemaphoreType.DMA((NTILE,)),
            pltpu.SemaphoreType.DMA((2,)),
            pltpu.SemaphoreType.DMA((NCHUNK, 12)),
            pltpu.SemaphoreType.DMA((NSLAB,)),
        ],
        compiler_params=pltpu.CompilerParams(vmem_limit_bytes=120 * 1024 * 1024),
    )(A_x[0].T, A_wqkv, A_wo, B_w_gate, B_w_up, B_w_down.T)
    return out_t.T[None]
```

```python
import math

import jax
import jax.numpy as jnp
from jax import lax
import jax.experimental.pallas as pl
import jax.experimental.pallas.tpu as pltpu

f32 = jnp.float32
bf16 = jnp.bfloat16
u32 = jnp.uint32

S, D, F = 2048, 576, 4608
H, DH, WIN, DIL = 32, 18, 8, 2
EPS = 1e-5
LOG2E = math.log2(math.e)
NSLAB = S // 128
TILE = 512
NTILE = S // TILE
FC = 512
NCHUNK = F // FC
MB = D // 4
HALO = 16
NTR = D // 8
WC_ROWS = 800 * 16
WD_ROWS = 448 * 16
NT = (((1,), (1,)), ((), ()))
AUG = (0, 1, 2, 5)

OPT = dict(qtok=1, att=1, skip_ffn=False, skip_attn=False, prep=1, a0=0, aper=6, alat=35, ldue=32, hdue=40)
DN_PLAN = dict(u1=(0, 0, 0, 0, 4, 4, 6), g2=(4, 0, 0, 0, 0, 0, 0), u2=(0, 0, 0, 0, 4, 4, 4))


def _up(v):
    return pltpu.bitcast(v, bf16)


def _quad(x):
    n = len(x) // 2
    return ([r[:n] for r in x[:n]], [r[n:] for r in x[:n]],
            [r[:n] for r in x[n:]], [r[n:] for r in x[n:]])


def _badd(x, y):
    return [[a + b for a, b in zip(r, s)] for r, s in zip(x, y)]


def _bsub(x, y):
    return [[a - b for a, b in zip(r, s)] for r, s in zip(x, y)]


def _lhs_terms(a):
    a11, a12, a21, a22 = _quad(a)
    return [lambda: _badd(a11, a22), lambda: _badd(a21, a22), lambda: a11, lambda: a22,
            lambda: _badd(a11, a12), lambda: _bsub(a21, a11), lambda: _bsub(a12, a22)]


def _rhs_terms(b):
    b11, b12, b21, b22 = _quad(b)
    return [lambda: _badd(b11, b22), lambda: b11, lambda: _bsub(b12, b22), lambda: _bsub(b21, b11),
            lambda: b22, lambda: _badd(b11, b12), lambda: _badd(b21, b22)]


def _combos(x, terms, emit):
    for o, fo in enumerate(terms(x)):
        y = fo()
        for i, fi in enumerate(terms(y)):
            emit(o * 7 + i, fi()[0][0])


_LHS_SPEC = (((0, 0), (1, 1), 1), ((1, 0), (1, 1), 1), ((0, 0), None, 0), ((1, 1), None, 0),
             ((0, 0), (0, 1), 1), ((1, 0), (0, 0), -1), ((0, 1), (1, 1), -1))
_RHS_SPEC = (((0, 0), (1, 1), 1), ((0, 0), None, 0), ((0, 1), (1, 1), -1), ((1, 0), (0, 0), -1),
             ((1, 1), None, 0), ((0, 0), (0, 1), 1), ((1, 0), (1, 1), 1))


def _outer_term(load, spec, o):
    p, q, sign = spec[o]
    out = []
    for y in range(2):
        row = []
        for z in range(2):
            v = load(2 * p[0] + y, 2 * p[1] + z)
            if sign:
                w = load(2 * q[0] + y, 2 * q[1] + z)
                v = v + w if sign > 0 else v - w
            row.append(v)
        out.append(row)
    return out


def _inner_terms(y, terms, o, emit):
    for i, fi in enumerate(terms(y)):
        emit(o * 7 + i, fi()[0][0])


def _lhs_ext(e):
    n = len(e) // 2
    return {0: e[:n], 1: e[n:], 2: e[:n], 5: [y - x for x, y in zip(e[:n], e[n:])]}


def _rhs_ext(e):
    n = len(e) // 2
    return {0: e[:n], 1: e[:n], 2: e[n:], 5: [x + y for x, y in zip(e[:n], e[n:])]}


def _ext_combos(e, fn, emit):
    for oi, o in enumerate(AUG):
        d = fn(fn(e)[o])
        for ii, i in enumerate(AUG):
            emit(oi * 4 + ii, d[i][0])


def _adv(gen, n):
    for _ in range(n):
        try:
            next(gen)
        except StopIteration:
            return


def _ld(ref, idx):
    n = ref.shape[-2] // 2
    return jnp.concatenate([ref[idx, :n, :], ref[idx, n:, :]], axis=0)


class _Temps:
    def __init__(self, ref):
        self.ref = ref
        self.n = 0

    def put(self, v):
        i = self.n % self.ref.shape[0]
        self.n += 1
        self.ref[i] = v
        return i

    def get(self, i):
        return _ld(self.ref, i)


def _recombine(prod, fin, ti, to):
    def inner(o, sink):
        a = ti.put(prod(o, 0))
        b = ti.put(prod(o, 1))
        c = ti.put(prod(o, 2))
        sink(1, 1, ti.get(a) - ti.get(b) + ti.get(c) + prod(o, 5))
        m3 = prod(o, 3)
        m4 = prod(o, 4)
        m6 = prod(o, 6)
        sink(1, 0, ti.get(b) + m3)
        sink(0, 1, ti.get(c) + m4)
        sink(0, 0, ti.get(a) + m3 - m4 + m6)

    m = {}
    for o in (0, 1, 2):
        def keep(y, z, v, o=o):
            m[o, y, z] = to.put(v)
        inner(o, keep)
        yield

    def s5(y, z, v):
        fin(2 + y, 2 + z, to.get(m[0, y, z]) - to.get(m[1, y, z]) + to.get(m[2, y, z]) + v)
    inner(5, s5)
    yield

    def s3(y, z, v):
        fin(2 + y, z, to.get(m[1, y, z]) + v)
        m[3, y, z] = to.put(to.get(m[0, y, z]) + v)
    inner(3, s3)
    yield

    def s4(y, z, v):
        fin(y, 2 + z, to.get(m[2, y, z]) + v)
        m[3, y, z] = to.put(to.get(m[3, y, z]) - v)
    inner(4, s4)
    yield

    def s6(y, z, v):
        fin(y, z, to.get(m[3, y, z]) + v)
    inner(6, s6)
    yield


def _kernel(xt_hbm, wqkv_hbm, wo_hbm, wg_hbm, wu_hbm, wdt_hbm, out_hbm,
            xin, xa, xb, ost, wq_raw, wo_raw, wtmp, wqb, wob, raw, wcb, web, wdcb,
            xnb, qkv, ob, xn2, acb, aeb, gs, hs, hcb, acc, tin, tout, tin2, tout2, zero,
            sem_x, sem_w, sem_c, sem_o):
    wq, wo, wc, we, wdc, xn, o32, ac, ae, hc, raw32 = [
        r.bitcast(u32) for r in (wqb, wob, wcb, web, wdcb, xnb, ob, acb, aeb, hcb, raw)]

    def x_copy(t):
        return pltpu.make_async_copy(
            xt_hbm.at[:, pl.ds(t * TILE, TILE)], xin.at[:, pl.ds(t * TILE, TILE)], sem_x.at[t])

    def chunk_copies(j):
        rows = pl.ds(pl.multiple_of(j * 32, 32), 32)
        return [pltpu.make_async_copy(src.at[:, rows, :], raw.at[j, pl.ds(m * NTR, NTR)],
                                      sem_c.at[j, m])
                for m, src in enumerate((wg_hbm, wu_hbm, wdt_hbm))]

    def out_copy(p):
        return pltpu.make_async_copy(
            ost.at[p], out_hbm.at[:, pl.ds(pl.multiple_of(p * 128, 128), 128)], sem_o.at[p])

    wq_copy = pltpu.make_async_copy(wqkv_hbm, wq_raw, sem_w.at[0])
    wo_copy = pltpu.make_async_copy(wo_hbm, wo_raw, sem_w.at[1])
    zero[0] = 0
    wq_copy.start()
    x_copy(0).start()
    wo_copy.start()
    wq_copy.wait()
    for cp in chunk_copies(0):
        cp.start()

    def wq_transpose(n, carry):
        c0 = pl.multiple_of(n * 128, 128)
        t = wq_raw[:, pl.ds(c0, 128)].astype(f32).T
        for k in range(4):
            wtmp[k, pl.ds(c0, 128), :] = t[:, k * 128:(k + 1) * 128]
        wtmp[4, pl.ds(c0, 128), 0:64] = t[:, 512:576]
        return carry
    lax.fori_loop(0, 13, wq_transpose, 0, unroll=True)
    t = wq_raw[:, 1664:1728].astype(f32).T
    for k in range(4):
        wtmp[k, 1664:1728, :] = t[:, k * 128:(k + 1) * 128]
    wtmp[4, 1664:1728, 0:64] = t[:, 512:576]
    for k in range(5):
        lanes = slice(0, 128) if k < 4 else slice(0, 64)
        for part in range(3):
            for d in range(DH):
                if d < 16:
                    row = part * 512 + d * 32
                else:
                    row = (1536, 1664, 1600)[part] + (d - 16) * 32
                wqb[k, row:row + 32, lanes] = wtmp[
                    k, pl.ds(part * D + d, H, stride=DH), lanes].astype(bf16)
        wqb[k, 1728:1792, lanes] = jnp.zeros((64, lanes.stop), bf16)
    wqb[4, :, 64:128] = jnp.zeros((1792, 64), bf16)
    xnb[:, 4, :, 64:128] = jnp.zeros((2, 128, 64), bf16)
    ob[1] = jnp.zeros((5, 128, 128), bf16)

    for j in range(1, 3):
        for cp in chunk_copies(j):
            cp.start()
    x_copy(1).start()

    wo_copy.wait()
    for n in range(5):
        w = 128 if n < 4 else 64
        wtmp[n, 0:D, 0:w] = wo_raw[:, n * 128:n * 128 + w].astype(f32)
    for n in range(5):
        w = 128 if n < 4 else 64
        for c in range(5):
            if c < 4:
                rows = [wtmp[n, pl.ds(4 * c + g, H, stride=DH), 0:w] for g in range(4)]
            else:
                rows = [jnp.zeros((64, w), f32)] + [
                    wtmp[n, pl.ds(16 + g, H, stride=DH), 0:w] for g in range(2)]
            wob[c, n * 128:n * 128 + w, :] = jnp.concatenate(rows, axis=0).T.astype(bf16)

    for j in range(3, NCHUNK):
        for cp in chunk_copies(j):
            cp.start()
        if j in (4, 6):
            x_copy(j // 2).start()

    def after(v, row=0):
        return lax.bitcast_convert_type(v[row:row + 1, 0:1], jnp.int32)[0, 0] & zero[0]

    never = zero[0] != 0

    def held(v, z):
        if z is None:
            return v
        return jnp.where(never, pltpu.bitcast(z, v.dtype), v)

    def prep_chunk(j):
        def loader(m, z):
            seen = {}

            def pair(tr, cp):
                if (tr, cp) not in seen:
                    v = raw32[j, m * NTR + tr, cp * 8:cp * 8 + 8, :]
                    seen[tr, cp] = _up(held(v, z)).astype(f32)
                return seen[tr, cp]

            def load(row, c):
                h = slice((c % 2) * 8, (c % 2) * 8 + 8)
                return jnp.concatenate(
                    [pair(row // 8, c // 2)[h], pair(row // 8 + 1, c // 2)[h]], axis=0)
            return load
        for m in range(2):
            for s in range(8):
                def emit(i, v, m=m, s=s):
                    r = (m * 49 + i) * 128 + s * 16
                    wcb[j, r:r + 16, :] = v.astype(bf16)
                for o in range(7):
                    load = loader(m, (yield))
                    y = _outer_term(lambda k, c: load(k * 128 + s * 16, c), _RHS_SPEC, o)
                    _inner_terms(y, _rhs_terms, o, emit)
            for s in range(4):
                load = loader(m, (yield))
                e = [load(512 + s * 16, c) for c in range(4)]

                def emit_e(i, v, m=m, s=s):
                    web[j, m * 16 + i, s * 16:(s + 1) * 16, :] = v.astype(bf16)
                _ext_combos(e, _rhs_ext, emit_e)
        for s in range(9):
            def emit_d(i, v, s=s):
                r = i * MB + s * 16
                wdcb[j, r:r + 16, :] = v.astype(bf16)
            for o in range(7):
                load = loader(2, (yield))
                y = _outer_term(lambda r, k: load(r * MB + s * 16, k), _LHS_SPEC, o)
                _inner_terms(y, _lhs_terms, o, emit_d)

    def feed(gen, z, n):
        for _ in range(n):
            try:
                gen.send(z)
            except StopIteration:
                return

    def layer(li, carry):
        first = li == 0

        class Pace:
            def __init__(self):
                self.tok = 0
                self.plan = []
                self.due = []

            def add(self, gen, t0, period, count=1, lat=None):
                next(gen)
                self.plan.append((gen, t0, period, count, lat))

            def step(self, z):
                for gen, t0, period, count, lat in self.plan:
                    if self.tok >= t0 and (self.tok - t0) % period == 0:
                        for _ in range(count):
                            try:
                                v = gen.send(z)
                            except StopIteration:
                                break
                            if v is not None and lat is not None:
                                self.due.append((self.tok + lat, v))
                self.tok += 1

            def tokens(self, r, n):
                for k in range(n):
                    self.step(r[k * 16:k * 16 + 8])

            def gate(self, v):
                now = [x for t, x in self.due if t <= self.tok]
                self.due = [(t, x) for t, x in self.due if t > self.tok]
                if not now:
                    return v
                head = jnp.where(never, pltpu.bitcast(tree(now), u32), v[0:8])
                return jnp.concatenate([head, v[8:]], axis=0)

            def drain(self):
                for gen, *_ in self.plan:
                    feed(gen, None, 1000)

        def tree(vals):
            while len(vals) > 1:
                vals = [a + b for a, b in zip(vals[::2], vals[1::2])] + vals[len(vals) & ~1:]
            return vals[0]

        def norm_slab(src, p0, emit):
            def total(x):
                return tree([x[k * 8:(k + 1) * 8] for k in range(D // 8)])
            t = total(src[p0, 0:D, :])
            mu = jnp.sum(t, axis=0, keepdims=True) * (1.0 / D)
            xc = src[jnp.clip(p0 + after(t), 0, NSLAB - 1), 0:D, :] - mu
            t = total(xc * xc)
            rs = lax.rsqrt(jnp.sum(t, axis=0, keepdims=True) * (1.0 / D) + EPS)
            p = jnp.clip(p0 + after(t), 0, NSLAB - 1)
            ends = []
            for k in (4, 0, 1, 2, 3):
                y = ((src[p, k * 128:min((k + 1) * 128, D), :] - mu) * rs).T
                emit(k, y)
                ends.append(y[120:128] if k < 4 else jnp.concatenate([y[120:128]] * 2, axis=1))
            return tree(ends)

        def ln1(p, b):
            def emit(k, y):
                xnb[b, k, :, 0:y.shape[1]] = y.astype(bf16)
            return norm_slab(xa, p, emit)

        def widen(t):
            for r in range(4):
                c0 = pl.multiple_of(t * TILE + r * 128, 128)
                xa[t * 4 + r, 0:D, :] = xin[:, pl.ds(c0, 128)].astype(f32)

        def qkv_proj(b, pace):
            for grp in ((4, 5, 6, 7), (13, 0, 1, 2), (3, 12, 8, 9), (10, 11)):
                for n in grp:
                    qkv[b, n, HALO:HALO + 128, :] = lax.dot_general(
                        _up(xn[b, 4]), _up(wq[4, n * 64:(n + 1) * 64, :]), NT,
                        preferred_element_type=f32)
                for n in grp:
                    rows = slice(n * 64, (n + 1) * 64)
                    lhs = jnp.concatenate(
                        [_up(pace.gate(xn[b, 0]))] + [_up(xn[b, k]) for k in range(1, 4)], axis=1)
                    rhs = jnp.concatenate([_up(wq[k, rows, :]) for k in range(4)], axis=1)
                    r = lax.dot_general(lhs, rhs, NT, preferred_element_type=f32)
                    r = r + jnp.concatenate([qkv[b, n, HALO:HALO + 64, :],
                                             qkv[b, n, HALO + 64:HALO + 128, :]], axis=0)
                    if n in (4, 5, 6, 7, 13):
                        r = r * (DH ** -0.5 * LOG2E)
                    qkv[b, n, HALO:HALO + 128, :] = r
                    pace.tokens(r, 7)

        def halo(b):
            for n in range(4, 14):
                qkv[b, n, 0:HALO, :] = qkv[1 - b, n, 128:128 + HALO, :]

        def attend(b, row0):
            qs, ks, vs = (0, 1, 2, 3, 12), (4, 5, 6, 7, 13), (8, 9, 10, 11, 12)
            v = None
            for s in range(16 * OPT["att"]):
                z = yield v
                r = HALO + s * 8
                q = [held(qkv[b, n, r:r + 8, :], z if OPT["qtok"] else None) for n in qs]
                logit = []
                for w in range(WIN):
                    rw = r - DIL * w
                    part = tree([q[c] * qkv[b, ks[c], rw:rw + 8, :] for c in range(5)])
                    part = part + pltpu.roll(part, 64, 1)
                    part = part + pltpu.roll(part, 32, 1)
                    if row0 is not None and s * 8 < DIL * w:
                        pos = row0 + s * 8 + lax.broadcasted_iota(jnp.int32, (8, 128), 0)
                        part = jnp.where(pos >= DIL * w, part, -1e9 * LOG2E)
                    logit.append(part)
                mx = logit
                while len(mx) > 1:
                    mx = [jnp.maximum(a, c) for a, c in zip(mx[::2], mx[1::2])]
                e = [jnp.exp2(l - mx[0]) for l in logit]
                inv = 1.0 / tree(e)
                outs = []
                for c in range(5):
                    o = e[0] * qkv[b, vs[c], r:r + 8, :]
                    for w in range(1, WIN):
                        rw = r - DIL * w
                        o = o + e[w] * qkv[b, vs[c], rw:rw + 8, :]
                    o = o * inv
                    outs.append(o)
                    ob[b, c, s * 8:(s + 1) * 8, :] = o.astype(bf16)
                v = tree(outs)
            yield v

        def out_proj(p, b, pace):
            h = MB // 2
            for m in range(4):
                xb[p, m * MB:(m + 1) * MB, :] = xa[p, m * MB:(m + 1) * MB, :] + lax.dot_general(
                    _up(wo[4, m * h:(m + 1) * h, :]), _up(o32[b, 4]), NT, preferred_element_type=f32)
            rhs = jnp.concatenate([_up(o32[b, c]) for c in range(4)], axis=1)
            for m in range(4):
                rows = slice(m * h, (m + 1) * h)
                lhs = jnp.concatenate(
                    [_up(pace.gate(wo[0, rows, :]))] + [_up(wo[c, rows, :]) for c in range(1, 4)],
                    axis=1)
                r = lax.dot_general(lhs, rhs, NT, preferred_element_type=f32)
                r = r + jnp.concatenate([xb[p, m * MB:m * MB + h, :],
                                         xb[p, m * MB + h:(m + 1) * MB, :]], axis=0)
                xb[p, m * MB:(m + 1) * MB, :] = r
                pace.tokens(r, 8)

        def ffn_lhs(t):
            for r in range(4):
                def emit_n(k, y, r=r):
                    xn2[r * 5 + k, :, 0:y.shape[1]] = y
                norm_slab(xb, t * 4 + r, emit_n)
            for s in range(8):
                rows = slice(s * 16, (s + 1) * 16)
                a = [[xn2[r * 5 + k, rows, :] for k in range(4)] for r in range(4)]

                def emit(i, v, rows=rows):
                    acb[i, rows, :] = v.astype(bf16)
                _combos(a, _lhs_terms, emit)
                e = [xn2[r * 5 + 4, rows, 0:64] for r in range(4)]

                def emit_e(i, v, rows=rows):
                    aeb[i, rows, 0:64] = v.astype(bf16)
                _ext_combos(e, _lhs_ext, emit_e)

        @pl.when(first)
        def _():
            x_copy(0).wait()
            widen(0)
            for cp in chunk_copies(0):
                cp.wait()

        for n in range(4, 14):
            qkv[0, n, 0:HALO, :] = jnp.zeros((HALO, 128), f32)
        ln1(0, 0)
        pace = Pace()
        pace.add(prep_chunk(0), 0, 1, 2 * OPT["prep"])
        pace.due.append((OPT["hdue"], ln1(1, 1)))
        qkv_proj(0, pace)

        def attn_step(i, c):
            @pl.when(first)
            def _():
                for cp in chunk_copies(i + 1):
                    cp.wait()

            @pl.when(jnp.logical_and(first, jnp.logical_and(i % 2 == 1, i < 7)))
            def _():
                x_copy((i + 1) // 2).wait()
                widen((i + 1) // 2)

            side = prep_chunk(i + 1)
            next(side)
            for b in (1, 0):
                pace = Pace()
                if OPT["prep"]:
                    for t0 in (0, 1, 2):
                        pace.plan.append((side, t0, 4, 1, None))
                pace.due.append((OPT["ldue"], ln1(jnp.minimum(2 * i + 3 - b, NSLAB - 1), 1 - b)))
                pace.add(attend(1 - b, i * 256 if b == 1 else None),
                         OPT["a0"], OPT["aper"], 1, OPT["alat"])
                out_proj(jnp.maximum(2 * i - 1, 0) if b == 1 else 2 * i, b, pace)
                halo(b)
                qkv_proj(b, pace)
                pace.plan = pace.plan[-1:]
                pace.drain()
            if OPT["prep"]:
                feed(side, None, 1000)
            return c
        if not OPT["skip_attn"]:
            lax.fori_loop(0, NSLAB // 2, attn_step, 0)

        out_proj(NSLAB - 1, 1, Pace())
        ffn_lhs(0)

        def ffn_group(t, g, last):
            ti = _Temps(tin)
            to = _Temps(tout)

            def proj(c, m):
                j = g * 3 + c

                def prod(o, i):
                    r = (m * 49 + o * 7 + i) * 64
                    p = jnp.dot(_up(ac[o * 7 + i]), _up(wc[j, r:r + 64, :]),
                                preferred_element_type=f32)
                    if o in AUG and i in AUG:
                        q = AUG.index(o) * 4 + AUG.index(i)
                        p = p + jnp.dot(_up(ae[q, :, 0:64]), _up(we[j, m * 16 + q]),
                                        preferred_element_type=f32)
                    return p
                return prod

            def gate(c):
                def fin(r, cc, v):
                    gs[(c % 2) * 16 + r * 4 + cc] = v
                return _recombine(proj(c, 0), fin, ti, to)

            def upgate(c):
                def fin(r, cc, v):
                    hs[c, r * 4 + cc] = _ld(gs, (c % 2) * 16 + r * 4 + cc) * v
                yield from _recombine(proj(c, 1), fin, ti, to)
                for s in range(8):
                    rows = slice(s * 16, (s + 1) * 16)
                    b = [[hs[c, r * 4 + cc, rows, :] for r in range(4)] for cc in range(4)]

                    def emit(i, v, rows=rows):
                        hcb[c, i, rows, :] = v.astype(bf16)
                    _combos(b, _rhs_terms, emit)

            def dprod(cs, i):
                p = None
                for c in cs:
                    r = i * (MB // 2)
                    q = lax.dot_general(_up(wdc[g * 3 + c, r:r + MB // 2, :]), _up(hc[c, i]), NT,
                                        preferred_element_type=f32)
                    p = q if p is None else p + q
                return p

            def down(cs, reset):
                for i in range(49):
                    a = _ld(acc, i)
                    if reset:
                        a = jnp.where(g == 0, 0.0, a)
                    acc[i] = a + dprod(cs, i)
                    yield

            def down_final(cs):
                def fin(mb, r, v):
                    rows = slice(mb * MB, (mb + 1) * MB)
                    y = xb[t * 4 + r, rows, :] + v
                    xa[t * 4 + r, rows, :] = y
                    ost[t * 4 + r, rows, :] = y.astype(bf16)
                return _recombine(lambda o, i: _ld(acc, o * 7 + i) + dprod(cs, o * 7 + i),
                                  fin, _Temps(tin2), _Temps(tout2))

            for gen in (gate(0), upgate(0), gate(1)):
                _adv(gen, 100)
            d0 = down((0,), not last)
            for gen, plan in ((upgate(1), DN_PLAN["u1"]), (gate(2), DN_PLAN["g2"]),
                              (upgate(2), DN_PLAN["u2"])):
                for n in plan:
                    _adv(gen, 1)
                    _adv(d0, n)
                _adv(gen, 100)
            if last:
                ffn_lhs((t + 1) % NTILE)
            _adv(d0, 100)
            _adv(down_final((1, 2)) if last else down((1, 2), False), 100)

        def ffn_tile(t, c):
            def grp(g, c2):
                ffn_group(t, g, False)
                return c2
            lax.fori_loop(0, 2, grp, 0)
            ffn_group(t, 2, True)

            @pl.when(li == 1)
            def _():
                for r in range(4):
                    out_copy(t * 4 + r).start()
            return c
        if not OPT["skip_ffn"]:
            lax.fori_loop(0, NTILE, ffn_tile, 0)
        else:
            r0 = pl.multiple_of(zero[0] * 16, 16)
            ost[0, 0:16, :] = wcb[li, pl.ds(r0, 16), :] + wdcb[li, pl.ds(r0, 16), :] + web[li, li, 0:16, :]
            ost[1, 0:16, :] = acb[li, 0:16, :] + aeb[li, 0:16, :] + qkv[li, li, 0:16, :].astype(bf16)
            ost[2] = xb[li, 0:D, :].astype(bf16)
            for r in range(8):
                out_copy(li * 8 + r).start()
        return carry

    lax.fori_loop(0, 2, layer, 0)
    for p in range(NSLAB):
        out_copy(p).wait()


def _tiles(w):
    return w.reshape(NTR, 8, F // 128, 128).transpose(0, 2, 1, 3).reshape(NTR, F // 16, 128)


@jax.jit
def pallas_interleave_layers__sliding_local_dilated__glu_gated_bilinear__prompt_kernel(
    A_x: jax.Array,
    A_wqkv: jax.Array,
    A_wo: jax.Array,
    B_x: jax.Array,
    B_w_gate: jax.Array,
    B_w_up: jax.Array,
    B_w_down: jax.Array,
):
    del B_x
    vm = pltpu.VMEM
    hbm = pl.BlockSpec(memory_space=pl.ANY)
    out_t = pl.pallas_call(
        _kernel,
        in_specs=[hbm] * 6,
        out_specs=hbm,
        out_shape=jax.ShapeDtypeStruct((D, S), bf16),
        scratch_shapes=[
            vm((D, S), bf16),
            vm((NSLAB, 768, 128), f32),
            vm((NSLAB, 768, 128), f32),
            vm((NSLAB, D, 128), bf16),
            vm((D, 3 * D), bf16),
            vm((D, D), bf16),
            vm((5, 3 * D, 128), f32),
            vm((5, 1792, 128), bf16),
            vm((5, D, 128), bf16),
            vm((NCHUNK, 224, 32, 128), bf16),
            vm((NCHUNK, WC_ROWS, 128), bf16),
            vm((NCHUNK, 32, 64, 128), bf16),
            vm((NCHUNK, WD_ROWS, 128), bf16),
            vm((2, 5, 128, 128), bf16),
            vm((2, 14, HALO + 128, 128), f32),
            vm((2, 5, 128, 128), bf16),
            vm((20, 128, 128), f32),
            vm((49, 128, 128), bf16),
            vm((16, 128, 128), bf16),
            vm((32, 128, 128), f32),
            vm((3, 16, 128, 128), f32),
            vm((3, 49, 128, 128), bf16),
            vm((49, MB, 128), f32),
            vm((12, 128, 128), f32),
            vm((40, 128, 128), f32),
            vm((12, MB, 128), f32),
            vm((20, MB, 128), f32),
            pltpu.SMEM((1,), jnp.int32),
            pltpu.SemaphoreType.DMA((NTILE,)),
            pltpu.SemaphoreType.DMA((2,)),
            pltpu.SemaphoreType.DMA((NCHUNK, 3)),
            pltpu.SemaphoreType.DMA((NSLAB,)),
        ],
        compiler_params=pltpu.CompilerParams(vmem_limit_bytes=120 * 1024 * 1024),
    )(A_x[0].T, A_wqkv, A_wo, _tiles(B_w_gate), _tiles(B_w_up), _tiles(B_w_down.T))
    return out_t.T[None]
```

```python
import math

import jax
import jax.numpy as jnp
from jax import lax
import jax.experimental.pallas as pl
import jax.experimental.pallas.tpu as pltpu

f32 = jnp.float32
bf16 = jnp.bfloat16
u32 = jnp.uint32

S, D, F = 2048, 576, 4608
H, DH, WIN, DIL = 32, 18, 8, 2
EPS = 1e-5
LOG2E = math.log2(math.e)
NSLAB = S // 128
TILE = 512
NTILE = S // TILE
FC = 512
NCHUNK = F // FC
MB = D // 4
HALO = 16
NTR = D // 8
WC_ROWS = 800 * 16
WD_ROWS = 448 * 16
NT = (((1,), (1,)), ((), ()))
AUG = (0, 1, 2, 5)

OPT = dict(skip_ffn=False, hdue=40,
           p=dict(qtok=1, a0=0, aper=6, alat=35, ldue=32, pt=(0, 1, 2), pper=4),
           n=dict(qtok=1, a0=0, aper=6, alat=35, ldue=32))
DN_PLAN = dict(u1=(0, 0, 0, 0, 4, 4, 6), g2=(4, 0, 0, 0, 0, 0, 0), u2=(0, 0, 0, 0, 4, 4, 4))


def _up(v):
    return pltpu.bitcast(v, bf16)


def _quad(x):
    n = len(x) // 2
    return ([r[:n] for r in x[:n]], [r[n:] for r in x[:n]],
            [r[:n] for r in x[n:]], [r[n:] for r in x[n:]])


def _badd(x, y):
    return [[a + b for a, b in zip(r, s)] for r, s in zip(x, y)]


def _bsub(x, y):
    return [[a - b for a, b in zip(r, s)] for r, s in zip(x, y)]


def _lhs_terms(a):
    a11, a12, a21, a22 = _quad(a)
    return [lambda: _badd(a11, a22), lambda: _badd(a21, a22), lambda: a11, lambda: a22,
            lambda: _badd(a11, a12), lambda: _bsub(a21, a11), lambda: _bsub(a12, a22)]


def _rhs_terms(b):
    b11, b12, b21, b22 = _quad(b)
    return [lambda: _badd(b11, b22), lambda: b11, lambda: _bsub(b12, b22), lambda: _bsub(b21, b11),
            lambda: b22, lambda: _badd(b11, b12), lambda: _badd(b21, b22)]


def _combos(x, terms, emit):
    for o, fo in enumerate(terms(x)):
        y = fo()
        for i, fi in enumerate(terms(y)):
            emit(o * 7 + i, fi()[0][0])


_LHS_SPEC = (((0, 0), (1, 1), 1), ((1, 0), (1, 1), 1), ((0, 0), None, 0), ((1, 1), None, 0),
             ((0, 0), (0, 1), 1), ((1, 0), (0, 0), -1), ((0, 1), (1, 1), -1))
_RHS_SPEC = (((0, 0), (1, 1), 1), ((0, 0), None, 0), ((0, 1), (1, 1), -1), ((1, 0), (0, 0), -1),
             ((1, 1), None, 0), ((0, 0), (0, 1), 1), ((1, 0), (1, 1), 1))


def _outer_term(load, spec, o):
    p, q, sign = spec[o]
    out = []
    for y in range(2):
        row = []
        for z in range(2):
            v = load(2 * p[0] + y, 2 * p[1] + z)
            if sign:
                w = load(2 * q[0] + y, 2 * q[1] + z)
                v = v + w if sign > 0 else v - w
            row.append(v)
        out.append(row)
    return out


def _inner_terms(y, terms, o, emit):
    for i, fi in enumerate(terms(y)):
        emit(o * 7 + i, fi()[0][0])


def _lhs_ext(e):
    n = len(e) // 2
    return {0: e[:n], 1: e[n:], 2: e[:n], 5: [y - x for x, y in zip(e[:n], e[n:])]}


def _rhs_ext(e):
    n = len(e) // 2
    return {0: e[:n], 1: e[:n], 2: e[n:], 5: [x + y for x, y in zip(e[:n], e[n:])]}


def _ext_combos(e, fn, emit):
    for oi, o in enumerate(AUG):
        d = fn(fn(e)[o])
        for ii, i in enumerate(AUG):
            emit(oi * 4 + ii, d[i][0])


def _adv(gen, n):
    for _ in range(n):
        try:
            next(gen)
        except StopIteration:
            return


def _ld(ref, idx):
    n = ref.shape[-2] // 2
    return jnp.concatenate([ref[idx, :n, :], ref[idx, n:, :]], axis=0)


class _Temps:
    def __init__(self, ref):
        self.ref = ref
        self.n = 0

    def put(self, v):
        i = self.n % self.ref.shape[0]
        self.n += 1
        self.ref[i] = v
        return i

    def get(self, i):
        return _ld(self.ref, i)


def _recombine(prod, fin, ti, to):
    def inner(o, sink):
        a = ti.put(prod(o, 0))
        b = ti.put(prod(o, 1))
        c = ti.put(prod(o, 2))
        sink(1, 1, ti.get(a) - ti.get(b) + ti.get(c) + prod(o, 5))
        m3 = prod(o, 3)
        m4 = prod(o, 4)
        m6 = prod(o, 6)
        sink(1, 0, ti.get(b) + m3)
        sink(0, 1, ti.get(c) + m4)
        sink(0, 0, ti.get(a) + m3 - m4 + m6)

    m = {}
    for o in (0, 1, 2):
        def keep(y, z, v, o=o):
            m[o, y, z] = to.put(v)
        inner(o, keep)
        yield

    def s5(y, z, v):
        fin(2 + y, 2 + z, to.get(m[0, y, z]) - to.get(m[1, y, z]) + to.get(m[2, y, z]) + v)
    inner(5, s5)
    yield

    def s3(y, z, v):
        fin(2 + y, z, to.get(m[1, y, z]) + v)
        m[3, y, z] = to.put(to.get(m[0, y, z]) + v)
    inner(3, s3)
    yield

    def s4(y, z, v):
        fin(y, 2 + z, to.get(m[2, y, z]) + v)
        m[3, y, z] = to.put(to.get(m[3, y, z]) - v)
    inner(4, s4)
    yield

    def s6(y, z, v):
        fin(y, z, to.get(m[3, y, z]) + v)
    inner(6, s6)
    yield


def _kernel(xt_hbm, wqkv_hbm, wo_hbm, wg_hbm, wu_hbm, wdt_hbm, out_hbm,
            xin, xa, xb, ost, wq_raw, wo_raw, wtmp, wqb, wob, raw, wcb, web, wdcb,
            xnb, qkv, ob, xn2, acb, aeb, gs, hs, hcb, acc, tin, tout, tin2, tout2, zero,
            sem_x, sem_w, sem_c, sem_o):
    wq, wo, wc, we, wdc, xn, o32, ac, ae, hc, raw32 = [
        r.bitcast(u32) for r in (wqb, wob, wcb, web, wdcb, xnb, ob, acb, aeb, hcb, raw)]

    def x_copy(t):
        return pltpu.make_async_copy(
            xt_hbm.at[:, pl.ds(t * TILE, TILE)], xin.at[:, pl.ds(t * TILE, TILE)], sem_x.at[t])

    def chunk_copies(j):
        rows = pl.ds(pl.multiple_of(j * 32, 32), 32)
        return [pltpu.make_async_copy(src.at[:, rows, :], raw.at[j, pl.ds(m * NTR, NTR)],
                                      sem_c.at[j, m])
                for m, src in enumerate((wg_hbm, wu_hbm, wdt_hbm))]

    def out_copy(p):
        return pltpu.make_async_copy(
            ost.at[p], out_hbm.at[:, pl.ds(pl.multiple_of(p * 128, 128), 128)], sem_o.at[p])

    wq_copy = pltpu.make_async_copy(wqkv_hbm, wq_raw, sem_w.at[0])
    wo_copy = pltpu.make_async_copy(wo_hbm, wo_raw, sem_w.at[1])
    zero[0] = 0
    wq_copy.start()
    x_copy(0).start()
    wo_copy.start()
    wq_copy.wait()
    for cp in chunk_copies(0):
        cp.start()

    def wq_transpose(n, carry):
        c0 = pl.multiple_of(n * 128, 128)
        t = wq_raw[:, pl.ds(c0, 128)].astype(f32).T
        for k in range(4):
            wtmp[k, pl.ds(c0, 128), :] = t[:, k * 128:(k + 1) * 128]
        wtmp[4, pl.ds(c0, 128), 0:64] = t[:, 512:576]
        return carry
    lax.fori_loop(0, 13, wq_transpose, 0, unroll=True)
    t = wq_raw[:, 1664:1728].astype(f32).T
    for k in range(4):
        wtmp[k, 1664:1728, :] = t[:, k * 128:(k + 1) * 128]
    wtmp[4, 1664:1728, 0:64] = t[:, 512:576]
    for k in range(5):
        lanes = slice(0, 128) if k < 4 else slice(0, 64)
        for part in range(3):
            for d in range(DH):
                if d < 16:
                    row = part * 512 + d * 32
                else:
                    row = (1536, 1664, 1600)[part] + (d - 16) * 32
                wqb[k, row:row + 32, lanes] = wtmp[
                    k, pl.ds(part * D + d, H, stride=DH), lanes].astype(bf16)
        wqb[k, 1728:1792, lanes] = jnp.zeros((64, lanes.stop), bf16)
    wqb[4, :, 64:128] = jnp.zeros((1792, 64), bf16)
    xnb[:, 4, :, 64:128] = jnp.zeros((2, 128, 64), bf16)
    ob[1] = jnp.zeros((5, 128, 128), bf16)

    for j in range(1, 3):
        for cp in chunk_copies(j):
            cp.start()
    x_copy(1).start()

    wo_copy.wait()
    for n in range(5):
        w = 128 if n < 4 else 64
        wtmp[n, 0:D, 0:w] = wo_raw[:, n * 128:n * 128 + w].astype(f32)
    for n in range(5):
        w = 128 if n < 4 else 64
        for c in range(5):
            if c < 4:
                rows = [wtmp[n, pl.ds(4 * c + g, H, stride=DH), 0:w] for g in range(4)]
            else:
                rows = [jnp.zeros((64, w), f32)] + [
                    wtmp[n, pl.ds(16 + g, H, stride=DH), 0:w] for g in range(2)]
            wob[c, n * 128:n * 128 + w, :] = jnp.concatenate(rows, axis=0).T.astype(bf16)

    for j in range(3, NCHUNK):
        for cp in chunk_copies(j):
            cp.start()
        if j in (4, 6):
            x_copy(j // 2).start()

    def after(v, row=0):
        return lax.bitcast_convert_type(v[row:row + 1, 0:1], jnp.int32)[0, 0] & zero[0]

    never = zero[0] != 0

    def held(v, z):
        if z is None:
            return v
        return jnp.where(never, pltpu.bitcast(z, v.dtype), v)

    def prep_chunk(j):
        def loader(m, z):
            seen = {}

            def pair(tr, cp):
                if (tr, cp) not in seen:
                    v = raw32[j, m * NTR + tr, cp * 8:cp * 8 + 8, :]
                    seen[tr, cp] = _up(held(v, z)).astype(f32)
                return seen[tr, cp]

            def load(row, c):
                h = slice((c % 2) * 8, (c % 2) * 8 + 8)
                return jnp.concatenate(
                    [pair(row // 8, c // 2)[h], pair(row // 8 + 1, c // 2)[h]], axis=0)
            return load
        for m in range(2):
            for s in range(8):
                def emit(i, v, m=m, s=s):
                    r = (m * 49 + i) * 128 + s * 16
                    wcb[j, r:r + 16, :] = v.astype(bf16)
                for o in range(7):
                    load = loader(m, (yield))
                    y = _outer_term(lambda k, c: load(k * 128 + s * 16, c), _RHS_SPEC, o)
                    _inner_terms(y, _rhs_terms, o, emit)
            for s in range(4):
                load = loader(m, (yield))
                e = [load(512 + s * 16, c) for c in range(4)]

                def emit_e(i, v, m=m, s=s):
                    web[j, m * 16 + i, s * 16:(s + 1) * 16, :] = v.astype(bf16)
                _ext_combos(e, _rhs_ext, emit_e)
        for s in range(9):
            def emit_d(i, v, s=s):
                r = i * MB + s * 16
                wdcb[j, r:r + 16, :] = v.astype(bf16)
            for o in range(7):
                load = loader(2, (yield))
                y = _outer_term(lambda r, k: load(r * MB + s * 16, k), _LHS_SPEC, o)
                _inner_terms(y, _lhs_terms, o, emit_d)

    def feed(gen, z, n):
        for _ in range(n):
            try:
                gen.send(z)
            except StopIteration:
                return

    def layer(li, carry):
        first = li == 0

        class Pace:
            def __init__(self):
                self.tok = 0
                self.plan = []
                self.due = []

            def add(self, gen, t0, period, count=1, lat=None):
                next(gen)
                self.plan.append((gen, t0, period, count, lat))

            def step(self, z):
                for gen, t0, period, count, lat in self.plan:
                    if self.tok >= t0 and (self.tok - t0) % period == 0:
                        for _ in range(count):
                            try:
                                v = gen.send(z)
                            except StopIteration:
                                break
                            if v is not None and lat is not None:
                                self.due.append((self.tok + lat, v))
                self.tok += 1

            def tokens(self, r, n):
                for k in range(n):
                    self.step(r[k * 16:k * 16 + 8])

            def gate(self, v):
                now = [x for t, x in self.due if t <= self.tok]
                self.due = [(t, x) for t, x in self.due if t > self.tok]
                if not now:
                    return v
                head = jnp.where(never, pltpu.bitcast(tree(now), u32), v[0:8])
                return jnp.concatenate([head, v[8:]], axis=0)

            def drain(self):
                for gen, *_ in self.plan:
                    feed(gen, None, 1000)

        def tree(vals):
            while len(vals) > 1:
                vals = [a + b for a, b in zip(vals[::2], vals[1::2])] + vals[len(vals) & ~1:]
            return vals[0]

        def norm_slab(src, p0, emit):
            def total(x):
                return tree([x[k * 8:(k + 1) * 8] for k in range(D // 8)])
            t = total(src[p0, 0:D, :])
            mu = jnp.sum(t, axis=0, keepdims=True) * (1.0 / D)
            xc = src[jnp.clip(p0 + after(t), 0, NSLAB - 1), 0:D, :] - mu
            t = total(xc * xc)
            rs = lax.rsqrt(jnp.sum(t, axis=0, keepdims=True) * (1.0 / D) + EPS)
            p = jnp.clip(p0 + after(t), 0, NSLAB - 1)
            ends = []
            for k in (4, 0, 1, 2, 3):
                y = ((src[p, k * 128:min((k + 1) * 128, D), :] - mu) * rs).T
                emit(k, y)
                ends.append(y[120:128] if k < 4 else jnp.concatenate([y[120:128]] * 2, axis=1))
            return tree(ends)

        def ln1(p, b):
            def emit(k, y):
                xnb[b, k, :, 0:y.shape[1]] = y.astype(bf16)
            return norm_slab(xa, p, emit)

        def widen(t):
            for r in range(4):
                c0 = pl.multiple_of(t * TILE + r * 128, 128)
                xa[t * 4 + r, 0:D, :] = xin[:, pl.ds(c0, 128)].astype(f32)

        def qkv_proj(b, pace):
            for grp in ((4, 5, 6, 7), (13, 0, 1, 2), (3, 12, 8, 9), (10, 11)):
                for n in grp:
                    qkv[b, n, HALO:HALO + 128, :] = lax.dot_general(
                        _up(xn[b, 4]), _up(wq[4, n * 64:(n + 1) * 64, :]), NT,
                        preferred_element_type=f32)
                for n in grp:
                    rows = slice(n * 64, (n + 1) * 64)
                    lhs = jnp.concatenate(
                        [_up(pace.gate(xn[b, 0]))] + [_up(xn[b, k]) for k in range(1, 4)], axis=1)
                    rhs = jnp.concatenate([_up(wq[k, rows, :]) for k in range(4)], axis=1)
                    r = lax.dot_general(lhs, rhs, NT, preferred_element_type=f32)
                    r = r + jnp.concatenate([qkv[b, n, HALO:HALO + 64, :],
                                             qkv[b, n, HALO + 64:HALO + 128, :]], axis=0)
                    if n in (4, 5, 6, 7, 13):
                        r = r * (DH ** -0.5 * LOG2E)
                    qkv[b, n, HALO:HALO + 128, :] = r
                    pace.tokens(r, 7)

        def halo(b):
            for n in range(4, 14):
                qkv[b, n, 0:HALO, :] = qkv[1 - b, n, 128:128 + HALO, :]

        def attend(b, row0, qtok):
            qs, ks, vs = (0, 1, 2, 3, 12), (4, 5, 6, 7, 13), (8, 9, 10, 11, 12)
            v = None
            for s in range(16):
                z = yield v
                r = HALO + s * 8
                q = [held(qkv[b, n, r:r + 8, :], z if qtok else None) for n in qs]
                logit = []
                for w in range(WIN):
                    rw = r - DIL * w
                    part = tree([q[c] * qkv[b, ks[c], rw:rw + 8, :] for c in range(5)])
                    part = part + pltpu.roll(part, 64, 1)
                    part = part + pltpu.roll(part, 32, 1)
                    if row0 is not None and s * 8 < DIL * w:
                        pos = row0 + s * 8 + lax.broadcasted_iota(jnp.int32, (8, 128), 0)
                        part = jnp.where(pos >= DIL * w, part, -1e9 * LOG2E)
                    logit.append(part)
                mx = logit
                while len(mx) > 1:
                    mx = [jnp.maximum(a, c) for a, c in zip(mx[::2], mx[1::2])]
                e = [jnp.exp2(l - mx[0]) for l in logit]
                inv = 1.0 / tree(e)
                outs = []
                for c in range(5):
                    o = e[0] * qkv[b, vs[c], r:r + 8, :]
                    for w in range(1, WIN):
                        rw = r - DIL * w
                        o = o + e[w] * qkv[b, vs[c], rw:rw + 8, :]
                    o = o * inv
                    outs.append(o)
                    ob[b, c, s * 8:(s + 1) * 8, :] = o.astype(bf16)
                v = tree(outs)
            yield v

        def out_proj(p, b, pace):
            h = MB // 2
            for m in range(4):
                xb[p, m * MB:(m + 1) * MB, :] = xa[p, m * MB:(m + 1) * MB, :] + lax.dot_general(
                    _up(wo[4, m * h:(m + 1) * h, :]), _up(o32[b, 4]), NT, preferred_element_type=f32)
            rhs = jnp.concatenate([_up(o32[b, c]) for c in range(4)], axis=1)
            for m in range(4):
                rows = slice(m * h, (m + 1) * h)
                lhs = jnp.concatenate(
                    [_up(pace.gate(wo[0, rows, :]))] + [_up(wo[c, rows, :]) for c in range(1, 4)],
                    axis=1)
                r = lax.dot_general(lhs, rhs, NT, preferred_element_type=f32)
                r = r + jnp.concatenate([xb[p, m * MB:m * MB + h, :],
                                         xb[p, m * MB + h:(m + 1) * MB, :]], axis=0)
                xb[p, m * MB:(m + 1) * MB, :] = r
                pace.tokens(r, 8)

        def ffn_lhs(t):
            for r in range(4):
                def emit_n(k, y, r=r):
                    xn2[r * 5 + k, :, 0:y.shape[1]] = y
                norm_slab(xb, t * 4 + r, emit_n)
            for s in range(8):
                rows = slice(s * 16, (s + 1) * 16)
                a = [[xn2[r * 5 + k, rows, :] for k in range(4)] for r in range(4)]

                def emit(i, v, rows=rows):
                    acb[i, rows, :] = v.astype(bf16)
                _combos(a, _lhs_terms, emit)
                e = [xn2[r * 5 + 4, rows, 0:64] for r in range(4)]

                def emit_e(i, v, rows=rows):
                    aeb[i, rows, 0:64] = v.astype(bf16)
                _ext_combos(e, _lhs_ext, emit_e)

        @pl.when(first)
        def _():
            x_copy(0).wait()
            widen(0)
            for cp in chunk_copies(0):
                cp.wait()

        for n in range(4, 14):
            qkv[0, n, 0:HALO, :] = jnp.zeros((HALO, 128), f32)
        ln1(0, 0)
        pace = Pace()
        pace.add(prep_chunk(0), 0, 1, 2)
        pace.due.append((OPT["hdue"], ln1(1, 1)))
        qkv_proj(0, pace)

        def attn_step(i, prep):
            o = OPT["p"] if prep else OPT["n"]
            if prep:
                for cp in chunk_copies(i + 1):
                    cp.wait()

                @pl.when(jnp.logical_and(i % 2 == 1, i < 7))
                def _():
                    x_copy((i + 1) // 2).wait()
                    widen((i + 1) // 2)

                side = prep_chunk(i + 1)
                next(side)
            for b in (1, 0):
                pace = Pace()
                if prep:
                    for t0 in o["pt"]:
                        pace.plan.append((side, t0, o["pper"], 1, None))
                pace.due.append((o["ldue"], ln1(jnp.minimum(2 * i + 3 - b, NSLAB - 1), 1 - b)))
                pace.add(attend(1 - b, i * 256 if b == 1 else None, o["qtok"]),
                         o["a0"], o["aper"], 1, o["alat"])
                out_proj(jnp.maximum(2 * i - 1, 0) if b == 1 else 2 * i, b, pace)
                halo(b)
                qkv_proj(b, pace)
                pace.plan = pace.plan[-1:]
                pace.drain()
            if prep:
                feed(side, None, 1000)

        @pl.when(first)
        def _():
            pl.loop(0, NSLAB // 2)(lambda i: attn_step(i, True))

        @pl.when(li != 0)
        def _():
            pl.loop(0, NSLAB // 2)(lambda i: attn_step(i, False))

        out_proj(NSLAB - 1, 1, Pace())
        ffn_lhs(0)

        def ffn_group(t, g, last):
            ti = _Temps(tin)
            to = _Temps(tout)

            def proj(c, m):
                j = g * 3 + c

                def prod(o, i):
                    r = (m * 49 + o * 7 + i) * 64
                    p = jnp.dot(_up(ac[o * 7 + i]), _up(wc[j, r:r + 64, :]),
                                preferred_element_type=f32)
                    if o in AUG and i in AUG:
                        q = AUG.index(o) * 4 + AUG.index(i)
                        p = p + jnp.dot(_up(ae[q, :, 0:64]), _up(we[j, m * 16 + q]),
                                        preferred_element_type=f32)
                    return p
                return prod

            def gate(c):
                def fin(r, cc, v):
                    gs[(c % 2) * 16 + r * 4 + cc] = v
                return _recombine(proj(c, 0), fin, ti, to)

            def upgate(c):
                def fin(r, cc, v):
                    hs[c, r * 4 + cc] = _ld(gs, (c % 2) * 16 + r * 4 + cc) * v
                yield from _recombine(proj(c, 1), fin, ti, to)
                for s in range(8):
                    rows = slice(s * 16, (s + 1) * 16)
                    b = [[hs[c, r * 4 + cc, rows, :] for r in range(4)] for cc in range(4)]

                    def emit(i, v, rows=rows):
                        hcb[c, i, rows, :] = v.astype(bf16)
                    _combos(b, _rhs_terms, emit)

            def dprod(cs, i):
                p = None
                for c in cs:
                    r = i * (MB // 2)
                    q = lax.dot_general(_up(wdc[g * 3 + c, r:r + MB // 2, :]), _up(hc[c, i]), NT,
                                        preferred_element_type=f32)
                    p = q if p is None else p + q
                return p

            def down(cs, reset):
                for i in range(49):
                    a = _ld(acc, i)
                    if reset:
                        a = jnp.where(g == 0, 0.0, a)
                    acc[i] = a + dprod(cs, i)
                    yield

            def down_final(cs):
                def fin(mb, r, v):
                    rows = slice(mb * MB, (mb + 1) * MB)
                    y = xb[t * 4 + r, rows, :] + v
                    xa[t * 4 + r, rows, :] = y
                    ost[t * 4 + r, rows, :] = y.astype(bf16)
                return _recombine(lambda o, i: _ld(acc, o * 7 + i) + dprod(cs, o * 7 + i),
                                  fin, _Temps(tin2), _Temps(tout2))

            for gen in (gate(0), upgate(0), gate(1)):
                _adv(gen, 100)
            d0 = down((0,), not last)
            for gen, plan in ((upgate(1), DN_PLAN["u1"]), (gate(2), DN_PLAN["g2"]),
                              (upgate(2), DN_PLAN["u2"])):
                for n in plan:
                    _adv(gen, 1)
                    _adv(d0, n)
                _adv(gen, 100)
            if last:
                ffn_lhs((t + 1) % NTILE)
            _adv(d0, 100)
            _adv(down_final((1, 2)) if last else down((1, 2), False), 100)

        def ffn_tile(t, c):
            def grp(g, c2):
                ffn_group(t, g, False)
                return c2
            lax.fori_loop(0, 2, grp, 0)
            ffn_group(t, 2, True)

            @pl.when(li == 1)
            def _():
                for r in range(4):
                    out_copy(t * 4 + r).start()
            return c
        if not OPT["skip_ffn"]:
            lax.fori_loop(0, NTILE, ffn_tile, 0)
        else:
            r0 = pl.multiple_of(zero[0] * 16, 16)
            ost[0, 0:16, :] = wcb[li, pl.ds(r0, 16), :] + wdcb[li, pl.ds(r0, 16), :] + web[li, li, 0:16, :]
            ost[1, 0:16, :] = acb[li, 0:16, :] + aeb[li, 0:16, :] + qkv[li, li, 0:16, :].astype(bf16)
            ost[2] = xb[li, 0:D, :].astype(bf16)
            for r in range(8):
                out_copy(li * 8 + r).start()
        return carry

    lax.fori_loop(0, 2, layer, 0)
    for p in range(NSLAB):
        out_copy(p).wait()


def _tiles(w):
    return w.reshape(NTR, 8, F // 128, 128).transpose(0, 2, 1, 3).reshape(NTR, F // 16, 128)


@jax.jit
def pallas_interleave_layers__sliding_local_dilated__glu_gated_bilinear__prompt_kernel(
    A_x: jax.Array,
    A_wqkv: jax.Array,
    A_wo: jax.Array,
    B_x: jax.Array,
    B_w_gate: jax.Array,
    B_w_up: jax.Array,
    B_w_down: jax.Array,
):
    del B_x
    vm = pltpu.VMEM
    hbm = pl.BlockSpec(memory_space=pl.ANY)
    out_t = pl.pallas_call(
        _kernel,
        in_specs=[hbm] * 6,
        out_specs=hbm,
        out_shape=jax.ShapeDtypeStruct((D, S), bf16),
        scratch_shapes=[
            vm((D, S), bf16),
            vm((NSLAB, 768, 128), f32),
            vm((NSLAB, 768, 128), f32),
            vm((NSLAB, D, 128), bf16),
            vm((D, 3 * D), bf16),
            vm((D, D), bf16),
            vm((5, 3 * D, 128), f32),
            vm((5, 1792, 128), bf16),
            vm((5, D, 128), bf16),
            vm((NCHUNK, 224, 32, 128), bf16),
            vm((NCHUNK, WC_ROWS, 128), bf16),
            vm((NCHUNK, 32, 64, 128), bf16),
            vm((NCHUNK, WD_ROWS, 128), bf16),
            vm((2, 5, 128, 128), bf16),
            vm((2, 14, HALO + 128, 128), f32),
            vm((2, 5, 128, 128), bf16),
            vm((20, 128, 128), f32),
            vm((49, 128, 128), bf16),
            vm((16, 128, 128), bf16),
            vm((32, 128, 128), f32),
            vm((3, 16, 128, 128), f32),
            vm((3, 49, 128, 128), bf16),
            vm((49, MB, 128), f32),
            vm((12, 128, 128), f32),
            vm((40, 128, 128), f32),
            vm((12, MB, 128), f32),
            vm((20, MB, 128), f32),
            pltpu.SMEM((1,), jnp.int32),
            pltpu.SemaphoreType.DMA((NTILE,)),
            pltpu.SemaphoreType.DMA((2,)),
            pltpu.SemaphoreType.DMA((NCHUNK, 3)),
            pltpu.SemaphoreType.DMA((NSLAB,)),
        ],
        compiler_params=pltpu.CompilerParams(vmem_limit_bytes=120 * 1024 * 1024),
    )(A_x[0].T, A_wqkv, A_wo, _tiles(B_w_gate), _tiles(B_w_up), _tiles(B_w_down.T))
    return out_t.T[None]
```

```python
import math

import jax
import jax.numpy as jnp
from jax import lax
import jax.experimental.pallas as pl
import jax.experimental.pallas.tpu as pltpu

f32 = jnp.float32
bf16 = jnp.bfloat16
u32 = jnp.uint32

S, D, F = 2048, 576, 4608
H, DH, WIN, DIL = 32, 18, 8, 2
EPS = 1e-5
LOG2E = math.log2(math.e)
NSLAB = S // 128
TILE = 512
NTILE = S // TILE
FC = 512
NCHUNK = F // FC
MB = D // 4
HALO = 16
NTR = D // 8
WC_ROWS = 800 * 16
WD_ROWS = 448 * 16
NT = (((1,), (1,)), ((), ()))
ORDER = (0, 1, 2, 5, 3, 4, 6)
AUG = (0, 1, 2, 5)

OPT = dict(skip_ffn=False, hdue=40,
           f=dict(h=((0, 1, 1), (0, 1, 1), (0, 1, 1)), n0=0, nper=2, l0=0, lper=2),
           p=dict(qtok=1, a0=0, aper=6, alat=35, ldue=32, pt=(0, 1, 2), pper=4),
           n=dict(qtok=1, a0=0, aper=6, alat=35, ldue=32))
DN_PLAN = dict(u1=(0, 0, 0, 0, 4, 4, 6), g2=(4, 0, 0, 0, 0, 0, 0), u2=(0, 0, 0, 0, 4, 4, 4))


def _up(v):
    return pltpu.bitcast(v, bf16)


def _quad(x):
    n = len(x) // 2
    return ([r[:n] for r in x[:n]], [r[n:] for r in x[:n]],
            [r[:n] for r in x[n:]], [r[n:] for r in x[n:]])


def _badd(x, y):
    return [[a + b for a, b in zip(r, s)] for r, s in zip(x, y)]


def _bsub(x, y):
    return [[a - b for a, b in zip(r, s)] for r, s in zip(x, y)]


def _lhs_terms(a):
    a11, a12, a21, a22 = _quad(a)
    return [lambda: _badd(a11, a22), lambda: _badd(a21, a22), lambda: a11, lambda: a22,
            lambda: _badd(a11, a12), lambda: _bsub(a21, a11), lambda: _bsub(a12, a22)]


def _rhs_terms(b):
    b11, b12, b21, b22 = _quad(b)
    return [lambda: _badd(b11, b22), lambda: b11, lambda: _bsub(b12, b22), lambda: _bsub(b21, b11),
            lambda: b22, lambda: _badd(b11, b12), lambda: _badd(b21, b22)]


def _combos(x, terms, emit):
    for o, fo in enumerate(terms(x)):
        y = fo()
        for i, fi in enumerate(terms(y)):
            emit(o * 7 + i, fi()[0][0])


_LHS_SPEC = (((0, 0), (1, 1), 1), ((1, 0), (1, 1), 1), ((0, 0), None, 0), ((1, 1), None, 0),
             ((0, 0), (0, 1), 1), ((1, 0), (0, 0), -1), ((0, 1), (1, 1), -1))
_RHS_SPEC = (((0, 0), (1, 1), 1), ((0, 0), None, 0), ((0, 1), (1, 1), -1), ((1, 0), (0, 0), -1),
             ((1, 1), None, 0), ((0, 0), (0, 1), 1), ((1, 0), (1, 1), 1))


def _outer_term(load, spec, o):
    p, q, sign = spec[o]
    out = []
    for y in range(2):
        row = []
        for z in range(2):
            v = load(2 * p[0] + y, 2 * p[1] + z)
            if sign:
                w = load(2 * q[0] + y, 2 * q[1] + z)
                v = v + w if sign > 0 else v - w
            row.append(v)
        out.append(row)
    return out


def _inner_terms(y, terms, o, emit):
    for i, fi in enumerate(terms(y)):
        emit(o * 7 + i, fi()[0][0])


def _lhs_ext(e):
    n = len(e) // 2
    return {0: e[:n], 1: e[n:], 2: e[:n], 5: [y - x for x, y in zip(e[:n], e[n:])]}


def _rhs_ext(e):
    n = len(e) // 2
    return {0: e[:n], 1: e[:n], 2: e[n:], 5: [x + y for x, y in zip(e[:n], e[n:])]}


def _ext_combos(e, fn, emit):
    for oi, o in enumerate(AUG):
        d = fn(fn(e)[o])
        for ii, i in enumerate(AUG):
            emit(oi * 4 + ii, d[i][0])


def _adv(gen, n):
    for _ in range(n):
        try:
            next(gen)
        except StopIteration:
            return


def _ld(ref, idx):
    n = ref.shape[-2] // 2
    return jnp.concatenate([ref[idx, :n, :], ref[idx, n:, :]], axis=0)


class _Temps:
    def __init__(self, ref):
        self.ref = ref
        self.n = 0

    def put(self, v):
        i = self.n % self.ref.shape[0]
        self.n += 1
        self.ref[i] = v
        return i

    def get(self, i):
        return _ld(self.ref, i)


def _recombine(prod, fin, ti, to):
    def inner(o, sink):
        a = ti.put(prod(o, 0))
        b = ti.put(prod(o, 1))
        c = ti.put(prod(o, 2))
        sink(1, 1, ti.get(a) - ti.get(b) + ti.get(c) + prod(o, 5))
        m3 = prod(o, 3)
        m4 = prod(o, 4)
        m6 = prod(o, 6)
        sink(1, 0, ti.get(b) + m3)
        sink(0, 1, ti.get(c) + m4)
        sink(0, 0, ti.get(a) + m3 - m4 + m6)

    m = {}
    for o in (0, 1, 2):
        def keep(y, z, v, o=o):
            m[o, y, z] = to.put(v)
        inner(o, keep)
        yield

    def s5(y, z, v):
        fin(2 + y, 2 + z, to.get(m[0, y, z]) - to.get(m[1, y, z]) + to.get(m[2, y, z]) + v)
    inner(5, s5)
    yield

    def s3(y, z, v):
        fin(2 + y, z, to.get(m[1, y, z]) + v)
        m[3, y, z] = to.put(to.get(m[0, y, z]) + v)
    inner(3, s3)
    yield

    def s4(y, z, v):
        fin(y, 2 + z, to.get(m[2, y, z]) + v)
        m[3, y, z] = to.put(to.get(m[3, y, z]) - v)
    inner(4, s4)
    yield

    def s6(y, z, v):
        fin(y, z, to.get(m[3, y, z]) + v)
    inner(6, s6)
    yield


def _kernel(xt_hbm, wqkv_hbm, wo_hbm, wg_hbm, wu_hbm, wdt_hbm, out_hbm,
            xin, xa, xb, ost, wq_raw, wo_raw, wtmp, wqb, wob, raw, wcb, web, wdcb,
            xnb, qkv, ob, xn2, acb, aeb, gs, hs, hcb, acc, tin, tout, tin2, tout2, zero,
            sem_x, sem_w, sem_c, sem_o):
    wq, wo, wc, we, wdc, xn, o32, ac, ae, hc, raw32 = [
        r.bitcast(u32) for r in (wqb, wob, wcb, web, wdcb, xnb, ob, acb, aeb, hcb, raw)]

    def x_copy(t):
        return pltpu.make_async_copy(
            xt_hbm.at[:, pl.ds(t * TILE, TILE)], xin.at[:, pl.ds(t * TILE, TILE)], sem_x.at[t])

    def chunk_copies(j):
        rows = pl.ds(pl.multiple_of(j * 32, 32), 32)
        return [pltpu.make_async_copy(src.at[:, rows, :], raw.at[j, pl.ds(m * NTR, NTR)],
                                      sem_c.at[j, m])
                for m, src in enumerate((wg_hbm, wu_hbm, wdt_hbm))]

    def out_copy(p):
        return pltpu.make_async_copy(
            ost.at[p], out_hbm.at[:, pl.ds(pl.multiple_of(p * 128, 128), 128)], sem_o.at[p])

    wq_copy = pltpu.make_async_copy(wqkv_hbm, wq_raw, sem_w.at[0])
    wo_copy = pltpu.make_async_copy(wo_hbm, wo_raw, sem_w.at[1])
    zero[0] = 0
    wq_copy.start()
    x_copy(0).start()
    wo_copy.start()
    wq_copy.wait()
    for cp in chunk_copies(0):
        cp.start()

    def wq_transpose(n, carry):
        c0 = pl.multiple_of(n * 128, 128)
        t = wq_raw[:, pl.ds(c0, 128)].astype(f32).T
        for k in range(4):
            wtmp[k, pl.ds(c0, 128), :] = t[:, k * 128:(k + 1) * 128]
        wtmp[4, pl.ds(c0, 128), 0:64] = t[:, 512:576]
        return carry
    lax.fori_loop(0, 13, wq_transpose, 0, unroll=True)
    t = wq_raw[:, 1664:1728].astype(f32).T
    for k in range(4):
        wtmp[k, 1664:1728, :] = t[:, k * 128:(k + 1) * 128]
    wtmp[4, 1664:1728, 0:64] = t[:, 512:576]
    for k in range(5):
        lanes = slice(0, 128) if k < 4 else slice(0, 64)
        for part in range(3):
            for d in range(DH):
                if d < 16:
                    row = part * 512 + d * 32
                else:
                    row = (1536, 1664, 1600)[part] + (d - 16) * 32
                wqb[k, row:row + 32, lanes] = wtmp[
                    k, pl.ds(part * D + d, H, stride=DH), lanes].astype(bf16)
        wqb[k, 1728:1792, lanes] = jnp.zeros((64, lanes.stop), bf16)
    wqb[4, :, 64:128] = jnp.zeros((1792, 64), bf16)
    xnb[:, 4, :, 64:128] = jnp.zeros((2, 128, 64), bf16)
    ob[1] = jnp.zeros((5, 128, 128), bf16)

    for j in range(1, 3):
        for cp in chunk_copies(j):
            cp.start()
    x_copy(1).start()

    wo_copy.wait()
    for n in range(5):
        w = 128 if n < 4 else 64
        wtmp[n, 0:D, 0:w] = wo_raw[:, n * 128:n * 128 + w].astype(f32)
    for n in range(5):
        w = 128 if n < 4 else 64
        for c in range(5):
            if c < 4:
                rows = [wtmp[n, pl.ds(4 * c + g, H, stride=DH), 0:w] for g in range(4)]
            else:
                rows = [jnp.zeros((64, w), f32)] + [
                    wtmp[n, pl.ds(16 + g, H, stride=DH), 0:w] for g in range(2)]
            wob[c, n * 128:n * 128 + w, :] = jnp.concatenate(rows, axis=0).T.astype(bf16)

    for j in range(3, NCHUNK):
        for cp in chunk_copies(j):
            cp.start()
        if j in (4, 6):
            x_copy(j // 2).start()

    never = zero[0] != 0

    def held(v, z):
        if z is None:
            return v
        return jnp.where(never, pltpu.bitcast(z, v.dtype), v)

    def prep_chunk(j):
        def loader(m, z):
            seen = {}

            def pair(tr, cp):
                if (tr, cp) not in seen:
                    v = raw32[j, m * NTR + tr, cp * 8:cp * 8 + 8, :]
                    seen[tr, cp] = _up(held(v, z)).astype(f32)
                return seen[tr, cp]

            def load(row, c):
                h = slice((c % 2) * 8, (c % 2) * 8 + 8)
                return jnp.concatenate(
                    [pair(row // 8, c // 2)[h], pair(row // 8 + 1, c // 2)[h]], axis=0)
            return load
        for m in range(2):
            for s in range(8):
                def emit(i, v, m=m, s=s):
                    r = (m * 49 + i) * 128 + s * 16
                    wcb[j, r:r + 16, :] = v.astype(bf16)
                for o in range(7):
                    load = loader(m, (yield))
                    y = _outer_term(lambda k, c: load(k * 128 + s * 16, c), _RHS_SPEC, o)
                    _inner_terms(y, _rhs_terms, o, emit)
            for s in range(4):
                load = loader(m, (yield))
                e = [load(512 + s * 16, c) for c in range(4)]

                def emit_e(i, v, m=m, s=s):
                    web[j, m * 16 + i, s * 16:(s + 1) * 16, :] = v.astype(bf16)
                _ext_combos(e, _rhs_ext, emit_e)
        for s in range(9):
            def emit_d(i, v, s=s):
                r = i * MB + s * 16
                wdcb[j, r:r + 16, :] = v.astype(bf16)
            for o in range(7):
                load = loader(2, (yield))
                y = _outer_term(lambda r, k: load(r * MB + s * 16, k), _LHS_SPEC, o)
                _inner_terms(y, _lhs_terms, o, emit_d)

    def feed(gen, z, n):
        for _ in range(n):
            try:
                gen.send(z)
            except StopIteration:
                return

    def layer(li, carry):
        first = li == 0

        class Pace:
            def __init__(self):
                self.tok = 0
                self.plan = []
                self.due = []

            def add(self, gen, t0, period, count=1, lat=None):
                next(gen)
                self.plan.append((gen, t0, period, count, lat))

            def step(self, z):
                for gen, t0, period, count, lat in self.plan:
                    if self.tok >= t0 and (self.tok - t0) % period == 0:
                        for _ in range(count):
                            try:
                                v = gen.send(z)
                            except StopIteration:
                                break
                            if v is not None and lat is not None:
                                self.due.append((self.tok + lat, v))
                self.tok += 1

            def tokens(self, r, n):
                for k in range(n):
                    self.step(r[k * 16:k * 16 + 8])

            def gate(self, v):
                now = [x for t, x in self.due if t <= self.tok]
                self.due = [(t, x) for t, x in self.due if t > self.tok]
                if not now:
                    return v
                head = jnp.where(never, pltpu.bitcast(tree(now), u32), v[0:8])
                return jnp.concatenate([head, v[8:]], axis=0)

            def drain(self):
                for gen, *_ in self.plan:
                    feed(gen, None, 1000)

        def tree(vals):
            while len(vals) > 1:
                vals = [a + b for a, b in zip(vals[::2], vals[1::2])] + vals[len(vals) & ~1:]
            return vals[0]

        def norm_slab(src, p0, emit):
            def rows(p, lo, hi):
                return [src[p, r:r + 8, :] for r in range(lo, hi, 8)]

            def mean(vals):
                t = tree([sum(vals[k + 4::4], vals[k]) for k in range(4)])
                t = jnp.sum(t, axis=0, keepdims=True) * (1.0 / D)
                return jnp.broadcast_to(t, (8, 128))
            p1, p2 = [jnp.clip(p0 + k * zero[0], 0, NSLAB - 1) for k in (1, 2)]
            z = yield
            x = rows(p0, 0, D)
            mu = mean([held(v, z) for v in x[:4]] + x[4:])
            m = held(mu, (yield))
            rs = lax.rsqrt(mean([(v - m) * (v - m) for v in rows(p1, 0, D)]) + EPS)
            end = None
            for k in (4, 0, 1, 2, 3):
                m = held(mu, (yield end))
                y = jnp.concatenate(
                    [(v - m) * rs for v in rows(p2, k * 128, min((k + 1) * 128, D))], axis=0).T
                emit(k, y)
                end = y[120:128] if k < 4 else jnp.concatenate([y[120:128]] * 2, axis=1)
            yield end

        def flush(gen):
            return tree([v for v in gen if v is not None])

        def ln1(p, b):
            def emit(k, y):
                xnb[b, k, :, 0:y.shape[1]] = y.astype(bf16)
            return flush(norm_slab(xa, p, emit))

        def widen(t):
            for r in range(4):
                c0 = pl.multiple_of(t * TILE + r * 128, 128)
                xa[t * 4 + r, 0:D, :] = xin[:, pl.ds(c0, 128)].astype(f32)

        def qkv_proj(b, pace):
            for grp in ((4, 5, 6, 7), (13, 0, 1, 2), (3, 12, 8, 9), (10, 11)):
                for n in grp:
                    qkv[b, n, HALO:HALO + 128, :] = lax.dot_general(
                        _up(xn[b, 4]), _up(wq[4, n * 64:(n + 1) * 64, :]), NT,
                        preferred_element_type=f32)
                for n in grp:
                    rows = slice(n * 64, (n + 1) * 64)
                    lhs = jnp.concatenate(
                        [_up(pace.gate(xn[b, 0]))] + [_up(xn[b, k]) for k in range(1, 4)], axis=1)
                    rhs = jnp.concatenate([_up(wq[k, rows, :]) for k in range(4)], axis=1)
                    r = lax.dot_general(lhs, rhs, NT, preferred_element_type=f32)
                    r = r + jnp.concatenate([qkv[b, n, HALO:HALO + 64, :],
                                             qkv[b, n, HALO + 64:HALO + 128, :]], axis=0)
                    if n in (4, 5, 6, 7, 13):
                        r = r * (DH ** -0.5 * LOG2E)
                    qkv[b, n, HALO:HALO + 128, :] = r
                    pace.tokens(r, 7)

        def halo(b):
            for n in range(4, 14):
                qkv[b, n, 0:HALO, :] = qkv[1 - b, n, 128:128 + HALO, :]

        def attend(b, row0, qtok):
            qs, ks, vs = (0, 1, 2, 3, 12), (4, 5, 6, 7, 13), (8, 9, 10, 11, 12)
            v = None
            for s in range(16):
                z = yield v
                r = HALO + s * 8
                q = [held(qkv[b, n, r:r + 8, :], z if qtok else None) for n in qs]
                logit = []
                for w in range(WIN):
                    rw = r - DIL * w
                    part = tree([q[c] * qkv[b, ks[c], rw:rw + 8, :] for c in range(5)])
                    part = part + pltpu.roll(part, 64, 1)
                    part = part + pltpu.roll(part, 32, 1)
                    if row0 is not None and s * 8 < DIL * w:
                        pos = row0 + s * 8 + lax.broadcasted_iota(jnp.int32, (8, 128), 0)
                        part = jnp.where(pos >= DIL * w, part, -1e9 * LOG2E)
                    logit.append(part)
                mx = logit
                while len(mx) > 1:
                    mx = [jnp.maximum(a, c) for a, c in zip(mx[::2], mx[1::2])]
                e = [jnp.exp2(l - mx[0]) for l in logit]
                inv = 1.0 / tree(e)
                outs = []
                for c in range(5):
                    o = e[0] * qkv[b, vs[c], r:r + 8, :]
                    for w in range(1, WIN):
                        rw = r - DIL * w
                        o = o + e[w] * qkv[b, vs[c], rw:rw + 8, :]
                    o = o * inv
                    outs.append(o)
                    ob[b, c, s * 8:(s + 1) * 8, :] = o.astype(bf16)
                v = tree(outs)
            yield v

        def out_proj(p, b, pace):
            h = MB // 2
            for m in range(4):
                xb[p, m * MB:(m + 1) * MB, :] = xa[p, m * MB:(m + 1) * MB, :] + lax.dot_general(
                    _up(wo[4, m * h:(m + 1) * h, :]), _up(o32[b, 4]), NT, preferred_element_type=f32)
            rhs = jnp.concatenate([_up(o32[b, c]) for c in range(4)], axis=1)
            for m in range(4):
                rows = slice(m * h, (m + 1) * h)
                lhs = jnp.concatenate(
                    [_up(pace.gate(wo[0, rows, :]))] + [_up(wo[c, rows, :]) for c in range(1, 4)],
                    axis=1)
                r = lax.dot_general(lhs, rhs, NT, preferred_element_type=f32)
                r = r + jnp.concatenate([xb[p, m * MB:m * MB + h, :],
                                         xb[p, m * MB + h:(m + 1) * MB, :]], axis=0)
                xb[p, m * MB:(m + 1) * MB, :] = r
                pace.tokens(r, 8)

        def ffn_norm(t):
            for r in range(4):
                def emit_n(k, y, r=r):
                    xn2[r * 5 + k, :, 0:y.shape[1]] = y
                yield from norm_slab(xb, t * 4 + r, emit_n)

        def strips(load, spec, terms, o, dst):
            for s in range(8):
                z = yield
                rows = slice(s * 16, (s + 1) * 16)

                def ld(r, c):
                    v = load(r, c, rows)
                    if (r // 2, c // 2) == spec[o][0]:
                        v = jnp.concatenate([held(v[0:8], z), held(v[8:16], z)], axis=0)
                    return v

                def emit(i, v):
                    dst[i, rows, :] = v.astype(bf16)
                _inner_terms(_outer_term(ld, spec, o), terms, o, emit)

        def lhs_strips(o):
            yield from strips(lambda r, k, rows: xn2[r * 5 + k, rows, :],
                              _LHS_SPEC, _lhs_terms, o, acb)
            if o in AUG:
                for s in range(2):
                    z = yield
                    rows = slice(s * 64, (s + 1) * 64)
                    d = _lhs_ext(_lhs_ext([xn2[r * 5 + 4, rows, 0:64] for r in range(4)])[o])
                    for ii, i in enumerate(AUG):
                        aeb[AUG.index(o) * 4 + ii, rows, 0:64] = d[i][0].astype(bf16)

        def ffn_lhs(t):
            flush(ffn_norm(t))
            for s in range(8):
                rows = slice(s * 16, (s + 1) * 16)
                a = [[xn2[r * 5 + k, rows, :] for k in range(4)] for r in range(4)]

                def emit(i, v, rows=rows):
                    acb[i, rows, :] = v.astype(bf16)
                _combos(a, _lhs_terms, emit)
                e = [xn2[r * 5 + 4, rows, 0:64] for r in range(4)]

                def emit_e(i, v, rows=rows):
                    aeb[i, rows, 0:64] = v.astype(bf16)
                _ext_combos(e, _lhs_ext, emit_e)

        @pl.when(first)
        def _():
            x_copy(0).wait()
            widen(0)
            for cp in chunk_copies(0):
                cp.wait()

        for n in range(4, 14):
            qkv[0, n, 0:HALO, :] = jnp.zeros((HALO, 128), f32)
        ln1(0, 0)
        pace = Pace()
        pace.add(prep_chunk(0), 0, 1, 2)
        pace.due.append((OPT["hdue"], ln1(1, 1)))
        qkv_proj(0, pace)

        def attn_step(i, prep):
            o = OPT["p"] if prep else OPT["n"]
            if prep:
                for cp in chunk_copies(i + 1):
                    cp.wait()

                @pl.when(jnp.logical_and(i % 2 == 1, i < 7))
                def _():
                    x_copy((i + 1) // 2).wait()
                    widen((i + 1) // 2)

                side = prep_chunk(i + 1)
                next(side)
            for b in (1, 0):
                pace = Pace()
                if prep:
                    for t0 in o["pt"]:
                        pace.plan.append((side, t0, o["pper"], 1, None))
                pace.due.append((o["ldue"], ln1(jnp.minimum(2 * i + 3 - b, NSLAB - 1), 1 - b)))
                pace.add(attend(1 - b, i * 256 if b == 1 else None, o["qtok"]),
                         o["a0"], o["aper"], 1, o["alat"])
                out_proj(jnp.maximum(2 * i - 1, 0) if b == 1 else 2 * i, b, pace)
                halo(b)
                qkv_proj(b, pace)
                pace.plan = pace.plan[-1:]
                pace.drain()
            if prep:
                feed(side, None, 1000)

        @pl.when(first)
        def _():
            pl.loop(0, NSLAB // 2)(lambda i: attn_step(i, True))

        @pl.when(li != 0)
        def _():
            pl.loop(0, NSLAB // 2)(lambda i: attn_step(i, False))

        out_proj(NSLAB - 1, 1, Pace())
        ffn_lhs(0)

        def ffn_group(t, g, last):
            ti = _Temps(tin)
            to = _Temps(tout)
            pace = Pace()
            o_ = OPT["f"]

            def chain(gens):
                yield
                for gen in gens:
                    next(gen)
                    z = None
                    while True:
                        z = yield
                        try:
                            gen.send(z)
                        except StopIteration:
                            break

            def proj(c, m):
                j = g * 3 + c

                def prod(o, i):
                    r = (m * 49 + o * 7 + i) * 64
                    p = jnp.dot(_up(ac[o * 7 + i]), _up(wc[j, r:r + 64, :]),
                                preferred_element_type=f32)
                    pace.step(p[0:8])
                    if o in AUG and i in AUG:
                        q = AUG.index(o) * 4 + AUG.index(i)
                        e = jnp.dot(_up(ae[q, :, 0:64]), _up(we[j, m * 16 + q]),
                                    preferred_element_type=f32)
                        pace.step(e[0:8])
                        p = p + e
                    return p
                return prod

            def gate(c):
                def fin(r, cc, v):
                    gs[(c % 2) * 16 + r * 4 + cc] = v
                return _recombine(proj(c, 0), fin, ti, to)

            def upgate(c):
                def fin(r, cc, v):
                    hs[c, r * 4 + cc] = _ld(gs, (c % 2) * 16 + r * 4 + cc) * v
                yield from _recombine(proj(c, 1), fin, ti, to)
                t0, per, cnt = o_["h"][c]
                hgen[c] = chain([strips(lambda cc, r, rows: hs[c, r * 4 + cc, rows, :],
                                        _RHS_SPEC, _rhs_terms, o, hcb.at[c]) for o in ORDER])
                hdone[c] = 0
                pace.add(counted(c), pace.tok + t0, per, cnt)

            hgen, hdone = {}, {}

            def counted(c):
                next(hgen[c])
                next(hgen[c])
                while True:
                    z = yield
                    if hdone[c] < 56:
                        need(c, hdone[c] + 1, z)

            def need(c, n, z=None):
                while hdone[c] < n:
                    hdone[c] += 1
                    feed(hgen[c], z, 1)

            def dprod(cs, i):
                p = None
                for c in cs:
                    need(c, 8 * (ORDER.index(i // 7) + 1))
                    r = i * (MB // 2)
                    q = lax.dot_general(_up(wdc[g * 3 + c, r:r + MB // 2, :]), _up(hc[c, i]), NT,
                                        preferred_element_type=f32)
                    pace.step(q[0:8])
                    p = q if p is None else p + q
                return p

            def down(cs, reset):
                for i in [o * 7 + k for o in ORDER for k in range(7)]:
                    a = _ld(acc, i)
                    if reset:
                        a = jnp.where(g == 0, 0.0, a)
                    acc[i] = a + dprod(cs, i)
                    yield

            def down_final(cs):
                def fin(mb, r, v):
                    rows = slice(mb * MB, (mb + 1) * MB)
                    y = xb[t * 4 + r, rows, :] + v
                    xa[t * 4 + r, rows, :] = y
                    ost[t * 4 + r, rows, :] = y.astype(bf16)
                return _recombine(lambda o, i: _ld(acc, o * 7 + i) + dprod(cs, o * 7 + i),
                                  fin, _Temps(tin2), _Temps(tout2))

            if last:
                norm = ffn_norm((t + 1) % NTILE)
                pace.add(norm, o_["n0"], o_["nper"])
            for gen in (gate(0), upgate(0), gate(1)):
                _adv(gen, 100)
            d0 = down((0,), not last)
            queue = []

            def lhs_queue():
                while True:
                    z = yield
                    while queue:
                        try:
                            queue[0].send(z)
                            break
                        except StopIteration:
                            queue.pop(0)
                            break
            for gen, plan in ((upgate(1), "u1"), (gate(2), "g2"), (upgate(2), "u2")):
                if last and plan == "u2":
                    feed(norm, None, 1000)
                    pace.add(lhs_queue(), pace.tok + o_["l0"], o_["lper"])
                for k, n in enumerate(DN_PLAN[plan]):
                    _adv(gen, 1)
                    if last and plan == "u2":
                        queue.append(lhs_strips(ORDER[k]))
                        next(queue[-1])
                    _adv(d0, n)
                _adv(gen, 100)
            _adv(d0, 100)
            _adv(down_final((1, 2)) if last else down((1, 2), False), 100)
            for gen in queue:
                feed(gen, None, 1000)

        def ffn_tile(t, c):
            def grp(g, c2):
                ffn_group(t, g, False)
                return c2
            lax.fori_loop(0, 2, grp, 0)
            ffn_group(t, 2, True)

            @pl.when(li == 1)
            def _():
                for r in range(4):
                    out_copy(t * 4 + r).start()
            return c
        if not OPT["skip_ffn"]:
            lax.fori_loop(0, NTILE, ffn_tile, 0)
        else:
            r0 = pl.multiple_of(zero[0] * 16, 16)
            ost[0, 0:16, :] = wcb[li, pl.ds(r0, 16), :] + wdcb[li, pl.ds(r0, 16), :] + web[li, li, 0:16, :]
            ost[1, 0:16, :] = acb[li, 0:16, :] + aeb[li, 0:16, :] + qkv[li, li, 0:16, :].astype(bf16)
            ost[2] = xb[li, 0:D, :].astype(bf16)
            for r in range(8):
                out_copy(li * 8 + r).start()
        return carry

    lax.fori_loop(0, 2, layer, 0)
    for p in range(NSLAB):
        out_copy(p).wait()


def _tiles(w):
    return w.reshape(NTR, 8, F // 128, 128).transpose(0, 2, 1, 3).reshape(NTR, F // 16, 128)


@jax.jit
def pallas_interleave_layers__sliding_local_dilated__glu_gated_bilinear__prompt_kernel(
    A_x: jax.Array,
    A_wqkv: jax.Array,
    A_wo: jax.Array,
    B_x: jax.Array,
    B_w_gate: jax.Array,
    B_w_up: jax.Array,
    B_w_down: jax.Array,
):
    del B_x
    vm = pltpu.VMEM
    hbm = pl.BlockSpec(memory_space=pl.ANY)
    out_t = pl.pallas_call(
        _kernel,
        in_specs=[hbm] * 6,
        out_specs=hbm,
        out_shape=jax.ShapeDtypeStruct((D, S), bf16),
        scratch_shapes=[
            vm((D, S), bf16),
            vm((NSLAB, 768, 128), f32),
            vm((NSLAB, 768, 128), f32),
            vm((NSLAB, D, 128), bf16),
            vm((D, 3 * D), bf16),
            vm((D, D), bf16),
            vm((5, 3 * D, 128), f32),
            vm((5, 1792, 128), bf16),
            vm((5, D, 128), bf16),
            vm((NCHUNK, 224, 32, 128), bf16),
            vm((NCHUNK, WC_ROWS, 128), bf16),
            vm((NCHUNK, 32, 64, 128), bf16),
            vm((NCHUNK, WD_ROWS, 128), bf16),
            vm((2, 5, 128, 128), bf16),
            vm((2, 14, HALO + 128, 128), f32),
            vm((2, 5, 128, 128), bf16),
            vm((20, 128, 128), f32),
            vm((49, 128, 128), bf16),
            vm((16, 128, 128), bf16),
            vm((32, 128, 128), f32),
            vm((3, 16, 128, 128), f32),
            vm((3, 49, 128, 128), bf16),
            vm((49, MB, 128), f32),
            vm((12, 128, 128), f32),
            vm((40, 128, 128), f32),
            vm((12, MB, 128), f32),
            vm((20, MB, 128), f32),
            pltpu.SMEM((1,), jnp.int32),
            pltpu.SemaphoreType.DMA((NTILE,)),
            pltpu.SemaphoreType.DMA((2,)),
            pltpu.SemaphoreType.DMA((NCHUNK, 3)),
            pltpu.SemaphoreType.DMA((NSLAB,)),
        ],
        compiler_params=pltpu.CompilerParams(vmem_limit_bytes=120 * 1024 * 1024),
    )(A_x[0].T, A_wqkv, A_wo, _tiles(B_w_gate), _tiles(B_w_up), _tiles(B_w_down.T))
    return out_t.T[None]
```

```python
import math

import jax
import jax.numpy as jnp
from jax import lax
import jax.experimental.pallas as pl
import jax.experimental.pallas.tpu as pltpu

f32 = jnp.float32
bf16 = jnp.bfloat16
u32 = jnp.uint32

S, D, F = 2048, 576, 4608
H, DH, WIN, DIL = 32, 18, 8, 2
EPS = 1e-5
LOG2E = math.log2(math.e)
NSLAB = S // 128
TILE = 512
NTILE = S // TILE
FC = 512
NCHUNK = F // FC
MB = D // 4
HALO = 16
NTR = D // 8
WC_ROWS = 800 * 16
WD_ROWS = 448 * 16
NT = (((1,), (1,)), ((), ()))
ORDER = (0, 1, 2, 5, 3, 4, 6)
AUG = (0, 1, 2, 5)

OPT = dict(skip_ffn=False,
           f=dict(h=((0, 1, 1), (0, 1, 1), (0, 1, 1)), n0=0, nper=2, l0=0, lper=2),
           h=dict(qtok=1, a0=0, aper=5, alat=35, l0=10, lper=6, llat=None),
           e=dict(qtok=0, aper=2),
           p=dict(qtok=1, a0=0, aper=6, alat=35, l0=100, lper=4, llat=None, pt=(0, 1, 2), pper=4),
           n=dict(qtok=1, a0=0, aper=6, alat=35, l0=100, lper=4, llat=None))
DN_PLAN = dict(u1=(0, 0, 0, 0, 4, 4, 6), g2=(4, 0, 0, 0, 0, 0, 0), u2=(0, 0, 0, 0, 4, 4, 4))


def _up(v):
    return pltpu.bitcast(v, bf16)


def _quad(x):
    n = len(x) // 2
    return ([r[:n] for r in x[:n]], [r[n:] for r in x[:n]],
            [r[:n] for r in x[n:]], [r[n:] for r in x[n:]])


def _badd(x, y):
    return [[a + b for a, b in zip(r, s)] for r, s in zip(x, y)]


def _bsub(x, y):
    return [[a - b for a, b in zip(r, s)] for r, s in zip(x, y)]


def _lhs_terms(a):
    a11, a12, a21, a22 = _quad(a)
    return [lambda: _badd(a11, a22), lambda: _badd(a21, a22), lambda: a11, lambda: a22,
            lambda: _badd(a11, a12), lambda: _bsub(a21, a11), lambda: _bsub(a12, a22)]


def _rhs_terms(b):
    b11, b12, b21, b22 = _quad(b)
    return [lambda: _badd(b11, b22), lambda: b11, lambda: _bsub(b12, b22), lambda: _bsub(b21, b11),
            lambda: b22, lambda: _badd(b11, b12), lambda: _badd(b21, b22)]


def _combos(x, terms, emit):
    for o, fo in enumerate(terms(x)):
        y = fo()
        for i, fi in enumerate(terms(y)):
            emit(o * 7 + i, fi()[0][0])


_LHS_SPEC = (((0, 0), (1, 1), 1), ((1, 0), (1, 1), 1), ((0, 0), None, 0), ((1, 1), None, 0),
             ((0, 0), (0, 1), 1), ((1, 0), (0, 0), -1), ((0, 1), (1, 1), -1))
_RHS_SPEC = (((0, 0), (1, 1), 1), ((0, 0), None, 0), ((0, 1), (1, 1), -1), ((1, 0), (0, 0), -1),
             ((1, 1), None, 0), ((0, 0), (0, 1), 1), ((1, 0), (1, 1), 1))


def _outer_term(load, spec, o):
    p, q, sign = spec[o]
    out = []
    for y in range(2):
        row = []
        for z in range(2):
            v = load(2 * p[0] + y, 2 * p[1] + z)
            if sign:
                w = load(2 * q[0] + y, 2 * q[1] + z)
                v = v + w if sign > 0 else v - w
            row.append(v)
        out.append(row)
    return out


def _inner_terms(y, terms, o, emit):
    for i, fi in enumerate(terms(y)):
        emit(o * 7 + i, fi()[0][0])


def _lhs_ext(e):
    n = len(e) // 2
    return {0: e[:n], 1: e[n:], 2: e[:n], 5: [y - x for x, y in zip(e[:n], e[n:])]}


def _rhs_ext(e):
    n = len(e) // 2
    return {0: e[:n], 1: e[:n], 2: e[n:], 5: [x + y for x, y in zip(e[:n], e[n:])]}


def _ext_combos(e, fn, emit):
    for oi, o in enumerate(AUG):
        d = fn(fn(e)[o])
        for ii, i in enumerate(AUG):
            emit(oi * 4 + ii, d[i][0])


def _adv(gen, n):
    for _ in range(n):
        try:
            next(gen)
        except StopIteration:
            return


def _ld(ref, idx):
    n = ref.shape[-2] // 2
    return jnp.concatenate([ref[idx, :n, :], ref[idx, n:, :]], axis=0)


class _Temps:
    def __init__(self, ref):
        self.ref = ref
        self.n = 0

    def put(self, v):
        i = self.n % self.ref.shape[0]
        self.n += 1
        self.ref[i] = v
        return i

    def get(self, i):
        return _ld(self.ref, i)


def _recombine(prod, fin, ti, to):
    def inner(o, sink):
        a = ti.put(prod(o, 0))
        b = ti.put(prod(o, 1))
        c = ti.put(prod(o, 2))
        sink(1, 1, ti.get(a) - ti.get(b) + ti.get(c) + prod(o, 5))
        m3 = prod(o, 3)
        m4 = prod(o, 4)
        m6 = prod(o, 6)
        sink(1, 0, ti.get(b) + m3)
        sink(0, 1, ti.get(c) + m4)
        sink(0, 0, ti.get(a) + m3 - m4 + m6)

    m = {}
    for o in (0, 1, 2):
        def keep(y, z, v, o=o):
            m[o, y, z] = to.put(v)
        inner(o, keep)
        yield

    def s5(y, z, v):
        fin(2 + y, 2 + z, to.get(m[0, y, z]) - to.get(m[1, y, z]) + to.get(m[2, y, z]) + v)
    inner(5, s5)
    yield

    def s3(y, z, v):
        fin(2 + y, z, to.get(m[1, y, z]) + v)
        m[3, y, z] = to.put(to.get(m[0, y, z]) + v)
    inner(3, s3)
    yield

    def s4(y, z, v):
        fin(y, 2 + z, to.get(m[2, y, z]) + v)
        m[3, y, z] = to.put(to.get(m[3, y, z]) - v)
    inner(4, s4)
    yield

    def s6(y, z, v):
        fin(y, z, to.get(m[3, y, z]) + v)
    inner(6, s6)
    yield


def _kernel(xt_hbm, wqkv_hbm, wo_hbm, wg_hbm, wu_hbm, wdt_hbm, out_hbm,
            xin, xa, xb, ost, wq_raw, wo_raw, wtmp, wqb, wob, raw, wcb, web, wdcb,
            xnb, qkv, ob, xn2, acb, aeb, gs, hs, hcb, acc, tin, tout, tin2, tout2, zero,
            sem_x, sem_w, sem_c, sem_o):
    wq, wo, wc, we, wdc, xn, o32, ac, ae, hc, raw32, xin32 = [
        r.bitcast(u32) for r in (wqb, wob, wcb, web, wdcb, xnb, ob, acb, aeb, hcb, raw, xin)]

    def x_copy(q):
        return pltpu.make_async_copy(
            xt_hbm.at[:, pl.ds(pl.multiple_of(q * 16, 16), 16), :], xin.at[q, 0:NTR], sem_x.at[q])

    def chunk_copies(j):
        rows = pl.ds(pl.multiple_of(j * 32, 32), 32)
        return [pltpu.make_async_copy(src.at[:, rows, :], raw.at[j, pl.ds(m * NTR, NTR)],
                                      sem_c.at[j, m])
                for m, src in enumerate((wg_hbm, wu_hbm, wdt_hbm))]

    def out_copy(p):
        return pltpu.make_async_copy(
            ost.at[p], out_hbm.at[:, pl.ds(pl.multiple_of(p * 128, 128), 128)], sem_o.at[p])

    wq_copy = pltpu.make_async_copy(wqkv_hbm, wq_raw, sem_w.at[0])
    wo_copy = pltpu.make_async_copy(wo_hbm, wo_raw, sem_w.at[1])
    zero[0] = 0
    wq_copy.start()
    x_copy(0).start()
    wo_copy.start()
    wq_copy.wait()
    for cp in [x_copy(1)] + chunk_copies(0):
        cp.start()

    def wq_transpose(n, carry):
        c0 = pl.multiple_of(n * 128, 128)
        t = wq_raw[:, pl.ds(c0, 128)].astype(f32).T
        for k in range(4):
            wtmp[k, pl.ds(c0, 128), :] = t[:, k * 128:(k + 1) * 128]
        wtmp[4, pl.ds(c0, 128), 0:64] = t[:, 512:576]
        return carry
    lax.fori_loop(0, 13, wq_transpose, 0, unroll=True)
    t = wq_raw[:, 1664:1728].astype(f32).T
    for k in range(4):
        wtmp[k, 1664:1728, :] = t[:, k * 128:(k + 1) * 128]
    wtmp[4, 1664:1728, 0:64] = t[:, 512:576]
    for k in range(5):
        lanes = slice(0, 128) if k < 4 else slice(0, 64)
        for part in range(3):
            for d in range(DH):
                if d < 16:
                    row = part * 512 + d * 32
                else:
                    row = (1536, 1664, 1600)[part] + (d - 16) * 32
                wqb[k, row:row + 32, lanes] = wtmp[
                    k, pl.ds(part * D + d, H, stride=DH), lanes].astype(bf16)
        wqb[k, 1728:1792, lanes] = jnp.zeros((64, lanes.stop), bf16)
    wqb[4, :, 64:128] = jnp.zeros((1792, 64), bf16)
    xnb[:, 4, :, 64:128] = jnp.zeros((2, 128, 64), bf16)

    wo_copy.wait()
    for n in range(5):
        w = 128 if n < 4 else 64
        wtmp[n, 0:D, 0:w] = wo_raw[:, n * 128:n * 128 + w].astype(f32)
    for n in range(5):
        w = 128 if n < 4 else 64
        for c in range(5):
            if c < 4:
                rows = [wtmp[n, pl.ds(4 * c + g, H, stride=DH), 0:w] for g in range(4)]
            else:
                rows = [jnp.zeros((64, w), f32)] + [
                    wtmp[n, pl.ds(16 + g, H, stride=DH), 0:w] for g in range(2)]
            wob[c, n * 128:n * 128 + w, :] = jnp.concatenate(rows, axis=0).T.astype(bf16)

    never = zero[0] != 0

    def held(v, z):
        if z is None:
            return v
        return jnp.where(never, pltpu.bitcast(z, v.dtype), v)

    def prep_chunk(j):
        def loader(m, z):
            seen = {}

            def pair(tr, cp):
                if (tr, cp) not in seen:
                    v = raw32[j, m * NTR + tr, cp * 8:cp * 8 + 8, :]
                    seen[tr, cp] = _up(held(v, z)).astype(f32)
                return seen[tr, cp]

            def load(row, c):
                h = slice((c % 2) * 8, (c % 2) * 8 + 8)
                return jnp.concatenate(
                    [pair(row // 8, c // 2)[h], pair(row // 8 + 1, c // 2)[h]], axis=0)
            return load
        for m in range(2):
            for s in range(8):
                def emit(i, v, m=m, s=s):
                    r = (m * 49 + i) * 128 + s * 16
                    wcb[j, r:r + 16, :] = v.astype(bf16)
                for o in range(7):
                    load = loader(m, (yield))
                    y = _outer_term(lambda k, c: load(k * 128 + s * 16, c), _RHS_SPEC, o)
                    _inner_terms(y, _rhs_terms, o, emit)
            for s in range(4):
                load = loader(m, (yield))
                e = [load(512 + s * 16, c) for c in range(4)]

                def emit_e(i, v, m=m, s=s):
                    web[j, m * 16 + i, s * 16:(s + 1) * 16, :] = v.astype(bf16)
                _ext_combos(e, _rhs_ext, emit_e)
        for s in range(9):
            def emit_d(i, v, s=s):
                r = i * MB + s * 16
                wdcb[j, r:r + 16, :] = v.astype(bf16)
            for o in range(7):
                load = loader(2, (yield))
                y = _outer_term(lambda r, k: load(r * MB + s * 16, k), _LHS_SPEC, o)
                _inner_terms(y, _lhs_terms, o, emit_d)

    def feed(gen, z, n):
        for _ in range(n):
            try:
                gen.send(z)
            except StopIteration:
                return

    class Pace:
        def __init__(self):
            self.tok = 0
            self.plan = []
            self.due = []

        def add(self, gen, t0, period, count=1, lat=None):
            next(gen)
            self.plan.append((gen, t0, period, count, lat))

        def step(self, z):
            for gen, t0, period, count, lat in self.plan:
                if self.tok >= t0 and (self.tok - t0) % period == 0:
                    for _ in range(count):
                        try:
                            v = gen.send(z)
                        except StopIteration:
                            break
                        if v is not None and lat is not None:
                            self.due.append((self.tok + lat, v))
            self.tok += 1

        def tokens(self, r, n):
            for k in range(n):
                self.step(r[k * 16:k * 16 + 8])

        def gate(self, v):
            now = [x for t, x in self.due if t <= self.tok]
            self.due = [(t, x) for t, x in self.due if t > self.tok]
            if not now:
                return v
            head = jnp.where(never, pltpu.bitcast(tree(now), u32), v[0:8])
            return jnp.concatenate([head, v[8:]], axis=0)

        def drain(self):
            for gen, *_ in self.plan:
                feed(gen, None, 1000)

    def tree(vals):
        while len(vals) > 1:
            vals = [a + b for a, b in zip(vals[::2], vals[1::2])] + vals[len(vals) & ~1:]
        return vals[0]

    def norm_slab(src, p0, emit, first=None):
        def rows(p, lo, hi):
            return [src[p, r:r + 8, :] for r in range(lo, hi, 8)]

        def mean(vals):
            t = tree([sum(vals[k + 4::4], vals[k]) for k in range(4)])
            t = jnp.sum(t, axis=0, keepdims=True) * (1.0 / D)
            return jnp.broadcast_to(t, (8, 128))
        p1, p2 = [jnp.clip(p0 + k * zero[0], 0, NSLAB - 1) for k in (1, 2)]
        z = yield
        x = rows(p0, 0, D) if first is None else first()
        mu = mean([held(v, z) for v in x[:4]] + x[4:])
        m = held(mu, (yield))
        rs = lax.rsqrt(mean([(v - m) * (v - m) for v in rows(p1, 0, D)]) + EPS)
        end = None
        for k in (4, 0, 1, 2, 3):
            m = held(mu, (yield end))
            y = jnp.concatenate(
                [(v - m) * rs for v in rows(p2, k * 128, min((k + 1) * 128, D))], axis=0).T
            emit(k, y)
            end = y[120:128] if k < 4 else jnp.concatenate([y[120:128]] * 2, axis=1)
        yield end

    def flush(gen):
        return tree([v for v in gen if v is not None])

    def ln1(p, b, fresh):
        def emit(k, y):
            xnb[b, k, :, 0:y.shape[1]] = y.astype(bf16)

        def widen():
            x = [_up(xin32[p // 2, r])[b * 8:b * 8 + 8].astype(f32) for r in range(NTR)]
            for r in range(NTR):
                xa[p, r * 8:r * 8 + 8, :] = x[r]
            return x
        return norm_slab(xa, p, emit, widen if fresh else None)

    def qkv_proj(b, pace):
        for grp in ((4, 5, 6, 7), (13, 0, 1, 2), (3, 12, 8, 9), (10, 11)):
            for n in grp:
                qkv[b, n, HALO:HALO + 128, :] = lax.dot_general(
                    _up(xn[b, 4]), _up(wq[4, n * 64:(n + 1) * 64, :]), NT,
                    preferred_element_type=f32)
            for n in grp:
                rows = slice(n * 64, (n + 1) * 64)
                lhs = jnp.concatenate(
                    [_up(pace.gate(xn[b, 0]))] + [_up(xn[b, k]) for k in range(1, 4)], axis=1)
                rhs = jnp.concatenate([_up(wq[k, rows, :]) for k in range(4)], axis=1)
                r = lax.dot_general(lhs, rhs, NT, preferred_element_type=f32)
                r = r + jnp.concatenate([qkv[b, n, HALO:HALO + 64, :],
                                         qkv[b, n, HALO + 64:HALO + 128, :]], axis=0)
                if n in (4, 5, 6, 7, 13):
                    r = r * (DH ** -0.5 * LOG2E)
                qkv[b, n, HALO:HALO + 128, :] = r
                pace.tokens(r, 7)

    def halo(b):
        for n in range(4, 14):
            qkv[b, n, 0:HALO, :] = qkv[1 - b, n, 128:128 + HALO, :]

    def attend(b, row0, qtok):
        qs, ks, vs = (0, 1, 2, 3, 12), (4, 5, 6, 7, 13), (8, 9, 10, 11, 12)
        v = None
        for s in range(16):
            z = yield v
            r = HALO + s * 8
            q = [held(qkv[b, n, r:r + 8, :], z if qtok else None) for n in qs]
            logit = []
            for w in range(WIN):
                rw = r - DIL * w
                part = tree([q[c] * qkv[b, ks[c], rw:rw + 8, :] for c in range(5)])
                part = part + pltpu.roll(part, 64, 1)
                part = part + pltpu.roll(part, 32, 1)
                if row0 is not None and s * 8 < DIL * w:
                    pos = row0 + s * 8 + lax.broadcasted_iota(jnp.int32, (8, 128), 0)
                    part = jnp.where(pos >= DIL * w, part, -1e9 * LOG2E)
                logit.append(part)
            mx = logit
            while len(mx) > 1:
                mx = [jnp.maximum(a, c) for a, c in zip(mx[::2], mx[1::2])]
            e = [jnp.exp2(l - mx[0]) for l in logit]
            inv = 1.0 / tree(e)
            outs = []
            for c in range(5):
                o = e[0] * qkv[b, vs[c], r:r + 8, :]
                for w in range(1, WIN):
                    rw = r - DIL * w
                    o = o + e[w] * qkv[b, vs[c], rw:rw + 8, :]
                o = o * inv
                outs.append(o)
                ob[b, c, s * 8:(s + 1) * 8, :] = o.astype(bf16)
            v = tree(outs)
        yield v

    def out_proj(p, b, pace):
        h = MB // 2
        for m in range(4):
            xb[p, m * MB:(m + 1) * MB, :] = xa[p, m * MB:(m + 1) * MB, :] + lax.dot_general(
                _up(wo[4, m * h:(m + 1) * h, :]), _up(o32[b, 4]), NT, preferred_element_type=f32)
        rhs = jnp.concatenate([_up(o32[b, c]) for c in range(4)], axis=1)
        for m in range(4):
            rows = slice(m * h, (m + 1) * h)
            lhs = jnp.concatenate(
                [_up(pace.gate(wo[0, rows, :]))] + [_up(wo[c, rows, :]) for c in range(1, 4)],
                axis=1)
            r = lax.dot_general(lhs, rhs, NT, preferred_element_type=f32)
            r = r + jnp.concatenate([xb[p, m * MB:m * MB + h, :],
                                     xb[p, m * MB + h:(m + 1) * MB, :]], axis=0)
            xb[p, m * MB:(m + 1) * MB, :] = r
            pace.tokens(r, 8)

    def ffn_norm(t):
        for r in range(4):
            def emit_n(k, y, r=r):
                xn2[r * 5 + k, :, 0:y.shape[1]] = y
            yield from norm_slab(xb, t * 4 + r, emit_n)

    def strips(load, spec, terms, o, dst):
        for s in range(8):
            z = yield
            rows = slice(s * 16, (s + 1) * 16)

            def ld(r, c):
                v = load(r, c, rows)
                if (r // 2, c // 2) == spec[o][0]:
                    v = jnp.concatenate([held(v[0:8], z), held(v[8:16], z)], axis=0)
                return v

            def emit(i, v):
                dst[i, rows, :] = v.astype(bf16)
            _inner_terms(_outer_term(ld, spec, o), terms, o, emit)

    def lhs_strips(o):
        yield from strips(lambda r, k, rows: xn2[r * 5 + k, rows, :],
                          _LHS_SPEC, _lhs_terms, o, acb)
        if o in AUG:
            for s in range(2):
                z = yield
                rows = slice(s * 64, (s + 1) * 64)
                d = _lhs_ext(_lhs_ext([xn2[r * 5 + 4, rows, 0:64] for r in range(4)])[o])
                for ii, i in enumerate(AUG):
                    aeb[AUG.index(o) * 4 + ii, rows, 0:64] = d[i][0].astype(bf16)

    def ffn_lhs(t):
        flush(ffn_norm(t))
        for s in range(8):
            rows = slice(s * 16, (s + 1) * 16)
            a = [[xn2[r * 5 + k, rows, :] for k in range(4)] for r in range(4)]

            def emit(i, v, rows=rows):
                acb[i, rows, :] = v.astype(bf16)
            _combos(a, _lhs_terms, emit)
            e = [xn2[r * 5 + 4, rows, 0:64] for r in range(4)]

            def emit_e(i, v, rows=rows):
                aeb[i, rows, 0:64] = v.astype(bf16)
            _ext_combos(e, _lhs_ext, emit_e)

    def attn_pair(h, o, fresh, side=None, head=False):
        flush(ln1(h % NSLAB, 0, fresh))
        for b in (0, 1):
            pace = Pace()
            if side is not None:
                for t0 in o["pt"]:
                    pace.plan.append((side, t0, o["pper"], 1, None))
            if b == 0:
                pace.add(ln1((h + 1) % NSLAB, 1, fresh), o["l0"], o["lper"], 1, o["llat"])
            if b == 1 or not head:
                row0 = None if b == 0 or (fresh and not head) else (h % NSLAB) * 128
                pace.add(attend(1 - b, row0, o["qtok"]), o["a0"], o["aper"], 1, o["alat"])
                if not head:
                    out_proj((h + b - 2) % NSLAB, b, pace)
                halo(b)
            qkv_proj(b, pace)
            pace.plan = [e for e in pace.plan if e[0] is not side]
            pace.drain()
        if side is not None:
            feed(side, None, 1000)

    x_copy(0).wait()
    for cp in [x_copy(2)] + chunk_copies(1):
        cp.start()
    for n in range(4, 14):
        qkv[0, n, 0:HALO, :] = jnp.zeros((HALO, 128), f32)
    attn_pair(0, OPT["h"], True, head=True)

    @pl.loop(0, 7)
    def _(i):
        for cp in [x_copy(i + 1)] + chunk_copies(i):
            cp.wait()
        for cp in chunk_copies(i + 2):
            cp.start()

        @pl.when(i + 3 < NSLAB // 2)
        def _():
            x_copy(i + 3).start()
        side = prep_chunk(i)
        next(side)
        attn_pair(2 * i + 2, OPT["p"], True, side)

    @pl.loop(7, NCHUNK)
    def _(j):
        for cp in chunk_copies(j):
            cp.wait()
        feed(prep_chunk(j), None, 1000)

    ffn_lhs(0)

    def ffn_group(t, g, last):
        ti = _Temps(tin)
        to = _Temps(tout)
        pace = Pace()
        o_ = OPT["f"]

        def chain(gens):
            yield
            for gen in gens:
                next(gen)
                z = None
                while True:
                    z = yield
                    try:
                        gen.send(z)
                    except StopIteration:
                        break

        def proj(c, m):
            j = g * 3 + c

            def prod(o, i):
                r = (m * 49 + o * 7 + i) * 64
                p = jnp.dot(_up(ac[o * 7 + i]), _up(wc[j, r:r + 64, :]),
                            preferred_element_type=f32)
                pace.step(p[0:8])
                if o in AUG and i in AUG:
                    q = AUG.index(o) * 4 + AUG.index(i)
                    e = jnp.dot(_up(ae[q, :, 0:64]), _up(we[j, m * 16 + q]),
                                preferred_element_type=f32)
                    pace.step(e[0:8])
                    p = p + e
                return p
            return prod

        def gate(c):
            def fin(r, cc, v):
                gs[(c % 2) * 16 + r * 4 + cc] = v
            return _recombine(proj(c, 0), fin, ti, to)

        def upgate(c):
            def fin(r, cc, v):
                hs[c, r * 4 + cc] = _ld(gs, (c % 2) * 16 + r * 4 + cc) * v
            yield from _recombine(proj(c, 1), fin, ti, to)
            t0, per, cnt = o_["h"][c]
            hgen[c] = chain([strips(lambda cc, r, rows: hs[c, r * 4 + cc, rows, :],
                                    _RHS_SPEC, _rhs_terms, o, hcb.at[c]) for o in ORDER])
            hdone[c] = 0
            pace.add(counted(c), pace.tok + t0, per, cnt)

        hgen, hdone = {}, {}

        def counted(c):
            next(hgen[c])
            next(hgen[c])
            while True:
                z = yield
                if hdone[c] < 56:
                    need(c, hdone[c] + 1, z)

        def need(c, n, z=None):
            while hdone[c] < n:
                hdone[c] += 1
                feed(hgen[c], z, 1)

        def dprod(cs, i):
            p = None
            for c in cs:
                need(c, 8 * (ORDER.index(i // 7) + 1))
                r = i * (MB // 2)
                q = lax.dot_general(_up(wdc[g * 3 + c, r:r + MB // 2, :]), _up(hc[c, i]), NT,
                                    preferred_element_type=f32)
                pace.step(q[0:8])
                p = q if p is None else p + q
            return p

        def down(cs, reset):
            for i in [o * 7 + k for o in ORDER for k in range(7)]:
                a = _ld(acc, i)
                if reset:
                    a = jnp.where(g == 0, 0.0, a)
                acc[i] = a + dprod(cs, i)
                yield

        def down_final(cs):
            def fin(mb, r, v):
                rows = slice(mb * MB, (mb + 1) * MB)
                y = xb[t * 4 + r, rows, :] + v
                xa[t * 4 + r, rows, :] = y
                ost[t * 4 + r, rows, :] = y.astype(bf16)
            return _recombine(lambda o, i: _ld(acc, o * 7 + i) + dprod(cs, o * 7 + i),
                              fin, _Temps(tin2), _Temps(tout2))

        if last:
            norm = ffn_norm((t + 1) % NTILE)
            pace.add(norm, o_["n0"], o_["nper"])
        for gen in (gate(0), upgate(0), gate(1)):
            _adv(gen, 100)
        d0 = down((0,), not last)
        queue = []

        def lhs_queue():
            while True:
                z = yield
                while queue:
                    try:
                        queue[0].send(z)
                        break
                    except StopIteration:
                        queue.pop(0)
                        break
        for gen, plan in ((upgate(1), "u1"), (gate(2), "g2"), (upgate(2), "u2")):
            if last and plan == "u2":
                feed(norm, None, 1000)
                pace.add(lhs_queue(), pace.tok + o_["l0"], o_["lper"])
            for k, n in enumerate(DN_PLAN[plan]):
                _adv(gen, 1)
                if last and plan == "u2":
                    queue.append(lhs_strips(ORDER[k]))
                    next(queue[-1])
                _adv(d0, n)
            _adv(gen, 100)
        _adv(d0, 100)
        _adv(down_final((1, 2)) if last else down((1, 2), False), 100)
        for gen in queue:
            feed(gen, None, 1000)

    @pl.loop(0, 2 * NTILE)
    def _(tile):
        t = tile % NTILE
        steps = jnp.where(jnp.logical_and(tile >= 1, tile <= NTILE), 2, 0)

        @pl.loop(0, steps)
        def _(k):
            attn_pair(4 * t + 2 * k + 12, OPT["n"], False)

        @pl.when(tile == NTILE + 1)
        def _():
            o = OPT["e"]
            pace = Pace()
            pace.add(attend(1, None, o["qtok"]), 0, o["aper"], 1, None)
            out_proj(NSLAB - 2, 0, pace)
            pace.drain()
            out_proj(NSLAB - 1, 1, Pace())

        if not OPT["skip_ffn"]:
            @pl.loop(0, 2)
            def _(g):
                ffn_group(t, g, False)
            ffn_group(t, 2, True)
        else:
            r0 = pl.multiple_of(zero[0] * 16, 16)
            ost[0, 0:16, :] = wcb[t, pl.ds(r0, 16), :] + wdcb[t, pl.ds(r0, 16), :] + web[t, t, 0:16, :]
            ost[1, 0:16, :] = acb[t, 0:16, :] + aeb[t, 0:16, :]
            ost[2] = xb[t, 0:D, :].astype(bf16)

        @pl.when(tile >= NTILE)
        def _():
            for r in range(4):
                out_copy(t * 4 + r).start()

    for p in range(NSLAB):
        out_copy(p).wait()


def _tiles(w):
    n = w.shape[1]
    return w.reshape(NTR, 8, n // 128, 128).transpose(0, 2, 1, 3).reshape(NTR, n // 16, 128)


@jax.jit
def pallas_interleave_layers__sliding_local_dilated__glu_gated_bilinear__prompt_kernel(
    A_x: jax.Array,
    A_wqkv: jax.Array,
    A_wo: jax.Array,
    B_x: jax.Array,
    B_w_gate: jax.Array,
    B_w_up: jax.Array,
    B_w_down: jax.Array,
):
    del B_x
    vm = pltpu.VMEM
    hbm = pl.BlockSpec(memory_space=pl.ANY)
    out_t = pl.pallas_call(
        _kernel,
        in_specs=[hbm] * 6,
        out_specs=hbm,
        out_shape=jax.ShapeDtypeStruct((D, S), bf16),
        scratch_shapes=[
            vm((NSLAB // 2, 96, 16, 128), bf16),
            vm((NSLAB, 768, 128), f32),
            vm((NSLAB, 768, 128), f32),
            vm((NSLAB, D, 128), bf16),
            vm((D, 3 * D), bf16),
            vm((D, D), bf16),
            vm((5, 3 * D, 128), f32),
            vm((5, 1792, 128), bf16),
            vm((5, D, 128), bf16),
            vm((NCHUNK, 224, 32, 128), bf16),
            vm((NCHUNK, WC_ROWS, 128), bf16),
            vm((NCHUNK, 32, 64, 128), bf16),
            vm((NCHUNK, WD_ROWS, 128), bf16),
            vm((2, 5, 128, 128), bf16),
            vm((2, 14, HALO + 128, 128), f32),
            vm((2, 5, 128, 128), bf16),
            vm((20, 128, 128), f32),
            vm((49, 128, 128), bf16),
            vm((16, 128, 128), bf16),
            vm((32, 128, 128), f32),
            vm((3, 16, 128, 128), f32),
            vm((3, 49, 128, 128), bf16),
            vm((49, MB, 128), f32),
            vm((12, 128, 128), f32),
            vm((40, 128, 128), f32),
            vm((12, MB, 128), f32),
            vm((20, MB, 128), f32),
            pltpu.SMEM((1,), jnp.int32),
            pltpu.SemaphoreType.DMA((NSLAB // 2,)),
            pltpu.SemaphoreType.DMA((2,)),
            pltpu.SemaphoreType.DMA((NCHUNK, 3)),
            pltpu.SemaphoreType.DMA((NSLAB,)),
        ],
        compiler_params=pltpu.CompilerParams(vmem_limit_bytes=120 * 1024 * 1024),
    )(_tiles(A_x[0].T), A_wqkv, A_wo, _tiles(B_w_gate), _tiles(B_w_up), _tiles(B_w_down.T))
    return out_t.T[None]
```

```python
import math

import jax
import jax.numpy as jnp
from jax import lax
import jax.experimental.pallas as pl
import jax.experimental.pallas.tpu as pltpu

f32 = jnp.float32
bf16 = jnp.bfloat16
u32 = jnp.uint32

S, D, F = 2048, 576, 4608
H, DH, WIN, DIL = 32, 18, 8, 2
EPS = 1e-5
LOG2E = math.log2(math.e)
NSLAB = S // 128
TILE = 512
NTILE = S // TILE
FC = 512
NCHUNK = F // FC
MB = D // 4
HALO = 16
NTR = D // 8
WC_ROWS = 800 * 16
WD_ROWS = 448 * 16
NT = (((1,), (1,)), ((), ()))
ORDER = (0, 1, 2, 5, 3, 4, 6)
AUG = (0, 1, 2, 5)

OPT = dict(
    skip_ffn=False,
    fa=dict(h=((0, 1), (0, 1), (0, 1)), tr=0,
            u1=(0, 0, 0, 0, 4, 4, 6), g2=(4, 0, 0, 0, 0, 0, 0), u2=(0, 0, 0, 0, 4, 4, 4)),
    fb=dict(h=((0, 1), (0, 1), (0, 1)), tr=0, n0=0, nper=2, l0=0, lper=2,
            u1=(0, 0, 0, 0, 4, 4, 6), g2=(4, 0, 0, 0, 0, 0, 0), u2=(0, 0, 0, 0, 4, 4, 4)),
    h=dict(qtok=1, a=((0, 5, 35), (0, 5, 35)), l0=10, lper=6, llat=None, w0=8, wper=2),
    e=dict(qtok=0, aper=2),
    p=dict(qtok=1, a=((0, 6, 35), (0, 6, 35)), l0=60, lper=8, llat=None, w0=5, wper=6,
           pn=79, pw=((0, 126), (0, 126))),
    n=dict(qtok=1, a=((0, 6, 35), (0, 6, 35)), l0=80, lper=6, llat=None))


def _up(v):
    return pltpu.bitcast(v, bf16)


def _quad(x):
    n = len(x) // 2
    return ([r[:n] for r in x[:n]], [r[n:] for r in x[:n]],
            [r[:n] for r in x[n:]], [r[n:] for r in x[n:]])


def _badd(x, y):
    return [[a + b for a, b in zip(r, s)] for r, s in zip(x, y)]


def _bsub(x, y):
    return [[a - b for a, b in zip(r, s)] for r, s in zip(x, y)]


def _lhs_terms(a):
    a11, a12, a21, a22 = _quad(a)
    return [lambda: _badd(a11, a22), lambda: _badd(a21, a22), lambda: a11, lambda: a22,
            lambda: _badd(a11, a12), lambda: _bsub(a21, a11), lambda: _bsub(a12, a22)]


def _rhs_terms(b):
    b11, b12, b21, b22 = _quad(b)
    return [lambda: _badd(b11, b22), lambda: b11, lambda: _bsub(b12, b22), lambda: _bsub(b21, b11),
            lambda: b22, lambda: _badd(b11, b12), lambda: _badd(b21, b22)]


def _combos(x, terms, emit):
    for o, fo in enumerate(terms(x)):
        y = fo()
        for i, fi in enumerate(terms(y)):
            emit(o * 7 + i, fi()[0][0])


_LHS_SPEC = (((0, 0), (1, 1), 1), ((1, 0), (1, 1), 1), ((0, 0), None, 0), ((1, 1), None, 0),
             ((0, 0), (0, 1), 1), ((1, 0), (0, 0), -1), ((0, 1), (1, 1), -1))
_RHS_SPEC = (((0, 0), (1, 1), 1), ((0, 0), None, 0), ((0, 1), (1, 1), -1), ((1, 0), (0, 0), -1),
             ((1, 1), None, 0), ((0, 0), (0, 1), 1), ((1, 0), (1, 1), 1))


def _outer_term(load, spec, o):
    p, q, sign = spec[o]
    out = []
    for y in range(2):
        row = []
        for z in range(2):
            v = load(2 * p[0] + y, 2 * p[1] + z)
            if sign:
                w = load(2 * q[0] + y, 2 * q[1] + z)
                v = v + w if sign > 0 else v - w
            row.append(v)
        out.append(row)
    return out


def _inner_terms(y, terms, o, emit):
    for i, fi in enumerate(terms(y)):
        emit(o * 7 + i, fi()[0][0])


def _lhs_ext(e):
    n = len(e) // 2
    return {0: e[:n], 1: e[n:], 2: e[:n], 5: [y - x for x, y in zip(e[:n], e[n:])]}


def _rhs_ext(e):
    n = len(e) // 2
    return {0: e[:n], 1: e[:n], 2: e[n:], 5: [x + y for x, y in zip(e[:n], e[n:])]}


def _ext_combos(e, fn, emit):
    for oi, o in enumerate(AUG):
        d = fn(fn(e)[o])
        for ii, i in enumerate(AUG):
            emit(oi * 4 + ii, d[i][0])


def _adv(gen, n):
    for _ in range(n):
        try:
            next(gen)
        except StopIteration:
            return


def _ld(ref, idx):
    n = ref.shape[-2] // 2
    return jnp.concatenate([ref[idx, :n, :], ref[idx, n:, :]], axis=0)


class _Temps:
    def __init__(self, ref):
        self.ref = ref
        self.n = 0

    def put(self, v):
        i = self.n % self.ref.shape[0]
        self.n += 1
        self.ref[i] = v
        return i

    def get(self, i):
        return _ld(self.ref, i)


def _recombine(prod, fin, ti, to):
    def inner(o, sink):
        a = ti.put(prod(o, 0))
        b = ti.put(prod(o, 1))
        c = ti.put(prod(o, 2))
        sink(1, 1, ti.get(a) - ti.get(b) + ti.get(c) + prod(o, 5))
        m3 = prod(o, 3)
        m4 = prod(o, 4)
        m6 = prod(o, 6)
        sink(1, 0, ti.get(b) + m3)
        sink(0, 1, ti.get(c) + m4)
        sink(0, 0, ti.get(a) + m3 - m4 + m6)

    m = {}
    for o in (0, 1, 2):
        def keep(y, z, v, o=o):
            m[o, y, z] = to.put(v)
        inner(o, keep)
        yield

    def s5(y, z, v):
        fin(2 + y, 2 + z, to.get(m[0, y, z]) - to.get(m[1, y, z]) + to.get(m[2, y, z]) + v)
    inner(5, s5)
    yield

    def s3(y, z, v):
        fin(2 + y, z, to.get(m[1, y, z]) + v)
        m[3, y, z] = to.put(to.get(m[0, y, z]) + v)
    inner(3, s3)
    yield

    def s4(y, z, v):
        fin(y, 2 + z, to.get(m[2, y, z]) + v)
        m[3, y, z] = to.put(to.get(m[3, y, z]) - v)
    inner(4, s4)
    yield

    def s6(y, z, v):
        fin(y, z, to.get(m[3, y, z]) + v)
    inner(6, s6)
    yield


def _kernel(xt_hbm, wqkv_hbm, wo_hbm, wg_hbm, wu_hbm, wdt_hbm, out_hbm,
            xin, xa, xb, ost, wq_raw, wo_raw, wtmp, wqb, wob, raw, wcb, web, wdcb,
            xnb, qkv, ob, xn2, acb, aeb, gs, hs, hcb, acc, tin, tout, tin2, tout2, zero,
            sem_x, sem_w, sem_c, sem_o):
    wq, wo, wc, we, wdc, xn, o32, ac, ae, hc, raw32, xin32 = [
        r.bitcast(u32) for r in (wqb, wob, wcb, web, wdcb, xnb, ob, acb, aeb, hcb, raw, xin)]

    def x_copy(q):
        return pltpu.make_async_copy(
            xt_hbm.at[:, pl.ds(pl.multiple_of(q * 16, 16), 16), :], xin.at[q, 0:NTR], sem_x.at[q])

    def chunk_copies(j):
        rows = pl.ds(pl.multiple_of(j * 32, 32), 32)
        return [pltpu.make_async_copy(src.at[:, rows, :], raw.at[j, pl.ds(m * NTR, NTR)],
                                      sem_c.at[j, m])
                for m, src in enumerate((wg_hbm, wu_hbm, wdt_hbm))]

    def out_copy(p):
        return pltpu.make_async_copy(
            ost.at[p], out_hbm.at[:, pl.ds(pl.multiple_of(p * 128, 128), 128)], sem_o.at[p])

    edges = (0, 640, 1152, 1536, 3 * D)
    wq_copies = [pltpu.make_async_copy(wqkv_hbm.at[:, lo:hi], wq_raw.at[:, lo:hi], sem_w.at[k])
                 for k, (lo, hi) in enumerate(zip(edges, edges[1:]))]
    wo_copy = pltpu.make_async_copy(wo_hbm, wo_raw, sem_w.at[4])
    for cp in [x_copy(0)] + wq_copies + [wo_copy]:
        cp.start()
    zero[0] = 0
    never = zero[0] != 0

    def held(v, z):
        if z is None:
            return v
        return jnp.where(never, pltpu.bitcast(z, v.dtype), v)

    def prep_chunk(j):
        def pair(m, row, cp, z):
            v = [_up(held(raw32[j, m * NTR + row // 8 + k, cp * 8:cp * 8 + 8, :], z)).astype(f32)
                 for k in range(2)]
            return [jnp.concatenate([v[0][h:h + 8], v[1][h:h + 8]], axis=0) for h in (0, 8)]

        def strip(m, step, row, spec, terms, path, emit):
            live = {}
            for o in path:
                used = [q for q in spec[o][:2] if q is not None]
                live = {q: live[q] for q in used if q in live}
                for q in used:
                    if q not in live:
                        z = yield
                        live[q] = [pair(m, (2 * q[0] + y) * step + row, q[1], z) for y in range(2)]
                y = _outer_term(lambda r, c: live[r // 2, c // 2][r % 2][c % 2], spec, o)
                _inner_terms(y, terms, o, emit)

        for m in range(2):
            for s in range(8):
                def emit(i, v, m=m, s=s):
                    r = (m * 49 + i) * 128 + s * 16
                    wcb[j, r:r + 16, :] = v.astype(bf16)
                yield from strip(m, 128, s * 16, _RHS_SPEC, _rhs_terms, (1, 0, 4, 2, 5, 3, 6), emit)
            for s in range(4):
                z = yield
                e = pair(m, 512 + s * 16, 0, z) + pair(m, 512 + s * 16, 1, z)

                def emit_e(i, v, m=m, s=s):
                    web[j, m * 16 + i, s * 16:(s + 1) * 16, :] = v.astype(bf16)
                _ext_combos(e, _rhs_ext, emit_e)
        for s in range(9):
            def emit_d(i, v, s=s):
                r = i * MB + s * 16
                wdcb[j, r:r + 16, :] = v.astype(bf16)
            yield from strip(2, MB, s * 16, _LHS_SPEC, _lhs_terms, (2, 0, 3, 6, 4, 5, 1), emit_d)

    def feed(gen, z, n):
        for _ in range(n):
            try:
                gen.send(z)
            except StopIteration:
                return

    class Pace:
        def __init__(self):
            self.tok = 0
            self.plan = []
            self.due = []

        def add(self, gen, t0, period, lat=None, n=1000, primed=False):
            if not primed:
                next(gen)
            when = [self.tok + int(t0 + k * period) for k in range(n)]
            self.plan.append((gen, when, lat))

        def step(self, z):
            for gen, when, lat in self.plan:
                for _ in range(when.count(self.tok)):
                    try:
                        v = gen.send(z)
                    except StopIteration:
                        break
                    if v is not None and lat is not None:
                        self.due.append((self.tok + lat, v))
            self.tok += 1

        def tokens(self, r, n):
            for k in range(n):
                self.step(r[k * 16:k * 16 + 8])

        def gate(self, v):
            now = [x for t, x in self.due if t <= self.tok]
            self.due = [(t, x) for t, x in self.due if t > self.tok]
            if not now:
                return v
            head = jnp.where(never, pltpu.bitcast(tree(now), u32), v[0:8])
            return jnp.concatenate([head, v[8:]], axis=0)

        def drain(self):
            for gen, *_ in self.plan:
                feed(gen, None, 1000)

    def tree(vals):
        while len(vals) > 1:
            vals = [a + b for a, b in zip(vals[::2], vals[1::2])] + vals[len(vals) & ~1:]
        return vals[0]

    def norm_slab(row, emit):
        def rows(k, lo, hi):
            return [row(k, r) for r in range(lo // 8, hi // 8)]

        def mean(vals):
            t = tree([sum(vals[k + 4::4], vals[k]) for k in range(4)])
            t = jnp.sum(t, axis=0, keepdims=True) * (1.0 / D)
            return jnp.broadcast_to(t, (8, 128))
        z = yield
        x = rows(0, 0, D)
        mu = mean([held(v, z) for v in x[:4]] + x[4:])
        m = held(mu, (yield))
        rs = lax.rsqrt(mean([(v - m) * (v - m) for v in rows(1, 0, D)]) + EPS)
        end = None
        for k in (4, 0, 1, 2, 3):
            m = held(mu, (yield end))
            y = jnp.concatenate(
                [(v - m) * rs for v in rows(2, k * 128, min((k + 1) * 128, D))], axis=0).T
            emit(k, y)
            end = y[120:128] if k < 4 else jnp.concatenate([y[120:128]] * 2, axis=1)
        yield end

    def alias(p, n):
        return [jnp.clip(p + k * zero[0], 0, n - 1) for k in range(3)]

    def slab_rows(src, p):
        q = alias(p, NSLAB)
        return lambda k, r: src[q[k], r * 8:r * 8 + 8, :]

    def flush(gen):
        return tree([v for v in gen if v is not None])

    def ln1(p, b):
        def emit(k, y):
            xnb[b, k, :, 0:y.shape[1]] = y.astype(bf16)
        return norm_slab(slab_rows(xa, p), emit)

    def widen(q):
        for r in range(NTR):
            if r % 4 == 0:
                z = yield
            v = _up(held(xin32[q, r], z)).astype(f32)
            for b in range(2):
                xa[2 * q + b, r * 8:r * 8 + 8, :] = v[b * 8:b * 8 + 8]

    def qkv_proj(b, pace):
        for grp in ((4, 5, 6, 7), (13, 0, 1, 2), (3, 12, 8, 9), (10, 11)):
            for n in grp:
                qkv[b, n, HALO:HALO + 128, :] = lax.dot_general(
                    _up(xn[b, 4]), _up(wq[4, n * 64:(n + 1) * 64, :]), NT,
                    preferred_element_type=f32)
            for n in grp:
                rows = slice(n * 64, (n + 1) * 64)
                lhs = jnp.concatenate(
                    [_up(pace.gate(xn[b, 0]))] + [_up(xn[b, k]) for k in range(1, 4)], axis=1)
                rhs = jnp.concatenate([_up(wq[k, rows, :]) for k in range(4)], axis=1)
                r = lax.dot_general(lhs, rhs, NT, preferred_element_type=f32)
                r = r + jnp.concatenate([qkv[b, n, HALO:HALO + 64, :],
                                         qkv[b, n, HALO + 64:HALO + 128, :]], axis=0)
                if n in (4, 5, 6, 7, 13):
                    r = r * (DH ** -0.5 * LOG2E)
                qkv[b, n, HALO:HALO + 128, :] = r
                pace.tokens(r, 7)

    def halo(b):
        for n in range(4, 14):
            qkv[b, n, 0:HALO, :] = qkv[1 - b, n, 128:128 + HALO, :]

    def attend(b, row0, qtok):
        qs, ks, vs = (0, 1, 2, 3, 12), (4, 5, 6, 7, 13), (8, 9, 10, 11, 12)
        v = None
        for s in range(16):
            z = yield v
            r = HALO + s * 8
            q = [held(qkv[b, n, r:r + 8, :], z if qtok else None) for n in qs]
            logit = []
            for w in range(WIN):
                rw = r - DIL * w
                part = tree([q[c] * qkv[b, ks[c], rw:rw + 8, :] for c in range(5)])
                part = part + pltpu.roll(part, 64, 1)
                part = part + pltpu.roll(part, 32, 1)
                if row0 is not None and s * 8 < DIL * w:
                    pos = row0 + s * 8 + lax.broadcasted_iota(jnp.int32, (8, 128), 0)
                    part = jnp.where(pos >= DIL * w, part, -1e9 * LOG2E)
                logit.append(part)
            mx = logit
            while len(mx) > 1:
                mx = [jnp.maximum(a, c) for a, c in zip(mx[::2], mx[1::2])]
            e = [jnp.exp2(l - mx[0]) for l in logit]
            inv = 1.0 / tree(e)
            outs = []
            for c in range(5):
                o = e[0] * qkv[b, vs[c], r:r + 8, :]
                for w in range(1, WIN):
                    rw = r - DIL * w
                    o = o + e[w] * qkv[b, vs[c], rw:rw + 8, :]
                o = o * inv
                outs.append(o)
                ob[b, c, s * 8:(s + 1) * 8, :] = o.astype(bf16)
            v = tree(outs)
        yield v

    def out_proj(p, b, pace):
        h = MB // 2
        for m in range(4):
            xb[p, m * MB:(m + 1) * MB, :] = xa[p, m * MB:(m + 1) * MB, :] + lax.dot_general(
                _up(wo[4, m * h:(m + 1) * h, :]), _up(o32[b, 4]), NT, preferred_element_type=f32)
        rhs = jnp.concatenate([_up(o32[b, c]) for c in range(4)], axis=1)
        for m in range(4):
            rows = slice(m * h, (m + 1) * h)
            lhs = jnp.concatenate(
                [_up(pace.gate(wo[0, rows, :]))] + [_up(wo[c, rows, :]) for c in range(1, 4)],
                axis=1)
            r = lax.dot_general(lhs, rhs, NT, preferred_element_type=f32)
            r = r + jnp.concatenate([xb[p, m * MB:m * MB + h, :],
                                     xb[p, m * MB + h:(m + 1) * MB, :]], axis=0)
            xb[p, m * MB:(m + 1) * MB, :] = r
            pace.tokens(r, 8)

    def ffn_norm(t):
        for r in range(4):
            def emit_n(k, y, r=r):
                xn2[r * 5 + k, :, 0:y.shape[1]] = y
            yield from norm_slab(slab_rows(xb, t * 4 + r), emit_n)

    def strips(load, spec, terms, o, dst):
        for s in range(8):
            z = yield
            rows = slice(s * 16, (s + 1) * 16)

            def ld(r, c):
                v = load(r, c, rows)
                if (r // 2, c // 2) == spec[o][0]:
                    v = jnp.concatenate([held(v[0:8], z), held(v[8:16], z)], axis=0)
                return v

            def emit(i, v):
                dst[i, rows, :] = v.astype(bf16)
            _inner_terms(_outer_term(ld, spec, o), terms, o, emit)

    def lhs_strips(o):
        yield from strips(lambda r, k, rows: xn2[r * 5 + k, rows, :],
                          _LHS_SPEC, _lhs_terms, o, acb)
        if o in AUG:
            for s in range(2):
                z = yield
                rows = slice(s * 64, (s + 1) * 64)
                d = _lhs_ext(_lhs_ext([xn2[r * 5 + 4, rows, 0:64] for r in range(4)])[o])
                for ii, i in enumerate(AUG):
                    aeb[AUG.index(o) * 4 + ii, rows, 0:64] = d[i][0].astype(bf16)

    def ffn_lhs(t):
        flush(ffn_norm(t))
        for s in range(8):
            rows = slice(s * 16, (s + 1) * 16)
            a = [[xn2[r * 5 + k, rows, :] for k in range(4)] for r in range(4)]

            def emit(i, v, rows=rows):
                acb[i, rows, :] = v.astype(bf16)
            _combos(a, _lhs_terms, emit)
            e = [xn2[r * 5 + 4, rows, 0:64] for r in range(4)]

            def emit_e(i, v, rows=rows):
                aeb[i, rows, 0:64] = v.astype(bf16)
            _ext_combos(e, _lhs_ext, emit_e)

    def attn_pair(h, o, mask, side=None, late=None, head=False):
        if not head:
            flush(ln1(h % NSLAB, 0))
        for b in (0, 1):
            pace = Pace()
            if side is not None:
                n = o["pn"] if b == 0 else 158 - o["pn"]
                lo, hi = o["pw"][b]
                pace.add(side, lo, (hi - lo) / n, n=n, primed=True)
            if b == 0:
                pace.add(ln1((h + 1) % NSLAB, 1), o["l0"], o["lper"], o["llat"])
            elif late is not None:
                pace.add(late, o["w0"], o["wper"])
            if b == 1 or not head:
                row0 = (h % NSLAB) * 128 if b == 1 and mask else None
                pace.add(attend(1 - b, row0, o["qtok"]), *o["a"][b])
                if not head:
                    out_proj((h + b - 2) % NSLAB, b, pace)
                halo(b)
            qkv_proj(b, pace)
            pace.plan = [e for e in pace.plan if e[0] is not side]
            pace.drain()
        if side is not None:
            feed(side, None, 1000)

    def wq_transpose(lo, hi):
        for c0 in range(lo, hi, 128):
            c1 = min(c0 + 128, hi)
            t = wq_raw[:, c0:c1].astype(f32).T
            for k in range(4):
                wtmp[k, c0:c1, :] = t[:, k * 128:(k + 1) * 128]
            wtmp[4, c0:c1, 0:64] = t[:, 512:D]

    def wq_gather(part):
        for k in range(5):
            lanes = slice(0, 128) if k < 4 else slice(0, 64)
            for d in range(DH):
                if d < 16:
                    row = part * 512 + d * 32
                else:
                    row = (1536, 1664, 1600)[part] + (d - 16) * 32
                wqb[k, row:row + 32, lanes] = wtmp[
                    k, pl.ds(part * D + d, H, stride=DH), lanes].astype(bf16)

    def wo_prep():
        for n in range(5):
            w = 128 if n < 4 else 64
            wtmp[n, 0:D, 0:w] = wo_raw[:, n * 128:n * 128 + w].astype(f32)
        for n in range(5):
            w = 128 if n < 4 else 64
            for c in range(5):
                z = yield
                rows = [held(wtmp[n, pl.ds(4 * c + g + k * 8 * DH, 8, stride=DH), :], z)[:, 0:w]
                        for g in range(4 if c < 4 else 2) for k in range(4)]
                if c == 4:
                    rows = [jnp.zeros((64, w), f32)] + rows
                wob[c, n * 128:n * 128 + w, :] = jnp.concatenate(rows, axis=0).T.astype(bf16)

    def head_late():
        for cp in (wo_copy, x_copy(1)):
            cp.wait()
        for cp in [x_copy(2)] + chunk_copies(1):
            cp.start()
        yield from wo_prep()
        yield from widen(1)

    wqb[:, 1728:1792, :] = jnp.zeros((5, 64, 128), bf16)
    wqb[4, 0:1728, 64:128] = jnp.zeros((1728, 64), bf16)
    xnb[:, 4, :, 64:128] = jnp.zeros((2, 128, 64), bf16)
    for n in range(4, 14):
        qkv[0, n, 0:HALO, :] = jnp.zeros((HALO, 128), f32)
    x_copy(0).wait()
    feed(widen(0), None, 1000)
    flush(ln1(0, 0))
    for k in range(4):
        wq_copies[k].wait()
        if k == 1:
            for cp in [x_copy(1)] + chunk_copies(0):
                cp.start()
        wq_transpose(edges[k], edges[k + 1])
        if k != 2:
            wq_gather(min(k, 2))
    attn_pair(0, OPT["h"], True, late=head_late(), head=True)

    @pl.loop(0, 7)
    def _(i):
        for cp in chunk_copies(i):
            cp.wait()

        @pl.when(i + 2 < NSLAB // 2)
        def _():
            x_copy(i + 2).wait()

        @pl.when(i + 3 < NSLAB // 2)
        def _():
            x_copy(i + 3).start()
        for cp in chunk_copies(i + 2):
            cp.start()
        side = prep_chunk(i)
        next(side)
        attn_pair(2 * i + 2, OPT["p"], False, side, widen(jnp.minimum(i + 2, NSLAB // 2 - 1)))

    @pl.loop(7, NCHUNK)
    def _(j):
        for cp in chunk_copies(j):
            cp.wait()
        feed(prep_chunk(j), None, 1000)

    ffn_lhs(0)

    def ffn_group(t, g, last):
        ti = _Temps(tin)
        to = _Temps(tout)
        pace = Pace()
        o_ = OPT["fb" if last else "fa"]

        tr = o_["tr"]

        def chain(gens):
            yield
            for gen in gens:
                next(gen)
                z = None
                while True:
                    z = yield
                    try:
                        gen.send(z)
                    except StopIteration:
                        break

        def proj(c, m):
            j = g * 3 + c

            def prod(o, i):
                r = (m * 49 + o * 7 + i) * 64
                p = jnp.dot(_up(ac[o * 7 + i]), _up(wc[j, r:r + 64, :]),
                            preferred_element_type=f32)
                pace.step(p[tr:tr + 8])
                if o in AUG and i in AUG:
                    q = AUG.index(o) * 4 + AUG.index(i)
                    e = jnp.dot(_up(ae[q, :, 0:64]), _up(we[j, m * 16 + q]),
                                preferred_element_type=f32)
                    pace.step(e[tr:tr + 8])
                    p = p + e
                return p
            return prod

        def gate(c):
            def fin(r, cc, v):
                gs[(c % 2) * 16 + r * 4 + cc] = v
            return _recombine(proj(c, 0), fin, ti, to)

        def upgate(c):
            def fin(r, cc, v):
                hs[c, r * 4 + cc] = _ld(gs, (c % 2) * 16 + r * 4 + cc) * v
            yield from _recombine(proj(c, 1), fin, ti, to)
            hgen[c] = chain([strips(lambda cc, r, rows: hs[c, r * 4 + cc, rows, :],
                                    _RHS_SPEC, _rhs_terms, o, hcb.at[c]) for o in ORDER])
            hdone[c] = 0
            pace.add(counted(c), *o_["h"][c])

        hgen, hdone = {}, {}

        def counted(c):
            next(hgen[c])
            next(hgen[c])
            while True:
                z = yield
                if hdone[c] < 56:
                    need(c, hdone[c] + 1, z)

        def need(c, n, z=None):
            while hdone[c] < n:
                hdone[c] += 1
                feed(hgen[c], z, 1)

        def dprod(cs, i):
            p = None
            for c in cs:
                need(c, 8 * (ORDER.index(i // 7) + 1))
                r = i * (MB // 2)
                q = lax.dot_general(_up(wdc[g * 3 + c, r:r + MB // 2, :]), _up(hc[c, i]), NT,
                                    preferred_element_type=f32)
                pace.step(q[tr:tr + 8])
                p = q if p is None else p + q
            return p

        def down(cs, reset):
            for i in [o * 7 + k for o in ORDER for k in range(7)]:
                a = _ld(acc, i)
                if reset:
                    a = jnp.where(g == 0, 0.0, a)
                acc[i] = a + dprod(cs, i)
                yield

        def down_final(cs):
            def fin(mb, r, v):
                rows = slice(mb * MB, (mb + 1) * MB)
                y = xb[t * 4 + r, rows, :] + v
                xa[t * 4 + r, rows, :] = y
                ost[t * 4 + r, rows, :] = y.astype(bf16)
            return _recombine(lambda o, i: _ld(acc, o * 7 + i) + dprod(cs, o * 7 + i),
                              fin, _Temps(tin2), _Temps(tout2))

        if last:
            norm = ffn_norm((t + 1) % NTILE)
            pace.add(norm, o_["n0"], o_["nper"])
        for gen in (gate(0), upgate(0), gate(1)):
            _adv(gen, 100)
        d0 = down((0,), not last)
        queue = []

        def lhs_queue():
            while True:
                z = yield
                while queue:
                    try:
                        queue[0].send(z)
                        break
                    except StopIteration:
                        queue.pop(0)
                        break
        for gen, plan in ((upgate(1), "u1"), (gate(2), "g2"), (upgate(2), "u2")):
            if last and plan == "u2":
                feed(norm, None, 1000)
                pace.add(lhs_queue(), o_["l0"], o_["lper"])
            for k, n in enumerate(o_[plan]):
                _adv(gen, 1)
                if last and plan == "u2":
                    queue.append(lhs_strips(ORDER[k]))
                    next(queue[-1])
                _adv(d0, n)
            _adv(gen, 100)
        _adv(d0, 100)
        _adv(down_final((1, 2)) if last else down((1, 2), False), 100)
        for gen in queue:
            feed(gen, None, 1000)

    @pl.loop(0, 2 * NTILE)
    def _(tile):
        t = tile % NTILE
        steps = jnp.where(jnp.logical_and(tile >= 1, tile <= NTILE), 2, 0)

        @pl.loop(0, steps)
        def _(k):
            attn_pair(4 * t + 2 * k + 12, OPT["n"], True)

        @pl.when(tile == NTILE + 1)
        def _():
            o = OPT["e"]
            pace = Pace()
            pace.add(attend(1, None, o["qtok"]), 0, o["aper"])
            out_proj(NSLAB - 2, 0, pace)
            pace.drain()
            out_proj(NSLAB - 1, 1, Pace())

        if not OPT["skip_ffn"]:
            @pl.loop(0, 2)
            def _(g):
                ffn_group(t, g, False)
            ffn_group(t, 2, True)
        else:
            r0 = pl.multiple_of(zero[0] * 16, 16)
            ost[0, 0:16, :] = wcb[t, pl.ds(r0, 16), :] + wdcb[t, pl.ds(r0, 16), :] + web[t, t, 0:16, :]
            ost[1, 0:16, :] = acb[t, 0:16, :] + aeb[t, 0:16, :]
            ost[2] = xb[t, 0:D, :].astype(bf16)

        @pl.when(tile >= NTILE)
        def _():
            for r in range(4):
                out_copy(t * 4 + r).start()

    for p in range(NSLAB):
        out_copy(p).wait()


def _tiles(w):
    n = w.shape[1]
    return w.reshape(NTR, 8, n // 128, 128).transpose(0, 2, 1, 3).reshape(NTR, n // 16, 128)


@jax.jit
def pallas_interleave_layers__sliding_local_dilated__glu_gated_bilinear__prompt_kernel(
    A_x: jax.Array,
    A_wqkv: jax.Array,
    A_wo: jax.Array,
    B_x: jax.Array,
    B_w_gate: jax.Array,
    B_w_up: jax.Array,
    B_w_down: jax.Array,
):
    del B_x
    vm = pltpu.VMEM
    hbm = pl.BlockSpec(memory_space=pl.ANY)
    out_t = pl.pallas_call(
        _kernel,
        in_specs=[hbm] * 6,
        out_specs=hbm,
        out_shape=jax.ShapeDtypeStruct((D, S), bf16),
        scratch_shapes=[
            vm((NSLAB // 2, 96, 16, 128), bf16),
            vm((NSLAB, 768, 128), f32),
            vm((NSLAB, 768, 128), f32),
            vm((NSLAB, D, 128), bf16),
            vm((D, 3 * D), bf16),
            vm((D, D), bf16),
            vm((5, 3 * D, 128), f32),
            vm((5, 1792, 128), bf16),
            vm((5, D, 128), bf16),
            vm((NCHUNK, 224, 32, 128), bf16),
            vm((NCHUNK, WC_ROWS, 128), bf16),
            vm((NCHUNK, 32, 64, 128), bf16),
            vm((NCHUNK, WD_ROWS, 128), bf16),
            vm((2, 5, 128, 128), bf16),
            vm((2, 14, HALO + 128, 128), f32),
            vm((2, 5, 128, 128), bf16),
            vm((20, 128, 128), f32),
            vm((49, 128, 128), bf16),
            vm((16, 128, 128), bf16),
            vm((32, 128, 128), f32),
            vm((3, 16, 128, 128), f32),
            vm((3, 49, 128, 128), bf16),
            vm((49, MB, 128), f32),
            vm((12, 128, 128), f32),
            vm((40, 128, 128), f32),
            vm((12, MB, 128), f32),
            vm((20, MB, 128), f32),
            pltpu.SMEM((1,), jnp.int32),
            pltpu.SemaphoreType.DMA((NSLAB // 2,)),
            pltpu.SemaphoreType.DMA((5,)),
            pltpu.SemaphoreType.DMA((NCHUNK, 3)),
            pltpu.SemaphoreType.DMA((NSLAB,)),
        ],
        compiler_params=pltpu.CompilerParams(vmem_limit_bytes=120 * 1024 * 1024),
    )(_tiles(A_x[0].T), A_wqkv, A_wo, _tiles(B_w_gate), _tiles(B_w_up), _tiles(B_w_down.T))
    return out_t.T[None]
```

```python
import math

import jax
import jax.numpy as jnp
from jax import lax
import jax.experimental.pallas as pl
import jax.experimental.pallas.tpu as pltpu

f32 = jnp.float32
bf16 = jnp.bfloat16
u32 = jnp.uint32

S, D, F = 2048, 576, 4608
H, DH, WIN, DIL = 32, 18, 8, 2
EPS = 1e-5
LOG2E = math.log2(math.e)
NSLAB = S // 128
TILE = 512
NTILE = S // TILE
FC = 512
NCHUNK = F // FC
MB = D // 4
HALO = 16
NTR = D // 8
WC_ROWS = 800 * 16
WD_ROWS = 448 * 16
NT = (((1,), (1,)), ((), ()))
ORDER = (0, 1, 2, 5, 3, 4, 6)
AUG = (0, 1, 2, 5)

OPT = dict(
    skip_ffn=False, dma=(0, 1), edges=(0, 640, 1152, 1280, 1728),
    fa=dict(h=((0, 1), (0, 1), (0, 1)), tr=0, hg=1,
            u1=(0, 0, 0, 0, 4, 4, 6), g2=(4, 0, 0, 0, 0, 0, 0), u2=(0, 0, 0, 0, 4, 4, 4)),
    fb=dict(h=((0, 1), (0, 1), (0, 1)), tr=0, n0=0, nper=2, l0=0, lper=2, hg=1, lg=1, ng=1,
            u1=(0, 0, 0, 0, 4, 4, 6), g2=(4, 0, 0, 0, 0, 0, 0), u2=(0, 0, 0, 0, 4, 4, 4)),
    h=dict(a=((0, 5, 35), (0, 5, 35)), l0=10, lper=6, llat=None, w0=8, wper=2,
           ag=1, lg=1, wg=1),
    e=dict(ag=0, aper=2),
    p=dict(a=((0, 6, 35), (0, 6, 35)), l0=60, lper=8, llat=None, w0=5, wper=6,
           pn=79, pw=((0, 126), (0, 126)), ag=1, lg=1, wg=1, pg=1),
    n=dict(a=((0, 6, 35), (0, 6, 35)), l0=80, lper=6, llat=None, ag=1, lg=1))


def _up(v):
    return pltpu.bitcast(v, bf16)


def _quad(x):
    n = len(x) // 2
    return ([r[:n] for r in x[:n]], [r[n:] for r in x[:n]],
            [r[:n] for r in x[n:]], [r[n:] for r in x[n:]])


def _badd(x, y):
    return [[a + b for a, b in zip(r, s)] for r, s in zip(x, y)]


def _bsub(x, y):
    return [[a - b for a, b in zip(r, s)] for r, s in zip(x, y)]


def _lhs_terms(a):
    a11, a12, a21, a22 = _quad(a)
    return [lambda: _badd(a11, a22), lambda: _badd(a21, a22), lambda: a11, lambda: a22,
            lambda: _badd(a11, a12), lambda: _bsub(a21, a11), lambda: _bsub(a12, a22)]


def _rhs_terms(b):
    b11, b12, b21, b22 = _quad(b)
    return [lambda: _badd(b11, b22), lambda: b11, lambda: _bsub(b12, b22), lambda: _bsub(b21, b11),
            lambda: b22, lambda: _badd(b11, b12), lambda: _badd(b21, b22)]


def _combos(x, terms, emit):
    for o, fo in enumerate(terms(x)):
        y = fo()
        for i, fi in enumerate(terms(y)):
            emit(o * 7 + i, fi()[0][0])


_LHS_SPEC = (((0, 0), (1, 1), 1), ((1, 0), (1, 1), 1), ((0, 0), None, 0), ((1, 1), None, 0),
             ((0, 0), (0, 1), 1), ((1, 0), (0, 0), -1), ((0, 1), (1, 1), -1))
_RHS_SPEC = (((0, 0), (1, 1), 1), ((0, 0), None, 0), ((0, 1), (1, 1), -1), ((1, 0), (0, 0), -1),
             ((1, 1), None, 0), ((0, 0), (0, 1), 1), ((1, 0), (1, 1), 1))


def _outer_term(load, spec, o):
    p, q, sign = spec[o]
    out = []
    for y in range(2):
        row = []
        for z in range(2):
            v = load(2 * p[0] + y, 2 * p[1] + z)
            if sign:
                w = load(2 * q[0] + y, 2 * q[1] + z)
                v = v + w if sign > 0 else v - w
            row.append(v)
        out.append(row)
    return out


def _inner_terms(y, terms, o, emit):
    for i, fi in enumerate(terms(y)):
        emit(o * 7 + i, fi()[0][0])


def _lhs_ext(e):
    n = len(e) // 2
    return {0: e[:n], 1: e[n:], 2: e[:n], 5: [y - x for x, y in zip(e[:n], e[n:])]}


def _rhs_ext(e):
    n = len(e) // 2
    return {0: e[:n], 1: e[:n], 2: e[n:], 5: [x + y for x, y in zip(e[:n], e[n:])]}


def _ext_combos(e, fn, emit):
    for oi, o in enumerate(AUG):
        d = fn(fn(e)[o])
        for ii, i in enumerate(AUG):
            emit(oi * 4 + ii, d[i][0])


def _adv(gen, n):
    for _ in range(n):
        try:
            next(gen)
        except StopIteration:
            return


def _ld(ref, idx):
    n = ref.shape[-2] // 2
    return jnp.concatenate([ref[idx, :n, :], ref[idx, n:, :]], axis=0)


class _Temps:
    def __init__(self, ref):
        self.ref = ref
        self.n = 0

    def put(self, v):
        i = self.n % self.ref.shape[0]
        self.n += 1
        self.ref[i] = v
        return i

    def get(self, i):
        return _ld(self.ref, i)


def _recombine(prod, fin, ti, to):
    def inner(o, sink):
        a = ti.put(prod(o, 0))
        b = ti.put(prod(o, 1))
        c = ti.put(prod(o, 2))
        sink(1, 1, ti.get(a) - ti.get(b) + ti.get(c) + prod(o, 5))
        m3 = prod(o, 3)
        m4 = prod(o, 4)
        m6 = prod(o, 6)
        sink(1, 0, ti.get(b) + m3)
        sink(0, 1, ti.get(c) + m4)
        sink(0, 0, ti.get(a) + m3 - m4 + m6)

    m = {}
    for o in (0, 1, 2):
        def keep(y, z, v, o=o):
            m[o, y, z] = to.put(v)
        inner(o, keep)
        yield

    def s5(y, z, v):
        fin(2 + y, 2 + z, to.get(m[0, y, z]) - to.get(m[1, y, z]) + to.get(m[2, y, z]) + v)
    inner(5, s5)
    yield

    def s3(y, z, v):
        fin(2 + y, z, to.get(m[1, y, z]) + v)
        m[3, y, z] = to.put(to.get(m[0, y, z]) + v)
    inner(3, s3)
    yield

    def s4(y, z, v):
        fin(y, 2 + z, to.get(m[2, y, z]) + v)
        m[3, y, z] = to.put(to.get(m[3, y, z]) - v)
    inner(4, s4)
    yield

    def s6(y, z, v):
        fin(y, z, to.get(m[3, y, z]) + v)
    inner(6, s6)
    yield


def _kernel(xt_hbm, wqkv_hbm, wo_hbm, wg_hbm, wu_hbm, wdt_hbm, out_hbm,
            xin, xa, xb, ost, wq_raw, wo_raw, wtmp, wqb, wob, raw, wcb, web, wdcb,
            xnb, qkv, ob, xn2, acb, aeb, gs, hs, hcb, acc, tin, tout, tin2, tout2, zero,
            sem_x, sem_w, sem_c, sem_o):
    wq, wo, wc, we, wdc, xn, o32, ac, ae, hc, raw32, xin32 = [
        r.bitcast(u32) for r in (wqb, wob, wcb, web, wdcb, xnb, ob, acb, aeb, hcb, raw, xin)]

    def x_copy(q):
        return pltpu.make_async_copy(
            xt_hbm.at[:, pl.ds(pl.multiple_of(q * 16, 16), 16), :], xin.at[q, 0:NTR], sem_x.at[q])

    def chunk_copies(j):
        rows = pl.ds(pl.multiple_of(j * 32, 32), 32)
        return [pltpu.make_async_copy(src.at[:, rows, :], raw.at[j, pl.ds(m * NTR, NTR)],
                                      sem_c.at[j, m])
                for m, src in enumerate((wg_hbm, wu_hbm, wdt_hbm))]

    def out_copy(p):
        return pltpu.make_async_copy(
            ost.at[p], out_hbm.at[:, pl.ds(pl.multiple_of(p * 128, 128), 128)], sem_o.at[p])

    edges = OPT["edges"]
    wq_copies = [pltpu.make_async_copy(wqkv_hbm.at[:, lo:hi], wq_raw.at[:, lo:hi], sem_w.at[k])
                 for k, (lo, hi) in enumerate(zip(edges, edges[1:]))]
    wo_copy = pltpu.make_async_copy(wo_hbm, wo_raw, sem_w.at[4])
    for cp in [x_copy(0)] + wq_copies:
        cp.start()
    zero[0] = 0
    never = [zero[0] != 0]

    def held(v, z):
        if z is None:
            return v
        return jnp.where(never[z[1]], pltpu.bitcast(z[0], v.dtype), v)

    def prep_chunk(j):
        def pair(m, row, cp, z):
            v = [_up(held(raw32[j, m * NTR + row // 8 + k, cp * 8:cp * 8 + 8, :], z)).astype(f32)
                 for k in range(2)]
            return [jnp.concatenate([v[0][h:h + 8], v[1][h:h + 8]], axis=0) for h in (0, 8)]

        def strip(m, step, row, spec, terms, path, emit):
            live = {}
            for o in path:
                used = [q for q in spec[o][:2] if q is not None]
                live = {q: live[q] for q in used if q in live}
                for q in used:
                    if q not in live:
                        z = yield
                        live[q] = [pair(m, (2 * q[0] + y) * step + row, q[1], z) for y in range(2)]
                y = _outer_term(lambda r, c: live[r // 2, c // 2][r % 2][c % 2], spec, o)
                _inner_terms(y, terms, o, emit)

        for m in range(2):
            for s in range(8):
                def emit(i, v, m=m, s=s):
                    r = (m * 49 + i) * 128 + s * 16
                    wcb[j, r:r + 16, :] = v.astype(bf16)
                yield from strip(m, 128, s * 16, _RHS_SPEC, _rhs_terms, (1, 0, 4, 2, 5, 3, 6), emit)
            for s in range(4):
                z = yield
                e = pair(m, 512 + s * 16, 0, z) + pair(m, 512 + s * 16, 1, z)

                def emit_e(i, v, m=m, s=s):
                    web[j, m * 16 + i, s * 16:(s + 1) * 16, :] = v.astype(bf16)
                _ext_combos(e, _rhs_ext, emit_e)
        for s in range(9):
            def emit_d(i, v, s=s):
                r = i * MB + s * 16
                wdcb[j, r:r + 16, :] = v.astype(bf16)
            yield from strip(2, MB, s * 16, _LHS_SPEC, _lhs_terms, (2, 0, 3, 6, 4, 5, 1), emit_d)

    def feed(gen, z, n):
        for _ in range(n):
            try:
                gen.send(z)
            except StopIteration:
                return

    class Pace:
        def __init__(self):
            self.tok = 0
            self.plan = []
            self.due = []

        def add(self, gen, t0, period, lat=None, gated=0, n=1000, primed=False):
            if not primed:
                next(gen)
            when = [self.tok + int(t0 + k * period) for k in range(n)]
            self.plan.append((gen, when, lat, gated))

        def step(self, z):
            for gen, when, lat, gated in self.plan:
                for _ in range(when.count(self.tok)):
                    try:
                        v = gen.send((z, gated - 1) if gated else None)
                    except StopIteration:
                        break
                    if v is not None and lat is not None:
                        self.due.append((self.tok + lat, v))
            self.tok += 1

        def tokens(self, r, n):
            for k in range(n):
                self.step(r[k * 16:k * 16 + 8])

        def gate(self, v):
            now = [x for t, x in self.due if t <= self.tok]
            self.due = [(t, x) for t, x in self.due if t > self.tok]
            if not now:
                return v
            head = jnp.where(never[0], pltpu.bitcast(tree(now), u32), v[0:8])
            return jnp.concatenate([head, v[8:]], axis=0)

        def drain(self):
            for gen, *_ in self.plan:
                feed(gen, None, 1000)

    def tree(vals):
        while len(vals) > 1:
            vals = [a + b for a, b in zip(vals[::2], vals[1::2])] + vals[len(vals) & ~1:]
        return vals[0]

    def norm_slab(row, emit):
        def rows(k, lo, hi):
            return [row(k, r) for r in range(lo // 8, hi // 8)]

        def mean(vals):
            t = tree([sum(vals[k + 4::4], vals[k]) for k in range(4)])
            t = jnp.sum(t, axis=0, keepdims=True) * (1.0 / D)
            return jnp.broadcast_to(t, (8, 128))
        z = yield
        x = rows(0, 0, D)
        mu = mean([held(v, z) for v in x[:4]] + x[4:])
        m = held(mu, (yield))
        rs = lax.rsqrt(mean([(v - m) * (v - m) for v in rows(1, 0, D)]) + EPS)
        end = None
        for k in (4, 0, 1, 2, 3):
            m = held(mu, (yield end))
            y = jnp.concatenate(
                [(v - m) * rs for v in rows(2, k * 128, min((k + 1) * 128, D))], axis=0).T
            emit(k, y)
            end = y[120:128] if k < 4 else jnp.concatenate([y[120:128]] * 2, axis=1)
        yield end

    def alias(p, n):
        return [jnp.clip(p + k * zero[0], 0, n - 1) for k in range(3)]

    def slab_rows(src, p):
        q = alias(p, NSLAB)
        return lambda k, r: src[q[k], r * 8:r * 8 + 8, :]

    def flush(gen):
        return tree([v for v in gen if v is not None])

    def ln1(p, b):
        def emit(k, y):
            xnb[b, k, :, 0:y.shape[1]] = y.astype(bf16)
        return norm_slab(slab_rows(xa, p), emit)

    def widen(q):
        for r in range(NTR):
            if r % 4 == 0:
                z = yield
            v = _up(held(xin32[q, r], z)).astype(f32)
            for b in range(2):
                xa[2 * q + b, r * 8:r * 8 + 8, :] = v[b * 8:b * 8 + 8]

    def qkv_proj(b, pace):
        for grp in ((4, 5, 6, 7), (13, 0, 1, 2), (3, 12, 8, 9), (10, 11)):
            for n in grp:
                qkv[b, n, HALO:HALO + 128, :] = lax.dot_general(
                    _up(xn[b, 4]), _up(wq[4, n * 64:(n + 1) * 64, :]), NT,
                    preferred_element_type=f32)
            for n in grp:
                rows = slice(n * 64, (n + 1) * 64)
                lhs = jnp.concatenate(
                    [_up(pace.gate(xn[b, 0]))] + [_up(xn[b, k]) for k in range(1, 4)], axis=1)
                rhs = jnp.concatenate([_up(wq[k, rows, :]) for k in range(4)], axis=1)
                r = lax.dot_general(lhs, rhs, NT, preferred_element_type=f32)
                r = r + jnp.concatenate([qkv[b, n, HALO:HALO + 64, :],
                                         qkv[b, n, HALO + 64:HALO + 128, :]], axis=0)
                if n in (4, 5, 6, 7, 13):
                    r = r * (DH ** -0.5 * LOG2E)
                qkv[b, n, HALO:HALO + 128, :] = r
                pace.tokens(r, 7)

    def halo(b):
        for n in range(4, 14):
            qkv[b, n, 0:HALO, :] = qkv[1 - b, n, 128:128 + HALO, :]

    def attend(b, row0):
        qs, ks, vs = (0, 1, 2, 3, 12), (4, 5, 6, 7, 13), (8, 9, 10, 11, 12)
        v = None
        for s in range(16):
            z = yield v
            r = HALO + s * 8
            q = [held(qkv[b, n, r:r + 8, :], z) for n in qs]
            logit = []
            for w in range(WIN):
                rw = r - DIL * w
                part = tree([q[c] * qkv[b, ks[c], rw:rw + 8, :] for c in range(5)])
                part = part + pltpu.roll(part, 64, 1)
                part = part + pltpu.roll(part, 32, 1)
                if row0 is not None and s * 8 < DIL * w:
                    pos = row0 + s * 8 + lax.broadcasted_iota(jnp.int32, (8, 128), 0)
                    part = jnp.where(pos >= DIL * w, part, -1e9 * LOG2E)
                logit.append(part)
            mx = logit
            while len(mx) > 1:
                mx = [jnp.maximum(a, c) for a, c in zip(mx[::2], mx[1::2])]
            e = [jnp.exp2(l - mx[0]) for l in logit]
            inv = 1.0 / tree(e)
            outs = []
            for c in range(5):
                o = e[0] * qkv[b, vs[c], r:r + 8, :]
                for w in range(1, WIN):
                    rw = r - DIL * w
                    o = o + e[w] * qkv[b, vs[c], rw:rw + 8, :]
                o = o * inv
                outs.append(o)
                ob[b, c, s * 8:(s + 1) * 8, :] = o.astype(bf16)
            v = tree(outs)
        yield v

    def out_proj(p, b, pace):
        h = MB // 2
        for m in range(4):
            xb[p, m * MB:(m + 1) * MB, :] = xa[p, m * MB:(m + 1) * MB, :] + lax.dot_general(
                _up(wo[4, m * h:(m + 1) * h, :]), _up(o32[b, 4]), NT, preferred_element_type=f32)
        rhs = jnp.concatenate([_up(o32[b, c]) for c in range(4)], axis=1)
        for m in range(4):
            rows = slice(m * h, (m + 1) * h)
            lhs = jnp.concatenate(
                [_up(pace.gate(wo[0, rows, :]))] + [_up(wo[c, rows, :]) for c in range(1, 4)],
                axis=1)
            r = lax.dot_general(lhs, rhs, NT, preferred_element_type=f32)
            r = r + jnp.concatenate([xb[p, m * MB:m * MB + h, :],
                                     xb[p, m * MB + h:(m + 1) * MB, :]], axis=0)
            xb[p, m * MB:(m + 1) * MB, :] = r
            pace.tokens(r, 8)

    def ffn_norm(t):
        for r in range(4):
            def emit_n(k, y, r=r):
                xn2[r * 5 + k, :, 0:y.shape[1]] = y
            yield from norm_slab(slab_rows(xb, t * 4 + r), emit_n)

    def strips(load, spec, terms, o, dst):
        for s in range(8):
            z = yield
            rows = slice(s * 16, (s + 1) * 16)

            def ld(r, c):
                v = load(r, c, rows)
                if (r // 2, c // 2) == spec[o][0]:
                    v = jnp.concatenate([held(v[0:8], z), held(v[8:16], z)], axis=0)
                return v

            def emit(i, v):
                dst[i, rows, :] = v.astype(bf16)
            _inner_terms(_outer_term(ld, spec, o), terms, o, emit)

    def lhs_strips(o):
        yield from strips(lambda r, k, rows: xn2[r * 5 + k, rows, :],
                          _LHS_SPEC, _lhs_terms, o, acb)
        if o in AUG:
            for s in range(2):
                z = yield
                rows = slice(s * 64, (s + 1) * 64)
                d = _lhs_ext(_lhs_ext([xn2[r * 5 + 4, rows, 0:64] for r in range(4)])[o])
                for ii, i in enumerate(AUG):
                    aeb[AUG.index(o) * 4 + ii, rows, 0:64] = d[i][0].astype(bf16)

    def ffn_lhs(t):
        flush(ffn_norm(t))
        for s in range(8):
            rows = slice(s * 16, (s + 1) * 16)
            a = [[xn2[r * 5 + k, rows, :] for k in range(4)] for r in range(4)]

            def emit(i, v, rows=rows):
                acb[i, rows, :] = v.astype(bf16)
            _combos(a, _lhs_terms, emit)
            e = [xn2[r * 5 + 4, rows, 0:64] for r in range(4)]

            def emit_e(i, v, rows=rows):
                aeb[i, rows, 0:64] = v.astype(bf16)
            _ext_combos(e, _lhs_ext, emit_e)

    def attn_pair(h, o, mask, side=None, late=None, head=False):
        if not head:
            flush(ln1(h % NSLAB, 0))
        for b in (0, 1):
            pace = Pace()
            if side is not None:
                n = o["pn"] if b == 0 else 158 - o["pn"]
                lo, hi = o["pw"][b]
                pace.add(side, lo, (hi - lo) / n, gated=o["pg"], n=n, primed=True)
            if b == 0:
                pace.add(ln1((h + 1) % NSLAB, 1), o["l0"], o["lper"], o["llat"], o["lg"])
            elif late is not None:
                pace.add(late, o["w0"], o["wper"], gated=o["wg"])
            if b == 1 or not head:
                row0 = (h % NSLAB) * 128 if b == 1 and mask else None
                pace.add(attend(1 - b, row0), *o["a"][b], o["ag"])
                if not head:
                    out_proj((h + b - 2) % NSLAB, b, pace)
                halo(b)
            qkv_proj(b, pace)
            pace.plan = [e for e in pace.plan if e[0] is not side]
            pace.drain()
        if side is not None:
            feed(side, None, 1000)

    def wq_transpose(lo, hi):
        for c0 in range(lo, hi, 128):
            c1 = min(c0 + 128, hi)
            t = wq_raw[:, c0:c1].astype(f32).T
            for k in range(4):
                wtmp[k, c0:c1, :] = t[:, k * 128:(k + 1) * 128]
            wtmp[4, c0:c1, 0:64] = t[:, 512:D]

    def wq_gather(part):
        for k in range(5):
            lanes = slice(0, 128) if k < 4 else slice(0, 64)
            for d in range(DH):
                if d < 16:
                    row = part * 512 + d * 32
                else:
                    row = (1536, 1664, 1600)[part] + (d - 16) * 32
                wqb[k, row:row + 32, lanes] = wtmp[
                    k, pl.ds(part * D + d, H, stride=DH), lanes].astype(bf16)

    def wo_prep():
        for n in range(5):
            w = 128 if n < 4 else 64
            wtmp[n, 0:D, 0:w] = wo_raw[:, n * 128:n * 128 + w].astype(f32)
        for n in range(5):
            w = 128 if n < 4 else 64
            for c in range(5):
                z = yield
                rows = [held(wtmp[n, pl.ds(4 * c + g + k * 8 * DH, 8, stride=DH), :], z)[:, 0:w]
                        for g in range(4 if c < 4 else 2) for k in range(4)]
                if c == 4:
                    rows = [jnp.zeros((64, w), f32)] + rows
                wob[c, n * 128:n * 128 + w, :] = jnp.concatenate(rows, axis=0).T.astype(bf16)

    def head_late():
        for cp in (wo_copy, x_copy(1)):
            cp.wait()
        for cp in [x_copy(2)] + chunk_copies(1):
            cp.start()
        yield from wo_prep()
        yield from widen(1)

    wqb[:, 1728:1792, :] = jnp.zeros((5, 64, 128), bf16)
    wqb[4, 0:1728, 64:128] = jnp.zeros((1728, 64), bf16)
    xnb[:, 4, :, 64:128] = jnp.zeros((2, 128, 64), bf16)
    for n in range(4, 14):
        qkv[0, n, 0:HALO, :] = jnp.zeros((HALO, 128), f32)
    x_copy(0).wait()
    never.append(zero[0] != 0)
    feed(widen(0), None, 1000)
    flush(ln1(0, 0))
    for k in range(4):
        wq_copies[k].wait()
        if k == OPT["dma"][0]:
            wo_copy.start()
        if k == OPT["dma"][1]:
            for cp in [x_copy(1)] + chunk_copies(0):
                cp.start()
        wq_transpose(edges[k], edges[k + 1])
        if k != 2:
            wq_gather(min(k, 2))
    attn_pair(0, OPT["h"], True, late=head_late(), head=True)

    @pl.loop(0, 7)
    def _(i):
        for cp in chunk_copies(i):
            cp.wait()

        @pl.when(i + 2 < NSLAB // 2)
        def _():
            x_copy(i + 2).wait()

        @pl.when(i + 3 < NSLAB // 2)
        def _():
            x_copy(i + 3).start()
        for cp in chunk_copies(i + 2):
            cp.start()
        side = prep_chunk(i)
        next(side)
        attn_pair(2 * i + 2, OPT["p"], False, side, widen(jnp.minimum(i + 2, NSLAB // 2 - 1)))

    @pl.loop(7, NCHUNK)
    def _(j):
        for cp in chunk_copies(j):
            cp.wait()
        feed(prep_chunk(j), None, 1000)

    ffn_lhs(0)

    def ffn_group(t, g, last):
        ti = _Temps(tin)
        to = _Temps(tout)
        pace = Pace()
        o_ = OPT["fb" if last else "fa"]

        tr = o_["tr"]

        def chain(gens):
            yield
            for gen in gens:
                next(gen)
                z = None
                while True:
                    z = yield
                    try:
                        gen.send(z)
                    except StopIteration:
                        break

        def proj(c, m):
            j = g * 3 + c

            def prod(o, i):
                r = (m * 49 + o * 7 + i) * 64
                p = jnp.dot(_up(ac[o * 7 + i]), _up(wc[j, r:r + 64, :]),
                            preferred_element_type=f32)
                pace.step(p[tr:tr + 8])
                if o in AUG and i in AUG:
                    q = AUG.index(o) * 4 + AUG.index(i)
                    e = jnp.dot(_up(ae[q, :, 0:64]), _up(we[j, m * 16 + q]),
                                preferred_element_type=f32)
                    pace.step(e[tr:tr + 8])
                    p = p + e
                return p
            return prod

        def gate(c):
            def fin(r, cc, v):
                gs[(c % 2) * 16 + r * 4 + cc] = v
            return _recombine(proj(c, 0), fin, ti, to)

        def upgate(c):
            def fin(r, cc, v):
                hs[c, r * 4 + cc] = _ld(gs, (c % 2) * 16 + r * 4 + cc) * v
            yield from _recombine(proj(c, 1), fin, ti, to)
            hgen[c] = chain([strips(lambda cc, r, rows: hs[c, r * 4 + cc, rows, :],
                                    _RHS_SPEC, _rhs_terms, o, hcb.at[c]) for o in ORDER])
            hdone[c] = 0
            pace.add(counted(c), *o_["h"][c], gated=o_["hg"])

        hgen, hdone = {}, {}

        def counted(c):
            next(hgen[c])
            next(hgen[c])
            while True:
                z = yield
                if hdone[c] < 56:
                    need(c, hdone[c] + 1, z)

        def need(c, n, z=None):
            while hdone[c] < n:
                hdone[c] += 1
                feed(hgen[c], z, 1)

        def dprod(cs, i):
            p = None
            for c in cs:
                need(c, 8 * (ORDER.index(i // 7) + 1))
                r = i * (MB // 2)
                q = lax.dot_general(_up(wdc[g * 3 + c, r:r + MB // 2, :]), _up(hc[c, i]), NT,
                                    preferred_element_type=f32)
                pace.step(q[tr:tr + 8])
                p = q if p is None else p + q
            return p

        def down(cs, reset):
            for i in [o * 7 + k for o in ORDER for k in range(7)]:
                a = _ld(acc, i)
                if reset:
                    a = jnp.where(g == 0, 0.0, a)
                acc[i] = a + dprod(cs, i)
                yield

        def down_final(cs):
            def fin(mb, r, v):
                rows = slice(mb * MB, (mb + 1) * MB)
                y = xb[t * 4 + r, rows, :] + v
                xa[t * 4 + r, rows, :] = y
                ost[t * 4 + r, rows, :] = y.astype(bf16)
            return _recombine(lambda o, i: _ld(acc, o * 7 + i) + dprod(cs, o * 7 + i),
                              fin, _Temps(tin2), _Temps(tout2))

        if last:
            norm = ffn_norm((t + 1) % NTILE)
            pace.add(norm, o_["n0"], o_["nper"], gated=o_["ng"])
        for gen in (gate(0), upgate(0), gate(1)):
            _adv(gen, 100)
        d0 = down((0,), not last)
        queue = []

        def lhs_queue():
            while True:
                z = yield
                while queue:
                    try:
                        queue[0].send(z)
                        break
                    except StopIteration:
                        queue.pop(0)
                        break
        for gen, plan in ((upgate(1), "u1"), (gate(2), "g2"), (upgate(2), "u2")):
            if last and plan == "u2":
                feed(norm, None, 1000)
                pace.add(lhs_queue(), o_["l0"], o_["lper"], gated=o_["lg"])
            for k, n in enumerate(o_[plan]):
                _adv(gen, 1)
                if last and plan == "u2":
                    queue.append(lhs_strips(ORDER[k]))
                    next(queue[-1])
                _adv(d0, n)
            _adv(gen, 100)
        _adv(d0, 100)
        _adv(down_final((1, 2)) if last else down((1, 2), False), 100)
        for gen in queue:
            feed(gen, None, 1000)

    @pl.loop(0, 2 * NTILE)
    def _(tile):
        t = tile % NTILE
        if not OPT["skip_ffn"]:
            @pl.loop(0, 2)
            def _(g):
                ffn_group(t, g, False)
            ffn_group(t, 2, True)
        else:
            r0 = pl.multiple_of(zero[0] * 16, 16)
            ost[0, 0:16, :] = wcb[t, pl.ds(r0, 16), :] + wdcb[t, pl.ds(r0, 16), :] + web[t, t, 0:16, :]
            ost[1, 0:16, :] = acb[t, 0:16, :] + aeb[t, 0:16, :]
            ost[2] = xb[t, 0:D, :].astype(bf16)

        @pl.when(tile >= NTILE)
        def _():
            for r in range(4):
                out_copy(t * 4 + r).start()

        @pl.loop(0, jnp.where(tile < NTILE, 2, 0))
        def _(k):
            attn_pair(4 * t + 2 * k + NSLAB, OPT["n"], True)

        @pl.when(tile == NTILE - 1)
        def _():
            o = OPT["e"]
            pace = Pace()
            pace.add(attend(1, None), 0, o["aper"], gated=o["ag"])
            out_proj(NSLAB - 2, 0, pace)
            pace.drain()
            out_proj(NSLAB - 1, 1, Pace())

    for p in range(NSLAB):
        out_copy(p).wait()


def _tiles(w):
    n = w.shape[1]
    return w.reshape(NTR, 8, n // 128, 128).transpose(0, 2, 1, 3).reshape(NTR, n // 16, 128)


@jax.jit
def pallas_interleave_layers__sliding_local_dilated__glu_gated_bilinear__prompt_kernel(
    A_x: jax.Array,
    A_wqkv: jax.Array,
    A_wo: jax.Array,
    B_x: jax.Array,
    B_w_gate: jax.Array,
    B_w_up: jax.Array,
    B_w_down: jax.Array,
):
    del B_x
    vm = pltpu.VMEM
    hbm = pl.BlockSpec(memory_space=pl.ANY)
    out_t = pl.pallas_call(
        _kernel,
        in_specs=[hbm] * 6,
        out_specs=hbm,
        out_shape=jax.ShapeDtypeStruct((D, S), bf16),
        scratch_shapes=[
            vm((NSLAB // 2, 96, 16, 128), bf16),
            vm((NSLAB, 768, 128), f32),
            vm((NSLAB, 768, 128), f32),
            vm((NSLAB, D, 128), bf16),
            vm((D, 3 * D), bf16),
            vm((D, D), bf16),
            vm((5, 3 * D, 128), f32),
            vm((5, 1792, 128), bf16),
            vm((5, D, 128), bf16),
            vm((NCHUNK, 224, 32, 128), bf16),
            vm((NCHUNK, WC_ROWS, 128), bf16),
            vm((NCHUNK, 32, 64, 128), bf16),
            vm((NCHUNK, WD_ROWS, 128), bf16),
            vm((2, 5, 128, 128), bf16),
            vm((2, 14, HALO + 128, 128), f32),
            vm((2, 5, 128, 128), bf16),
            vm((20, 128, 128), f32),
            vm((49, 128, 128), bf16),
            vm((16, 128, 128), bf16),
            vm((32, 128, 128), f32),
            vm((3, 16, 128, 128), f32),
            vm((3, 49, 128, 128), bf16),
            vm((49, MB, 128), f32),
            vm((12, 128, 128), f32),
            vm((40, 128, 128), f32),
            vm((12, MB, 128), f32),
            vm((20, MB, 128), f32),
            pltpu.SMEM((1,), jnp.int32),
            pltpu.SemaphoreType.DMA((NSLAB // 2,)),
            pltpu.SemaphoreType.DMA((5,)),
            pltpu.SemaphoreType.DMA((NCHUNK, 3)),
            pltpu.SemaphoreType.DMA((NSLAB,)),
        ],
        compiler_params=pltpu.CompilerParams(vmem_limit_bytes=120 * 1024 * 1024),
    )(_tiles(A_x[0].T), A_wqkv, A_wo, _tiles(B_w_gate), _tiles(B_w_up), _tiles(B_w_down.T))
    return out_t.T[None]
```

```python
import math

import jax
import jax.numpy as jnp
from jax import lax
import jax.experimental.pallas as pl
import jax.experimental.pallas.tpu as pltpu

f32 = jnp.float32
bf16 = jnp.bfloat16
u32 = jnp.uint32

S, D, F = 2048, 576, 4608
H, DH, WIN, DIL = 32, 18, 8, 2
EPS = 1e-5
LOG2E = math.log2(math.e)
NSLAB = S // 128
TILE = 512
NTILE = S // TILE
FC = 512
NCHUNK = F // FC
MB = D // 4
HALO = 16
NTR = D // 8
WC_ROWS = 800 * 16
WD_ROWS = 448 * 16
NT = (((1,), (1,)), ((), ()))
ORDER = (0, 1, 2, 5, 3, 4, 6)
AUG = (0, 1, 2, 5)

OPT = {'skip_ffn': False,
 'dma': (0, 1),
 'edges': (0, 640, 1152, 1280, 1728),
 'fa': {'h': ((0, 1), (0, 1), (0, 1)),
        'tr': 0,
        'hg': 1,
        'u1': (0, 0, 0, 4, 5, 4, 6),
        'g2': (4, 0, 0, 0, 0, 0, 0),
        'u2': (0, 0, 0, 0, 4, 4, 4)},
 'fb': {'h': ((0, 1), (0, 0.59), (0, 1)),
        'tr': 0,
        'n0': 0,
        'nper': 1.4,
        'l0': 0,
        'lper': 2,
        'hg': 1,
        'lg': 1,
        'ng': 1,
        'u1': (0, 0, 0, 0, 4, 4, 6),
        'g2': (4, 0, 0, 0, 0, 0, 0),
        'u2': (0, 0, 0, 0, 4, 4, 4)},
 'h': {'a': ((0, 5, 35), (0, 4.4, 35)),
       'l0': 13,
       'lper': 5.1,
       'llat': None,
       'w0': 2,
       'wper': 2.8,
       'ag': 1,
       'lg': 1,
       'wg': 1},
 'e': {'ag': 0, 'aper': 2},
 'p': {'a': ((0, 6, 35), (0, 6, 35)),
       'l0': 60,
       'lper': 8,
       'llat': None,
       'w0': 65,
       'wper': 5.1,
       'pn': 79,
       'pw': ((0, 126), (0, 126)),
       'ag': 0,
       'lg': 1,
       'wg': 1,
       'pg': 1},
 'n': {'a': ((0, 6, 35), (0, 6.6, 35)), 'l0': 80, 'lper': 5.1, 'llat': None, 'ag': 1, 'lg': 2}}


def _up(v):
    return pltpu.bitcast(v, bf16)


def _quad(x):
    n = len(x) // 2
    return ([r[:n] for r in x[:n]], [r[n:] for r in x[:n]],
            [r[:n] for r in x[n:]], [r[n:] for r in x[n:]])


def _badd(x, y):
    return [[a + b for a, b in zip(r, s)] for r, s in zip(x, y)]


def _bsub(x, y):
    return [[a - b for a, b in zip(r, s)] for r, s in zip(x, y)]


def _lhs_terms(a):
    a11, a12, a21, a22 = _quad(a)
    return [lambda: _badd(a11, a22), lambda: _badd(a21, a22), lambda: a11, lambda: a22,
            lambda: _badd(a11, a12), lambda: _bsub(a21, a11), lambda: _bsub(a12, a22)]


def _rhs_terms(b):
    b11, b12, b21, b22 = _quad(b)
    return [lambda: _badd(b11, b22), lambda: b11, lambda: _bsub(b12, b22), lambda: _bsub(b21, b11),
            lambda: b22, lambda: _badd(b11, b12), lambda: _badd(b21, b22)]


def _combos(x, terms, emit):
    for o, fo in enumerate(terms(x)):
        y = fo()
        for i, fi in enumerate(terms(y)):
            emit(o * 7 + i, fi()[0][0])


_LHS_SPEC = (((0, 0), (1, 1), 1), ((1, 0), (1, 1), 1), ((0, 0), None, 0), ((1, 1), None, 0),
             ((0, 0), (0, 1), 1), ((1, 0), (0, 0), -1), ((0, 1), (1, 1), -1))
_RHS_SPEC = (((0, 0), (1, 1), 1), ((0, 0), None, 0), ((0, 1), (1, 1), -1), ((1, 0), (0, 0), -1),
             ((1, 1), None, 0), ((0, 0), (0, 1), 1), ((1, 0), (1, 1), 1))


def _outer_term(load, spec, o):
    p, q, sign = spec[o]
    out = []
    for y in range(2):
        row = []
        for z in range(2):
            v = load(2 * p[0] + y, 2 * p[1] + z)
            if sign:
                w = load(2 * q[0] + y, 2 * q[1] + z)
                v = v + w if sign > 0 else v - w
            row.append(v)
        out.append(row)
    return out


def _inner_terms(y, terms, o, emit):
    for i, fi in enumerate(terms(y)):
        emit(o * 7 + i, fi()[0][0])


def _lhs_ext(e):
    n = len(e) // 2
    return {0: e[:n], 1: e[n:], 2: e[:n], 5: [y - x for x, y in zip(e[:n], e[n:])]}


def _rhs_ext(e):
    n = len(e) // 2
    return {0: e[:n], 1: e[:n], 2: e[n:], 5: [x + y for x, y in zip(e[:n], e[n:])]}


def _ext_combos(e, fn, emit):
    for oi, o in enumerate(AUG):
        d = fn(fn(e)[o])
        for ii, i in enumerate(AUG):
            emit(oi * 4 + ii, d[i][0])


def _adv(gen, n):
    for _ in range(n):
        try:
            next(gen)
        except StopIteration:
            return


def _ld(ref, idx):
    n = ref.shape[-2] // 2
    return jnp.concatenate([ref[idx, :n, :], ref[idx, n:, :]], axis=0)


class _Temps:
    def __init__(self, ref):
        self.ref = ref
        self.n = 0

    def put(self, v):
        i = self.n % self.ref.shape[0]
        self.n += 1
        self.ref[i] = v
        return i

    def get(self, i):
        return _ld(self.ref, i)


def _recombine(prod, fin, ti, to):
    def inner(o, sink):
        a = ti.put(prod(o, 0))
        b = ti.put(prod(o, 1))
        c = ti.put(prod(o, 2))
        sink(1, 1, ti.get(a) - ti.get(b) + ti.get(c) + prod(o, 5))
        m3 = prod(o, 3)
        m4 = prod(o, 4)
        m6 = prod(o, 6)
        sink(1, 0, ti.get(b) + m3)
        sink(0, 1, ti.get(c) + m4)
        sink(0, 0, ti.get(a) + m3 - m4 + m6)

    m = {}
    for o in (0, 1, 2):
        def keep(y, z, v, o=o):
            m[o, y, z] = to.put(v)
        inner(o, keep)
        yield

    def s5(y, z, v):
        fin(2 + y, 2 + z, to.get(m[0, y, z]) - to.get(m[1, y, z]) + to.get(m[2, y, z]) + v)
    inner(5, s5)
    yield

    def s3(y, z, v):
        fin(2 + y, z, to.get(m[1, y, z]) + v)
        m[3, y, z] = to.put(to.get(m[0, y, z]) + v)
    inner(3, s3)
    yield

    def s4(y, z, v):
        fin(y, 2 + z, to.get(m[2, y, z]) + v)
        m[3, y, z] = to.put(to.get(m[3, y, z]) - v)
    inner(4, s4)
    yield

    def s6(y, z, v):
        fin(y, z, to.get(m[3, y, z]) + v)
    inner(6, s6)
    yield


def _kernel(xt_hbm, wqkv_hbm, wo_hbm, wg_hbm, wu_hbm, wdt_hbm, out_hbm,
            xin, xa, xb, ost, wq_raw, wo_raw, wtmp, wqb, wob, raw, wcb, web, wdcb,
            xnb, qkv, ob, xn2, acb, aeb, gs, hs, hcb, acc, tin, tout, tin2, tout2, zero,
            sem_x, sem_w, sem_c, sem_o):
    wq, wo, wc, we, wdc, xn, o32, ac, ae, hc, raw32, xin32 = [
        r.bitcast(u32) for r in (wqb, wob, wcb, web, wdcb, xnb, ob, acb, aeb, hcb, raw, xin)]

    def x_copy(q):
        return pltpu.make_async_copy(
            xt_hbm.at[:, pl.ds(pl.multiple_of(q * 16, 16), 16), :], xin.at[q, 0:NTR], sem_x.at[q])

    def chunk_copies(j):
        rows = pl.ds(pl.multiple_of(j * 32, 32), 32)
        return [pltpu.make_async_copy(src.at[:, rows, :], raw.at[j, pl.ds(m * NTR, NTR)],
                                      sem_c.at[j, m])
                for m, src in enumerate((wg_hbm, wu_hbm, wdt_hbm))]

    def out_copy(p):
        return pltpu.make_async_copy(
            ost.at[p], out_hbm.at[:, pl.ds(pl.multiple_of(p * 128, 128), 128)], sem_o.at[p])

    edges = OPT["edges"]
    wq_copies = [pltpu.make_async_copy(wqkv_hbm.at[:, lo:hi], wq_raw.at[:, lo:hi], sem_w.at[k])
                 for k, (lo, hi) in enumerate(zip(edges, edges[1:]))]
    wo_copy = pltpu.make_async_copy(wo_hbm, wo_raw, sem_w.at[4])
    for cp in [x_copy(0)] + wq_copies:
        cp.start()
    zero[0] = 0
    never = [zero[0] != 0]

    def held(v, z):
        if z is None:
            return v
        return jnp.where(never[z[1]], pltpu.bitcast(z[0], v.dtype), v)

    def prep_chunk(j):
        def pair(m, row, cp, z):
            v = [_up(held(raw32[j, m * NTR + row // 8 + k, cp * 8:cp * 8 + 8, :], z)).astype(f32)
                 for k in range(2)]
            return [jnp.concatenate([v[0][h:h + 8], v[1][h:h + 8]], axis=0) for h in (0, 8)]

        def strip(m, step, row, spec, terms, path, emit):
            live = {}
            for o in path:
                used = [q for q in spec[o][:2] if q is not None]
                live = {q: live[q] for q in used if q in live}
                for q in used:
                    if q not in live:
                        z = yield
                        live[q] = [pair(m, (2 * q[0] + y) * step + row, q[1], z) for y in range(2)]
                y = _outer_term(lambda r, c: live[r // 2, c // 2][r % 2][c % 2], spec, o)
                _inner_terms(y, terms, o, emit)

        for m in range(2):
            for s in range(8):
                def emit(i, v, m=m, s=s):
                    r = (m * 49 + i) * 128 + s * 16
                    wcb[j, r:r + 16, :] = v.astype(bf16)
                yield from strip(m, 128, s * 16, _RHS_SPEC, _rhs_terms, (1, 0, 4, 2, 5, 3, 6), emit)
            for s in range(4):
                z = yield
                e = pair(m, 512 + s * 16, 0, z) + pair(m, 512 + s * 16, 1, z)

                def emit_e(i, v, m=m, s=s):
                    web[j, m * 16 + i, s * 16:(s + 1) * 16, :] = v.astype(bf16)
                _ext_combos(e, _rhs_ext, emit_e)
        for s in range(9):
            def emit_d(i, v, s=s):
                r = i * MB + s * 16
                wdcb[j, r:r + 16, :] = v.astype(bf16)
            yield from strip(2, MB, s * 16, _LHS_SPEC, _lhs_terms, (2, 0, 3, 6, 4, 5, 1), emit_d)

    def feed(gen, z, n):
        for _ in range(n):
            try:
                gen.send(z)
            except StopIteration:
                return

    class Pace:
        def __init__(self):
            self.tok = 0
            self.plan = []
            self.due = []

        def add(self, gen, t0, period, lat=None, gated=0, n=1000, primed=False):
            if not primed:
                next(gen)
            when = [self.tok + int(t0 + k * period) for k in range(n)]
            self.plan.append((gen, when, lat, gated))

        def step(self, z):
            for gen, when, lat, gated in self.plan:
                for _ in range(when.count(self.tok)):
                    try:
                        v = gen.send((z, gated - 1) if gated else None)
                    except StopIteration:
                        break
                    if v is not None and lat is not None:
                        self.due.append((self.tok + lat, v))
            self.tok += 1

        def tokens(self, r, n):
            for k in range(n):
                self.step(r[k * 16:k * 16 + 8])

        def gate(self, v):
            now = [x for t, x in self.due if t <= self.tok]
            self.due = [(t, x) for t, x in self.due if t > self.tok]
            if not now:
                return v
            head = jnp.where(never[0], pltpu.bitcast(tree(now), u32), v[0:8])
            return jnp.concatenate([head, v[8:]], axis=0)

        def drain(self):
            for gen, *_ in self.plan:
                feed(gen, None, 1000)

    def tree(vals):
        while len(vals) > 1:
            vals = [a + b for a, b in zip(vals[::2], vals[1::2])] + vals[len(vals) & ~1:]
        return vals[0]

    def norm_slab(row, emit):
        def rows(k, lo, hi):
            return [row(k, r) for r in range(lo // 8, hi // 8)]

        def mean(vals):
            t = tree([sum(vals[k + 4::4], vals[k]) for k in range(4)])
            t = jnp.sum(t, axis=0, keepdims=True) * (1.0 / D)
            return jnp.broadcast_to(t, (8, 128))
        z = yield
        x = rows(0, 0, D)
        mu = mean([held(v, z) for v in x[:4]] + x[4:])
        m = held(mu, (yield))
        rs = lax.rsqrt(mean([(v - m) * (v - m) for v in rows(1, 0, D)]) + EPS)
        end = None
        for k in (4, 0, 1, 2, 3):
            m = held(mu, (yield end))
            y = jnp.concatenate(
                [(v - m) * rs for v in rows(2, k * 128, min((k + 1) * 128, D))], axis=0).T
            emit(k, y)
            end = y[120:128] if k < 4 else jnp.concatenate([y[120:128]] * 2, axis=1)
        yield end

    def alias(p, n):
        return [jnp.clip(p + k * zero[0], 0, n - 1) for k in range(3)]

    def slab_rows(src, p):
        q = alias(p, NSLAB)
        return lambda k, r: src[q[k], r * 8:r * 8 + 8, :]

    def flush(gen):
        return tree([v for v in gen if v is not None])

    def ln1(p, b):
        def emit(k, y):
            xnb[b, k, :, 0:y.shape[1]] = y.astype(bf16)
        return norm_slab(slab_rows(xa, p), emit)

    def widen(q):
        for r in range(NTR):
            if r % 4 == 0:
                z = yield
            v = _up(held(xin32[q, r], z)).astype(f32)
            for b in range(2):
                xa[2 * q + b, r * 8:r * 8 + 8, :] = v[b * 8:b * 8 + 8]

    def qkv_proj(b, pace):
        for grp in ((4, 5, 6, 7), (13, 0, 1, 2), (3, 12, 8, 9), (10, 11)):
            for n in grp:
                qkv[b, n, HALO:HALO + 128, :] = lax.dot_general(
                    _up(xn[b, 4]), _up(wq[4, n * 64:(n + 1) * 64, :]), NT,
                    preferred_element_type=f32)
            for n in grp:
                rows = slice(n * 64, (n + 1) * 64)
                lhs = jnp.concatenate(
                    [_up(pace.gate(xn[b, 0]))] + [_up(xn[b, k]) for k in range(1, 4)], axis=1)
                rhs = jnp.concatenate([_up(wq[k, rows, :]) for k in range(4)], axis=1)
                r = lax.dot_general(lhs, rhs, NT, preferred_element_type=f32)
                r = r + jnp.concatenate([qkv[b, n, HALO:HALO + 64, :],
                                         qkv[b, n, HALO + 64:HALO + 128, :]], axis=0)
                if n in (4, 5, 6, 7, 13):
                    r = r * (DH ** -0.5 * LOG2E)
                qkv[b, n, HALO:HALO + 128, :] = r
                pace.tokens(r, 7)

    def halo(b):
        for n in range(4, 14):
            qkv[b, n, 0:HALO, :] = qkv[1 - b, n, 128:128 + HALO, :]

    def attend(b, row0):
        qs, ks, vs = (0, 1, 2, 3, 12), (4, 5, 6, 7, 13), (8, 9, 10, 11, 12)
        v = None
        for s in range(16):
            z = yield v
            r = HALO + s * 8
            q = [held(qkv[b, n, r:r + 8, :], z) for n in qs]
            logit = []
            for w in range(WIN):
                rw = r - DIL * w
                part = tree([q[c] * qkv[b, ks[c], rw:rw + 8, :] for c in range(5)])
                part = part + pltpu.roll(part, 64, 1)
                part = part + pltpu.roll(part, 32, 1)
                if row0 is not None and s * 8 < DIL * w:
                    pos = row0 + s * 8 + lax.broadcasted_iota(jnp.int32, (8, 128), 0)
                    part = jnp.where(pos >= DIL * w, part, -1e9 * LOG2E)
                logit.append(part)
            mx = logit
            while len(mx) > 1:
                mx = [jnp.maximum(a, c) for a, c in zip(mx[::2], mx[1::2])]
            e = [jnp.exp2(l - mx[0]) for l in logit]
            inv = 1.0 / tree(e)
            outs = []
            for c in range(5):
                o = e[0] * qkv[b, vs[c], r:r + 8, :]
                for w in range(1, WIN):
                    rw = r - DIL * w
                    o = o + e[w] * qkv[b, vs[c], rw:rw + 8, :]
                o = o * inv
                outs.append(o)
                ob[b, c, s * 8:(s + 1) * 8, :] = o.astype(bf16)
            v = tree(outs)
        yield v

    def out_proj(p, b, pace):
        h = MB // 2
        for m in range(4):
            xb[p, m * MB:(m + 1) * MB, :] = xa[p, m * MB:(m + 1) * MB, :] + lax.dot_general(
                _up(wo[4, m * h:(m + 1) * h, :]), _up(o32[b, 4]), NT, preferred_element_type=f32)
        rhs = jnp.concatenate([_up(o32[b, c]) for c in range(4)], axis=1)
        for m in range(4):
            rows = slice(m * h, (m + 1) * h)
            lhs = jnp.concatenate(
                [_up(pace.gate(wo[0, rows, :]))] + [_up(wo[c, rows, :]) for c in range(1, 4)],
                axis=1)
            r = lax.dot_general(lhs, rhs, NT, preferred_element_type=f32)
            r = r + jnp.concatenate([xb[p, m * MB:m * MB + h, :],
                                     xb[p, m * MB + h:(m + 1) * MB, :]], axis=0)
            xb[p, m * MB:(m + 1) * MB, :] = r
            pace.tokens(r, 8)

    def ffn_norm(t):
        for r in range(4):
            def emit_n(k, y, r=r):
                xn2[r * 5 + k, :, 0:y.shape[1]] = y
            yield from norm_slab(slab_rows(xb, t * 4 + r), emit_n)

    def strips(load, spec, terms, o, dst):
        for s in range(8):
            z = yield
            rows = slice(s * 16, (s + 1) * 16)

            def ld(r, c):
                v = load(r, c, rows)
                if (r // 2, c // 2) == spec[o][0]:
                    v = jnp.concatenate([held(v[0:8], z), held(v[8:16], z)], axis=0)
                return v

            def emit(i, v):
                dst[i, rows, :] = v.astype(bf16)
            _inner_terms(_outer_term(ld, spec, o), terms, o, emit)

    def lhs_strips(o):
        yield from strips(lambda r, k, rows: xn2[r * 5 + k, rows, :],
                          _LHS_SPEC, _lhs_terms, o, acb)
        if o in AUG:
            for s in range(2):
                z = yield
                rows = slice(s * 64, (s + 1) * 64)
                d = _lhs_ext(_lhs_ext([xn2[r * 5 + 4, rows, 0:64] for r in range(4)])[o])
                for ii, i in enumerate(AUG):
                    aeb[AUG.index(o) * 4 + ii, rows, 0:64] = d[i][0].astype(bf16)

    def ffn_lhs(t):
        flush(ffn_norm(t))
        for s in range(8):
            rows = slice(s * 16, (s + 1) * 16)
            a = [[xn2[r * 5 + k, rows, :] for k in range(4)] for r in range(4)]

            def emit(i, v, rows=rows):
                acb[i, rows, :] = v.astype(bf16)
            _combos(a, _lhs_terms, emit)
            e = [xn2[r * 5 + 4, rows, 0:64] for r in range(4)]

            def emit_e(i, v, rows=rows):
                aeb[i, rows, 0:64] = v.astype(bf16)
            _ext_combos(e, _lhs_ext, emit_e)

    def attn_pair(h, o, mask, side=None, late=None, head=False):
        if not head:
            flush(ln1(h % NSLAB, 0))
        for b in (0, 1):
            pace = Pace()
            if side is not None:
                n = o["pn"] if b == 0 else 158 - o["pn"]
                lo, hi = o["pw"][b]
                pace.add(side, lo, (hi - lo) / n, gated=o["pg"], n=n, primed=True)
            if b == 0:
                pace.add(ln1((h + 1) % NSLAB, 1), o["l0"], o["lper"], o["llat"], o["lg"])
            elif late is not None:
                pace.add(late, o["w0"], o["wper"], gated=o["wg"])
            if b == 1 or not head:
                row0 = (h % NSLAB) * 128 if b == 1 and mask else None
                pace.add(attend(1 - b, row0), *o["a"][b], o["ag"])
                if not head:
                    out_proj((h + b - 2) % NSLAB, b, pace)
                halo(b)
            qkv_proj(b, pace)
            pace.plan = [e for e in pace.plan if e[0] is not side]
            pace.drain()
        if side is not None:
            feed(side, None, 1000)

    def wq_transpose(lo, hi):
        for c0 in range(lo, hi, 128):
            c1 = min(c0 + 128, hi)
            t = wq_raw[:, c0:c1].astype(f32).T
            for k in range(4):
                wtmp[k, c0:c1, :] = t[:, k * 128:(k + 1) * 128]
            wtmp[4, c0:c1, 0:64] = t[:, 512:D]

    def wq_gather(part):
        for k in range(5):
            lanes = slice(0, 128) if k < 4 else slice(0, 64)
            for d in range(DH):
                if d < 16:
                    row = part * 512 + d * 32
                else:
                    row = (1536, 1664, 1600)[part] + (d - 16) * 32
                wqb[k, row:row + 32, lanes] = wtmp[
                    k, pl.ds(part * D + d, H, stride=DH), lanes].astype(bf16)

    def wo_prep():
        for n in range(5):
            w = 128 if n < 4 else 64
            wtmp[n, 0:D, 0:w] = wo_raw[:, n * 128:n * 128 + w].astype(f32)
        for n in range(5):
            w = 128 if n < 4 else 64
            for c in range(5):
                z = yield
                rows = [held(wtmp[n, pl.ds(4 * c + g + k * 8 * DH, 8, stride=DH), :], z)[:, 0:w]
                        for g in range(4 if c < 4 else 2) for k in range(4)]
                if c == 4:
                    rows = [jnp.zeros((64, w), f32)] + rows
                wob[c, n * 128:n * 128 + w, :] = jnp.concatenate(rows, axis=0).T.astype(bf16)

    def head_late():
        for cp in (wo_copy, x_copy(1)):
            cp.wait()
        for cp in [x_copy(2)] + chunk_copies(1):
            cp.start()
        yield from wo_prep()
        yield from widen(1)

    wqb[:, 1728:1792, :] = jnp.zeros((5, 64, 128), bf16)
    wqb[4, 0:1728, 64:128] = jnp.zeros((1728, 64), bf16)
    xnb[:, 4, :, 64:128] = jnp.zeros((2, 128, 64), bf16)
    for n in range(4, 14):
        qkv[0, n, 0:HALO, :] = jnp.zeros((HALO, 128), f32)
    x_copy(0).wait()
    never.append(zero[0] != 0)
    feed(widen(0), None, 1000)
    flush(ln1(0, 0))
    for k in range(4):
        wq_copies[k].wait()
        if k == OPT["dma"][0]:
            wo_copy.start()
        if k == OPT["dma"][1]:
            for cp in [x_copy(1)] + chunk_copies(0):
                cp.start()
        wq_transpose(edges[k], edges[k + 1])
        if k != 2:
            wq_gather(min(k, 2))
    attn_pair(0, OPT["h"], True, late=head_late(), head=True)

    @pl.loop(0, 7)
    def _(i):
        for cp in chunk_copies(i):
            cp.wait()

        @pl.when(i + 2 < NSLAB // 2)
        def _():
            x_copy(i + 2).wait()

        @pl.when(i + 3 < NSLAB // 2)
        def _():
            x_copy(i + 3).start()
        for cp in chunk_copies(i + 2):
            cp.start()
        side = prep_chunk(i)
        next(side)
        attn_pair(2 * i + 2, OPT["p"], False, side, widen(jnp.minimum(i + 2, NSLAB // 2 - 1)))

    @pl.loop(7, NCHUNK)
    def _(j):
        for cp in chunk_copies(j):
            cp.wait()
        feed(prep_chunk(j), None, 1000)

    ffn_lhs(0)

    def ffn_group(t, g, last):
        ti = _Temps(tin)
        to = _Temps(tout)
        pace = Pace()
        o_ = OPT["fb" if last else "fa"]

        tr = o_["tr"]

        def chain(gens):
            yield
            for gen in gens:
                next(gen)
                z = None
                while True:
                    z = yield
                    try:
                        gen.send(z)
                    except StopIteration:
                        break

        def proj(c, m):
            j = g * 3 + c

            def prod(o, i):
                r = (m * 49 + o * 7 + i) * 64
                p = jnp.dot(_up(ac[o * 7 + i]), _up(wc[j, r:r + 64, :]),
                            preferred_element_type=f32)
                pace.step(p[tr:tr + 8])
                if o in AUG and i in AUG:
                    q = AUG.index(o) * 4 + AUG.index(i)
                    e = jnp.dot(_up(ae[q, :, 0:64]), _up(we[j, m * 16 + q]),
                                preferred_element_type=f32)
                    pace.step(e[tr:tr + 8])
                    p = p + e
                return p
            return prod

        def gate(c):
            def fin(r, cc, v):
                gs[(c % 2) * 16 + r * 4 + cc] = v
            return _recombine(proj(c, 0), fin, ti, to)

        def upgate(c):
            def fin(r, cc, v):
                hs[c, r * 4 + cc] = _ld(gs, (c % 2) * 16 + r * 4 + cc) * v
            yield from _recombine(proj(c, 1), fin, ti, to)
            hgen[c] = chain([strips(lambda cc, r, rows: hs[c, r * 4 + cc, rows, :],
                                    _RHS_SPEC, _rhs_terms, o, hcb.at[c]) for o in ORDER])
            hdone[c] = 0
            pace.add(counted(c), *o_["h"][c], gated=o_["hg"])

        hgen, hdone = {}, {}

        def counted(c):
            next(hgen[c])
            next(hgen[c])
            while True:
                z = yield
                if hdone[c] < 56:
                    need(c, hdone[c] + 1, z)

        def need(c, n, z=None):
            while hdone[c] < n:
                hdone[c] += 1
                feed(hgen[c], z, 1)

        def dprod(cs, i):
            p = None
            for c in cs:
                need(c, 8 * (ORDER.index(i // 7) + 1))
                r = i * (MB // 2)
                q = lax.dot_general(_up(wdc[g * 3 + c, r:r + MB // 2, :]), _up(hc[c, i]), NT,
                                    preferred_element_type=f32)
                pace.step(q[tr:tr + 8])
                p = q if p is None else p + q
            return p

        def down(cs, reset):
            for i in [o * 7 + k for o in ORDER for k in range(7)]:
                a = _ld(acc, i)
                if reset:
                    a = jnp.where(g == 0, 0.0, a)
                acc[i] = a + dprod(cs, i)
                yield

        def down_final(cs):
            def fin(mb, r, v):
                rows = slice(mb * MB, (mb + 1) * MB)
                y = xb[t * 4 + r, rows, :] + v
                xa[t * 4 + r, rows, :] = y
                ost[t * 4 + r, rows, :] = y.astype(bf16)
            return _recombine(lambda o, i: _ld(acc, o * 7 + i) + dprod(cs, o * 7 + i),
                              fin, _Temps(tin2), _Temps(tout2))

        if last:
            norm = ffn_norm((t + 1) % NTILE)
            pace.add(norm, o_["n0"], o_["nper"], gated=o_["ng"])
        for gen in (gate(0), upgate(0), gate(1)):
            _adv(gen, 100)
        d0 = down((0,), not last)
        queue = []

        def lhs_queue():
            while True:
                z = yield
                while queue:
                    try:
                        queue[0].send(z)
                        break
                    except StopIteration:
                        queue.pop(0)
                        break
        for gen, plan in ((upgate(1), "u1"), (gate(2), "g2"), (upgate(2), "u2")):
            if last and plan == "u2":
                feed(norm, None, 1000)
                pace.add(lhs_queue(), o_["l0"], o_["lper"], gated=o_["lg"])
            for k, n in enumerate(o_[plan]):
                _adv(gen, 1)
                if last and plan == "u2":
                    queue.append(lhs_strips(ORDER[k]))
                    next(queue[-1])
                _adv(d0, n)
            _adv(gen, 100)
        _adv(d0, 100)
        _adv(down_final((1, 2)) if last else down((1, 2), False), 100)
        for gen in queue:
            feed(gen, None, 1000)

    @pl.loop(0, 2 * NTILE)
    def _(tile):
        t = tile % NTILE
        if not OPT["skip_ffn"]:
            @pl.loop(0, 2)
            def _(g):
                ffn_group(t, g, False)
            ffn_group(t, 2, True)
        else:
            r0 = pl.multiple_of(zero[0] * 16, 16)
            ost[0, 0:16, :] = wcb[t, pl.ds(r0, 16), :] + wdcb[t, pl.ds(r0, 16), :] + web[t, t, 0:16, :]
            ost[1, 0:16, :] = acb[t, 0:16, :] + aeb[t, 0:16, :]
            ost[2] = xb[t, 0:D, :].astype(bf16)

        @pl.when(tile >= NTILE)
        def _():
            for r in range(4):
                out_copy(t * 4 + r).start()

        @pl.loop(0, jnp.where(tile < NTILE, 2, 0))
        def _(k):
            attn_pair(4 * t + 2 * k + NSLAB, OPT["n"], True)

        @pl.when(tile == NTILE - 1)
        def _():
            o = OPT["e"]
            pace = Pace()
            pace.add(attend(1, None), 0, o["aper"], gated=o["ag"])
            out_proj(NSLAB - 2, 0, pace)
            pace.drain()
            out_proj(NSLAB - 1, 1, Pace())

    for p in range(NSLAB):
        out_copy(p).wait()


def _tiles(w):
    n = w.shape[1]
    return w.reshape(NTR, 8, n // 128, 128).transpose(0, 2, 1, 3).reshape(NTR, n // 16, 128)


@jax.jit
def pallas_interleave_layers__sliding_local_dilated__glu_gated_bilinear__prompt_kernel(
    A_x: jax.Array,
    A_wqkv: jax.Array,
    A_wo: jax.Array,
    B_x: jax.Array,
    B_w_gate: jax.Array,
    B_w_up: jax.Array,
    B_w_down: jax.Array,
):
    del B_x
    vm = pltpu.VMEM
    hbm = pl.BlockSpec(memory_space=pl.ANY)
    out_t = pl.pallas_call(
        _kernel,
        in_specs=[hbm] * 6,
        out_specs=hbm,
        out_shape=jax.ShapeDtypeStruct((D, S), bf16),
        scratch_shapes=[
            vm((NSLAB // 2, 96, 16, 128), bf16),
            vm((NSLAB, 768, 128), f32),
            vm((NSLAB, 768, 128), f32),
            vm((NSLAB, D, 128), bf16),
            vm((D, 3 * D), bf16),
            vm((D, D), bf16),
            vm((5, 3 * D, 128), f32),
            vm((5, 1792, 128), bf16),
            vm((5, D, 128), bf16),
            vm((NCHUNK, 224, 32, 128), bf16),
            vm((NCHUNK, WC_ROWS, 128), bf16),
            vm((NCHUNK, 32, 64, 128), bf16),
            vm((NCHUNK, WD_ROWS, 128), bf16),
            vm((2, 5, 128, 128), bf16),
            vm((2, 14, HALO + 128, 128), f32),
            vm((2, 5, 128, 128), bf16),
            vm((20, 128, 128), f32),
            vm((49, 128, 128), bf16),
            vm((16, 128, 128), bf16),
            vm((32, 128, 128), f32),
            vm((3, 16, 128, 128), f32),
            vm((3, 49, 128, 128), bf16),
            vm((49, MB, 128), f32),
            vm((12, 128, 128), f32),
            vm((40, 128, 128), f32),
            vm((12, MB, 128), f32),
            vm((20, MB, 128), f32),
            pltpu.SMEM((1,), jnp.int32),
            pltpu.SemaphoreType.DMA((NSLAB // 2,)),
            pltpu.SemaphoreType.DMA((5,)),
            pltpu.SemaphoreType.DMA((NCHUNK, 3)),
            pltpu.SemaphoreType.DMA((NSLAB,)),
        ],
        compiler_params=pltpu.CompilerParams(vmem_limit_bytes=120 * 1024 * 1024),
    )(_tiles(A_x[0].T), A_wqkv, A_wo, _tiles(B_w_gate), _tiles(B_w_up), _tiles(B_w_down.T))
    return out_t.T[None]
```

```python
import math

import jax
import jax.numpy as jnp
from jax import lax
import jax.experimental.pallas as pl
import jax.experimental.pallas.tpu as pltpu

f32 = jnp.float32
bf16 = jnp.bfloat16
u32 = jnp.uint32

S, D, F = 2048, 576, 4608
H, DH, WIN, DIL = 32, 18, 8, 2
EPS = 1e-5
LOG2E = math.log2(math.e)
NSLAB = S // 128
TILE = 512
NTILE = S // TILE
FC = 512
NCHUNK = F // FC
MB = D // 4
HALO = 16
NPREP = 158
NTR = D // 8
WC_ROWS = 800 * 16
WD_ROWS = 448 * 16
NT = (((1,), (1,)), ((), ()))
ORDER = (0, 1, 2, 5, 3, 4, 6)
AUG = (0, 1, 2, 5)

OPT = {'skip_ffn': False,
 'dma': (0, 1),
 'edges': (0, 640, 1152, 1280, 1728),
 'fa': {'h': ((0, 1), (0, 1), (0, 1)),
        'tr': 0,
        'hg': 1,
        'u1': (0, 0, 0, 4, 5, 4, 6),
        'g2': (4, 0, 0, 0, 0, 0, 0),
        'u2': (0, 0, 0, 0, 4, 4, 4)},
 'fb': {'h': ((0, 1), (0, 0.59), (0, 1)),
        'tr': 0,
        'n0': 0,
        'nper': 1.4,
        'l0': 0,
        'lper': 2,
        'hg': 1,
        'lg': 1,
        'ng': 1,
        'u1': (0, 0, 0, 0, 4, 4, 6),
        'g2': (4, 0, 0, 0, 0, 0, 0),
        'u2': (0, 0, 0, 0, 4, 4, 4)},
 'h': {'grp': ((4, 5, 6, 7), (0, 1, 2, 3), (12, 13, 8, 9, 10, 11)),
       'a': ((0, 5, 35), (0, 3.8, 35)),
       'l0': 13,
       'lper': 7.14,
       'llat': None,
       'w0': 2,
       'wper': 2.8,
       'ag': 1,
       'lg': 1,
       'wg': 1},
 'e': {'ag': 0, 'aper': 2.3},
 'p': {'x0': 30,
       'xper': 8,
       'xg': 1,
       'grp': ((4, 13), (5, 6, 7, 0), (1, 2, 3, 12), (8, 9, 10, 11)),
       'a': ((0, 6, 25), (0, 6, 35)),
       'l0': 52,
       'lper': 7.82,
       'llat': None,
       'w0': 59,
       'wper': 5.1,
       'pn': 71,
       'pw': ((0, 130), (0, 126)),
       'ag': 0,
       'lg': 1,
       'wg': 1,
       'pg': 1},
 'n': {'grp': ((4, 5, 6, 13), (7, 0, 1, 2, 3, 12), (8, 9, 10, 11)),
       'a': ((1, 6, 35), (0, 6.6, 35)),
       'l0': 85,
       'lper': 8.04,
       'llat': None,
       'ag': 1,
       'lg': 2}}


def _up(v):
    return pltpu.bitcast(v, bf16)


def _quad(x):
    n = len(x) // 2
    return ([r[:n] for r in x[:n]], [r[n:] for r in x[:n]],
            [r[:n] for r in x[n:]], [r[n:] for r in x[n:]])


def _badd(x, y):
    return [[a + b for a, b in zip(r, s)] for r, s in zip(x, y)]


def _bsub(x, y):
    return [[a - b for a, b in zip(r, s)] for r, s in zip(x, y)]


def _lhs_terms(a):
    a11, a12, a21, a22 = _quad(a)
    return [lambda: _badd(a11, a22), lambda: _badd(a21, a22), lambda: a11, lambda: a22,
            lambda: _badd(a11, a12), lambda: _bsub(a21, a11), lambda: _bsub(a12, a22)]


def _rhs_terms(b):
    b11, b12, b21, b22 = _quad(b)
    return [lambda: _badd(b11, b22), lambda: b11, lambda: _bsub(b12, b22), lambda: _bsub(b21, b11),
            lambda: b22, lambda: _badd(b11, b12), lambda: _badd(b21, b22)]


def _combos(x, terms, emit):
    for o, fo in enumerate(terms(x)):
        y = fo()
        for i, fi in enumerate(terms(y)):
            emit(o * 7 + i, fi()[0][0])


_LHS_SPEC = (((0, 0), (1, 1), 1), ((1, 0), (1, 1), 1), ((0, 0), None, 0), ((1, 1), None, 0),
             ((0, 0), (0, 1), 1), ((1, 0), (0, 0), -1), ((0, 1), (1, 1), -1))
_RHS_SPEC = (((0, 0), (1, 1), 1), ((0, 0), None, 0), ((0, 1), (1, 1), -1), ((1, 0), (0, 0), -1),
             ((1, 1), None, 0), ((0, 0), (0, 1), 1), ((1, 0), (1, 1), 1))


def _outer_term(load, spec, o):
    p, q, sign = spec[o]
    out = []
    for y in range(2):
        row = []
        for z in range(2):
            v = load(2 * p[0] + y, 2 * p[1] + z)
            if sign:
                w = load(2 * q[0] + y, 2 * q[1] + z)
                v = v + w if sign > 0 else v - w
            row.append(v)
        out.append(row)
    return out


def _inner_terms(y, terms, o, emit):
    for i, fi in enumerate(terms(y)):
        emit(o * 7 + i, fi()[0][0])


def _lhs_ext(e):
    n = len(e) // 2
    return {0: e[:n], 1: e[n:], 2: e[:n], 5: [y - x for x, y in zip(e[:n], e[n:])]}


def _rhs_ext(e):
    n = len(e) // 2
    return {0: e[:n], 1: e[:n], 2: e[n:], 5: [x + y for x, y in zip(e[:n], e[n:])]}


def _ext_combos(e, fn, emit):
    for oi, o in enumerate(AUG):
        d = fn(fn(e)[o])
        for ii, i in enumerate(AUG):
            emit(oi * 4 + ii, d[i][0])


def _adv(gen, n):
    for _ in range(n):
        try:
            next(gen)
        except StopIteration:
            return


def _ld(ref, idx):
    n = ref.shape[-2] // 2
    return jnp.concatenate([ref[idx, :n, :], ref[idx, n:, :]], axis=0)


class _Temps:
    def __init__(self, ref):
        self.ref = ref
        self.n = 0

    def put(self, v):
        i = self.n % self.ref.shape[0]
        self.n += 1
        self.ref[i] = v
        return i

    def get(self, i):
        return _ld(self.ref, i)


def _recombine(prod, fin, ti, to):
    def inner(o, sink):
        a = ti.put(prod(o, 0))
        b = ti.put(prod(o, 1))
        c = ti.put(prod(o, 2))
        sink(1, 1, ti.get(a) - ti.get(b) + ti.get(c) + prod(o, 5))
        m3 = prod(o, 3)
        m4 = prod(o, 4)
        m6 = prod(o, 6)
        sink(1, 0, ti.get(b) + m3)
        sink(0, 1, ti.get(c) + m4)
        sink(0, 0, ti.get(a) + m3 - m4 + m6)

    m = {}
    for o in (0, 1, 2):
        def keep(y, z, v, o=o):
            m[o, y, z] = to.put(v)
        inner(o, keep)
        yield

    def s5(y, z, v):
        fin(2 + y, 2 + z, to.get(m[0, y, z]) - to.get(m[1, y, z]) + to.get(m[2, y, z]) + v)
    inner(5, s5)
    yield

    def s3(y, z, v):
        fin(2 + y, z, to.get(m[1, y, z]) + v)
        m[3, y, z] = to.put(to.get(m[0, y, z]) + v)
    inner(3, s3)
    yield

    def s4(y, z, v):
        fin(y, 2 + z, to.get(m[2, y, z]) + v)
        m[3, y, z] = to.put(to.get(m[3, y, z]) - v)
    inner(4, s4)
    yield

    def s6(y, z, v):
        fin(y, z, to.get(m[3, y, z]) + v)
    inner(6, s6)
    yield


def _kernel(xt_hbm, wqkv_hbm, wo_hbm, wg_hbm, wu_hbm, wdt_hbm, out_hbm,
            xin, xa, xb, ost, wq_raw, wo_raw, wtmp, wqb, wob, raw, wcb, web, wdcb,
            xnb, qkv, ob, xn2, acb, aeb, gs, hs, hcb, acc, tin, tout, tin2, tout2, ktail, zero,
            sem_x, sem_w, sem_c, sem_o):
    wq, wo, wc, we, wdc, xn, o32, ac, ae, hc, raw32, xin32 = [
        r.bitcast(u32) for r in (wqb, wob, wcb, web, wdcb, xnb, ob, acb, aeb, hcb, raw, xin)]

    def x_copy(q):
        return pltpu.make_async_copy(
            xt_hbm.at[:, pl.ds(pl.multiple_of(q * 16, 16), 16), :], xin.at[q, 0:NTR], sem_x.at[q])

    def weight_copy(j, m):
        rows = pl.ds(pl.multiple_of(j * 32, 32), 32)
        return pltpu.make_async_copy((wg_hbm, wu_hbm, wdt_hbm)[m].at[:, rows, :],
                                     raw.at[j, pl.ds(m * NTR, NTR)], sem_c.at[j, m])

    def chunk_copies(j):
        return [weight_copy(j, m) for m in range(3)]

    def out_copy(p):
        return pltpu.make_async_copy(
            ost.at[p], out_hbm.at[:, pl.ds(pl.multiple_of(p * 128, 128), 128)], sem_o.at[p])

    edges = OPT["edges"]
    wq_copies = [pltpu.make_async_copy(wqkv_hbm.at[:, lo:hi], wq_raw.at[:, lo:hi], sem_w.at[k])
                 for k, (lo, hi) in enumerate(zip(edges, edges[1:]))]
    wo_copy = pltpu.make_async_copy(wo_hbm, wo_raw, sem_w.at[4])
    for cp in [x_copy(0)] + wq_copies:
        cp.start()
    zero[0] = 0
    never = [zero[0] != 0]

    def held(v, z):
        if z is None:
            return v
        return jnp.where(never[z[1]], pltpu.bitcast(z[0], v.dtype), v)

    def raw_pair(j, tr, cp, z):
        v = [_up(held(raw32[j, tr + k, cp * 8:cp * 8 + 8, :], z)).astype(f32) for k in range(2)]
        return [jnp.concatenate([v[0][h:h + 8], v[1][h:h + 8]], axis=0) for h in (0, 8)]

    def prep_strip(j, tr, step, spec, terms, path, emit):
        live = {}
        for o in path:
            used = [q for q in spec[o][:2] if q is not None]
            live = {q: live[q] for q in used if q in live}
            for q in used:
                if q not in live:
                    z = yield
                    live[q] = [raw_pair(j, tr + (2 * q[0] + y) * step, q[1], z) for y in range(2)]
            y = _outer_term(lambda r, c: live[r // 2, c // 2][r % 2][c % 2], spec, o)
            _inner_terms(y, terms, o, emit)

    def prep_gu(j, m, s):
        base = m * (49 * 128) + s * 16

        def emit(i, v):
            wcb[j, pl.ds(base + i * 128, 16), :] = v.astype(bf16)
        return prep_strip(j, m * NTR + 2 * s, 16, _RHS_SPEC, _rhs_terms, (1, 0, 4, 2, 5, 3, 6), emit)

    def prep_ext(j, m, s):
        z = yield
        tr = m * NTR + 64 + 2 * s

        def emit(i, v):
            web[j, m * 16 + i, pl.ds(s * 16, 16), :] = v.astype(bf16)
        _ext_combos(raw_pair(j, tr, 0, z) + raw_pair(j, tr, 1, z), _rhs_ext, emit)

    def prep_down(j, s):
        def emit(i, v):
            wdcb[j, pl.ds(s * 16 + i * MB, 16), :] = v.astype(bf16)
        return prep_strip(j, 2 * NTR + 2 * s, MB // 8, _LHS_SPEC, _lhs_terms,
                          (2, 0, 3, 6, 4, 5, 1), emit)

    def prep_chunk(j):
        for m in range(2):
            for s in range(8):
                yield from prep_gu(j, m, s)
            for s in range(4):
                yield from prep_ext(j, m, s)
        for s in range(9):
            yield from prep_down(j, s)

    def feed(gen, z, n):
        for _ in range(n):
            try:
                gen.send(z)
            except StopIteration:
                return

    class Pace:
        def __init__(self):
            self.tok = 0
            self.plan = []
            self.due = []

        def add(self, gen, t0, period, lat=None, gated=0, n=1000, primed=False):
            if not primed:
                next(gen)
            when = [self.tok + int(t0 + k * period) for k in range(n)]
            self.plan.append((gen, when, lat, gated))

        def step(self, z):
            for gen, when, lat, gated in self.plan:
                for _ in range(when.count(self.tok)):
                    try:
                        v = gen.send((z, gated - 1) if gated else None)
                    except StopIteration:
                        break
                    if v is not None and lat is not None:
                        self.due.append((self.tok + lat, v))
            self.tok += 1

        def tokens(self, r, n):
            for k in range(n):
                self.step(r[k * 16:k * 16 + 8])

        def gate(self, v):
            now = [x for t, x in self.due if t <= self.tok]
            self.due = [(t, x) for t, x in self.due if t > self.tok]
            if not now:
                return v
            head = jnp.where(never[0], pltpu.bitcast(tree(now), u32), v[0:8])
            return jnp.concatenate([head, v[8:]], axis=0)

        def drain(self):
            for gen, *_ in self.plan:
                feed(gen, None, 1000)

    def tree(vals):
        while len(vals) > 1:
            vals = [a + b for a, b in zip(vals[::2], vals[1::2])] + vals[len(vals) & ~1:]
        return vals[0]

    def norm_slab(row, emit):
        def rows(k, lo, hi):
            return [row(k, r) for r in range(lo // 8, hi // 8)]

        def mean(vals):
            t = tree([sum(vals[k + 4::4], vals[k]) for k in range(4)])
            t = jnp.sum(t, axis=0, keepdims=True) * (1.0 / D)
            return jnp.broadcast_to(t, (8, 128))
        z = yield
        x = rows(0, 0, D)
        mu = mean([held(v, z) for v in x[:4]] + x[4:])
        m = held(mu, (yield))
        rs = lax.rsqrt(mean([(v - m) * (v - m) for v in rows(1, 0, D)]) + EPS)
        end = None
        for k in (4, 0, 1, 2, 3):
            m = held(mu, (yield end))
            y = jnp.concatenate(
                [(v - m) * rs for v in rows(2, k * 128, min((k + 1) * 128, D))], axis=0).T
            emit(k, y)
            end = y[120:128] if k < 4 else jnp.concatenate([y[120:128]] * 2, axis=1)
        yield end

    def alias(p, n):
        return [jnp.clip(p + k * zero[0], 0, n - 1) for k in range(3)]

    def slab_rows(src, p):
        q = alias(p, NSLAB)
        return lambda k, r: src[q[k], r * 8:r * 8 + 8, :]

    def flush(gen):
        return tree([v for v in gen if v is not None])

    def ln1(p, b):
        def emit(k, y):
            xnb[b, k, :, 0:y.shape[1]] = y.astype(bf16)
        return norm_slab(slab_rows(xa, p), emit)

    def widen(q):
        for r in range(NTR):
            if r % 4 == 0:
                z = yield
            v = _up(held(xin32[q, r], z)).astype(f32)
            for b in range(2):
                xa[2 * q + b, r * 8:r * 8 + 8, :] = v[b * 8:b * 8 + 8]

    def qkv_proj(b, pace, groups):
        scale = DH ** -0.5 * LOG2E
        for grp in groups:
            for n in grp:
                if n == 13:
                    ktail[...] = lax.dot_general(
                        _up(wq[4, n * 64:n * 64 + 32, :]), _up(xn[b, 4]), NT,
                        preferred_element_type=f32)
                else:
                    qkv[b, n, HALO:HALO + 128, :] = lax.dot_general(
                        _up(xn[b, 4]), _up(wq[4, n * 64:(n + 1) * 64, :]), NT,
                        preferred_element_type=f32)
            for n in grp:
                rows = slice(n * 64, n * 64 + (32 if n == 13 else 64))
                x = jnp.concatenate(
                    [_up(pace.gate(xn[b, 0]))] + [_up(xn[b, k]) for k in range(1, 4)], axis=1)
                w = jnp.concatenate([_up(wq[k, rows, :]) for k in range(4)], axis=1)
                if n == 13:
                    r = lax.dot_general(w, x, NT, preferred_element_type=f32)
                    r = r + jnp.concatenate([ktail[0:32, :], ktail[32:64, :]], axis=0)
                    qkv[b, n, HALO:HALO + 128, 0:64] = (r * scale).T
                    pace.tokens(r, 4)
                    continue
                r = lax.dot_general(x, w, NT, preferred_element_type=f32)
                r = r + jnp.concatenate([qkv[b, n, HALO:HALO + 64, :],
                                         qkv[b, n, HALO + 64:HALO + 128, :]], axis=0)
                if n in (4, 5, 6, 7):
                    r = r * scale
                qkv[b, n, HALO:HALO + 128, :] = r
                pace.tokens(r, 7)

    def halo(b):
        for n in range(4, 14):
            qkv[b, n, 0:HALO, :] = qkv[1 - b, n, 128:128 + HALO, :]

    def attend(b, row0):
        qs, ks, vs = (0, 1, 2, 3, 12), (4, 5, 6, 7, 13), (8, 9, 10, 11, 12)
        v = None
        for s in range(16):
            z = yield v
            r = HALO + s * 8
            q = [held(qkv[b, n, r:r + 8, :], z) for n in qs]
            logit = []
            for w in range(WIN):
                rw = r - DIL * w
                part = tree([q[c] * qkv[b, ks[c], rw:rw + 8, :] for c in range(5)])
                part = part + pltpu.roll(part, 64, 1)
                part = part + pltpu.roll(part, 32, 1)
                if row0 is not None and s * 8 < DIL * w:
                    pos = row0 + s * 8 + lax.broadcasted_iota(jnp.int32, (8, 128), 0)
                    part = jnp.where(pos >= DIL * w, part, -1e9 * LOG2E)
                logit.append(part)
            mx = logit
            while len(mx) > 1:
                mx = [jnp.maximum(a, c) for a, c in zip(mx[::2], mx[1::2])]
            e = [jnp.exp2(l - mx[0]) for l in logit]
            inv = 1.0 / tree(e)
            outs = []
            for c in range(5):
                o = e[0] * qkv[b, vs[c], r:r + 8, :]
                for w in range(1, WIN):
                    rw = r - DIL * w
                    o = o + e[w] * qkv[b, vs[c], rw:rw + 8, :]
                o = o * inv
                outs.append(o)
                ob[b, c, s * 8:(s + 1) * 8, :] = o.astype(bf16)
            v = tree(outs)
        yield v

    def out_proj(p, b, pace):
        h = MB // 2
        for m in range(4):
            xb[p, m * MB:(m + 1) * MB, :] = xa[p, m * MB:(m + 1) * MB, :] + lax.dot_general(
                _up(wo[4, m * h:(m + 1) * h, :]), _up(o32[b, 4]), NT, preferred_element_type=f32)
        rhs = jnp.concatenate([_up(o32[b, c]) for c in range(4)], axis=1)
        for m in range(4):
            rows = slice(m * h, (m + 1) * h)
            lhs = jnp.concatenate(
                [_up(pace.gate(wo[0, rows, :]))] + [_up(wo[c, rows, :]) for c in range(1, 4)],
                axis=1)
            r = lax.dot_general(lhs, rhs, NT, preferred_element_type=f32)
            r = r + jnp.concatenate([xb[p, m * MB:m * MB + h, :],
                                     xb[p, m * MB + h:(m + 1) * MB, :]], axis=0)
            xb[p, m * MB:(m + 1) * MB, :] = r
            pace.tokens(r, 8)

    def ffn_norm_slab(p, r):
        def emit(k, y):
            xn2[r * 6 + k, :, 0:y.shape[1]] = y
        return norm_slab(slab_rows(xb, p), emit)

    def ffn_norm(t):
        for r in range(4):
            yield from ffn_norm_slab(t * 4 + r, r)

    def strips(load, spec, terms, o, dst):
        for s in range(8):
            z = yield
            rows = slice(s * 16, (s + 1) * 16)

            def ld(r, c):
                v = load(r, c, rows)
                if (r // 2, c // 2) == spec[o][0]:
                    v = jnp.concatenate([held(v[0:8], z), held(v[8:16], z)], axis=0)
                return v

            def emit(i, v):
                dst[i, rows, :] = v.astype(bf16)
            _inner_terms(_outer_term(ld, spec, o), terms, o, emit)

    def lhs_strips(o):
        yield from strips(lambda r, k, rows: xn2[r * 6 + k, rows, :],
                          _LHS_SPEC, _lhs_terms, o, acb)
        if o in AUG:
            for s in range(2):
                z = yield
                rows = slice(s * 64, (s + 1) * 64)
                d = _lhs_ext(_lhs_ext([xn2[r * 6 + 4, rows, 0:64] for r in range(4)])[o])
                for ii, i in enumerate(AUG):
                    aeb[AUG.index(o) * 4 + ii, rows, 0:64] = d[i][0].astype(bf16)

    def ffn_combos():
        for s in range(8):
            rows = slice(s * 16, (s + 1) * 16)
            a = [[xn2[r * 6 + k, rows, :] for k in range(4)] for r in range(4)]

            def emit(i, v, rows=rows):
                acb[i, rows, :] = v.astype(bf16)
            _combos(a, _lhs_terms, emit)
            e = [xn2[r * 6 + 4, rows, 0:64] for r in range(4)]

            def emit_e(i, v, rows=rows):
                aeb[i, rows, 0:64] = v.astype(bf16)
            _ext_combos(e, _lhs_ext, emit_e)

    def attn_pair(h, o, mask, side=None, late=None, extra=None, head=False):
        if not head:
            flush(ln1(h % NSLAB, 0))
        for b in (0, 1):
            pace = Pace()
            if side is not None:
                n = o["pn"] if b == 0 else NPREP - o["pn"]
                lo, hi = o["pw"][b]
                pace.add(side, lo, (hi - lo) / n, gated=o["pg"], n=n, primed=True)
            if b == 0:
                pace.add(ln1((h + 1) % NSLAB, 1), o["l0"], o["lper"], o["llat"], o["lg"])
            elif late is not None:
                pace.add(late, o["w0"], o["wper"], gated=o["wg"])
            if b == 1 and extra is not None:
                pace.add(extra, 32 + o["x0"], o["xper"], gated=o["xg"])
            if b == 1 or not head:
                row0 = (h % NSLAB) * 128 if b == 1 and mask else None
                pace.add(attend(1 - b, row0), *o["a"][b], o["ag"])
                if not head:
                    out_proj((h + b - 2) % NSLAB, b, pace)
                halo(b)
            qkv_proj(b, pace, o["grp"])
            pace.plan = [e for e in pace.plan if e[0] is not side]
            pace.drain()
        if side is not None:
            feed(side, None, 1000)

    def wq_transpose(lo, hi):
        for c0 in range(lo, hi, 128):
            c1 = min(c0 + 128, hi)
            t = wq_raw[:, c0:c1].astype(f32).T
            for k in range(4):
                wtmp[k, c0:c1, :] = t[:, k * 128:(k + 1) * 128]
            wtmp[4, c0:c1, 0:64] = t[:, 512:D]

    def wq_gather(part):
        for k in range(5):
            lanes = slice(0, 128) if k < 4 else slice(0, 64)
            for d in range(DH):
                if d < 16:
                    row = part * 512 + d * 32
                else:
                    row = (1536, 1664, 1600)[part] + (d - 16) * 32
                wqb[k, row:row + 32, lanes] = wtmp[
                    k, pl.ds(part * D + d, H, stride=DH), lanes].astype(bf16)

    def wo_prep():
        for n in range(5):
            w = 128 if n < 4 else 64
            wtmp[n, 0:D, 0:w] = wo_raw[:, n * 128:n * 128 + w].astype(f32)
        for n in range(5):
            w = 128 if n < 4 else 64
            for c in range(5):
                z = yield
                rows = [held(wtmp[n, pl.ds(4 * c + g + k * 8 * DH, 8, stride=DH), :], z)[:, 0:w]
                        for g in range(4 if c < 4 else 2) for k in range(4)]
                if c == 4:
                    rows = [jnp.zeros((64, w), f32)] + rows
                wob[c, n * 128:n * 128 + w, :] = jnp.concatenate(rows, axis=0).T.astype(bf16)

    def head_late():
        for cp in (wo_copy, x_copy(1)):
            cp.wait()
        for cp in [x_copy(2)] + chunk_copies(1):
            cp.start()
        yield from wo_prep()
        yield from widen(1)

    wqb[4, :, 64:128] = jnp.zeros((3 * D, 64), bf16)
    qkv[:, 13] = jnp.zeros((2, HALO + 128, 128), f32)
    xnb[:, 4, :, 64:128] = jnp.zeros((2, 128, 64), bf16)
    for n in range(4, 13):
        qkv[0, n, 0:HALO, :] = jnp.zeros((HALO, 128), f32)
    x_copy(0).wait()
    never.append(zero[0] != 0)
    feed(widen(0), None, 1000)
    flush(ln1(0, 0))
    for k in range(4):
        wq_copies[k].wait()
        if k == OPT["dma"][0]:
            wo_copy.start()
        if k == OPT["dma"][1]:
            for cp in [x_copy(1)] + chunk_copies(0):
                cp.start()
        wq_transpose(edges[k], edges[k + 1])
        if k != 2:
            wq_gather(min(k, 2))
    attn_pair(0, OPT["h"], True, late=head_late(), head=True)

    @pl.loop(0, 7)
    def _(i):
        for cp in chunk_copies(i):
            cp.wait()

        @pl.when(i + 2 < NSLAB // 2)
        def _():
            x_copy(i + 2).wait()

        @pl.when(i + 3 < NSLAB // 2)
        def _():
            x_copy(i + 3).start()
        for cp in chunk_copies(i + 2):
            cp.start()
        side = prep_chunk(i)
        next(side)
        r = jnp.clip(i - 2, 0, 3)
        attn_pair(2 * i + 2, OPT["p"], False, side, widen(jnp.minimum(i + 2, NSLAB // 2 - 1)),
                  ffn_norm_slab(r, r))

    @pl.loop(7, NCHUNK)
    def _(j):
        for cp in chunk_copies(j):
            cp.wait()
        feed(prep_chunk(j), None, 1000)

    ffn_combos()

    def ffn_group(t, g, last):
        ti = _Temps(tin)
        to = _Temps(tout)
        pace = Pace()
        o_ = OPT["fb" if last else "fa"]

        tr = o_["tr"]

        def chain(gens):
            yield
            for gen in gens:
                next(gen)
                z = None
                while True:
                    z = yield
                    try:
                        gen.send(z)
                    except StopIteration:
                        break

        def proj(c, m):
            j = g * 3 + c

            def prod(o, i):
                r = (m * 49 + o * 7 + i) * 64
                p = jnp.dot(_up(ac[o * 7 + i]), _up(wc[j, r:r + 64, :]),
                            preferred_element_type=f32)
                pace.step(p[tr:tr + 8])
                if o in AUG and i in AUG:
                    q = AUG.index(o) * 4 + AUG.index(i)
                    e = jnp.dot(_up(ae[q, :, 0:64]), _up(we[j, m * 16 + q]),
                                preferred_element_type=f32)
                    pace.step(e[tr:tr + 8])
                    p = p + e
                return p
            return prod

        def gate(c):
            def fin(r, cc, v):
                gs[(c % 2) * 16 + r * 4 + cc] = v
            return _recombine(proj(c, 0), fin, ti, to)

        def upgate(c):
            def fin(r, cc, v):
                hs[c, r * 4 + cc] = _ld(gs, (c % 2) * 16 + r * 4 + cc) * v
            yield from _recombine(proj(c, 1), fin, ti, to)
            hgen[c] = chain([strips(lambda cc, r, rows: hs[c, r * 4 + cc, rows, :],
                                    _RHS_SPEC, _rhs_terms, o, hcb.at[c]) for o in ORDER])
            hdone[c] = 0
            pace.add(counted(c), *o_["h"][c], gated=o_["hg"])

        hgen, hdone = {}, {}

        def counted(c):
            next(hgen[c])
            next(hgen[c])
            while True:
                z = yield
                if hdone[c] < 56:
                    need(c, hdone[c] + 1, z)

        def need(c, n, z=None):
            while hdone[c] < n:
                hdone[c] += 1
                feed(hgen[c], z, 1)

        def dprod(cs, i):
            p = None
            for c in cs:
                need(c, 8 * (ORDER.index(i // 7) + 1))
                r = i * (MB // 2)
                q = lax.dot_general(_up(wdc[g * 3 + c, r:r + MB // 2, :]), _up(hc[c, i]), NT,
                                    preferred_element_type=f32)
                pace.step(q[tr:tr + 8])
                p = q if p is None else p + q
            return p

        def down(cs, reset):
            for i in [o * 7 + k for o in ORDER for k in range(7)]:
                a = _ld(acc, i)
                if reset:
                    a = jnp.where(g == 0, 0.0, a)
                acc[i] = a + dprod(cs, i)
                yield

        def down_final(cs):
            def fin(mb, r, v):
                rows = slice(mb * MB, (mb + 1) * MB)
                y = xb[t * 4 + r, rows, :] + v
                xa[t * 4 + r, rows, :] = y
                ost[t * 4 + r, rows, :] = y.astype(bf16)
            return _recombine(lambda o, i: _ld(acc, o * 7 + i) + dprod(cs, o * 7 + i),
                              fin, _Temps(tin2), _Temps(tout2))

        if last:
            norm = ffn_norm((t + 1) % NTILE)
            pace.add(norm, o_["n0"], o_["nper"], gated=o_["ng"])
        for gen in (gate(0), upgate(0), gate(1)):
            _adv(gen, 100)
        d0 = down((0,), not last)
        queue = []

        def lhs_queue():
            while True:
                z = yield
                while queue:
                    try:
                        queue[0].send(z)
                        break
                    except StopIteration:
                        queue.pop(0)
                        break
        for gen, plan in ((upgate(1), "u1"), (gate(2), "g2"), (upgate(2), "u2")):
            if last and plan == "u2":
                feed(norm, None, 1000)
                pace.add(lhs_queue(), o_["l0"], o_["lper"], gated=o_["lg"])
            for k, n in enumerate(o_[plan]):
                _adv(gen, 1)
                if last and plan == "u2":
                    queue.append(lhs_strips(ORDER[k]))
                    next(queue[-1])
                _adv(d0, n)
            _adv(gen, 100)
        _adv(d0, 100)
        _adv(down_final((1, 2)) if last else down((1, 2), False), 100)
        for gen in queue:
            feed(gen, None, 1000)

    @pl.loop(0, 2 * NTILE)
    def _(tile):
        t = tile % NTILE
        if not OPT["skip_ffn"]:
            @pl.loop(0, 2)
            def _(g):
                ffn_group(t, g, False)
            ffn_group(t, 2, True)
        else:
            r0 = pl.multiple_of(zero[0] * 16, 16)
            ost[0, 0:16, :] = wcb[t, pl.ds(r0, 16), :] + wdcb[t, pl.ds(r0, 16), :] + web[t, t, 0:16, :]
            ost[1, 0:16, :] = acb[t, 0:16, :] + aeb[t, 0:16, :]
            ost[2] = xb[t, 0:D, :].astype(bf16)

        @pl.when(tile >= NTILE)
        def _():
            for r in range(4):
                out_copy(t * 4 + r).start()

        @pl.loop(0, jnp.where(tile < NTILE, 2, 0))
        def _(k):
            attn_pair(4 * t + 2 * k + NSLAB, OPT["n"], True)

        @pl.when(tile == NTILE - 1)
        def _():
            o = OPT["e"]
            pace = Pace()
            pace.add(attend(1, None), 0, o["aper"], gated=o["ag"])
            out_proj(NSLAB - 2, 0, pace)
            pace.drain()
            out_proj(NSLAB - 1, 1, Pace())

    for p in range(NSLAB):
        out_copy(p).wait()


def _tiles(w):
    n = w.shape[1]
    return w.reshape(NTR, 8, n // 128, 128).transpose(0, 2, 1, 3).reshape(NTR, n // 16, 128)


@jax.jit
def pallas_interleave_layers__sliding_local_dilated__glu_gated_bilinear__prompt_kernel(
    A_x: jax.Array,
    A_wqkv: jax.Array,
    A_wo: jax.Array,
    B_x: jax.Array,
    B_w_gate: jax.Array,
    B_w_up: jax.Array,
    B_w_down: jax.Array,
):
    del B_x
    vm = pltpu.VMEM
    hbm = pl.BlockSpec(memory_space=pl.ANY)
    out_t = pl.pallas_call(
        _kernel,
        in_specs=[hbm] * 6,
        out_specs=hbm,
        out_shape=jax.ShapeDtypeStruct((D, S), bf16),
        scratch_shapes=[
            vm((NSLAB // 2, 96, 16, 128), bf16),
            vm((NSLAB, 768, 128), f32),
            vm((NSLAB, 768, 128), f32),
            vm((NSLAB, D, 128), bf16),
            vm((D, 3 * D), bf16),
            vm((D, D), bf16),
            vm((5, 3 * D, 128), f32),
            vm((5, 3 * D, 128), bf16),
            vm((5, D, 128), bf16),
            vm((NCHUNK, 224, 32, 128), bf16),
            vm((NCHUNK, WC_ROWS, 128), bf16),
            vm((NCHUNK, 32, 64, 128), bf16),
            vm((NCHUNK, WD_ROWS, 128), bf16),
            vm((2, 5, 128, 128), bf16),
            vm((2, 14, HALO + 128, 128), f32),
            vm((2, 5, 128, 128), bf16),
            vm((24, 128, 128), f32),
            vm((49, 128, 128), bf16),
            vm((16, 128, 128), bf16),
            vm((32, 128, 128), f32),
            vm((3, 16, 128, 128), f32),
            vm((3, 49, 128, 128), bf16),
            vm((49, MB, 128), f32),
            vm((12, 128, 128), f32),
            vm((40, 128, 128), f32),
            vm((12, MB, 128), f32),
            vm((20, MB, 128), f32),
            vm((64, 128), f32),
            pltpu.SMEM((1,), jnp.int32),
            pltpu.SemaphoreType.DMA((NSLAB // 2,)),
            pltpu.SemaphoreType.DMA((5,)),
            pltpu.SemaphoreType.DMA((NCHUNK, 3)),
            pltpu.SemaphoreType.DMA((NSLAB,)),
        ],
        compiler_params=pltpu.CompilerParams(vmem_limit_bytes=120 * 1024 * 1024),
    )(_tiles(A_x[0].T), A_wqkv, A_wo, _tiles(B_w_gate), _tiles(B_w_up), _tiles(B_w_down.T))
    return out_t.T[None]
```

```python
import math

import jax
import jax.numpy as jnp
from jax import lax
import jax.experimental.pallas as pl
import jax.experimental.pallas.tpu as pltpu

f32 = jnp.float32
bf16 = jnp.bfloat16
u32 = jnp.uint32

S, D, F = 2048, 576, 4608
H, DH, WIN, DIL = 32, 18, 8, 2
EPS = 1e-5
LOG2E = math.log2(math.e)
NSLAB = S // 128
TILE = 512
NTILE = S // TILE
FC = 512
NCHUNK = F // FC
MB = D // 4
HALO = 16
NPREP = 158
NTR = D // 8
WC_ROWS = 800 * 16
WD_ROWS = 448 * 16
NT = (((1,), (1,)), ((), ()))
ORDER = (0, 1, 2, 5, 3, 4, 6)
AUG = (0, 1, 2, 5)

OPT = {'skip_ffn': False,
 'dma': (0, 1),
 'edges': (0, 640, 1152, 1280, 1728),
 'fa': {'gm': 0, 'um': 0,
        'h': ((0, 1), (0, 1), (0, 1)),
        'tr': 0,
        'hg': 1,
        'u1': (0, 0, 0, 4, 5, 4, 6),
        'g2': (4, 0, 0, 0, 0, 0, 0),
        'u2': (0, 0, 0, 0, 4, 4, 4)},
 'fb': {'gm': 0, 'um': 0, 'dm': 0,
        'h': ((0, 1), (0, 0.59), (0, 1)),
        'tr': 0,
        'n0': 0,
        'nper': 1.4,
        'l0': 0,
        'lper': 2,
        'hg': 1,
        'lg': 1,
        'ng': 1,
        'u1': (0, 0, 0, 0, 4, 4, 6),
        'g2': (4, 0, 0, 0, 0, 0, 0),
        'u2': (0, 0, 0, 0, 4, 4, 4)},
 'h': {'grp': ((4, 5, 6, 7), (0, 1, 2, 3), (12, 13, 8, 9, 10, 11)),
       'a': ((0, 5, 35), (0, 3.8, 35)),
       'l0': 13,
       'lper': 7.14,
       'llat': None,
       'w0': 2,
       'wper': 2.8,
       'ag': 1,
       'lg': 1,
       'wg': 1},
 'e': {'ag': 0, 'aper': 2.3},
 'p': {'x0': 30,
       'xper': 8,
       'xg': 1,
       'grp': ((4, 13), (5, 6, 7, 0), (1, 2, 3, 12), (8, 9, 10, 11)),
       'a': ((0, 6, 25), (0, 6, 35)),
       'l0': 52,
       'lper': 7.82,
       'llat': None,
       'w0': 59,
       'wper': 5.1,
       'pn': 71,
       'pw': ((0, 130), (0, 126)),
       'ag': 0,
       'lg': 1,
       'wg': 1,
       'pg': 1},
 'n': {'grp': ((4, 5, 6, 13), (7, 0, 1, 2, 3, 12), (8, 9, 10, 11)),
       'a': ((1, 6, 35), (0, 6.6, 35)),
       'l0': 85,
       'lper': 8.04,
       'llat': None,
       'ag': 1,
       'lg': 2}}


def _up(v):
    return pltpu.bitcast(v, bf16)


def _quad(x):
    n = len(x) // 2
    return ([r[:n] for r in x[:n]], [r[n:] for r in x[:n]],
            [r[:n] for r in x[n:]], [r[n:] for r in x[n:]])


def _badd(x, y):
    return [[a + b for a, b in zip(r, s)] for r, s in zip(x, y)]


def _bsub(x, y):
    return [[a - b for a, b in zip(r, s)] for r, s in zip(x, y)]


def _lhs_terms(a):
    a11, a12, a21, a22 = _quad(a)
    return [lambda: _badd(a11, a22), lambda: _badd(a21, a22), lambda: a11, lambda: a22,
            lambda: _badd(a11, a12), lambda: _bsub(a21, a11), lambda: _bsub(a12, a22)]


def _rhs_terms(b):
    b11, b12, b21, b22 = _quad(b)
    return [lambda: _badd(b11, b22), lambda: b11, lambda: _bsub(b12, b22), lambda: _bsub(b21, b11),
            lambda: b22, lambda: _badd(b11, b12), lambda: _badd(b21, b22)]


def _combos(x, terms, emit):
    for o, fo in enumerate(terms(x)):
        y = fo()
        for i, fi in enumerate(terms(y)):
            emit(o * 7 + i, fi()[0][0])


_LHS_SPEC = (((0, 0), (1, 1), 1), ((1, 0), (1, 1), 1), ((0, 0), None, 0), ((1, 1), None, 0),
             ((0, 0), (0, 1), 1), ((1, 0), (0, 0), -1), ((0, 1), (1, 1), -1))
_RHS_SPEC = (((0, 0), (1, 1), 1), ((0, 0), None, 0), ((0, 1), (1, 1), -1), ((1, 0), (0, 0), -1),
             ((1, 1), None, 0), ((0, 0), (0, 1), 1), ((1, 0), (1, 1), 1))


def _outer_term(load, spec, o):
    p, q, sign = spec[o]
    out = []
    for y in range(2):
        row = []
        for z in range(2):
            v = load(2 * p[0] + y, 2 * p[1] + z)
            if sign:
                w = load(2 * q[0] + y, 2 * q[1] + z)
                v = v + w if sign > 0 else v - w
            row.append(v)
        out.append(row)
    return out


def _inner_terms(y, terms, o, emit):
    for i, fi in enumerate(terms(y)):
        emit(o * 7 + i, fi()[0][0])


def _lhs_ext(e):
    n = len(e) // 2
    return {0: e[:n], 1: e[n:], 2: e[:n], 5: [y - x for x, y in zip(e[:n], e[n:])]}


def _rhs_ext(e):
    n = len(e) // 2
    return {0: e[:n], 1: e[:n], 2: e[n:], 5: [x + y for x, y in zip(e[:n], e[n:])]}


def _ext_combos(e, fn, emit):
    for oi, o in enumerate(AUG):
        d = fn(fn(e)[o])
        for ii, i in enumerate(AUG):
            emit(oi * 4 + ii, d[i][0])


def _adv(gen, n):
    for _ in range(n):
        try:
            next(gen)
        except StopIteration:
            return


def _ld(ref, idx):
    n = ref.shape[-2] // 2
    return jnp.concatenate([ref[idx, :n, :], ref[idx, n:, :]], axis=0)


class _Temps:
    def __init__(self, ref):
        self.ref = ref
        self.n = 0

    def put(self, v):
        i = self.n % self.ref.shape[0]
        self.n += 1
        self.ref[i] = v
        return i

    def get(self, i):
        return _ld(self.ref, i)


def _recombine(prod, fin, ti, to, mode=0):
    def inner(o, sink):
        a = ti.put(prod(o, 0))
        b = ti.put(prod(o, 1))
        c = ti.put(prod(o, 2))
        sink(1, 1, ti.get(a) - ti.get(b) + ti.get(c) + prod(o, 5))
        if mode == 1 or (mode == 2 and o == 6):
            m3 = prod(o, 3)
            sink(1, 0, ti.get(b) + m3)
            d = ti.put(ti.get(a) + m3)
            m4 = prod(o, 4)
            sink(0, 1, ti.get(c) + m4)
            d = ti.put(ti.get(d) - m4)
            sink(0, 0, ti.get(d) + prod(o, 6))
            return
        if mode == 3:
            m3 = prod(o, 3)
            m4 = prod(o, 4)
            sink(1, 0, ti.get(b) + m3)
            sink(0, 1, ti.get(c) + m4)
            d = ti.put(ti.get(a) + m3 - m4)
            sink(0, 0, ti.get(d) + prod(o, 6))
            return
        m3 = prod(o, 3)
        m4 = prod(o, 4)
        m6 = prod(o, 6)
        sink(1, 0, ti.get(b) + m3)
        sink(0, 1, ti.get(c) + m4)
        sink(0, 0, ti.get(a) + m3 - m4 + m6)

    m = {}
    for o in (0, 1, 2):
        def keep(y, z, v, o=o):
            m[o, y, z] = to.put(v)
        inner(o, keep)
        yield

    def s5(y, z, v):
        fin(2 + y, 2 + z, to.get(m[0, y, z]) - to.get(m[1, y, z]) + to.get(m[2, y, z]) + v)
    inner(5, s5)
    yield

    def s3(y, z, v):
        fin(2 + y, z, to.get(m[1, y, z]) + v)
        m[3, y, z] = to.put(to.get(m[0, y, z]) + v)
    inner(3, s3)
    yield

    def s4(y, z, v):
        fin(y, 2 + z, to.get(m[2, y, z]) + v)
        m[3, y, z] = to.put(to.get(m[3, y, z]) - v)
    inner(4, s4)
    yield

    def s6(y, z, v):
        fin(y, z, to.get(m[3, y, z]) + v)
    inner(6, s6)
    yield


def _kernel(xt_hbm, wqkv_hbm, wo_hbm, wg_hbm, wu_hbm, wdt_hbm, out_hbm,
            xin, xa, xb, ost, wq_raw, wo_raw, wtmp, wqb, wob, raw, wcb, web, wdcb,
            xnb, qkv, ob, xn2, acb, aeb, gs, hs, hcb, acc, tin, tout, tin2, tout2, ktail, zero,
            sem_x, sem_w, sem_c, sem_o):
    wq, wo, wc, we, wdc, xn, o32, ac, ae, hc, raw32, xin32 = [
        r.bitcast(u32) for r in (wqb, wob, wcb, web, wdcb, xnb, ob, acb, aeb, hcb, raw, xin)]

    def x_copy(q):
        return pltpu.make_async_copy(
            xt_hbm.at[:, pl.ds(pl.multiple_of(q * 16, 16), 16), :], xin.at[q, 0:NTR], sem_x.at[q])

    def weight_copy(j, m):
        rows = pl.ds(pl.multiple_of(j * 32, 32), 32)
        return pltpu.make_async_copy((wg_hbm, wu_hbm, wdt_hbm)[m].at[:, rows, :],
                                     raw.at[j, pl.ds(m * NTR, NTR)], sem_c.at[j, m])

    def chunk_copies(j):
        return [weight_copy(j, m) for m in range(3)]

    def out_copy(q, h):
        rows = pl.ds(h * 2 * MB, 2 * MB)
        return pltpu.make_async_copy(
            ost.at[q, rows, :], out_hbm.at[rows, pl.ds(pl.multiple_of(q * 256, 256), 256)],
            sem_o.at[q, h])

    edges = OPT["edges"]
    wq_copies = [pltpu.make_async_copy(wqkv_hbm.at[:, lo:hi], wq_raw.at[:, lo:hi], sem_w.at[k])
                 for k, (lo, hi) in enumerate(zip(edges, edges[1:]))]
    wo_copy = pltpu.make_async_copy(wo_hbm, wo_raw, sem_w.at[4])
    for cp in [x_copy(0)] + wq_copies:
        cp.start()
    zero[0] = 0
    never = [zero[0] != 0]

    def held(v, z):
        if z is None:
            return v
        return jnp.where(never[z[1]], pltpu.bitcast(z[0], v.dtype), v)

    def raw_pair(j, tr, cp, z):
        v = [_up(held(raw32[j, tr + k, cp * 8:cp * 8 + 8, :], z)).astype(f32) for k in range(2)]
        return [jnp.concatenate([v[0][h:h + 8], v[1][h:h + 8]], axis=0) for h in (0, 8)]

    def prep_strip(j, tr, step, spec, terms, path, emit):
        live = {}
        for o in path:
            used = [q for q in spec[o][:2] if q is not None]
            live = {q: live[q] for q in used if q in live}
            for q in used:
                if q not in live:
                    z = yield
                    live[q] = [raw_pair(j, tr + (2 * q[0] + y) * step, q[1], z) for y in range(2)]
            y = _outer_term(lambda r, c: live[r // 2, c // 2][r % 2][c % 2], spec, o)
            _inner_terms(y, terms, o, emit)

    def prep_gu(j, m, s):
        base = m * (49 * 128) + s * 16

        def emit(i, v):
            wcb[j, pl.ds(base + i * 128, 16), :] = v.astype(bf16)
        return prep_strip(j, m * NTR + 2 * s, 16, _RHS_SPEC, _rhs_terms, (1, 0, 4, 2, 5, 3, 6), emit)

    def prep_ext(j, m, s):
        z = yield
        tr = m * NTR + 64 + 2 * s

        def emit(i, v):
            web[j, m * 16 + i, pl.ds(s * 16, 16), :] = v.astype(bf16)
        _ext_combos(raw_pair(j, tr, 0, z) + raw_pair(j, tr, 1, z), _rhs_ext, emit)

    def prep_down(j, s):
        def emit(i, v):
            wdcb[j, pl.ds(s * 16 + i * MB, 16), :] = v.astype(bf16)
        return prep_strip(j, 2 * NTR + 2 * s, MB // 8, _LHS_SPEC, _lhs_terms,
                          (2, 0, 3, 6, 4, 5, 1), emit)

    def prep_chunk(j):
        for m in range(2):
            for s in range(8):
                yield from prep_gu(j, m, s)
            for s in range(4):
                yield from prep_ext(j, m, s)
        for s in range(9):
            yield from prep_down(j, s)

    def feed(gen, z, n):
        for _ in range(n):
            try:
                gen.send(z)
            except StopIteration:
                return

    class Pace:
        def __init__(self):
            self.tok = 0
            self.plan = []
            self.due = []

        def add(self, gen, t0, period, lat=None, gated=0, n=1000, primed=False):
            if not primed:
                next(gen)
            when = [self.tok + int(t0 + k * period) for k in range(n)]
            self.plan.append((gen, when, lat, gated))

        def step(self, z):
            for gen, when, lat, gated in self.plan:
                for _ in range(when.count(self.tok)):
                    try:
                        v = gen.send((z, gated - 1) if gated else None)
                    except StopIteration:
                        break
                    if v is not None and lat is not None:
                        self.due.append((self.tok + lat, v))
            self.tok += 1

        def tokens(self, r, n):
            for k in range(n):
                self.step(r[k * 16:k * 16 + 8])

        def gate(self, v):
            now = [x for t, x in self.due if t <= self.tok]
            self.due = [(t, x) for t, x in self.due if t > self.tok]
            if not now:
                return v
            head = jnp.where(never[0], pltpu.bitcast(tree(now), u32), v[0:8])
            return jnp.concatenate([head, v[8:]], axis=0)

        def drain(self):
            for gen, *_ in self.plan:
                feed(gen, None, 1000)

    def tree(vals):
        while len(vals) > 1:
            vals = [a + b for a, b in zip(vals[::2], vals[1::2])] + vals[len(vals) & ~1:]
        return vals[0]

    def norm_slab(row, emit):
        def rows(k, lo, hi):
            return [row(k, r) for r in range(lo // 8, hi // 8)]

        def mean(vals):
            t = tree([sum(vals[k + 4::4], vals[k]) for k in range(4)])
            t = jnp.sum(t, axis=0, keepdims=True) * (1.0 / D)
            return jnp.broadcast_to(t, (8, 128))
        z = yield
        x = rows(0, 0, D)
        mu = mean([held(v, z) for v in x[:4]] + x[4:])
        m = held(mu, (yield))
        rs = lax.rsqrt(mean([(v - m) * (v - m) for v in rows(1, 0, D)]) + EPS)
        end = None
        for k in (4, 0, 1, 2, 3):
            m = held(mu, (yield end))
            y = jnp.concatenate(
                [(v - m) * rs for v in rows(2, k * 128, min((k + 1) * 128, D))], axis=0).T
            emit(k, y)
            end = y[120:128] if k < 4 else jnp.concatenate([y[120:128]] * 2, axis=1)
        yield end

    def alias(p, n):
        return [jnp.clip(p + k * zero[0], 0, n - 1) for k in range(3)]

    def slab_rows(src, p):
        q = alias(p, NSLAB)
        return lambda k, r: src[q[k], r * 8:r * 8 + 8, :]

    def flush(gen):
        return tree([v for v in gen if v is not None])

    def ln1(p, b):
        def emit(k, y):
            xnb[b, k, :, 0:y.shape[1]] = y.astype(bf16)
        return norm_slab(slab_rows(xa, p), emit)

    def widen(q):
        for r in range(NTR):
            if r % 4 == 0:
                z = yield
            v = _up(held(xin32[q, r], z)).astype(f32)
            for b in range(2):
                xa[2 * q + b, r * 8:r * 8 + 8, :] = v[b * 8:b * 8 + 8]

    def qkv_proj(b, pace, groups):
        scale = DH ** -0.5 * LOG2E
        for grp in groups:
            for n in grp:
                if n == 13:
                    ktail[...] = lax.dot_general(
                        _up(wq[4, n * 64:n * 64 + 32, :]), _up(xn[b, 4]), NT,
                        preferred_element_type=f32)
                else:
                    qkv[b, n, HALO:HALO + 128, :] = lax.dot_general(
                        _up(xn[b, 4]), _up(wq[4, n * 64:(n + 1) * 64, :]), NT,
                        preferred_element_type=f32)
            for n in grp:
                rows = slice(n * 64, n * 64 + (32 if n == 13 else 64))
                x = jnp.concatenate(
                    [_up(pace.gate(xn[b, 0]))] + [_up(xn[b, k]) for k in range(1, 4)], axis=1)
                w = jnp.concatenate([_up(wq[k, rows, :]) for k in range(4)], axis=1)
                if n == 13:
                    r = lax.dot_general(w, x, NT, preferred_element_type=f32)
                    r = r + jnp.concatenate([ktail[0:32, :], ktail[32:64, :]], axis=0)
                    qkv[b, n, HALO:HALO + 128, 0:64] = (r * scale).T
                    pace.tokens(r, 4)
                    continue
                r = lax.dot_general(x, w, NT, preferred_element_type=f32)
                r = r + jnp.concatenate([qkv[b, n, HALO:HALO + 64, :],
                                         qkv[b, n, HALO + 64:HALO + 128, :]], axis=0)
                if n in (4, 5, 6, 7):
                    r = r * scale
                qkv[b, n, HALO:HALO + 128, :] = r
                pace.tokens(r, 7)

    def halo(b):
        for n in range(4, 14):
            qkv[b, n, 0:HALO, :] = qkv[1 - b, n, 128:128 + HALO, :]

    def attend(b, row0):
        qs, ks, vs = (0, 1, 2, 3, 12), (4, 5, 6, 7, 13), (8, 9, 10, 11, 12)
        v = None
        for s in range(16):
            z = yield v
            r = HALO + s * 8
            q = [held(qkv[b, n, r:r + 8, :], z) for n in qs]
            logit = []
            for w in range(WIN):
                rw = r - DIL * w
                part = tree([q[c] * qkv[b, ks[c], rw:rw + 8, :] for c in range(5)])
                part = part + pltpu.roll(part, 64, 1)
                part = part + pltpu.roll(part, 32, 1)
                if row0 is not None and s * 8 < DIL * w:
                    pos = row0 + s * 8 + lax.broadcasted_iota(jnp.int32, (8, 128), 0)
                    part = jnp.where(pos >= DIL * w, part, -1e9 * LOG2E)
                logit.append(part)
            mx = logit
            while len(mx) > 1:
                mx = [jnp.maximum(a, c) for a, c in zip(mx[::2], mx[1::2])]
            e = [jnp.exp2(l - mx[0]) for l in logit]
            inv = 1.0 / tree(e)
            outs = []
            for c in range(5):
                o = e[0] * qkv[b, vs[c], r:r + 8, :]
                for w in range(1, WIN):
                    rw = r - DIL * w
                    o = o + e[w] * qkv[b, vs[c], rw:rw + 8, :]
                o = o * inv
                outs.append(o)
                ob[b, c, s * 8:(s + 1) * 8, :] = o.astype(bf16)
            v = tree(outs)
        yield v

    def out_proj(p, b, pace):
        h = MB // 2
        for m in range(4):
            xb[p, m * MB:(m + 1) * MB, :] = xa[p, m * MB:(m + 1) * MB, :] + lax.dot_general(
                _up(wo[4, m * h:(m + 1) * h, :]), _up(o32[b, 4]), NT, preferred_element_type=f32)
        rhs = jnp.concatenate([_up(o32[b, c]) for c in range(4)], axis=1)
        for m in range(4):
            rows = slice(m * h, (m + 1) * h)
            lhs = jnp.concatenate(
                [_up(pace.gate(wo[0, rows, :]))] + [_up(wo[c, rows, :]) for c in range(1, 4)],
                axis=1)
            r = lax.dot_general(lhs, rhs, NT, preferred_element_type=f32)
            r = r + jnp.concatenate([xb[p, m * MB:m * MB + h, :],
                                     xb[p, m * MB + h:(m + 1) * MB, :]], axis=0)
            xb[p, m * MB:(m + 1) * MB, :] = r
            pace.tokens(r, 8)

    def ffn_norm_slab(p, r):
        def emit(k, y):
            xn2[r * 6 + k, :, 0:y.shape[1]] = y
        return norm_slab(slab_rows(xb, p), emit)

    def ffn_norm(t):
        for r in range(4):
            yield from ffn_norm_slab(t * 4 + r, r)

    def strips(load, spec, terms, o, dst):
        for s in range(8):
            z = yield
            rows = slice(s * 16, (s + 1) * 16)

            def ld(r, c):
                v = load(r, c, rows)
                if (r // 2, c // 2) == spec[o][0]:
                    v = jnp.concatenate([held(v[0:8], z), held(v[8:16], z)], axis=0)
                return v

            def emit(i, v):
                dst[i, rows, :] = v.astype(bf16)
            _inner_terms(_outer_term(ld, spec, o), terms, o, emit)

    def lhs_strips(o):
        yield from strips(lambda r, k, rows: xn2[r * 6 + k, rows, :],
                          _LHS_SPEC, _lhs_terms, o, acb)
        if o in AUG:
            for s in range(2):
                z = yield
                rows = slice(s * 64, (s + 1) * 64)
                d = _lhs_ext(_lhs_ext([xn2[r * 6 + 4, rows, 0:64] for r in range(4)])[o])
                for ii, i in enumerate(AUG):
                    aeb[AUG.index(o) * 4 + ii, rows, 0:64] = d[i][0].astype(bf16)

    def ffn_combos():
        for s in range(8):
            rows = slice(s * 16, (s + 1) * 16)
            a = [[xn2[r * 6 + k, rows, :] for k in range(4)] for r in range(4)]

            def emit(i, v, rows=rows):
                acb[i, rows, :] = v.astype(bf16)
            _combos(a, _lhs_terms, emit)
            e = [xn2[r * 6 + 4, rows, 0:64] for r in range(4)]

            def emit_e(i, v, rows=rows):
                aeb[i, rows, 0:64] = v.astype(bf16)
            _ext_combos(e, _lhs_ext, emit_e)

    def attn_pair(h, o, mask, side=None, late=None, extra=None, head=False):
        if not head:
            flush(ln1(h % NSLAB, 0))
        for b in (0, 1):
            pace = Pace()
            if side is not None:
                n = o["pn"] if b == 0 else NPREP - o["pn"]
                lo, hi = o["pw"][b]
                pace.add(side, lo, (hi - lo) / n, gated=o["pg"], n=n, primed=True)
            if b == 0:
                pace.add(ln1((h + 1) % NSLAB, 1), o["l0"], o["lper"], o["llat"], o["lg"])
            elif late is not None:
                pace.add(late, o["w0"], o["wper"], gated=o["wg"])
            if b == 1 and extra is not None:
                pace.add(extra, 32 + o["x0"], o["xper"], gated=o["xg"])
            if b == 1 or not head:
                row0 = (h % NSLAB) * 128 if b == 1 and mask else None
                pace.add(attend(1 - b, row0), *o["a"][b], o["ag"])
                if not head:
                    out_proj((h + b - 2) % NSLAB, b, pace)
                halo(b)
            qkv_proj(b, pace, o["grp"])
            pace.plan = [e for e in pace.plan if e[0] is not side]
            pace.drain()
        if side is not None:
            feed(side, None, 1000)

    def wq_transpose(lo, hi):
        for c0 in range(lo, hi, 128):
            c1 = min(c0 + 128, hi)
            t = wq_raw[:, c0:c1].astype(f32).T
            for k in range(4):
                wtmp[k, c0:c1, :] = t[:, k * 128:(k + 1) * 128]
            wtmp[4, c0:c1, 0:64] = t[:, 512:D]

    def wq_gather(part):
        for k in range(5):
            lanes = slice(0, 128) if k < 4 else slice(0, 64)
            for d in range(DH):
                if d < 16:
                    row = part * 512 + d * 32
                else:
                    row = (1536, 1664, 1600)[part] + (d - 16) * 32
                wqb[k, row:row + 32, lanes] = wtmp[
                    k, pl.ds(part * D + d, H, stride=DH), lanes].astype(bf16)

    def wo_prep():
        for n in range(5):
            w = 128 if n < 4 else 64
            wtmp[n, 0:D, 0:w] = wo_raw[:, n * 128:n * 128 + w].astype(f32)
        for n in range(5):
            w = 128 if n < 4 else 64
            for c in range(5):
                z = yield
                rows = [held(wtmp[n, pl.ds(4 * c + g + k * 8 * DH, 8, stride=DH), :], z)[:, 0:w]
                        for g in range(4 if c < 4 else 2) for k in range(4)]
                if c == 4:
                    rows = [jnp.zeros((64, w), f32)] + rows
                wob[c, n * 128:n * 128 + w, :] = jnp.concatenate(rows, axis=0).T.astype(bf16)

    def head_late():
        for cp in (wo_copy, x_copy(1)):
            cp.wait()
        for cp in [x_copy(2)] + chunk_copies(1):
            cp.start()
        yield from wo_prep()
        yield from widen(1)

    wqb[4, :, 64:128] = jnp.zeros((3 * D, 64), bf16)
    qkv[:, 13] = jnp.zeros((2, HALO + 128, 128), f32)
    xnb[:, 4, :, 64:128] = jnp.zeros((2, 128, 64), bf16)
    for n in range(4, 13):
        qkv[0, n, 0:HALO, :] = jnp.zeros((HALO, 128), f32)
    x_copy(0).wait()
    never.append(zero[0] != 0)
    feed(widen(0), None, 1000)
    flush(ln1(0, 0))
    for k in range(4):
        wq_copies[k].wait()
        if k == OPT["dma"][0]:
            wo_copy.start()
        if k == OPT["dma"][1]:
            for cp in [x_copy(1)] + chunk_copies(0):
                cp.start()
        wq_transpose(edges[k], edges[k + 1])
        if k != 2:
            wq_gather(min(k, 2))
    attn_pair(0, OPT["h"], True, late=head_late(), head=True)

    @pl.loop(0, 7)
    def _(i):
        for cp in chunk_copies(i):
            cp.wait()

        @pl.when(i + 2 < NSLAB // 2)
        def _():
            x_copy(i + 2).wait()

        @pl.when(i + 3 < NSLAB // 2)
        def _():
            x_copy(i + 3).start()
        for cp in chunk_copies(i + 2):
            cp.start()
        side = prep_chunk(i)
        next(side)
        r = jnp.clip(i - 2, 0, 3)
        attn_pair(2 * i + 2, OPT["p"], False, side, widen(jnp.minimum(i + 2, NSLAB // 2 - 1)),
                  ffn_norm_slab(r, r))

    @pl.loop(7, NCHUNK)
    def _(j):
        for cp in chunk_copies(j):
            cp.wait()
        feed(prep_chunk(j), None, 1000)

    ffn_combos()

    def ffn_group(t, g, last, emit=None):
        ti = _Temps(tin)
        to = _Temps(tout)
        pace = Pace()
        o_ = OPT["fb" if last else "fa"]

        tr = o_["tr"]

        def chain(gens):
            yield
            for gen in gens:
                next(gen)
                z = None
                while True:
                    z = yield
                    try:
                        gen.send(z)
                    except StopIteration:
                        break

        def proj(c, m):
            j = g * 3 + c

            def prod(o, i):
                r = (m * 49 + o * 7 + i) * 64
                p = jnp.dot(_up(ac[o * 7 + i]), _up(wc[j, r:r + 64, :]),
                            preferred_element_type=f32)
                pace.step(p[tr:tr + 8])
                if o in AUG and i in AUG:
                    q = AUG.index(o) * 4 + AUG.index(i)
                    e = jnp.dot(_up(ae[q, :, 0:64]), _up(we[j, m * 16 + q]),
                                preferred_element_type=f32)
                    pace.step(e[tr:tr + 8])
                    p = p + e
                return p
            return prod

        def gate(c):
            def fin(r, cc, v):
                gs[(c % 2) * 16 + r * 4 + cc] = v
            return _recombine(proj(c, 0), fin, ti, to, o_["gm"])

        def upgate(c):
            def fin(r, cc, v):
                hs[c, r * 4 + cc] = _ld(gs, (c % 2) * 16 + r * 4 + cc) * v
            yield from _recombine(proj(c, 1), fin, ti, to, o_["um"])
            hgen[c] = chain([strips(lambda cc, r, rows: hs[c, r * 4 + cc, rows, :],
                                    _RHS_SPEC, _rhs_terms, o, hcb.at[c]) for o in ORDER])
            hdone[c] = 0
            pace.add(counted(c), *o_["h"][c], gated=o_["hg"])

        hgen, hdone = {}, {}

        def counted(c):
            next(hgen[c])
            next(hgen[c])
            while True:
                z = yield
                if hdone[c] < 56:
                    need(c, hdone[c] + 1, z)

        def need(c, n, z=None):
            while hdone[c] < n:
                hdone[c] += 1
                feed(hgen[c], z, 1)

        def dprod(cs, i):
            p = None
            for c in cs:
                need(c, 8 * (ORDER.index(i // 7) + 1))
                r = i * (MB // 2)
                q = lax.dot_general(_up(wdc[g * 3 + c, r:r + MB // 2, :]), _up(hc[c, i]), NT,
                                    preferred_element_type=f32)
                pace.step(q[tr:tr + 8])
                p = q if p is None else p + q
            return p

        def down(cs, reset):
            for i in [o * 7 + k for o in ORDER for k in range(7)]:
                a = _ld(acc, i)
                if reset:
                    a = jnp.where(g == 0, 0.0, a)
                acc[i] = a + dprod(cs, i)
                yield

        def down_final(cs):
            def fin(mb, r, v):
                rows = slice(mb * MB, (mb + 1) * MB)
                y = xb[t * 4 + r, rows, :] + v
                xa[t * 4 + r, rows, :] = y
                ost[t * 2 + r // 2, rows, (r % 2) * 128:(r % 2) * 128 + 128] = y.astype(bf16)
            return _recombine(lambda o, i: _ld(acc, o * 7 + i) + dprod(cs, o * 7 + i),
                              fin, _Temps(tin2), _Temps(tout2), o_["dm"])

        if last:
            norm = ffn_norm((t + 1) % NTILE)
            pace.add(norm, o_["n0"], o_["nper"], gated=o_["ng"])
        for gen in (gate(0), upgate(0), gate(1)):
            _adv(gen, 100)
        d0 = down((0,), not last)
        queue = []

        def lhs_queue():
            while True:
                z = yield
                while queue:
                    try:
                        queue[0].send(z)
                        break
                    except StopIteration:
                        queue.pop(0)
                        break
        for gen, plan in ((upgate(1), "u1"), (gate(2), "g2"), (upgate(2), "u2")):
            if last and plan == "u2":
                feed(norm, None, 1000)
                pace.add(lhs_queue(), o_["l0"], o_["lper"], gated=o_["lg"])
            for k, n in enumerate(o_[plan]):
                _adv(gen, 1)
                if last and plan == "u2":
                    queue.append(lhs_strips(ORDER[k]))
                    next(queue[-1])
                _adv(d0, n)
            _adv(gen, 100)
        _adv(d0, 100)
        if last:
            gen = down_final((1, 2))
            _adv(gen, 3)
            for q, h in ((1, 1), (0, 1), (1, 0), (0, 0)):
                _adv(gen, 1)
                pl.when(emit)(out_copy(t * 2 + q, h).start)
        else:
            _adv(down((1, 2), False), 100)
        for gen in queue:
            feed(gen, None, 1000)

    @pl.loop(0, 2 * NTILE)
    def _(tile):
        t = tile % NTILE
        if not OPT["skip_ffn"]:
            @pl.loop(0, 2)
            def _(g):
                ffn_group(t, g, False)
            ffn_group(t, 2, True, tile >= NTILE)
        else:
            r0 = pl.multiple_of(zero[0] * 16, 16)
            ost[0, 0:16, 0:128] = wcb[t, pl.ds(r0, 16), :] + wdcb[t, pl.ds(r0, 16), :] + web[t, t, 0:16, :]
            ost[1, 0:16, 0:128] = acb[t, 0:16, :] + aeb[t, 0:16, :]
            ost[2, 0:D, 0:128] = xb[t, 0:D, :].astype(bf16)
            for q, h in ((1, 1), (0, 1), (1, 0), (0, 0)):
                pl.when(tile >= NTILE)(out_copy(t * 2 + q, h).start)

        @pl.loop(0, jnp.where(tile < NTILE, 2, 0))
        def _(k):
            attn_pair(4 * t + 2 * k + NSLAB, OPT["n"], True)

        @pl.when(tile == NTILE - 1)
        def _():
            o = OPT["e"]
            pace = Pace()
            pace.add(attend(1, None), 0, o["aper"], gated=o["ag"])
            out_proj(NSLAB - 2, 0, pace)
            pace.drain()
            out_proj(NSLAB - 1, 1, Pace())

    for p in range(NSLAB):
        out_copy(p // 2, p % 2).wait()


def _tiles(w):
    n = w.shape[1]
    return w.reshape(NTR, 8, n // 128, 128).transpose(0, 2, 1, 3).reshape(NTR, n // 16, 128)


@jax.jit
def pallas_interleave_layers__sliding_local_dilated__glu_gated_bilinear__prompt_kernel(
    A_x: jax.Array,
    A_wqkv: jax.Array,
    A_wo: jax.Array,
    B_x: jax.Array,
    B_w_gate: jax.Array,
    B_w_up: jax.Array,
    B_w_down: jax.Array,
):
    del B_x
    vm = pltpu.VMEM
    hbm = pl.BlockSpec(memory_space=pl.ANY)
    out_t = pl.pallas_call(
        _kernel,
        in_specs=[hbm] * 6,
        out_specs=hbm,
        out_shape=jax.ShapeDtypeStruct((D, S), bf16),
        scratch_shapes=[
            vm((NSLAB // 2, 96, 16, 128), bf16),
            vm((NSLAB, 768, 128), f32),
            vm((NSLAB, 768, 128), f32),
            vm((NSLAB // 2, 768, 256), bf16),
            vm((D, 3 * D), bf16),
            vm((D, D), bf16),
            vm((5, 3 * D, 128), f32),
            vm((5, 3 * D, 128), bf16),
            vm((5, D, 128), bf16),
            vm((NCHUNK, 224, 32, 128), bf16),
            vm((NCHUNK, WC_ROWS, 128), bf16),
            vm((NCHUNK, 32, 64, 128), bf16),
            vm((NCHUNK, WD_ROWS, 128), bf16),
            vm((2, 5, 128, 128), bf16),
            vm((2, 14, HALO + 128, 128), f32),
            vm((2, 5, 128, 128), bf16),
            vm((24, 128, 128), f32),
            vm((49, 128, 128), bf16),
            vm((16, 128, 128), bf16),
            vm((32, 128, 128), f32),
            vm((3, 16, 128, 128), f32),
            vm((3, 49, 128, 128), bf16),
            vm((49, MB, 128), f32),
            vm((12, 128, 128), f32),
            vm((40, 128, 128), f32),
            vm((12, MB, 128), f32),
            vm((20, MB, 128), f32),
            vm((64, 128), f32),
            pltpu.SMEM((1,), jnp.int32),
            pltpu.SemaphoreType.DMA((NSLAB // 2,)),
            pltpu.SemaphoreType.DMA((5,)),
            pltpu.SemaphoreType.DMA((NCHUNK, 3)),
            pltpu.SemaphoreType.DMA((NSLAB // 2, 2)),
        ],
        compiler_params=pltpu.CompilerParams(vmem_limit_bytes=120 * 1024 * 1024),
    )(_tiles(A_x[0].T), A_wqkv, A_wo, _tiles(B_w_gate), _tiles(B_w_up), _tiles(B_w_down.T))
    return out_t.T[None]
```

```python
import math

import jax
import jax.numpy as jnp
from jax import lax
import jax.experimental.pallas as pl
import jax.experimental.pallas.tpu as pltpu

f32 = jnp.float32
bf16 = jnp.bfloat16
u32 = jnp.uint32

S, D, F = 2048, 576, 4608
H, DH, WIN, DIL = 32, 18, 8, 2
EPS = 1e-5
LOG2E = math.log2(math.e)
NSLAB = S // 128
TILE = 512
NTILE = S // TILE
FC = 512
NCHUNK = F // FC
MB = D // 4
HALO = 16
NPREP = 158
NTR = D // 8
WC_ROWS = 800 * 16
WD_ROWS = 448 * 16
NT = (((1,), (1,)), ((), ()))
ORDER = (0, 1, 2, 5, 3, 4, 6)
AUG = (0, 1, 2, 5)

OPT = {'skip_ffn': False,
 'dma': (0, 1),
 'edges': (0, 640, 1152, 1280, 1728),
 'fa': {'wts': (1, 0, 3, 1, 0, 1, 2, 3, 1, 2, 0, 0, 0, 0, 0, 1, 3, 4),
        'ng': 1,
        'gm': 0,
        'um': 0,
        'h': ((0, 0.7), (0, 1), (0, 1)),
        'tr': 0,
        'hg': 1,
        'u1': (0, 0, 0, 4, 5, 4, 6),
        'g2': (4, 0, 0, 0, 0, 0, 0),
        'u2': (0, 0, 0, 0, 4, 4, 4)},
 'fb': {'gm': 0,
        'um': 0,
        'dm': 0,
        'h': ((0, 1), (0, 0.59), (0, 1)),
        'tr': 0,
        'n0': 0,
        'nper': 1.4,
        'l0': 0,
        'lper': 2,
        'hg': 1,
        'lg': 1,
        'ng': 1,
        'u1': (0, 0, 0, 0, 4, 4, 6),
        'g2': (4, 0, 0, 0, 0, 0, 0),
        'u2': (0, 0, 0, 0, 4, 4, 4)},
 'h': {'grp': ((4, 5, 6, 7), (0, 1, 2, 3), (12, 13, 8, 9, 10, 11)),
       'a': ((0, 5, 35), (0, 3.8, 35)),
       'l0': 5,
       'lper': 5.0,
       'llat': None,
       'w0': 2,
       'wper': 2.8,
       'ag': 1,
       'lg': 1,
       'wg': 1},
 'e': {'ag': 0, 'aper': 2.3},
 'p': {'x0': 30,
       'xper': 8,
       'xg': 1,
       'grp': ((4, 13), (5, 6, 7, 0), (1, 2, 3, 12), (8, 9, 10, 11)),
       'a': ((0, 6, 25), (0, 6, 35)),
       'l0': 52,
       'lper': 7.82,
       'llat': None,
       'w0': 59,
       'wper': 4.33,
       'pn': 71,
       'pw': ((0, 130), (0, 126)),
       'ag': 0,
       'lg': 1,
       'wg': 1,
       'pg': 1},
 'n': {'grp': ((4, 5, 6, 13), (7, 0, 1, 2, 3, 12), (8, 9, 10, 11)),
       'a': ((1, 6, 35), (0, 6.6, 35)),
       'l0': 85,
       'lper': 8.04,
       'llat': 20,
       'ag': 1,
       'lg': 2}}


def _up(v):
    return pltpu.bitcast(v, bf16)


def _quad(x):
    n = len(x) // 2
    return ([r[:n] for r in x[:n]], [r[n:] for r in x[:n]],
            [r[:n] for r in x[n:]], [r[n:] for r in x[n:]])


def _badd(x, y):
    return [[a + b for a, b in zip(r, s)] for r, s in zip(x, y)]


def _bsub(x, y):
    return [[a - b for a, b in zip(r, s)] for r, s in zip(x, y)]


def _lhs_terms(a):
    a11, a12, a21, a22 = _quad(a)
    return [lambda: _badd(a11, a22), lambda: _badd(a21, a22), lambda: a11, lambda: a22,
            lambda: _badd(a11, a12), lambda: _bsub(a21, a11), lambda: _bsub(a12, a22)]


def _rhs_terms(b):
    b11, b12, b21, b22 = _quad(b)
    return [lambda: _badd(b11, b22), lambda: b11, lambda: _bsub(b12, b22), lambda: _bsub(b21, b11),
            lambda: b22, lambda: _badd(b11, b12), lambda: _badd(b21, b22)]


def _combos(x, terms, emit):
    for o, fo in enumerate(terms(x)):
        y = fo()
        for i, fi in enumerate(terms(y)):
            emit(o * 7 + i, fi()[0][0])


_LHS_SPEC = (((0, 0), (1, 1), 1), ((1, 0), (1, 1), 1), ((0, 0), None, 0), ((1, 1), None, 0),
             ((0, 0), (0, 1), 1), ((1, 0), (0, 0), -1), ((0, 1), (1, 1), -1))
_RHS_SPEC = (((0, 0), (1, 1), 1), ((0, 0), None, 0), ((0, 1), (1, 1), -1), ((1, 0), (0, 0), -1),
             ((1, 1), None, 0), ((0, 0), (0, 1), 1), ((1, 0), (1, 1), 1))


def _outer_term(load, spec, o):
    p, q, sign = spec[o]
    out = []
    for y in range(2):
        row = []
        for z in range(2):
            v = load(2 * p[0] + y, 2 * p[1] + z)
            if sign:
                w = load(2 * q[0] + y, 2 * q[1] + z)
                v = v + w if sign > 0 else v - w
            row.append(v)
        out.append(row)
    return out


def _inner_terms(y, terms, o, emit):
    for i, fi in enumerate(terms(y)):
        emit(o * 7 + i, fi()[0][0])


def _lhs_ext(e):
    n = len(e) // 2
    return {0: e[:n], 1: e[n:], 2: e[:n], 5: [y - x for x, y in zip(e[:n], e[n:])]}


def _rhs_ext(e):
    n = len(e) // 2
    return {0: e[:n], 1: e[:n], 2: e[n:], 5: [x + y for x, y in zip(e[:n], e[n:])]}


def _ext_combos(e, fn, emit):
    for oi, o in enumerate(AUG):
        d = fn(fn(e)[o])
        for ii, i in enumerate(AUG):
            emit(oi * 4 + ii, d[i][0])


def _spread(weights, span, n):
    total, acc, out = sum(weights), 0.0, []
    for k, w in enumerate(weights):
        lo, acc = acc, acc + w * n / total
        count = round(acc) - round(lo)
        out += [k * span + i * span // count for i in range(count)]
    return out


def _adv(gen, n):
    for _ in range(n):
        try:
            next(gen)
        except StopIteration:
            return


def _ld(ref, idx):
    n = ref.shape[-2] // 2
    return jnp.concatenate([ref[idx, :n, :], ref[idx, n:, :]], axis=0)


class _Temps:
    def __init__(self, ref):
        self.ref = ref
        self.n = 0

    def put(self, v):
        i = self.n % self.ref.shape[0]
        self.n += 1
        self.ref[i] = v
        return i

    def get(self, i):
        return _ld(self.ref, i)


def _recombine(prod, fin, ti, to, mode=0):
    def inner(o, sink):
        a = ti.put(prod(o, 0))
        b = ti.put(prod(o, 1))
        c = ti.put(prod(o, 2))
        sink(1, 1, ti.get(a) - ti.get(b) + ti.get(c) + prod(o, 5))
        if mode == 1 or (mode == 2 and o == 6):
            m3 = prod(o, 3)
            sink(1, 0, ti.get(b) + m3)
            d = ti.put(ti.get(a) + m3)
            m4 = prod(o, 4)
            sink(0, 1, ti.get(c) + m4)
            d = ti.put(ti.get(d) - m4)
            sink(0, 0, ti.get(d) + prod(o, 6))
            return
        if mode == 3:
            m3 = prod(o, 3)
            m4 = prod(o, 4)
            sink(1, 0, ti.get(b) + m3)
            sink(0, 1, ti.get(c) + m4)
            d = ti.put(ti.get(a) + m3 - m4)
            sink(0, 0, ti.get(d) + prod(o, 6))
            return
        m3 = prod(o, 3)
        m4 = prod(o, 4)
        m6 = prod(o, 6)
        sink(1, 0, ti.get(b) + m3)
        sink(0, 1, ti.get(c) + m4)
        sink(0, 0, ti.get(a) + m3 - m4 + m6)

    m = {}
    for o in (0, 1, 2):
        def keep(y, z, v, o=o):
            m[o, y, z] = to.put(v)
        inner(o, keep)
        yield

    def s5(y, z, v):
        fin(2 + y, 2 + z, to.get(m[0, y, z]) - to.get(m[1, y, z]) + to.get(m[2, y, z]) + v)
    inner(5, s5)
    yield

    def s3(y, z, v):
        fin(2 + y, z, to.get(m[1, y, z]) + v)
        m[3, y, z] = to.put(to.get(m[0, y, z]) + v)
    inner(3, s3)
    yield

    def s4(y, z, v):
        fin(y, 2 + z, to.get(m[2, y, z]) + v)
        m[3, y, z] = to.put(to.get(m[3, y, z]) - v)
    inner(4, s4)
    yield

    def s6(y, z, v):
        fin(y, z, to.get(m[3, y, z]) + v)
    inner(6, s6)
    yield


def _kernel(xt_hbm, wqkv_hbm, wo_hbm, wg_hbm, wu_hbm, wdt_hbm, out_hbm,
            xin, xa, xb, ost, wq_raw, wo_raw, wtmp, wqb, wob, raw, wcb, web, wdcb, wcb2, web2, wdcb2,
            xnb, qkv, ob, xn2, acb, aeb, gs, hs, hcb, acc, tin, tout, tin2, tout2, ktail, zero,
            sem_x, sem_w, sem_c, sem_o):
    wq, wo, wc, we, wdc, xn, o32, ac, ae, hc, raw32, xin32, wc2, we2, wdc2 = [
        r.bitcast(u32) for r in (wqb, wob, wcb, web, wdcb, xnb, ob, acb, aeb, hcb, raw, xin,
                                 wcb2, web2, wdcb2)]

    def x_copy(q):
        return pltpu.make_async_copy(
            xt_hbm.at[:, pl.ds(pl.multiple_of(q * 16, 16), 16), :], xin.at[q, 0:NTR], sem_x.at[q])

    def weight_copy(j, m):
        rows = pl.ds(pl.multiple_of(j * 32, 32), 32)
        return pltpu.make_async_copy((wg_hbm, wu_hbm, wdt_hbm)[m].at[:, rows, :],
                                     raw.at[j, pl.ds(m * NTR, NTR)], sem_c.at[j, m])

    def chunk_copies(j):
        return [weight_copy(j, m) for m in range(3)]

    def out_copy(q, h):
        rows = pl.ds(h * 2 * MB, 2 * MB)
        return pltpu.make_async_copy(
            ost.at[q, rows, :], out_hbm.at[rows, pl.ds(pl.multiple_of(q * 256, 256), 256)],
            sem_o.at[q, h])

    edges = OPT["edges"]
    wq_copies = [pltpu.make_async_copy(wqkv_hbm.at[:, lo:hi], wq_raw.at[:, lo:hi], sem_w.at[k])
                 for k, (lo, hi) in enumerate(zip(edges, edges[1:]))]
    wo_copy = pltpu.make_async_copy(wo_hbm, wo_raw, sem_w.at[4])
    for cp in [x_copy(0)] + wq_copies:
        cp.start()
    zero[0] = 0
    never = [zero[0] != 0]

    def held(v, z):
        if z is None:
            return v
        return jnp.where(never[z[1]], pltpu.bitcast(z[0], v.dtype), v)

    def raw_pair(j, tr, cp, z):
        v = [_up(held(raw32[j, tr + k, cp * 8:cp * 8 + 8, :], z)).astype(f32) for k in range(2)]
        return [jnp.concatenate([v[0][h:h + 8], v[1][h:h + 8]], axis=0) for h in (0, 8)]

    def prep_strip(j, tr, step, spec, terms, path, emit):
        live = {}
        for o in path:
            used = [q for q in spec[o][:2] if q is not None]
            live = {q: live[q] for q in used if q in live}
            for q in used:
                if q not in live:
                    z = yield
                    live[q] = [raw_pair(j, tr + (2 * q[0] + y) * step, q[1], z) for y in range(2)]
            y = _outer_term(lambda r, c: live[r // 2, c // 2][r % 2][c % 2], spec, o)
            _inner_terms(y, terms, o, emit)

    def prep_gu(j, dst, m, s):
        base = m * (49 * 128) + s * 16

        def emit(i, v):
            dst[pl.ds(base + i * 128, 16), :] = v.astype(bf16)
        return prep_strip(j, m * NTR + 2 * s, 16, _RHS_SPEC, _rhs_terms, (1, 0, 4, 2, 5, 3, 6), emit)

    def prep_ext(j, dst, m, s):
        z = yield
        tr = m * NTR + 64 + 2 * s

        def emit(i, v):
            dst[m * 16 + i, pl.ds(s * 16, 16), :] = v.astype(bf16)
        _ext_combos(raw_pair(j, tr, 0, z) + raw_pair(j, tr, 1, z), _rhs_ext, emit)

    def prep_down(j, dst, s):
        def emit(i, v):
            dst[pl.ds(s * 16 + i * MB, 16), :] = v.astype(bf16)
        return prep_strip(j, 2 * NTR + 2 * s, MB // 8, _LHS_SPEC, _lhs_terms,
                          (2, 0, 3, 6, 4, 5, 1), emit)

    def prep_chunk(j, dst):
        for m in range(2):
            for s in range(8):
                yield from prep_gu(j, dst[0], m, s)
            for s in range(4):
                yield from prep_ext(j, dst[1], m, s)
        for s in range(9):
            yield from prep_down(j, dst[2], s)

    def feed(gen, z, n):
        for _ in range(n):
            try:
                gen.send(z)
            except StopIteration:
                return

    class Pace:
        def __init__(self):
            self.tok = 0
            self.plan = []
            self.due = []

        def add(self, gen, t0, period, lat=None, gated=0, n=1000, primed=False):
            if not primed:
                next(gen)
            when = [self.tok + int(t0 + k * period) for k in range(n)]
            self.plan.append((gen, when, lat, gated))

        def step(self, z):
            for gen, when, lat, gated in self.plan:
                for _ in range(when.count(self.tok)):
                    try:
                        v = gen.send((z, gated - 1) if gated else None)
                    except StopIteration:
                        break
                    if v is not None and lat is not None:
                        self.due.append((self.tok + lat, v))
            self.tok += 1

        def tokens(self, r, n):
            for k in range(n):
                self.step(r[k * 16:k * 16 + 8])

        def gate(self, v):
            now = [x for t, x in self.due if t <= self.tok]
            self.due = [(t, x) for t, x in self.due if t > self.tok]
            if not now:
                return v
            head = jnp.where(never[0], pltpu.bitcast(tree(now), u32), v[0:8])
            return jnp.concatenate([head, v[8:]], axis=0)

        def drain(self):
            for gen, *_ in self.plan:
                feed(gen, None, 1000)

    def tree(vals):
        while len(vals) > 1:
            vals = [a + b for a, b in zip(vals[::2], vals[1::2])] + vals[len(vals) & ~1:]
        return vals[0]

    def norm_slab(row, emit):
        def rows(k, lo, hi):
            return [row(k, r) for r in range(lo // 8, hi // 8)]

        def mean(vals):
            t = tree([sum(vals[k + 4::4], vals[k]) for k in range(4)])
            t = jnp.sum(t, axis=0, keepdims=True) * (1.0 / D)
            return jnp.broadcast_to(t, (8, 128))
        z = yield
        x = rows(0, 0, D)
        mu = mean([held(v, z) for v in x[:4]] + x[4:])
        m = held(mu, (yield))
        rs = lax.rsqrt(mean([(v - m) * (v - m) for v in rows(1, 0, D)]) + EPS)
        end = None
        for k in (4, 0, 1, 2, 3):
            m = held(mu, (yield end))
            y = jnp.concatenate(
                [(v - m) * rs for v in rows(2, k * 128, min((k + 1) * 128, D))], axis=0).T
            emit(k, y)
            end = y[120:128] if k < 4 else jnp.concatenate([y[120:128]] * 2, axis=1)
        yield end

    def alias(p, n):
        return [jnp.clip(p + k * zero[0], 0, n - 1) for k in range(3)]

    def slab_rows(src, p):
        q = alias(p, NSLAB)
        return lambda k, r: src[q[k], r * 8:r * 8 + 8, :]

    def flush(gen):
        return tree([v for v in gen if v is not None])

    def ln1(p, b):
        def emit(k, y):
            xnb[b, k, :, 0:y.shape[1]] = y.astype(bf16)
        return norm_slab(slab_rows(xa, p), emit)

    def widen(q):
        for r in range(NTR):
            if r % 4 == 0:
                z = yield
            v = _up(held(xin32[q, r], z)).astype(f32)
            for b in range(2):
                xa[2 * q + b, r * 8:r * 8 + 8, :] = v[b * 8:b * 8 + 8]

    def qkv_proj(b, pace, groups):
        scale = DH ** -0.5 * LOG2E
        for grp in groups:
            for n in grp:
                if n == 13:
                    ktail[...] = lax.dot_general(
                        _up(wq[4, n * 64:n * 64 + 32, :]), _up(xn[b, 4]), NT,
                        preferred_element_type=f32)
                else:
                    qkv[b, n, HALO:HALO + 128, :] = lax.dot_general(
                        _up(xn[b, 4]), _up(wq[4, n * 64:(n + 1) * 64, :]), NT,
                        preferred_element_type=f32)
            for n in grp:
                rows = slice(n * 64, n * 64 + (32 if n == 13 else 64))
                x = jnp.concatenate(
                    [_up(pace.gate(xn[b, 0]))] + [_up(xn[b, k]) for k in range(1, 4)], axis=1)
                w = jnp.concatenate([_up(wq[k, rows, :]) for k in range(4)], axis=1)
                if n == 13:
                    r = lax.dot_general(w, x, NT, preferred_element_type=f32)
                    r = r + jnp.concatenate([ktail[0:32, :], ktail[32:64, :]], axis=0)
                    qkv[b, n, HALO:HALO + 128, 0:64] = (r * scale).T
                    pace.tokens(r, 4)
                    continue
                r = lax.dot_general(x, w, NT, preferred_element_type=f32)
                r = r + jnp.concatenate([qkv[b, n, HALO:HALO + 64, :],
                                         qkv[b, n, HALO + 64:HALO + 128, :]], axis=0)
                if n in (4, 5, 6, 7):
                    r = r * scale
                qkv[b, n, HALO:HALO + 128, :] = r
                pace.tokens(r, 7)

    def halo(b):
        for n in range(4, 14):
            qkv[b, n, 0:HALO, :] = qkv[1 - b, n, 128:128 + HALO, :]

    def attend(b, row0):
        qs, ks, vs = (0, 1, 2, 3, 12), (4, 5, 6, 7, 13), (8, 9, 10, 11, 12)
        v = None
        for s in range(16):
            z = yield v
            r = HALO + s * 8
            q = [held(qkv[b, n, r:r + 8, :], z) for n in qs]
            logit = []
            for w in range(WIN):
                rw = r - DIL * w
                part = tree([q[c] * qkv[b, ks[c], rw:rw + 8, :] for c in range(5)])
                part = part + pltpu.roll(part, 64, 1)
                part = part + pltpu.roll(part, 32, 1)
                if row0 is not None and s * 8 < DIL * w:
                    pos = row0 + s * 8 + lax.broadcasted_iota(jnp.int32, (8, 128), 0)
                    part = jnp.where(pos >= DIL * w, part, -1e9 * LOG2E)
                logit.append(part)
            mx = logit
            while len(mx) > 1:
                mx = [jnp.maximum(a, c) for a, c in zip(mx[::2], mx[1::2])]
            e = [jnp.exp2(l - mx[0]) for l in logit]
            inv = 1.0 / tree(e)
            outs = []
            for c in range(5):
                o = e[0] * qkv[b, vs[c], r:r + 8, :]
                for w in range(1, WIN):
                    rw = r - DIL * w
                    o = o + e[w] * qkv[b, vs[c], rw:rw + 8, :]
                o = o * inv
                outs.append(o)
                ob[b, c, s * 8:(s + 1) * 8, :] = o.astype(bf16)
            v = tree(outs)
        yield v

    def out_proj(p, b, pace):
        h = MB // 2
        for m in range(4):
            xb[p, m * MB:(m + 1) * MB, :] = xa[p, m * MB:(m + 1) * MB, :] + lax.dot_general(
                _up(wo[4, m * h:(m + 1) * h, :]), _up(o32[b, 4]), NT, preferred_element_type=f32)
        rhs = jnp.concatenate([_up(o32[b, c]) for c in range(4)], axis=1)
        for m in range(4):
            rows = slice(m * h, (m + 1) * h)
            lhs = jnp.concatenate(
                [_up(pace.gate(wo[0, rows, :]))] + [_up(wo[c, rows, :]) for c in range(1, 4)],
                axis=1)
            r = lax.dot_general(lhs, rhs, NT, preferred_element_type=f32)
            r = r + jnp.concatenate([xb[p, m * MB:m * MB + h, :],
                                     xb[p, m * MB + h:(m + 1) * MB, :]], axis=0)
            xb[p, m * MB:(m + 1) * MB, :] = r
            pace.tokens(r, 8)

    def ffn_norm_slab(p, r):
        def emit(k, y):
            xn2[r * 6 + k, :, 0:y.shape[1]] = y
        return norm_slab(slab_rows(xb, p), emit)

    def ffn_norm(t):
        for r in range(4):
            yield from ffn_norm_slab(t * 4 + r, r)

    def strips(load, spec, terms, o, dst):
        for s in range(8):
            z = yield
            rows = slice(s * 16, (s + 1) * 16)

            def ld(r, c):
                v = load(r, c, rows)
                if (r // 2, c // 2) == spec[o][0]:
                    v = jnp.concatenate([held(v[0:8], z), held(v[8:16], z)], axis=0)
                return v

            def emit(i, v):
                dst[i, rows, :] = v.astype(bf16)
            _inner_terms(_outer_term(ld, spec, o), terms, o, emit)

    def lhs_strips(o):
        yield from strips(lambda r, k, rows: xn2[r * 6 + k, rows, :],
                          _LHS_SPEC, _lhs_terms, o, acb)
        if o in AUG:
            for s in range(2):
                z = yield
                rows = slice(s * 64, (s + 1) * 64)
                d = _lhs_ext(_lhs_ext([xn2[r * 6 + 4, rows, 0:64] for r in range(4)])[o])
                for ii, i in enumerate(AUG):
                    aeb[AUG.index(o) * 4 + ii, rows, 0:64] = d[i][0].astype(bf16)

    def ffn_combos():
        for s in range(8):
            rows = slice(s * 16, (s + 1) * 16)
            a = [[xn2[r * 6 + k, rows, :] for k in range(4)] for r in range(4)]

            def emit(i, v, rows=rows):
                acb[i, rows, :] = v.astype(bf16)
            _combos(a, _lhs_terms, emit)
            e = [xn2[r * 6 + 4, rows, 0:64] for r in range(4)]

            def emit_e(i, v, rows=rows):
                aeb[i, rows, 0:64] = v.astype(bf16)
            _ext_combos(e, _lhs_ext, emit_e)

    def attn_pair(h, o, mask, side=None, late=None, extra=None, head=False):
        if not head:
            flush(ln1(h % NSLAB, 0))
        for b in (0, 1):
            pace = Pace()
            if side is not None:
                n = o["pn"] if b == 0 else NPREP - o["pn"]
                lo, hi = o["pw"][b]
                pace.add(side, lo, (hi - lo) / n, gated=o["pg"], n=n, primed=True)
            if b == 0:
                pace.add(ln1((h + 1) % NSLAB, 1), o["l0"], o["lper"], o["llat"], o["lg"])
            elif late is not None:
                pace.add(late, o["w0"], o["wper"], gated=o["wg"])
            if b == 1 and extra is not None:
                pace.add(extra, 32 + o["x0"], o["xper"], gated=o["xg"])
            if b == 1 or not head:
                row0 = (h % NSLAB) * 128 if b == 1 and mask else None
                pace.add(attend(1 - b, row0), *o["a"][b], o["ag"])
                if not head:
                    out_proj((h + b - 2) % NSLAB, b, pace)
                halo(b)
            qkv_proj(b, pace, o["grp"])
            pace.plan = [e for e in pace.plan if e[0] is not side]
            pace.drain()
        if side is not None:
            feed(side, None, 1000)

    def wq_transpose(lo, hi):
        for c0 in range(lo, hi, 128):
            c1 = min(c0 + 128, hi)
            t = wq_raw[:, c0:c1].astype(f32).T
            for k in range(4):
                wtmp[k, c0:c1, :] = t[:, k * 128:(k + 1) * 128]
            wtmp[4, c0:c1, 0:64] = t[:, 512:D]

    def wq_gather(part):
        for k in range(5):
            lanes = slice(0, 128) if k < 4 else slice(0, 64)
            for d in range(DH):
                if d < 16:
                    row = part * 512 + d * 32
                else:
                    row = (1536, 1664, 1600)[part] + (d - 16) * 32
                wqb[k, row:row + 32, lanes] = wtmp[
                    k, pl.ds(part * D + d, H, stride=DH), lanes].astype(bf16)

    def wo_prep():
        for n in range(5):
            w = 128 if n < 4 else 64
            wtmp[n, 0:D, 0:w] = wo_raw[:, n * 128:n * 128 + w].astype(f32)
        for n in range(5):
            w = 128 if n < 4 else 64
            for c in range(5):
                z = yield
                rows = [held(wtmp[n, pl.ds(4 * c + g + k * 8 * DH, 8, stride=DH), :], z)[:, 0:w]
                        for g in range(4 if c < 4 else 2) for k in range(4)]
                if c == 4:
                    rows = [jnp.zeros((64, w), f32)] + rows
                wob[c, n * 128:n * 128 + w, :] = jnp.concatenate(rows, axis=0).T.astype(bf16)

    def head_late():
        for cp in (wo_copy, x_copy(1)):
            cp.wait()
        for cp in [x_copy(2)] + chunk_copies(1):
            cp.start()
        yield from wo_prep()
        yield from widen(1)

    wqb[4, :, 64:128] = jnp.zeros((3 * D, 64), bf16)
    qkv[:, 13] = jnp.zeros((2, HALO + 128, 128), f32)
    xnb[:, 4, :, 64:128] = jnp.zeros((2, 128, 64), bf16)
    for n in range(4, 13):
        qkv[0, n, 0:HALO, :] = jnp.zeros((HALO, 128), f32)
    x_copy(0).wait()
    never.append(zero[0] != 0)
    feed(widen(0), None, 1000)
    flush(ln1(0, 0))
    for k in range(4):
        wq_copies[k].wait()
        if k == OPT["dma"][0]:
            wo_copy.start()
        if k == OPT["dma"][1]:
            for cp in [x_copy(1)] + chunk_copies(0):
                cp.start()
        wq_transpose(edges[k], edges[k + 1])
        if k != 2:
            wq_gather(min(k, 2))
    attn_pair(0, OPT["h"], True, late=head_late(), head=True)

    @pl.loop(0, 7)
    def _(i):
        for cp in chunk_copies(i):
            cp.wait()

        @pl.when(i + 2 < NSLAB // 2)
        def _():
            x_copy(i + 2).wait()

        @pl.when(i + 3 < NSLAB // 2)
        def _():
            x_copy(i + 3).start()
        for cp in chunk_copies(i + 2):
            cp.start()
        side = prep_chunk(i, [r.at[i] for r in (wcb, web, wdcb)])
        next(side)
        r = jnp.clip(i - 2, 0, 3)
        attn_pair(2 * i + 2, OPT["p"], False, side, widen(jnp.minimum(i + 2, NSLAB // 2 - 1)),
                  ffn_norm_slab(r, r))

    for cp in chunk_copies(7) + chunk_copies(8):
        cp.wait()
    ffn_combos()

    def ffn_group(t, g, last, emit=None):
        ti = _Temps(tin)
        to = _Temps(tout)
        pace = Pace()
        o_ = OPT["fb" if last else "fa"]

        tr = o_["tr"]

        def chain(gens):
            yield
            for gen in gens:
                next(gen)
                z = None
                while True:
                    z = yield
                    try:
                        gen.send(z)
                    except StopIteration:
                        break

        def weights(c):
            if last and c > 0:
                return [r.at[c - 1] for r in (wc2, we2, wdc2)]
            return [r.at[g * 3 + c] for r in (wc, we, wdc)]

        def proj(c, m):
            w, w_ext, _ = weights(c)

            def prod(o, i):
                r = (m * 49 + o * 7 + i) * 64
                p = jnp.dot(_up(ac[o * 7 + i]), _up(w[r:r + 64, :]),
                            preferred_element_type=f32)
                pace.step(p[tr:tr + 8])
                if o in AUG and i in AUG:
                    q = AUG.index(o) * 4 + AUG.index(i)
                    e = jnp.dot(_up(ae[q, :, 0:64]), _up(w_ext[m * 16 + q]),
                                preferred_element_type=f32)
                    pace.step(e[tr:tr + 8])
                    p = p + e
                return p
            return prod

        def gate(c):
            def fin(r, cc, v):
                gs[(c % 2) * 16 + r * 4 + cc] = v
            return _recombine(proj(c, 0), fin, ti, to, o_["gm"])

        def upgate(c):
            def fin(r, cc, v):
                hs[c, r * 4 + cc] = _ld(gs, (c % 2) * 16 + r * 4 + cc) * v
            yield from _recombine(proj(c, 1), fin, ti, to, o_["um"])
            hgen[c] = chain([strips(lambda cc, r, rows: hs[c, r * 4 + cc, rows, :],
                                    _RHS_SPEC, _rhs_terms, o, hcb.at[c]) for o in ORDER])
            hdone[c] = 0
            pace.add(counted(c), *o_["h"][c], gated=o_["hg"])

        hgen, hdone = {}, {}

        def counted(c):
            next(hgen[c])
            next(hgen[c])
            while True:
                z = yield
                if hdone[c] < 56:
                    need(c, hdone[c] + 1, z)

        def need(c, n, z=None):
            while hdone[c] < n:
                hdone[c] += 1
                feed(hgen[c], z, 1)

        def dprod(cs, i):
            p = None
            for c in cs:
                need(c, 8 * (ORDER.index(i // 7) + 1))
                r = i * (MB // 2)
                q = lax.dot_general(_up(weights(c)[2][r:r + MB // 2, :]), _up(hc[c, i]), NT,
                                    preferred_element_type=f32)
                pace.step(q[tr:tr + 8])
                p = q if p is None else p + q
            return p

        def down(cs, reset):
            for i in [o * 7 + k for o in ORDER for k in range(7)]:
                a = _ld(acc, i)
                if reset:
                    a = jnp.where(g == 0, 0.0, a)
                acc[i] = a + dprod(cs, i)
                yield

        def down_final(cs):
            def fin(mb, r, v):
                rows = slice(mb * MB, (mb + 1) * MB)
                y = xb[t * 4 + r, rows, :] + v
                xa[t * 4 + r, rows, :] = y
                ost[t * 2 + r // 2, rows, (r % 2) * 128:(r % 2) * 128 + 128] = y.astype(bf16)
            return _recombine(lambda o, i: _ld(acc, o * 7 + i) + dprod(cs, o * 7 + i),
                              fin, _Temps(tin2), _Temps(tout2), o_["dm"])

        if last:
            norm = ffn_norm((t + 1) % NTILE)
            pace.add(norm, o_["n0"], o_["nper"], gated=o_["ng"])
        else:
            late = prep_chunk(7 + g, [r.at[g] for r in (wcb2, web2, wdcb2)])
            next(late)
            pace.plan.append((late, _spread(o_["wts"], 30, NPREP), None, o_["ng"]))
        for gen in (gate(0), upgate(0), gate(1)):
            _adv(gen, 100)
        d0 = down((0,), not last)
        queue = []

        def lhs_queue():
            while True:
                z = yield
                while queue:
                    try:
                        queue[0].send(z)
                        break
                    except StopIteration:
                        queue.pop(0)
                        break
        for gen, plan in ((upgate(1), "u1"), (gate(2), "g2"), (upgate(2), "u2")):
            if last and plan == "u2":
                feed(norm, None, 1000)
                pace.add(lhs_queue(), o_["l0"], o_["lper"], gated=o_["lg"])
            for k, n in enumerate(o_[plan]):
                _adv(gen, 1)
                if last and plan == "u2":
                    queue.append(lhs_strips(ORDER[k]))
                    next(queue[-1])
                _adv(d0, n)
            _adv(gen, 100)
        _adv(d0, 100)
        if last:
            gen = down_final((1, 2))
            _adv(gen, 3)
            for q, h in ((1, 1), (0, 1), (1, 0), (0, 0)):
                _adv(gen, 1)
                pl.when(emit)(out_copy(t * 2 + q, h).start)
        else:
            _adv(down((1, 2), False), 100)
            feed(late, None, 1000)
        for gen in queue:
            feed(gen, None, 1000)

    @pl.loop(0, 2 * NTILE)
    def _(tile):
        t = tile % NTILE
        if not OPT["skip_ffn"]:
            @pl.loop(0, 2)
            def _(g):
                ffn_group(t, g, False)
            ffn_group(t, 2, True, tile >= NTILE)
        else:
            r0 = pl.multiple_of(zero[0] * 16, 16)
            ost[0, 0:16, 0:128] = wcb[t, pl.ds(r0, 16), :] + wdcb[t, pl.ds(r0, 16), :] + web[t, t, 0:16, :]
            ost[1, 0:16, 0:128] = acb[t, 0:16, :] + aeb[t, 0:16, :]
            ost[2, 0:D, 0:128] = xb[t, 0:D, :].astype(bf16)
            for q, h in ((1, 1), (0, 1), (1, 0), (0, 0)):
                pl.when(tile >= NTILE)(out_copy(t * 2 + q, h).start)

        @pl.loop(0, jnp.where(tile < NTILE, 2, 0))
        def _(k):
            attn_pair(4 * t + 2 * k + NSLAB, OPT["n"], True)

        @pl.when(tile == NTILE - 1)
        def _():
            o = OPT["e"]
            pace = Pace()
            pace.add(attend(1, None), 0, o["aper"], gated=o["ag"])
            out_proj(NSLAB - 2, 0, pace)
            pace.drain()
            out_proj(NSLAB - 1, 1, Pace())

    for p in range(NSLAB):
        out_copy(p // 2, p % 2).wait()


def _tiles(w):
    n = w.shape[1]
    return w.reshape(NTR, 8, n // 128, 128).transpose(0, 2, 1, 3).reshape(NTR, n // 16, 128)


@jax.jit
def pallas_interleave_layers__sliding_local_dilated__glu_gated_bilinear__prompt_kernel(
    A_x: jax.Array,
    A_wqkv: jax.Array,
    A_wo: jax.Array,
    B_x: jax.Array,
    B_w_gate: jax.Array,
    B_w_up: jax.Array,
    B_w_down: jax.Array,
):
    del B_x
    vm = pltpu.VMEM
    hbm = pl.BlockSpec(memory_space=pl.ANY)
    out_t = pl.pallas_call(
        _kernel,
        in_specs=[hbm] * 6,
        out_specs=hbm,
        out_shape=jax.ShapeDtypeStruct((D, S), bf16),
        scratch_shapes=[
            vm((NSLAB // 2, 96, 16, 128), bf16),
            vm((NSLAB, 768, 128), f32),
            vm((NSLAB, 768, 128), f32),
            vm((NSLAB // 2, 768, 256), bf16),
            vm((D, 3 * D), bf16),
            vm((D, D), bf16),
            vm((5, 3 * D, 128), f32),
            vm((5, 3 * D, 128), bf16),
            vm((5, D, 128), bf16),
            vm((NCHUNK, 224, 32, 128), bf16),
            vm((7, WC_ROWS, 128), bf16),
            vm((7, 32, 64, 128), bf16),
            vm((7, WD_ROWS, 128), bf16),
            vm((2, WC_ROWS, 128), bf16),
            vm((2, 32, 64, 128), bf16),
            vm((2, WD_ROWS, 128), bf16),
            vm((2, 5, 128, 128), bf16),
            vm((2, 14, HALO + 128, 128), f32),
            vm((2, 5, 128, 128), bf16),
            vm((24, 128, 128), f32),
            vm((49, 128, 128), bf16),
            vm((16, 128, 128), bf16),
            vm((32, 128, 128), f32),
            vm((3, 16, 128, 128), f32),
            vm((3, 49, 128, 128), bf16),
            vm((49, MB, 128), f32),
            vm((12, 128, 128), f32),
            vm((40, 128, 128), f32),
            vm((12, MB, 128), f32),
            vm((20, MB, 128), f32),
            vm((64, 128), f32),
            pltpu.SMEM((1,), jnp.int32),
            pltpu.SemaphoreType.DMA((NSLAB // 2,)),
            pltpu.SemaphoreType.DMA((5,)),
            pltpu.SemaphoreType.DMA((NCHUNK, 3)),
            pltpu.SemaphoreType.DMA((NSLAB // 2, 2)),
        ],
        compiler_params=pltpu.CompilerParams(vmem_limit_bytes=120 * 1024 * 1024),
    )(_tiles(A_x[0].T), A_wqkv, A_wo, _tiles(B_w_gate), _tiles(B_w_up), _tiles(B_w_down.T))
    return out_t.T[None]
```

```python
import math

import jax
import jax.numpy as jnp
from jax import lax
import jax.experimental.pallas as pl
import jax.experimental.pallas.tpu as pltpu

f32 = jnp.float32
bf16 = jnp.bfloat16
u32 = jnp.uint32

S, D, F = 2048, 576, 4608
H, DH, WIN, DIL = 32, 18, 8, 2
EPS = 1e-5
LOG2E = math.log2(math.e)
NSLAB = S // 128
TILE = 512
NTILE = S // TILE
FC = 512
NCHUNK = F // FC
MB = D // 4
HALO = 16
NPREP = 158
NTR = D // 8
WC_ROWS = 800 * 16
WD_ROWS = 448 * 16
NT = (((1,), (1,)), ((), ()))
ORDER = (0, 1, 2, 5, 3, 4, 6)
AUG = (0, 1, 2, 5)

OPT = {'unroll': 0,
 'skip_ffn': False,
 'dma': (0, 2),
 'xpos': 2,
 'parts': (1, 0, 2),
 'fa': {'wts': (1, 0, 3, 1, 0, 1, 2, 3, 1, 2, 0, 0, 0, 0, 0, 1, 3, 4),
        'ng': 1,
        'gm': 0,
        'um': 0,
        'h': ((0, 0.7), (0, 1), (0, 1)),
        'tr': 0,
        'hg': 1,
        'u1': (0, 0, 0, 4, 5, 4, 6),
        'g2': (4, 0, 0, 0, 0, 0, 0),
        'u2': (0, 0, 0, 0, 4, 4, 4)},
 'fb': {'gm': 0,
        'um': 0,
        'dm': 0,
        'h': ((0, 1), (0, 0.59), (0, 1)),
        'tr': 0,
        'n0': 0,
        'nper': 1.4,
        'l0': 0,
        'lper': 2,
        'hg': 1,
        'lg': 1,
        'ng': 1,
        'u1': (0, 0, 0, 0, 4, 4, 6),
        'g2': (4, 0, 0, 0, 0, 0, 0),
        'u2': (0, 0, 0, 0, 4, 4, 4)},
 'h': {'grp': ((4, 5, 6, 7), (0, 1, 2, 3), (12, 13, 8, 9, 10, 11)),
       'a': ((0, 5, 35), (0, 3.65, 35)),
       'l0': 13,
       'lper': 5.0,
       'llat': 40,
       'w0': 22,
       'wper': 2.8,
       'ag': 1,
       'lg': 2,
       'wg': 1},
 'e': {'ag': 0, 'aper': 3.04},
 'p': {'x0': 30,
       'xper': 5.6,
       'xg': 1,
       'grp': ((4, 13), (5, 6, 7, 0), (1, 2, 3, 12), (8, 9, 10, 11)),
       'a': ((0, 6, 25), (0, 6, 35)),
       'l0': 32,
       'lper': 5.47,
       'llat': None,
       'w0': 65,
       'wper': 6.06,
       'pn': 71,
       'pw': ((0, 130), (0, 126)),
       'ag': 0,
       'lg': 1,
       'wg': 1,
       'pg': 1},
 'n': {'grp': ((4, 5, 6, 13), (7, 0, 1, 2, 3, 12), (8, 9, 10, 11)),
       'a': ((1, 6, 35), (0, 6.6, 35)),
       'l0': 85,
       'lper': 8.04,
       'llat': 20,
       'ag': 1,
       'lg': 2}}


def _up(v):
    return pltpu.bitcast(v, bf16)


def _quad(x):
    n = len(x) // 2
    return ([r[:n] for r in x[:n]], [r[n:] for r in x[:n]],
            [r[:n] for r in x[n:]], [r[n:] for r in x[n:]])


def _badd(x, y):
    return [[a + b for a, b in zip(r, s)] for r, s in zip(x, y)]


def _bsub(x, y):
    return [[a - b for a, b in zip(r, s)] for r, s in zip(x, y)]


def _lhs_terms(a):
    a11, a12, a21, a22 = _quad(a)
    return [lambda: _badd(a11, a22), lambda: _badd(a21, a22), lambda: a11, lambda: a22,
            lambda: _badd(a11, a12), lambda: _bsub(a21, a11), lambda: _bsub(a12, a22)]


def _rhs_terms(b):
    b11, b12, b21, b22 = _quad(b)
    return [lambda: _badd(b11, b22), lambda: b11, lambda: _bsub(b12, b22), lambda: _bsub(b21, b11),
            lambda: b22, lambda: _badd(b11, b12), lambda: _badd(b21, b22)]


def _combos(x, terms, emit):
    for o, fo in enumerate(terms(x)):
        y = fo()
        for i, fi in enumerate(terms(y)):
            emit(o * 7 + i, fi()[0][0])


_LHS_SPEC = (((0, 0), (1, 1), 1), ((1, 0), (1, 1), 1), ((0, 0), None, 0), ((1, 1), None, 0),
             ((0, 0), (0, 1), 1), ((1, 0), (0, 0), -1), ((0, 1), (1, 1), -1))
_RHS_SPEC = (((0, 0), (1, 1), 1), ((0, 0), None, 0), ((0, 1), (1, 1), -1), ((1, 0), (0, 0), -1),
             ((1, 1), None, 0), ((0, 0), (0, 1), 1), ((1, 0), (1, 1), 1))


def _outer_term(load, spec, o):
    p, q, sign = spec[o]
    out = []
    for y in range(2):
        row = []
        for z in range(2):
            v = load(2 * p[0] + y, 2 * p[1] + z)
            if sign:
                w = load(2 * q[0] + y, 2 * q[1] + z)
                v = v + w if sign > 0 else v - w
            row.append(v)
        out.append(row)
    return out


def _inner_terms(y, terms, o, emit):
    for i, fi in enumerate(terms(y)):
        emit(o * 7 + i, fi()[0][0])


def _lhs_ext(e):
    n = len(e) // 2
    return {0: e[:n], 1: e[n:], 2: e[:n], 5: [y - x for x, y in zip(e[:n], e[n:])]}


def _rhs_ext(e):
    n = len(e) // 2
    return {0: e[:n], 1: e[:n], 2: e[n:], 5: [x + y for x, y in zip(e[:n], e[n:])]}


def _ext_combos(e, fn, emit):
    for oi, o in enumerate(AUG):
        d = fn(fn(e)[o])
        for ii, i in enumerate(AUG):
            emit(oi * 4 + ii, d[i][0])


def _spread(weights, span, n):
    total, acc, out = sum(weights), 0.0, []
    for k, w in enumerate(weights):
        lo, acc = acc, acc + w * n / total
        count = round(acc) - round(lo)
        out += [k * span + i * span // count for i in range(count)]
    return out


def _adv(gen, n):
    for _ in range(n):
        try:
            next(gen)
        except StopIteration:
            return


def _ld(ref, idx):
    n = ref.shape[-2] // 2
    return jnp.concatenate([ref[idx, :n, :], ref[idx, n:, :]], axis=0)


class _Temps:
    def __init__(self, ref):
        self.ref = ref
        self.n = 0

    def put(self, v):
        i = self.n % self.ref.shape[0]
        self.n += 1
        self.ref[i] = v
        return i

    def get(self, i):
        return _ld(self.ref, i)


def _recombine(prod, fin, ti, to, mode=0):
    def inner(o, sink):
        a = ti.put(prod(o, 0))
        b = ti.put(prod(o, 1))
        c = ti.put(prod(o, 2))
        sink(1, 1, ti.get(a) - ti.get(b) + ti.get(c) + prod(o, 5))
        if mode == 1 or (mode == 2 and o == 6):
            m3 = prod(o, 3)
            sink(1, 0, ti.get(b) + m3)
            d = ti.put(ti.get(a) + m3)
            m4 = prod(o, 4)
            sink(0, 1, ti.get(c) + m4)
            d = ti.put(ti.get(d) - m4)
            sink(0, 0, ti.get(d) + prod(o, 6))
            return
        if mode == 3:
            m3 = prod(o, 3)
            m4 = prod(o, 4)
            sink(1, 0, ti.get(b) + m3)
            sink(0, 1, ti.get(c) + m4)
            d = ti.put(ti.get(a) + m3 - m4)
            sink(0, 0, ti.get(d) + prod(o, 6))
            return
        m3 = prod(o, 3)
        m4 = prod(o, 4)
        m6 = prod(o, 6)
        sink(1, 0, ti.get(b) + m3)
        sink(0, 1, ti.get(c) + m4)
        sink(0, 0, ti.get(a) + m3 - m4 + m6)

    m = {}
    for o in (0, 1, 2):
        def keep(y, z, v, o=o):
            m[o, y, z] = to.put(v)
        inner(o, keep)
        yield

    def s5(y, z, v):
        fin(2 + y, 2 + z, to.get(m[0, y, z]) - to.get(m[1, y, z]) + to.get(m[2, y, z]) + v)
    inner(5, s5)
    yield

    def s3(y, z, v):
        fin(2 + y, z, to.get(m[1, y, z]) + v)
        m[3, y, z] = to.put(to.get(m[0, y, z]) + v)
    inner(3, s3)
    yield

    def s4(y, z, v):
        fin(y, 2 + z, to.get(m[2, y, z]) + v)
        m[3, y, z] = to.put(to.get(m[3, y, z]) - v)
    inner(4, s4)
    yield

    def s6(y, z, v):
        fin(y, z, to.get(m[3, y, z]) + v)
    inner(6, s6)
    yield


def _kernel(xt_hbm, wqkv_hbm, wo_hbm, wg_hbm, wu_hbm, wdt_hbm, out_hbm,
            xin, xa, xb, ost, raw, wcb, web, wdcb, wcb2, web2, wdcb2, xn2,
            wq_raw, wo_raw, wtmp, wqb, wob, xnb, qkv, ob, acb, aeb, gs, hs, hcb, acc, tin, tout, tin2, tout2, ktail, zero,
            sem_x, sem_w, sem_c, sem_o):
    wq, wo, wc, we, wdc, xn, o32, ac, ae, hc, raw32, xin32, wc2, we2, wdc2 = [
        r.bitcast(u32) for r in (wqb, wob, wcb, web, wdcb, xnb, ob, acb, aeb, hcb, raw, xin,
                                 wcb2, web2, wdcb2)]

    def x_copy(q):
        return pltpu.make_async_copy(
            xt_hbm.at[:, pl.ds(pl.multiple_of(q * 16, 16), 16), :], xin.at[q, 0:NTR], sem_x.at[q])

    def weight_copy(j, m):
        rows = pl.ds(pl.multiple_of(j * 32, 32), 32)
        return pltpu.make_async_copy((wg_hbm, wu_hbm, wdt_hbm)[m].at[:, rows, :],
                                     raw.at[j, pl.ds(m * NTR, NTR)], sem_c.at[j, m])

    def chunk_copies(j):
        return [weight_copy(j, m) for m in range(3)]

    def out_copy(q, h):
        rows = pl.ds(h * 2 * MB, 2 * MB)
        return pltpu.make_async_copy(
            ost.at[q, rows, :], out_hbm.at[rows, pl.ds(pl.multiple_of(q * 256, 256), 256)],
            sem_o.at[q, h])

    k_order = (4, 0, 1, 2, 3)
    wq_copies = [pltpu.make_async_copy(wqkv_hbm.at[k * 128:min(k * 128 + 128, D)],
                                       wq_raw.at[k * 128:min(k * 128 + 128, D)], sem_w.at[k])
                 for k in k_order]
    wo_copy = pltpu.make_async_copy(wo_hbm, wo_raw, sem_w.at[5])
    first = wq_copies[:OPT["xpos"]] + [x_copy(0)] + wq_copies[OPT["xpos"]:]
    for cp in first:
        cp.start()
    zero[0] = 0
    never = [zero[0] != 0]

    def held(v, z):
        if z is None:
            return v
        return jnp.where(never[z[1]], pltpu.bitcast(z[0], v.dtype), v)

    def raw_pair(j, tr, cp, z):
        v = [_up(held(raw32[j, tr + k, cp * 8:cp * 8 + 8, :], z)).astype(f32) for k in range(2)]
        return [jnp.concatenate([v[0][h:h + 8], v[1][h:h + 8]], axis=0) for h in (0, 8)]

    def prep_strip(j, tr, step, spec, terms, path, emit):
        live = {}
        for o in path:
            used = [q for q in spec[o][:2] if q is not None]
            live = {q: live[q] for q in used if q in live}
            for q in used:
                if q not in live:
                    z = yield
                    live[q] = [raw_pair(j, tr + (2 * q[0] + y) * step, q[1], z) for y in range(2)]
            y = _outer_term(lambda r, c: live[r // 2, c // 2][r % 2][c % 2], spec, o)
            _inner_terms(y, terms, o, emit)

    def prep_gu(j, dst, m, s):
        base = m * (49 * 128) + s * 16

        def emit(i, v):
            dst[pl.ds(base + i * 128, 16), :] = v.astype(bf16)
        return prep_strip(j, m * NTR + 2 * s, 16, _RHS_SPEC, _rhs_terms, (1, 0, 4, 2, 5, 3, 6), emit)

    def prep_ext(j, dst, m, s):
        z = yield
        tr = m * NTR + 64 + 2 * s

        def emit(i, v):
            dst[m * 16 + i, pl.ds(s * 16, 16), :] = v.astype(bf16)
        _ext_combos(raw_pair(j, tr, 0, z) + raw_pair(j, tr, 1, z), _rhs_ext, emit)

    def prep_down(j, dst, s):
        def emit(i, v):
            dst[pl.ds(s * 16 + i * MB, 16), :] = v.astype(bf16)
        return prep_strip(j, 2 * NTR + 2 * s, MB // 8, _LHS_SPEC, _lhs_terms,
                          (2, 0, 3, 6, 4, 5, 1), emit)

    def prep_chunk(j, dst):
        for m in range(2):
            for s in range(8):
                yield from prep_gu(j, dst[0], m, s)
            for s in range(4):
                yield from prep_ext(j, dst[1], m, s)
        for s in range(9):
            yield from prep_down(j, dst[2], s)

    def feed(gen, z, n):
        for _ in range(n):
            try:
                gen.send(z)
            except StopIteration:
                return

    class Pace:
        def __init__(self):
            self.tok = 0
            self.plan = []
            self.due = []

        def add(self, gen, t0, period, lat=None, gated=0, n=1000, primed=False):
            if not primed:
                next(gen)
            when = [self.tok + int(t0 + k * period) for k in range(n)]
            self.plan.append((gen, when, lat, gated))

        def step(self, z):
            for gen, when, lat, gated in self.plan:
                for _ in range(when.count(self.tok)):
                    try:
                        v = gen.send((z, gated - 1) if gated else None)
                    except StopIteration:
                        break
                    if v is not None and lat is not None:
                        self.due.append((self.tok + lat, v))
            self.tok += 1

        def tokens(self, r, n):
            for k in range(n):
                self.step(r[k * 16:k * 16 + 8])

        def gate(self, v):
            now = [x for t, x in self.due if t <= self.tok]
            self.due = [(t, x) for t, x in self.due if t > self.tok]
            if not now:
                return v
            head = jnp.where(never[0], pltpu.bitcast(tree(now), u32), v[0:8])
            return jnp.concatenate([head, v[8:]], axis=0)

        def drain(self):
            for gen, *_ in self.plan:
                feed(gen, None, 1000)

    def tree(vals):
        while len(vals) > 1:
            vals = [a + b for a, b in zip(vals[::2], vals[1::2])] + vals[len(vals) & ~1:]
        return vals[0]

    def norm_slab(row, emit):
        def rows(k, lo, hi):
            return [row(k, r) for r in range(lo // 8, hi // 8)]

        def mean(vals):
            t = tree([sum(vals[k + 4::4], vals[k]) for k in range(4)])
            t = jnp.sum(t, axis=0, keepdims=True) * (1.0 / D)
            return jnp.broadcast_to(t, (8, 128))
        z = yield
        x = rows(0, 0, D)
        mu = mean([held(v, z) for v in x[:4]] + x[4:])
        m = held(mu, (yield))
        rs = lax.rsqrt(mean([(v - m) * (v - m) for v in rows(1, 0, D)]) + EPS)
        end = None
        for k in (4, 0, 1, 2, 3):
            m = held(mu, (yield end))
            y = jnp.concatenate(
                [(v - m) * rs for v in rows(2, k * 128, min((k + 1) * 128, D))], axis=0).T
            emit(k, y)
            end = y[120:128] if k < 4 else jnp.concatenate([y[120:128]] * 2, axis=1)
        yield end

    def alias(p, n):
        return [jnp.clip(p + k * zero[0], 0, n - 1) for k in range(3)]

    def slab_rows(src, p):
        q = alias(p, NSLAB)
        return lambda k, r: src[q[k], r * 8:r * 8 + 8, :]

    def flush(gen):
        return tree([v for v in gen if v is not None])

    def ln1(p, b):
        def emit(k, y):
            xnb[b, k, :, 0:y.shape[1]] = y.astype(bf16)
        return norm_slab(slab_rows(xa, p), emit)

    def widen(q):
        for r in range(NTR):
            if r % 4 == 0:
                z = yield
            v = _up(held(xin32[q, r], z)).astype(f32)
            for b in range(2):
                xa[2 * q + b, r * 8:r * 8 + 8, :] = v[b * 8:b * 8 + 8]

    def qkv_proj(b, pace, groups):
        scale = DH ** -0.5 * LOG2E
        for grp in groups:
            for n in grp:
                if n == 13:
                    ktail[...] = lax.dot_general(
                        _up(wq[4, n * 64:n * 64 + 32, :]), _up(xn[b, 4]), NT,
                        preferred_element_type=f32)
                else:
                    qkv[b, n, HALO:HALO + 128, :] = lax.dot_general(
                        _up(xn[b, 4]), _up(wq[4, n * 64:(n + 1) * 64, :]), NT,
                        preferred_element_type=f32)
            for n in grp:
                rows = slice(n * 64, n * 64 + (32 if n == 13 else 64))
                x = jnp.concatenate(
                    [_up(pace.gate(xn[b, 0]))] + [_up(xn[b, k]) for k in range(1, 4)], axis=1)
                w = jnp.concatenate([_up(wq[k, rows, :]) for k in range(4)], axis=1)
                if n == 13:
                    r = lax.dot_general(w, x, NT, preferred_element_type=f32)
                    r = r + jnp.concatenate([ktail[0:32, :], ktail[32:64, :]], axis=0)
                    qkv[b, n, HALO:HALO + 128, 0:64] = (r * scale).T
                    pace.tokens(r, 4)
                    continue
                r = lax.dot_general(x, w, NT, preferred_element_type=f32)
                r = r + jnp.concatenate([qkv[b, n, HALO:HALO + 64, :],
                                         qkv[b, n, HALO + 64:HALO + 128, :]], axis=0)
                if n in (4, 5, 6, 7):
                    r = r * scale
                qkv[b, n, HALO:HALO + 128, :] = r
                pace.tokens(r, 7)

    def halo(b):
        for n in range(4, 14):
            qkv[b, n, 0:HALO, :] = qkv[1 - b, n, 128:128 + HALO, :]

    def attend(b, row0):
        qs, ks, vs = (0, 1, 2, 3, 12), (4, 5, 6, 7, 13), (8, 9, 10, 11, 12)
        v = None
        for s in range(16):
            z = yield v
            r = HALO + s * 8
            q = [held(qkv[b, n, r:r + 8, :], z) for n in qs]
            logit = []
            for w in range(WIN):
                rw = r - DIL * w
                part = tree([q[c] * qkv[b, ks[c], rw:rw + 8, :] for c in range(5)])
                part = part + pltpu.roll(part, 64, 1)
                part = part + pltpu.roll(part, 32, 1)
                if row0 is not None and s * 8 < DIL * w:
                    pos = row0 + s * 8 + lax.broadcasted_iota(jnp.int32, (8, 128), 0)
                    part = jnp.where(pos >= DIL * w, part, -1e9 * LOG2E)
                logit.append(part)
            mx = logit
            while len(mx) > 1:
                mx = [jnp.maximum(a, c) for a, c in zip(mx[::2], mx[1::2])]
            e = [jnp.exp2(l - mx[0]) for l in logit]
            inv = 1.0 / tree(e)
            outs = []
            for c in range(5):
                o = e[0] * qkv[b, vs[c], r:r + 8, :]
                for w in range(1, WIN):
                    rw = r - DIL * w
                    o = o + e[w] * qkv[b, vs[c], rw:rw + 8, :]
                o = o * inv
                outs.append(o)
                ob[b, c, s * 8:(s + 1) * 8, :] = o.astype(bf16)
            v = tree(outs)
        yield v

    def out_proj(p, b, pace):
        h = MB // 2
        for m in range(4):
            xb[p, m * MB:(m + 1) * MB, :] = xa[p, m * MB:(m + 1) * MB, :] + lax.dot_general(
                _up(wo[4, m * h:(m + 1) * h, :]), _up(o32[b, 4]), NT, preferred_element_type=f32)
        rhs = jnp.concatenate([_up(o32[b, c]) for c in range(4)], axis=1)
        for m in range(4):
            rows = slice(m * h, (m + 1) * h)
            lhs = jnp.concatenate(
                [_up(pace.gate(wo[0, rows, :]))] + [_up(wo[c, rows, :]) for c in range(1, 4)],
                axis=1)
            r = lax.dot_general(lhs, rhs, NT, preferred_element_type=f32)
            r = r + jnp.concatenate([xb[p, m * MB:m * MB + h, :],
                                     xb[p, m * MB + h:(m + 1) * MB, :]], axis=0)
            xb[p, m * MB:(m + 1) * MB, :] = r
            pace.tokens(r, 8)

    def ffn_norm_slab(p, r):
        def emit(k, y):
            xn2[r * 6 + k, :, 0:y.shape[1]] = y
        return norm_slab(slab_rows(xb, p), emit)

    def ffn_norm(t):
        for r in range(4):
            yield from ffn_norm_slab(t * 4 + r, r)

    def strips(load, spec, terms, o, dst):
        for s in range(8):
            z = yield
            rows = slice(s * 16, (s + 1) * 16)

            def ld(r, c):
                v = load(r, c, rows)
                if (r // 2, c // 2) == spec[o][0]:
                    v = jnp.concatenate([held(v[0:8], z), held(v[8:16], z)], axis=0)
                return v

            def emit(i, v):
                dst[i, rows, :] = v.astype(bf16)
            _inner_terms(_outer_term(ld, spec, o), terms, o, emit)

    def lhs_strips(o):
        yield from strips(lambda r, k, rows: xn2[r * 6 + k, rows, :],
                          _LHS_SPEC, _lhs_terms, o, acb)
        if o in AUG:
            for s in range(2):
                z = yield
                rows = slice(s * 64, (s + 1) * 64)
                d = _lhs_ext(_lhs_ext([xn2[r * 6 + 4, rows, 0:64] for r in range(4)])[o])
                for ii, i in enumerate(AUG):
                    aeb[AUG.index(o) * 4 + ii, rows, 0:64] = d[i][0].astype(bf16)

    def ffn_combos():
        for s in range(8):
            rows = slice(s * 16, (s + 1) * 16)
            a = [[xn2[r * 6 + k, rows, :] for k in range(4)] for r in range(4)]

            def emit(i, v, rows=rows):
                acb[i, rows, :] = v.astype(bf16)
            _combos(a, _lhs_terms, emit)
            e = [xn2[r * 6 + 4, rows, 0:64] for r in range(4)]

            def emit_e(i, v, rows=rows):
                aeb[i, rows, 0:64] = v.astype(bf16)
            _ext_combos(e, _lhs_ext, emit_e)

    def attn_pair(h, o, mask, side=None, late=None, extra=None, head=False):
        if not head:
            flush(ln1(h % NSLAB, 0))
        for b in (0, 1):
            pace = Pace()
            if side is not None:
                n = o["pn"] if b == 0 else NPREP - o["pn"]
                lo, hi = o["pw"][b]
                pace.add(side, lo, (hi - lo) / n, gated=o["pg"], n=n, primed=True)
            if b == 0:
                pace.add(ln1((h + 1) % NSLAB, 1), o["l0"], o["lper"], o["llat"], o["lg"])
            elif late is not None:
                pace.add(late, o["w0"], o["wper"], gated=o["wg"])
            if b == 1 and extra is not None:
                pace.add(extra, 32 + o["x0"], o["xper"], gated=o["xg"])
            if b == 1 or not head:
                row0 = (h % NSLAB) * 128 if b == 1 and mask else None
                pace.add(attend(1 - b, row0), *o["a"][b], o["ag"])
                if not head:
                    out_proj((h + b - 2) % NSLAB, b, pace)
                halo(b)
            qkv_proj(b, pace, o["grp"])
            pace.plan = [e for e in pace.plan if e[0] is not side]
            pace.drain()
        if side is not None:
            feed(side, None, 1000)

    def wq_prep(k):
        w = 128 if k < 4 else 64
        for c0 in range(0, 3 * D, 128):
            c1 = min(c0 + 128, 3 * D)
            wtmp[k, c0:c1, 0:w] = wq_raw[k * 128:k * 128 + w, c0:c1].astype(f32).T
        for part in OPT["parts"]:
            for d in range(DH):
                if d < 16:
                    row = part * 512 + d * 32
                else:
                    row = (1536, 1664, 1600)[part] + (d - 16) * 32
                wqb[k, row:row + 32, 0:w] = wtmp[
                    k, pl.ds(part * D + d, H, stride=DH), 0:w].astype(bf16)

    def wo_prep():
        for n in range(5):
            w = 128 if n < 4 else 64
            wtmp[n, 0:D, 0:w] = wo_raw[:, n * 128:n * 128 + w].astype(f32)
        for n in range(5):
            w = 128 if n < 4 else 64
            for c in range(5):
                z = yield
                rows = [held(wtmp[n, pl.ds(4 * c + g + k * 8 * DH, 8, stride=DH), :], z)[:, 0:w]
                        for g in range(4 if c < 4 else 2) for k in range(4)]
                if c == 4:
                    rows = [jnp.zeros((64, w), f32)] + rows
                wob[c, n * 128:n * 128 + w, :] = jnp.concatenate(rows, axis=0).T.astype(bf16)

    def head_late():
        for cp in (wo_copy, x_copy(1)):
            cp.wait()
        for cp in [x_copy(2)] + chunk_copies(1):
            cp.start()
        yield from wo_prep()
        yield from widen(1)

    wqb[4, :, 64:128] = jnp.zeros((3 * D, 64), bf16)
    qkv[:, 13] = jnp.zeros((2, HALO + 128, 128), f32)
    xnb[:, 4, :, 64:128] = jnp.zeros((2, 128, 64), bf16)
    for n in range(4, 13):
        qkv[0, n, 0:HALO, :] = jnp.zeros((HALO, 128), f32)
    todo = list(k_order)
    for n, cp in enumerate(first):
        cp.wait()
        if n == 0:
            never.append(zero[0] != 0)
        if n == OPT["dma"][0]:
            wo_copy.start()
        if n == OPT["dma"][1]:
            for c in [x_copy(1)] + chunk_copies(0):
                c.start()
        if n == OPT["xpos"]:
            feed(widen(0), None, 1000)
            flush(ln1(0, 0))
        else:
            wq_prep(todo.pop(0))
    attn_pair(0, OPT["h"], True, late=head_late(), head=True)

    @pl.loop(0, 7)
    def _(i):
        for cp in chunk_copies(i):
            cp.wait()

        @pl.when(i + 2 < NSLAB // 2)
        def _():
            x_copy(i + 2).wait()

        @pl.when(i + 3 < NSLAB // 2)
        def _():
            x_copy(i + 3).start()
        for cp in chunk_copies(i + 2):
            cp.start()
        side = prep_chunk(i, [r.at[i] for r in (wcb, web, wdcb)])
        next(side)
        r = jnp.clip(i - 2, 0, 3)
        attn_pair(2 * i + 2, OPT["p"], False, side, widen(jnp.minimum(i + 2, NSLAB // 2 - 1)),
                  ffn_norm_slab(r, r))

    for cp in chunk_copies(7) + chunk_copies(8):
        cp.wait()
    ffn_combos()

    def ffn_group(t, g, last, emit=None):
        ti = _Temps(tin)
        to = _Temps(tout)
        pace = Pace()
        o_ = OPT["fb" if last else "fa"]

        tr = o_["tr"]

        def chain(gens):
            yield
            for gen in gens:
                next(gen)
                z = None
                while True:
                    z = yield
                    try:
                        gen.send(z)
                    except StopIteration:
                        break

        def weights(c):
            if last and c > 0:
                return [r.at[c - 1] for r in (wc2, we2, wdc2)]
            return [r.at[g * 3 + c] for r in (wc, we, wdc)]

        def proj(c, m):
            w, w_ext, _ = weights(c)

            def prod(o, i):
                r = (m * 49 + o * 7 + i) * 64
                p = jnp.dot(_up(ac[o * 7 + i]), _up(w[r:r + 64, :]),
                            preferred_element_type=f32)
                pace.step(p[tr:tr + 8])
                if o in AUG and i in AUG:
                    q = AUG.index(o) * 4 + AUG.index(i)
                    e = jnp.dot(_up(ae[q, :, 0:64]), _up(w_ext[m * 16 + q]),
                                preferred_element_type=f32)
                    pace.step(e[tr:tr + 8])
                    p = p + e
                return p
            return prod

        def gate(c):
            def fin(r, cc, v):
                gs[(c % 2) * 16 + r * 4 + cc] = v
            return _recombine(proj(c, 0), fin, ti, to, o_["gm"])

        def upgate(c):
            def fin(r, cc, v):
                hs[c, r * 4 + cc] = _ld(gs, (c % 2) * 16 + r * 4 + cc) * v
            yield from _recombine(proj(c, 1), fin, ti, to, o_["um"])
            hgen[c] = chain([strips(lambda cc, r, rows: hs[c, r * 4 + cc, rows, :],
                                    _RHS_SPEC, _rhs_terms, o, hcb.at[c]) for o in ORDER])
            hdone[c] = 0
            pace.add(counted(c), *o_["h"][c], gated=o_["hg"])

        hgen, hdone = {}, {}

        def counted(c):
            next(hgen[c])
            next(hgen[c])
            while True:
                z = yield
                if hdone[c] < 56:
                    need(c, hdone[c] + 1, z)

        def need(c, n, z=None):
            while hdone[c] < n:
                hdone[c] += 1
                feed(hgen[c], z, 1)

        def dprod(cs, i):
            p = None
            for c in cs:
                need(c, 8 * (ORDER.index(i // 7) + 1))
                r = i * (MB // 2)
                q = lax.dot_general(_up(weights(c)[2][r:r + MB // 2, :]), _up(hc[c, i]), NT,
                                    preferred_element_type=f32)
                pace.step(q[tr:tr + 8])
                p = q if p is None else p + q
            return p

        def down(cs, reset):
            for i in [o * 7 + k for o in ORDER for k in range(7)]:
                a = _ld(acc, i)
                if reset:
                    a = jnp.where(g == 0, 0.0, a)
                acc[i] = a + dprod(cs, i)
                yield

        def down_final(cs):
            def fin(mb, r, v):
                rows = slice(mb * MB, (mb + 1) * MB)
                y = xb[t * 4 + r, rows, :] + v
                xa[t * 4 + r, rows, :] = y
                ost[t * 2 + r // 2, rows, (r % 2) * 128:(r % 2) * 128 + 128] = y.astype(bf16)
            return _recombine(lambda o, i: _ld(acc, o * 7 + i) + dprod(cs, o * 7 + i),
                              fin, _Temps(tin2), _Temps(tout2), o_["dm"])

        if last:
            norm = ffn_norm((t + 1) % NTILE)
            pace.add(norm, o_["n0"], o_["nper"], gated=o_["ng"])
        else:
            late = prep_chunk(7 + g, [r.at[g] for r in (wcb2, web2, wdcb2)])
            next(late)
            pace.plan.append((late, _spread(o_["wts"], 30, NPREP), None, o_["ng"]))
        for gen in (gate(0), upgate(0), gate(1)):
            _adv(gen, 100)
        d0 = down((0,), not last)
        queue = []

        def lhs_queue():
            while True:
                z = yield
                while queue:
                    try:
                        queue[0].send(z)
                        break
                    except StopIteration:
                        queue.pop(0)
                        break
        for gen, plan in ((upgate(1), "u1"), (gate(2), "g2"), (upgate(2), "u2")):
            if last and plan == "u2":
                feed(norm, None, 1000)
                pace.add(lhs_queue(), o_["l0"], o_["lper"], gated=o_["lg"])
            for k, n in enumerate(o_[plan]):
                _adv(gen, 1)
                if last and plan == "u2":
                    queue.append(lhs_strips(ORDER[k]))
                    next(queue[-1])
                _adv(d0, n)
            _adv(gen, 100)
        _adv(d0, 100)
        if last:
            gen = down_final((1, 2))
            _adv(gen, 3)
            for q, h in ((1, 1), (0, 1), (1, 0), (0, 0)):
                _adv(gen, 1)
                pl.when(emit)(out_copy(t * 2 + q, h).start)
        else:
            _adv(down((1, 2), False), 100)
            feed(late, None, 1000)
        for gen in queue:
            feed(gen, None, 1000)

    @pl.loop(0, 2 * NTILE)
    def _(tile):
        t = tile % NTILE
        if not OPT["skip_ffn"]:
            @pl.loop(0, 2)
            def _(g):
                ffn_group(t, g, False)
            ffn_group(t, 2, True, tile >= NTILE)
        else:
            r0 = pl.multiple_of(zero[0] * 16, 16)
            ost[0, 0:16, 0:128] = wcb[t, pl.ds(r0, 16), :] + wdcb[t, pl.ds(r0, 16), :] + web[t, t, 0:16, :]
            ost[1, 0:16, 0:128] = acb[t, 0:16, :] + aeb[t, 0:16, :]
            ost[2, 0:D, 0:128] = xb[t, 0:D, :].astype(bf16)
            for q, h in ((1, 1), (0, 1), (1, 0), (0, 0)):
                pl.when(tile >= NTILE)(out_copy(t * 2 + q, h).start)

        if OPT["unroll"]:
            @pl.when(tile < NTILE)
            def _():
                for k in range(2):
                    attn_pair(4 * t + 2 * k + NSLAB, OPT["n"], k == 0)
        else:
            @pl.loop(0, jnp.where(tile < NTILE, 2, 0))
            def _(k):
                attn_pair(4 * t + 2 * k + NSLAB, OPT["n"], True)

        @pl.when(tile == NTILE - 1)
        def _():
            o = OPT["e"]
            pace = Pace()
            pace.add(attend(1, None), 0, o["aper"], gated=o["ag"])
            out_proj(NSLAB - 2, 0, pace)
            pace.drain()
            out_proj(NSLAB - 1, 1, Pace())

    for p in range(NSLAB):
        out_copy(p // 2, p % 2).wait()


def _tiles(w):
    n = w.shape[1]
    return w.reshape(NTR, 8, n // 128, 128).transpose(0, 2, 1, 3).reshape(NTR, n // 16, 128)


@jax.jit
def pallas_interleave_layers__sliding_local_dilated__glu_gated_bilinear__prompt_kernel(
    A_x: jax.Array,
    A_wqkv: jax.Array,
    A_wo: jax.Array,
    B_x: jax.Array,
    B_w_gate: jax.Array,
    B_w_up: jax.Array,
    B_w_down: jax.Array,
):
    del B_x
    vm = pltpu.VMEM
    hbm = pl.BlockSpec(memory_space=pl.ANY)
    out_t = pl.pallas_call(
        _kernel,
        in_specs=[hbm] * 6,
        out_specs=hbm,
        out_shape=jax.ShapeDtypeStruct((D, S), bf16),
        scratch_shapes=[
            vm((NSLAB // 2, 96, 16, 128), bf16),
            vm((NSLAB, 768, 128), f32),
            vm((NSLAB, 768, 128), f32),
            vm((NSLAB // 2, 768, 256), bf16),
            vm((NCHUNK, 224, 32, 128), bf16),
            vm((7, WC_ROWS, 128), bf16),
            vm((7, 32, 64, 128), bf16),
            vm((7, WD_ROWS, 128), bf16),
            vm((2, WC_ROWS, 128), bf16),
            vm((2, 32, 64, 128), bf16),
            vm((2, WD_ROWS, 128), bf16),
            vm((24, 128, 128), f32),
            vm((D, 3 * D), bf16),
            vm((D, D), bf16),
            vm((5, 3 * D, 128), f32),
            vm((5, 3 * D, 128), bf16),
            vm((5, D, 128), bf16),
            vm((2, 5, 128, 128), bf16),
            vm((2, 14, HALO + 128, 128), f32),
            vm((2, 5, 128, 128), bf16),
            vm((49, 128, 128), bf16),
            vm((16, 128, 128), bf16),
            vm((32, 128, 128), f32),
            vm((3, 16, 128, 128), f32),
            vm((3, 49, 128, 128), bf16),
            vm((49, MB, 128), f32),
            vm((12, 128, 128), f32),
            vm((40, 128, 128), f32),
            vm((12, MB, 128), f32),
            vm((20, MB, 128), f32),
            vm((64, 128), f32),
            pltpu.SMEM((1,), jnp.int32),
            pltpu.SemaphoreType.DMA((NSLAB // 2,)),
            pltpu.SemaphoreType.DMA((6,)),
            pltpu.SemaphoreType.DMA((NCHUNK, 3)),
            pltpu.SemaphoreType.DMA((NSLAB // 2, 2)),
        ],
        compiler_params=pltpu.CompilerParams(vmem_limit_bytes=120 * 1024 * 1024),
    )(_tiles(A_x[0].T), A_wqkv, A_wo, _tiles(B_w_gate), _tiles(B_w_up), _tiles(B_w_down.T))
    return out_t.T[None]
```

```python
import math

import jax
import jax.numpy as jnp
from jax import lax
import jax.experimental.pallas as pl
import jax.experimental.pallas.tpu as pltpu

f32 = jnp.float32
bf16 = jnp.bfloat16
u32 = jnp.uint32

S, D, F = 2048, 576, 4608
H, DH, WIN, DIL = 32, 18, 8, 2
EPS = 1e-5
LOG2E = math.log2(math.e)
NSLAB = S // 128
TILE = 512
NTILE = S // TILE
FC = 512
NCHUNK = F // FC
MB = D // 4
HALO = 16
NPREP = 158
NTR = D // 8
WC_ROWS = 800 * 16
WD_ROWS = 448 * 16
NT = (((1,), (1,)), ((), ()))
ORDER = (0, 1, 2, 5, 3, 4, 6)
AUG = (0, 1, 2, 5)

OPT = {'skip_ffn': False,
 'dma': (0, 2),
 'xpos': 2,
 'parts': (1, 0, 2),
 'fa': {'wts': (1, 0, 3, 1, 0, 1, 2, 3, 1, 2, 0, 0, 0, 0, 0, 1, 3, 4),
        'ng': 1,
        'gm': 0,
        'um': 0,
        'h': ((0, 0.7), (0, 1), (0, 1)),
        'tr': 0,
        'hg': 1,
        'u1': (0, 0, 0, 4, 5, 4, 6),
        'g2': (4, 0, 0, 0, 0, 0, 0),
        'u2': (0, 0, 0, 0, 4, 4, 4)},
 'fb': {'gm': 0,
        'um': 0,
        'dm': 0,
        'h': ((0, 1), (0, 0.59), (0, 1)),
        'tr': 0,
        'n0': 0,
        'nper': 1.4,
        'l0': 0,
        'lper': 2,
        'hg': 1,
        'lg': 1,
        'ng': 1,
        'u1': (0, 0, 0, 0, 4, 4, 6),
        'g2': (4, 0, 0, 0, 0, 0, 0),
        'u2': (0, 0, 0, 0, 4, 4, 4)},
 'h': {'grp': ((4, 5, 6, 7), (0, 1, 2, 3), (12, 13, 8, 9, 10, 11)),
       'a': ((0, 5, 35), (0, 3.65, 35)),
       'w0': 22,
       'wper': 2.8,
       'ag': 1,
       'lg': 2,
       'wg': 1,
       'ls': ((13, 5.0, 40),)},
 'e': {'ag': 0, 'aper': 3.04},
 'p': {'x0': 30,
       'xper': 5.6,
       'xg': 1,
       'grp': ((4, 13), (5, 6, 7, 0), (1, 2, 3, 12), (8, 9, 10, 11)),
       'a': ((0, 6, 25), (0, 6, 35)),
       'w0': 65,
       'wper': 6.06,
       'pn': 71,
       'pw': ((0, 130), (0, 126)),
       'ag': 0,
       'lg': 1,
       'wg': 1,
       'pg': 1,
       'ls': ((32, 5.47, None),)},
 'n': {'grp': ((4, 5, 6, 7), (0, 1, 2, 3), (12, 13, 8, 9, 10, 11)),
       'a': ((1, 6, 35), (1, 5.4, 35), (1, 6.03, 35), (6, 6.9, 35)),
       'ag': 1,
       'lg': 1,
       'ls': ((77, 5.51, None), (69, 9.25, None), (80, 6.83, None))}}


def _up(v):
    return pltpu.bitcast(v, bf16)


def _quad(x):
    n = len(x) // 2
    return ([r[:n] for r in x[:n]], [r[n:] for r in x[:n]],
            [r[:n] for r in x[n:]], [r[n:] for r in x[n:]])


def _badd(x, y):
    return [[a + b for a, b in zip(r, s)] for r, s in zip(x, y)]


def _bsub(x, y):
    return [[a - b for a, b in zip(r, s)] for r, s in zip(x, y)]


def _lhs_terms(a):
    a11, a12, a21, a22 = _quad(a)
    return [lambda: _badd(a11, a22), lambda: _badd(a21, a22), lambda: a11, lambda: a22,
            lambda: _badd(a11, a12), lambda: _bsub(a21, a11), lambda: _bsub(a12, a22)]


def _rhs_terms(b):
    b11, b12, b21, b22 = _quad(b)
    return [lambda: _badd(b11, b22), lambda: b11, lambda: _bsub(b12, b22), lambda: _bsub(b21, b11),
            lambda: b22, lambda: _badd(b11, b12), lambda: _badd(b21, b22)]


def _combos(x, terms, emit):
    for o, fo in enumerate(terms(x)):
        y = fo()
        for i, fi in enumerate(terms(y)):
            emit(o * 7 + i, fi()[0][0])


_LHS_SPEC = (((0, 0), (1, 1), 1), ((1, 0), (1, 1), 1), ((0, 0), None, 0), ((1, 1), None, 0),
             ((0, 0), (0, 1), 1), ((1, 0), (0, 0), -1), ((0, 1), (1, 1), -1))
_RHS_SPEC = (((0, 0), (1, 1), 1), ((0, 0), None, 0), ((0, 1), (1, 1), -1), ((1, 0), (0, 0), -1),
             ((1, 1), None, 0), ((0, 0), (0, 1), 1), ((1, 0), (1, 1), 1))


def _outer_term(load, spec, o):
    p, q, sign = spec[o]
    out = []
    for y in range(2):
        row = []
        for z in range(2):
            v = load(2 * p[0] + y, 2 * p[1] + z)
            if sign:
                w = load(2 * q[0] + y, 2 * q[1] + z)
                v = v + w if sign > 0 else v - w
            row.append(v)
        out.append(row)
    return out


def _inner_terms(y, terms, o, emit):
    for i, fi in enumerate(terms(y)):
        emit(o * 7 + i, fi()[0][0])


def _lhs_ext(e):
    n = len(e) // 2
    return {0: e[:n], 1: e[n:], 2: e[:n], 5: [y - x for x, y in zip(e[:n], e[n:])]}


def _rhs_ext(e):
    n = len(e) // 2
    return {0: e[:n], 1: e[:n], 2: e[n:], 5: [x + y for x, y in zip(e[:n], e[n:])]}


def _ext_combos(e, fn, emit):
    for oi, o in enumerate(AUG):
        d = fn(fn(e)[o])
        for ii, i in enumerate(AUG):
            emit(oi * 4 + ii, d[i][0])


def _spread(weights, span, n):
    total, acc, out = sum(weights), 0.0, []
    for k, w in enumerate(weights):
        lo, acc = acc, acc + w * n / total
        count = round(acc) - round(lo)
        out += [k * span + i * span // count for i in range(count)]
    return out


def _adv(gen, n):
    for _ in range(n):
        try:
            next(gen)
        except StopIteration:
            return


def _ld(ref, idx):
    n = ref.shape[-2] // 2
    return jnp.concatenate([ref[idx, :n, :], ref[idx, n:, :]], axis=0)


class _Temps:
    def __init__(self, ref):
        self.ref = ref
        self.n = 0

    def put(self, v):
        i = self.n % self.ref.shape[0]
        self.n += 1
        self.ref[i] = v
        return i

    def get(self, i):
        return _ld(self.ref, i)


def _recombine(prod, fin, ti, to, mode=0):
    def inner(o, sink):
        a = ti.put(prod(o, 0))
        b = ti.put(prod(o, 1))
        c = ti.put(prod(o, 2))
        sink(1, 1, ti.get(a) - ti.get(b) + ti.get(c) + prod(o, 5))
        if mode == 1 or (mode == 2 and o == 6):
            m3 = prod(o, 3)
            sink(1, 0, ti.get(b) + m3)
            d = ti.put(ti.get(a) + m3)
            m4 = prod(o, 4)
            sink(0, 1, ti.get(c) + m4)
            d = ti.put(ti.get(d) - m4)
            sink(0, 0, ti.get(d) + prod(o, 6))
            return
        if mode == 3:
            m3 = prod(o, 3)
            m4 = prod(o, 4)
            sink(1, 0, ti.get(b) + m3)
            sink(0, 1, ti.get(c) + m4)
            d = ti.put(ti.get(a) + m3 - m4)
            sink(0, 0, ti.get(d) + prod(o, 6))
            return
        m3 = prod(o, 3)
        m4 = prod(o, 4)
        m6 = prod(o, 6)
        sink(1, 0, ti.get(b) + m3)
        sink(0, 1, ti.get(c) + m4)
        sink(0, 0, ti.get(a) + m3 - m4 + m6)

    m = {}
    for o in (0, 1, 2):
        def keep(y, z, v, o=o):
            m[o, y, z] = to.put(v)
        inner(o, keep)
        yield

    def s5(y, z, v):
        fin(2 + y, 2 + z, to.get(m[0, y, z]) - to.get(m[1, y, z]) + to.get(m[2, y, z]) + v)
    inner(5, s5)
    yield

    def s3(y, z, v):
        fin(2 + y, z, to.get(m[1, y, z]) + v)
        m[3, y, z] = to.put(to.get(m[0, y, z]) + v)
    inner(3, s3)
    yield

    def s4(y, z, v):
        fin(y, 2 + z, to.get(m[2, y, z]) + v)
        m[3, y, z] = to.put(to.get(m[3, y, z]) - v)
    inner(4, s4)
    yield

    def s6(y, z, v):
        fin(y, z, to.get(m[3, y, z]) + v)
    inner(6, s6)
    yield


def _kernel(xt_hbm, wqkv_hbm, wo_hbm, wg_hbm, wu_hbm, wdt_hbm, out_hbm,
            xin, xa, xb, ost, raw, wcb, web, wdcb, wcb2, web2, wdcb2, xn2,
            wq_raw, wo_raw, wtmp, wqb, wob, xnb, qkv, ob, acb, aeb, gs, hs, hcb, acc, tin, tout, tin2, tout2, ktail, zero,
            sem_x, sem_w, sem_c, sem_o):
    wq, wo, wc, we, wdc, xn, o32, ac, ae, hc, raw32, xin32, wc2, we2, wdc2 = [
        r.bitcast(u32) for r in (wqb, wob, wcb, web, wdcb, xnb, ob, acb, aeb, hcb, raw, xin,
                                 wcb2, web2, wdcb2)]

    def x_copy(q):
        return pltpu.make_async_copy(
            xt_hbm.at[:, pl.ds(pl.multiple_of(q * 16, 16), 16), :], xin.at[q, 0:NTR], sem_x.at[q])

    def weight_copy(j, m):
        rows = pl.ds(pl.multiple_of(j * 32, 32), 32)
        return pltpu.make_async_copy((wg_hbm, wu_hbm, wdt_hbm)[m].at[:, rows, :],
                                     raw.at[j, pl.ds(m * NTR, NTR)], sem_c.at[j, m])

    def chunk_copies(j):
        return [weight_copy(j, m) for m in range(3)]

    def out_copy(q, h):
        rows = pl.ds(h * 2 * MB, 2 * MB)
        return pltpu.make_async_copy(
            ost.at[q, rows, :], out_hbm.at[rows, pl.ds(pl.multiple_of(q * 256, 256), 256)],
            sem_o.at[q, h])

    k_order = (4, 0, 1, 2, 3)
    wq_copies = [pltpu.make_async_copy(wqkv_hbm.at[k * 128:min(k * 128 + 128, D)],
                                       wq_raw.at[k * 128:min(k * 128 + 128, D)], sem_w.at[k])
                 for k in k_order]
    wo_copy = pltpu.make_async_copy(wo_hbm, wo_raw, sem_w.at[5])
    first = wq_copies[:OPT["xpos"]] + [x_copy(0)] + wq_copies[OPT["xpos"]:]
    for cp in first:
        cp.start()
    zero[0] = 0
    never = [zero[0] != 0]

    def held(v, z):
        if z is None:
            return v
        return jnp.where(never[z[1]], pltpu.bitcast(z[0], v.dtype), v)

    def raw_pair(j, tr, cp, z):
        v = [_up(held(raw32[j, tr + k, cp * 8:cp * 8 + 8, :], z)).astype(f32) for k in range(2)]
        return [jnp.concatenate([v[0][h:h + 8], v[1][h:h + 8]], axis=0) for h in (0, 8)]

    def prep_strip(j, tr, step, spec, terms, path, emit):
        live = {}
        for o in path:
            used = [q for q in spec[o][:2] if q is not None]
            live = {q: live[q] for q in used if q in live}
            for q in used:
                if q not in live:
                    z = yield
                    live[q] = [raw_pair(j, tr + (2 * q[0] + y) * step, q[1], z) for y in range(2)]
            y = _outer_term(lambda r, c: live[r // 2, c // 2][r % 2][c % 2], spec, o)
            _inner_terms(y, terms, o, emit)

    def prep_gu(j, dst, m, s):
        base = m * (49 * 128) + s * 16

        def emit(i, v):
            dst[pl.ds(base + i * 128, 16), :] = v.astype(bf16)
        return prep_strip(j, m * NTR + 2 * s, 16, _RHS_SPEC, _rhs_terms, (1, 0, 4, 2, 5, 3, 6), emit)

    def prep_ext(j, dst, m, s):
        z = yield
        tr = m * NTR + 64 + 2 * s

        def emit(i, v):
            dst[m * 16 + i, pl.ds(s * 16, 16), :] = v.astype(bf16)
        _ext_combos(raw_pair(j, tr, 0, z) + raw_pair(j, tr, 1, z), _rhs_ext, emit)

    def prep_down(j, dst, s):
        def emit(i, v):
            dst[pl.ds(s * 16 + i * MB, 16), :] = v.astype(bf16)
        return prep_strip(j, 2 * NTR + 2 * s, MB // 8, _LHS_SPEC, _lhs_terms,
                          (2, 0, 3, 6, 4, 5, 1), emit)

    def prep_chunk(j, dst):
        for m in range(2):
            for s in range(8):
                yield from prep_gu(j, dst[0], m, s)
            for s in range(4):
                yield from prep_ext(j, dst[1], m, s)
        for s in range(9):
            yield from prep_down(j, dst[2], s)

    def feed(gen, z, n):
        for _ in range(n):
            try:
                gen.send(z)
            except StopIteration:
                return

    class Pace:
        def __init__(self):
            self.tok = 0
            self.plan = []
            self.due = []

        def add(self, gen, t0, period, lat=None, gated=0, n=1000, primed=False):
            if not primed:
                next(gen)
            when = [self.tok + int(t0 + k * period) for k in range(n)]
            self.plan.append((gen, when, lat, gated))

        def step(self, z):
            for gen, when, lat, gated in self.plan:
                for _ in range(when.count(self.tok)):
                    try:
                        v = gen.send((z, gated - 1) if gated else None)
                    except StopIteration:
                        break
                    if v is not None and lat is not None:
                        self.due.append((self.tok + lat, v))
            self.tok += 1

        def tokens(self, r, n):
            for k in range(n):
                self.step(r[k * 16:k * 16 + 8])

        def gate(self, v):
            now = [x for t, x in self.due if t <= self.tok]
            self.due = [(t, x) for t, x in self.due if t > self.tok]
            if not now:
                return v
            head = jnp.where(never[0], pltpu.bitcast(tree(now), u32), v[0:8])
            return jnp.concatenate([head, v[8:]], axis=0)

        def drain(self):
            for gen, *_ in self.plan:
                feed(gen, None, 1000)

    def tree(vals):
        while len(vals) > 1:
            vals = [a + b for a, b in zip(vals[::2], vals[1::2])] + vals[len(vals) & ~1:]
        return vals[0]

    def norm_slab(row, emit):
        def rows(k, lo, hi):
            return [row(k, r) for r in range(lo // 8, hi // 8)]

        def mean(vals):
            t = tree([sum(vals[k + 4::4], vals[k]) for k in range(4)])
            t = jnp.sum(t, axis=0, keepdims=True) * (1.0 / D)
            return jnp.broadcast_to(t, (8, 128))
        z = yield
        x = rows(0, 0, D)
        mu = mean([held(v, z) for v in x[:4]] + x[4:])
        m = held(mu, (yield))
        rs = lax.rsqrt(mean([(v - m) * (v - m) for v in rows(1, 0, D)]) + EPS)
        end = None
        for k in (4, 0, 1, 2, 3):
            m = held(mu, (yield end))
            y = jnp.concatenate(
                [(v - m) * rs for v in rows(2, k * 128, min((k + 1) * 128, D))], axis=0).T
            emit(k, y)
            end = y[120:128] if k < 4 else jnp.concatenate([y[120:128]] * 2, axis=1)
        yield end

    def alias(p, n):
        return [jnp.clip(p + k * zero[0], 0, n - 1) for k in range(3)]

    def slab_rows(src, p):
        q = alias(p, NSLAB)
        return lambda k, r: src[q[k], r * 8:r * 8 + 8, :]

    def flush(gen):
        return tree([v for v in gen if v is not None])

    def ln1(p, b):
        def emit(k, y):
            xnb[b, k, :, 0:y.shape[1]] = y.astype(bf16)
        return norm_slab(slab_rows(xa, p), emit)

    def widen(q):
        for r in range(NTR):
            if r % 4 == 0:
                z = yield
            v = _up(held(xin32[q, r], z)).astype(f32)
            for b in range(2):
                xa[2 * q + b, r * 8:r * 8 + 8, :] = v[b * 8:b * 8 + 8]

    def qkv_proj(b, pace, groups):
        scale = DH ** -0.5 * LOG2E
        for grp in groups:
            for n in grp:
                if n == 13:
                    ktail[...] = lax.dot_general(
                        _up(wq[4, n * 64:n * 64 + 32, :]), _up(xn[b, 4]), NT,
                        preferred_element_type=f32)
                else:
                    qkv[b, n, HALO:HALO + 128, :] = lax.dot_general(
                        _up(xn[b, 4]), _up(wq[4, n * 64:(n + 1) * 64, :]), NT,
                        preferred_element_type=f32)
            for n in grp:
                rows = slice(n * 64, n * 64 + (32 if n == 13 else 64))
                x = jnp.concatenate(
                    [_up(pace.gate(xn[b, 0]))] + [_up(xn[b, k]) for k in range(1, 4)], axis=1)
                w = jnp.concatenate([_up(wq[k, rows, :]) for k in range(4)], axis=1)
                if n == 13:
                    r = lax.dot_general(w, x, NT, preferred_element_type=f32)
                    r = r + jnp.concatenate([ktail[0:32, :], ktail[32:64, :]], axis=0)
                    qkv[b, n, HALO:HALO + 128, 0:64] = (r * scale).T
                    pace.tokens(r, 4)
                    continue
                r = lax.dot_general(x, w, NT, preferred_element_type=f32)
                r = r + jnp.concatenate([qkv[b, n, HALO:HALO + 64, :],
                                         qkv[b, n, HALO + 64:HALO + 128, :]], axis=0)
                if n in (4, 5, 6, 7):
                    r = r * scale
                qkv[b, n, HALO:HALO + 128, :] = r
                pace.tokens(r, 7)

    def halo(b):
        for n in range(4, 14):
            qkv[b, n, 0:HALO, :] = qkv[1 - b, n, 128:128 + HALO, :]

    def attend(b, row0):
        qs, ks, vs = (0, 1, 2, 3, 12), (4, 5, 6, 7, 13), (8, 9, 10, 11, 12)
        v = None
        for s in range(16):
            z = yield v
            r = HALO + s * 8
            q = [held(qkv[b, n, r:r + 8, :], z) for n in qs]
            logit = []
            for w in range(WIN):
                rw = r - DIL * w
                part = tree([q[c] * qkv[b, ks[c], rw:rw + 8, :] for c in range(5)])
                part = part + pltpu.roll(part, 64, 1)
                part = part + pltpu.roll(part, 32, 1)
                if row0 is not None and s * 8 < DIL * w:
                    pos = row0 + s * 8 + lax.broadcasted_iota(jnp.int32, (8, 128), 0)
                    part = jnp.where(pos >= DIL * w, part, -1e9 * LOG2E)
                logit.append(part)
            mx = logit
            while len(mx) > 1:
                mx = [jnp.maximum(a, c) for a, c in zip(mx[::2], mx[1::2])]
            e = [jnp.exp2(l - mx[0]) for l in logit]
            inv = 1.0 / tree(e)
            outs = []
            for c in range(5):
                o = e[0] * qkv[b, vs[c], r:r + 8, :]
                for w in range(1, WIN):
                    rw = r - DIL * w
                    o = o + e[w] * qkv[b, vs[c], rw:rw + 8, :]
                o = o * inv
                outs.append(o)
                ob[b, c, s * 8:(s + 1) * 8, :] = o.astype(bf16)
            v = tree(outs)
        yield v

    def out_proj(p, b, pace):
        h = MB // 2
        for m in range(4):
            xb[p, m * MB:(m + 1) * MB, :] = xa[p, m * MB:(m + 1) * MB, :] + lax.dot_general(
                _up(wo[4, m * h:(m + 1) * h, :]), _up(o32[b, 4]), NT, preferred_element_type=f32)
        rhs = jnp.concatenate([_up(o32[b, c]) for c in range(4)], axis=1)
        for m in range(4):
            rows = slice(m * h, (m + 1) * h)
            lhs = jnp.concatenate(
                [_up(pace.gate(wo[0, rows, :]))] + [_up(wo[c, rows, :]) for c in range(1, 4)],
                axis=1)
            r = lax.dot_general(lhs, rhs, NT, preferred_element_type=f32)
            r = r + jnp.concatenate([xb[p, m * MB:m * MB + h, :],
                                     xb[p, m * MB + h:(m + 1) * MB, :]], axis=0)
            xb[p, m * MB:(m + 1) * MB, :] = r
            pace.tokens(r, 8)

    def ffn_norm_slab(p, r):
        def emit(k, y):
            xn2[r * 6 + k, :, 0:y.shape[1]] = y
        return norm_slab(slab_rows(xb, p), emit)

    def ffn_norm(t):
        for r in range(4):
            yield from ffn_norm_slab(t * 4 + r, r)

    def strips(load, spec, terms, o, dst):
        for s in range(8):
            z = yield
            rows = slice(s * 16, (s + 1) * 16)

            def ld(r, c):
                v = load(r, c, rows)
                if (r // 2, c // 2) == spec[o][0]:
                    v = jnp.concatenate([held(v[0:8], z), held(v[8:16], z)], axis=0)
                return v

            def emit(i, v):
                dst[i, rows, :] = v.astype(bf16)
            _inner_terms(_outer_term(ld, spec, o), terms, o, emit)

    def lhs_strips(o):
        yield from strips(lambda r, k, rows: xn2[r * 6 + k, rows, :],
                          _LHS_SPEC, _lhs_terms, o, acb)
        if o in AUG:
            for s in range(2):
                z = yield
                rows = slice(s * 64, (s + 1) * 64)
                d = _lhs_ext(_lhs_ext([xn2[r * 6 + 4, rows, 0:64] for r in range(4)])[o])
                for ii, i in enumerate(AUG):
                    aeb[AUG.index(o) * 4 + ii, rows, 0:64] = d[i][0].astype(bf16)

    def ffn_combos():
        for s in range(8):
            rows = slice(s * 16, (s + 1) * 16)
            a = [[xn2[r * 6 + k, rows, :] for k in range(4)] for r in range(4)]

            def emit(i, v, rows=rows):
                acb[i, rows, :] = v.astype(bf16)
            _combos(a, _lhs_terms, emit)
            e = [xn2[r * 6 + 4, rows, 0:64] for r in range(4)]

            def emit_e(i, v, rows=rows):
                aeb[i, rows, 0:64] = v.astype(bf16)
            _ext_combos(e, _lhs_ext, emit_e)

    def attn_run(h, count, o, mask, side=None, late=None, extra=None, head=False):
        if not head:
            flush(ln1(h % NSLAB, 0))
        for k in range(count):
            b = k % 2
            pace = Pace()
            if side is not None:
                n = o["pn"] if k == 0 else NPREP - o["pn"]
                lo, hi = o["pw"][k]
                pace.add(side, lo, (hi - lo) / n, gated=o["pg"], n=n, primed=True)
            if k + 1 < count:
                pace.add(ln1((h + k + 1) % NSLAB, 1 - b), *o["ls"][k], o["lg"])
            elif late is not None:
                pace.add(late, o["w0"], o["wper"], gated=o["wg"])
            if k == 1 and extra is not None:
                pace.add(extra, 32 + o["x0"], o["xper"], gated=o["xg"])
            if k > 0 or not head:
                row0 = (h % NSLAB) * 128 if k == 1 and mask else None
                pace.add(attend(1 - b, row0), *o["a"][k], o["ag"])
                if not head:
                    out_proj((h + k - 2) % NSLAB, b, pace)
                halo(b)
            qkv_proj(b, pace, o["grp"])
            pace.plan = [e for e in pace.plan if e[0] is not side]
            pace.drain()
        if side is not None:
            feed(side, None, 1000)

    def wq_prep(k):
        w = 128 if k < 4 else 64
        for c0 in range(0, 3 * D, 128):
            c1 = min(c0 + 128, 3 * D)
            wtmp[k, c0:c1, 0:w] = wq_raw[k * 128:k * 128 + w, c0:c1].astype(f32).T
        for part in OPT["parts"]:
            for d in range(DH):
                if d < 16:
                    row = part * 512 + d * 32
                else:
                    row = (1536, 1664, 1600)[part] + (d - 16) * 32
                wqb[k, row:row + 32, 0:w] = wtmp[
                    k, pl.ds(part * D + d, H, stride=DH), 0:w].astype(bf16)

    def wo_prep():
        for n in range(5):
            w = 128 if n < 4 else 64
            wtmp[n, 0:D, 0:w] = wo_raw[:, n * 128:n * 128 + w].astype(f32)
        for n in range(5):
            w = 128 if n < 4 else 64
            for c in range(5):
                z = yield
                rows = [held(wtmp[n, pl.ds(4 * c + g + k * 8 * DH, 8, stride=DH), :], z)[:, 0:w]
                        for g in range(4 if c < 4 else 2) for k in range(4)]
                if c == 4:
                    rows = [jnp.zeros((64, w), f32)] + rows
                wob[c, n * 128:n * 128 + w, :] = jnp.concatenate(rows, axis=0).T.astype(bf16)

    def head_late():
        for cp in (wo_copy, x_copy(1)):
            cp.wait()
        for cp in [x_copy(2)] + chunk_copies(1):
            cp.start()
        yield from wo_prep()
        yield from widen(1)

    wqb[4, :, 64:128] = jnp.zeros((3 * D, 64), bf16)
    qkv[:, 13] = jnp.zeros((2, HALO + 128, 128), f32)
    xnb[:, 4, :, 64:128] = jnp.zeros((2, 128, 64), bf16)
    for n in range(4, 13):
        qkv[0, n, 0:HALO, :] = jnp.zeros((HALO, 128), f32)
    todo = list(k_order)
    for n, cp in enumerate(first):
        cp.wait()
        if n == 0:
            never.append(zero[0] != 0)
        if n == OPT["dma"][0]:
            wo_copy.start()
        if n == OPT["dma"][1]:
            for c in [x_copy(1)] + chunk_copies(0):
                c.start()
        if n == OPT["xpos"]:
            feed(widen(0), None, 1000)
            flush(ln1(0, 0))
        else:
            wq_prep(todo.pop(0))
    attn_run(0, 2, OPT["h"], True, late=head_late(), head=True)

    @pl.loop(0, 7)
    def _(i):
        for cp in chunk_copies(i):
            cp.wait()

        @pl.when(i + 2 < NSLAB // 2)
        def _():
            x_copy(i + 2).wait()

        @pl.when(i + 3 < NSLAB // 2)
        def _():
            x_copy(i + 3).start()
        for cp in chunk_copies(i + 2):
            cp.start()
        side = prep_chunk(i, [r.at[i] for r in (wcb, web, wdcb)])
        next(side)
        r = jnp.clip(i - 2, 0, 3)
        attn_run(2 * i + 2, 2, OPT["p"], False, side, widen(jnp.minimum(i + 2, NSLAB // 2 - 1)),
                 ffn_norm_slab(r, r))

    for cp in chunk_copies(7) + chunk_copies(8):
        cp.wait()
    ffn_combos()

    def ffn_group(t, g, last, emit=None):
        ti = _Temps(tin)
        to = _Temps(tout)
        pace = Pace()
        o_ = OPT["fb" if last else "fa"]

        tr = o_["tr"]

        def chain(gens):
            yield
            for gen in gens:
                next(gen)
                z = None
                while True:
                    z = yield
                    try:
                        gen.send(z)
                    except StopIteration:
                        break

        def weights(c):
            if last and c > 0:
                return [r.at[c - 1] for r in (wc2, we2, wdc2)]
            return [r.at[g * 3 + c] for r in (wc, we, wdc)]

        def proj(c, m):
            w, w_ext, _ = weights(c)

            def prod(o, i):
                r = (m * 49 + o * 7 + i) * 64
                p = jnp.dot(_up(ac[o * 7 + i]), _up(w[r:r + 64, :]),
                            preferred_element_type=f32)
                pace.step(p[tr:tr + 8])
                if o in AUG and i in AUG:
                    q = AUG.index(o) * 4 + AUG.index(i)
                    e = jnp.dot(_up(ae[q, :, 0:64]), _up(w_ext[m * 16 + q]),
                                preferred_element_type=f32)
                    pace.step(e[tr:tr + 8])
                    p = p + e
                return p
            return prod

        def gate(c):
            def fin(r, cc, v):
                gs[(c % 2) * 16 + r * 4 + cc] = v
            return _recombine(proj(c, 0), fin, ti, to, o_["gm"])

        def upgate(c):
            def fin(r, cc, v):
                hs[c, r * 4 + cc] = _ld(gs, (c % 2) * 16 + r * 4 + cc) * v
            yield from _recombine(proj(c, 1), fin, ti, to, o_["um"])
            hgen[c] = chain([strips(lambda cc, r, rows: hs[c, r * 4 + cc, rows, :],
                                    _RHS_SPEC, _rhs_terms, o, hcb.at[c]) for o in ORDER])
            hdone[c] = 0
            pace.add(counted(c), *o_["h"][c], gated=o_["hg"])

        hgen, hdone = {}, {}

        def counted(c):
            next(hgen[c])
            next(hgen[c])
            while True:
                z = yield
                if hdone[c] < 56:
                    need(c, hdone[c] + 1, z)

        def need(c, n, z=None):
            while hdone[c] < n:
                hdone[c] += 1
                feed(hgen[c], z, 1)

        def dprod(cs, i):
            p = None
            for c in cs:
                need(c, 8 * (ORDER.index(i // 7) + 1))
                r = i * (MB // 2)
                q = lax.dot_general(_up(weights(c)[2][r:r + MB // 2, :]), _up(hc[c, i]), NT,
                                    preferred_element_type=f32)
                pace.step(q[tr:tr + 8])
                p = q if p is None else p + q
            return p

        def down(cs, reset):
            for i in [o * 7 + k for o in ORDER for k in range(7)]:
                a = _ld(acc, i)
                if reset:
                    a = jnp.where(g == 0, 0.0, a)
                acc[i] = a + dprod(cs, i)
                yield

        def down_final(cs):
            def fin(mb, r, v):
                rows = slice(mb * MB, (mb + 1) * MB)
                y = xb[t * 4 + r, rows, :] + v
                xa[t * 4 + r, rows, :] = y
                ost[t * 2 + r // 2, rows, (r % 2) * 128:(r % 2) * 128 + 128] = y.astype(bf16)
            return _recombine(lambda o, i: _ld(acc, o * 7 + i) + dprod(cs, o * 7 + i),
                              fin, _Temps(tin2), _Temps(tout2), o_["dm"])

        if last:
            norm = ffn_norm((t + 1) % NTILE)
            pace.add(norm, o_["n0"], o_["nper"], gated=o_["ng"])
        else:
            late = prep_chunk(7 + g, [r.at[g] for r in (wcb2, web2, wdcb2)])
            next(late)
            pace.plan.append((late, _spread(o_["wts"], 30, NPREP), None, o_["ng"]))
        for gen in (gate(0), upgate(0), gate(1)):
            _adv(gen, 100)
        d0 = down((0,), not last)
        queue = []

        def lhs_queue():
            while True:
                z = yield
                while queue:
                    try:
                        queue[0].send(z)
                        break
                    except StopIteration:
                        queue.pop(0)
                        break
        for gen, plan in ((upgate(1), "u1"), (gate(2), "g2"), (upgate(2), "u2")):
            if last and plan == "u2":
                feed(norm, None, 1000)
                pace.add(lhs_queue(), o_["l0"], o_["lper"], gated=o_["lg"])
            for k, n in enumerate(o_[plan]):
                _adv(gen, 1)
                if last and plan == "u2":
                    queue.append(lhs_strips(ORDER[k]))
                    next(queue[-1])
                _adv(d0, n)
            _adv(gen, 100)
        _adv(d0, 100)
        if last:
            gen = down_final((1, 2))
            _adv(gen, 3)
            for q, h in ((1, 1), (0, 1), (1, 0), (0, 0)):
                _adv(gen, 1)
                pl.when(emit)(out_copy(t * 2 + q, h).start)
        else:
            _adv(down((1, 2), False), 100)
            feed(late, None, 1000)
        for gen in queue:
            feed(gen, None, 1000)

    @pl.loop(0, 2 * NTILE)
    def _(tile):
        t = tile % NTILE
        if not OPT["skip_ffn"]:
            @pl.loop(0, 2)
            def _(g):
                ffn_group(t, g, False)
            ffn_group(t, 2, True, tile >= NTILE)
        else:
            r0 = pl.multiple_of(zero[0] * 16, 16)
            ost[0, 0:16, 0:128] = wcb[t, pl.ds(r0, 16), :] + wdcb[t, pl.ds(r0, 16), :] + web[t, t, 0:16, :]
            ost[1, 0:16, 0:128] = acb[t, 0:16, :] + aeb[t, 0:16, :]
            ost[2, 0:D, 0:128] = xb[t, 0:D, :].astype(bf16)
            for q, h in ((1, 1), (0, 1), (1, 0), (0, 0)):
                pl.when(tile >= NTILE)(out_copy(t * 2 + q, h).start)

        @pl.when(tile < NTILE)
        def _():
            attn_run(4 * t + NSLAB, 4, OPT["n"], True)

        @pl.when(tile == NTILE - 1)
        def _():
            o = OPT["e"]
            pace = Pace()
            pace.add(attend(1, None), 0, o["aper"], gated=o["ag"])
            out_proj(NSLAB - 2, 0, pace)
            pace.drain()
            out_proj(NSLAB - 1, 1, Pace())

    for p in range(NSLAB):
        out_copy(p // 2, p % 2).wait()


def _tiles(w):
    n = w.shape[1]
    return w.reshape(NTR, 8, n // 128, 128).transpose(0, 2, 1, 3).reshape(NTR, n // 16, 128)


@jax.jit
def pallas_interleave_layers__sliding_local_dilated__glu_gated_bilinear__prompt_kernel(
    A_x: jax.Array,
    A_wqkv: jax.Array,
    A_wo: jax.Array,
    B_x: jax.Array,
    B_w_gate: jax.Array,
    B_w_up: jax.Array,
    B_w_down: jax.Array,
):
    del B_x
    vm = pltpu.VMEM
    hbm = pl.BlockSpec(memory_space=pl.ANY)
    out_t = pl.pallas_call(
        _kernel,
        in_specs=[hbm] * 6,
        out_specs=hbm,
        out_shape=jax.ShapeDtypeStruct((D, S), bf16),
        scratch_shapes=[
            vm((NSLAB // 2, 96, 16, 128), bf16),
            vm((NSLAB, 768, 128), f32),
            vm((NSLAB, 768, 128), f32),
            vm((NSLAB // 2, 768, 256), bf16),
            vm((NCHUNK, 224, 32, 128), bf16),
            vm((7, WC_ROWS, 128), bf16),
            vm((7, 32, 64, 128), bf16),
            vm((7, WD_ROWS, 128), bf16),
            vm((2, WC_ROWS, 128), bf16),
            vm((2, 32, 64, 128), bf16),
            vm((2, WD_ROWS, 128), bf16),
            vm((24, 128, 128), f32),
            vm((D, 3 * D), bf16),
            vm((D, D), bf16),
            vm((5, 3 * D, 128), f32),
            vm((5, 3 * D, 128), bf16),
            vm((5, D, 128), bf16),
            vm((2, 5, 128, 128), bf16),
            vm((2, 14, HALO + 128, 128), f32),
            vm((2, 5, 128, 128), bf16),
            vm((49, 128, 128), bf16),
            vm((16, 128, 128), bf16),
            vm((32, 128, 128), f32),
            vm((3, 16, 128, 128), f32),
            vm((3, 49, 128, 128), bf16),
            vm((49, MB, 128), f32),
            vm((12, 128, 128), f32),
            vm((40, 128, 128), f32),
            vm((12, MB, 128), f32),
            vm((20, MB, 128), f32),
            vm((64, 128), f32),
            pltpu.SMEM((1,), jnp.int32),
            pltpu.SemaphoreType.DMA((NSLAB // 2,)),
            pltpu.SemaphoreType.DMA((6,)),
            pltpu.SemaphoreType.DMA((NCHUNK, 3)),
            pltpu.SemaphoreType.DMA((NSLAB // 2, 2)),
        ],
        compiler_params=pltpu.CompilerParams(vmem_limit_bytes=120 * 1024 * 1024),
    )(_tiles(A_x[0].T), A_wqkv, A_wo, _tiles(B_w_gate), _tiles(B_w_up), _tiles(B_w_down.T))
    return out_t.T[None]
```

```python
import math

import jax
import jax.numpy as jnp
from jax import lax
import jax.experimental.pallas as pl
import jax.experimental.pallas.tpu as pltpu

f32 = jnp.float32
bf16 = jnp.bfloat16
u32 = jnp.uint32

S, D, F = 2048, 576, 4608
H, DH, WIN, DIL = 32, 18, 8, 2
EPS = 1e-5
LOG2E = math.log2(math.e)
NSLAB = S // 128
TILE = 512
NTILE = S // TILE
FC = 512
NCHUNK = F // FC
MB = D // 4
HALO = 16
NPREP = 158
NTR = D // 8
WC_ROWS = 800 * 16
WD_ROWS = 448 * 16
NT = (((1,), (1,)), ((), ()))
ORDER = (0, 1, 2, 5, 3, 4, 6)
AUG = (0, 1, 2, 5)

OPT = {'dma': (0, 2),
 'xpos': 2,
 'parts': (1, 0, 2),
 'fa': {'wts': (1, 0, 3, 1, 0, 1, 2, 3, 1, 2, 0, 0, 0, 0, 0, 1, 3, 4),
        'h': ((0, 0.7), (0, 1), (0, 1)),
        'u1': (0, 0, 0, 4, 5, 4, 6),
        'g2': (4, 0, 0, 0, 0, 0, 0),
        'u2': (0, 0, 0, 0, 4, 4, 4)},
 'fb': {'h': ((0, 1), (0, 0.59), (0, 1)),
        'n0': 0,
        'nper': 1.4,
        'l0': 0,
        'lper': 2.3,
        'u1': (0, 0, 0, 0, 4, 4, 6),
        'g2': (4, 0, 0, 0, 0, 0, 0),
        'u2': (0, 0, 0, 0, 4, 4, 4)},
 'h': {'grp': ((4, 5, 6, 7), (0, 1, 2, 3), (12, 13, 8, 9, 10, 11)),
       'a': ((0, 5, 35), (0, 3.65, 35)),
       'w0': 22,
       'wper': 2.8,
       'ag': 1,
       'ls': ((13, 5.0, 40),)},
 'e': {'aper': 3.04},
 'p': {'x0': 30,
       'xper': 5.6,
       'grp': ((4, 13), (5, 6, 7, 0), (1, 2, 3, 12), (8, 9, 10, 11)),
       'a': ((0, 6, 25), (0, 6, 35)),
       'w0': 65,
       'wper': 6.06,
       'pn': 71,
       'pw': ((0, 130), (0, 126)),
       'ag': 0,
       'ls': ((32, 5.47, None),)},
 'n': {'grp': ((4, 5, 6, 7), (0, 1, 2, 3), (12, 13, 8, 9, 10, 11)),
       'a': ((1, 6, 35), (1, 5.4, 35), (1, 6.03, 35), (6, 6.9, 35)),
       'ag': 1,
       'ls': ((77, 5.51, None), (69, 9.25, None), (80, 6.83, None))}}


def _up(v):
    return pltpu.bitcast(v, bf16)


def _quad(x):
    n = len(x) // 2
    return ([r[:n] for r in x[:n]], [r[n:] for r in x[:n]],
            [r[:n] for r in x[n:]], [r[n:] for r in x[n:]])


def _badd(x, y):
    return [[a + b for a, b in zip(r, s)] for r, s in zip(x, y)]


def _bsub(x, y):
    return [[a - b for a, b in zip(r, s)] for r, s in zip(x, y)]


def _lhs_terms(a):
    a11, a12, a21, a22 = _quad(a)
    return [lambda: _badd(a11, a22), lambda: _badd(a21, a22), lambda: a11, lambda: a22,
            lambda: _badd(a11, a12), lambda: _bsub(a21, a11), lambda: _bsub(a12, a22)]


def _rhs_terms(b):
    b11, b12, b21, b22 = _quad(b)
    return [lambda: _badd(b11, b22), lambda: b11, lambda: _bsub(b12, b22), lambda: _bsub(b21, b11),
            lambda: b22, lambda: _badd(b11, b12), lambda: _badd(b21, b22)]


def _combos(x, terms, emit):
    for o, fo in enumerate(terms(x)):
        y = fo()
        for i, fi in enumerate(terms(y)):
            emit(o * 7 + i, fi()[0][0])


_LHS_SPEC = (((0, 0), (1, 1), 1), ((1, 0), (1, 1), 1), ((0, 0), None, 0), ((1, 1), None, 0),
             ((0, 0), (0, 1), 1), ((1, 0), (0, 0), -1), ((0, 1), (1, 1), -1))
_RHS_SPEC = (((0, 0), (1, 1), 1), ((0, 0), None, 0), ((0, 1), (1, 1), -1), ((1, 0), (0, 0), -1),
             ((1, 1), None, 0), ((0, 0), (0, 1), 1), ((1, 0), (1, 1), 1))


def _outer_term(load, spec, o):
    p, q, sign = spec[o]
    out = []
    for y in range(2):
        row = []
        for z in range(2):
            v = load(2 * p[0] + y, 2 * p[1] + z)
            if sign:
                w = load(2 * q[0] + y, 2 * q[1] + z)
                v = v + w if sign > 0 else v - w
            row.append(v)
        out.append(row)
    return out


def _inner_terms(y, terms, o, emit):
    for i, fi in enumerate(terms(y)):
        emit(o * 7 + i, fi()[0][0])


def _lhs_ext(e):
    n = len(e) // 2
    return {0: e[:n], 1: e[n:], 2: e[:n], 5: [y - x for x, y in zip(e[:n], e[n:])]}


def _rhs_ext(e):
    n = len(e) // 2
    return {0: e[:n], 1: e[:n], 2: e[n:], 5: [x + y for x, y in zip(e[:n], e[n:])]}


def _ext_combos(e, fn, emit):
    for oi, o in enumerate(AUG):
        d = fn(fn(e)[o])
        for ii, i in enumerate(AUG):
            emit(oi * 4 + ii, d[i][0])


def _spread(weights, span, n):
    total, acc, out = sum(weights), 0.0, []
    for k, w in enumerate(weights):
        lo, acc = acc, acc + w * n / total
        count = round(acc) - round(lo)
        out += [k * span + i * span // count for i in range(count)]
    return out


def _adv(gen, n):
    for _ in range(n):
        try:
            next(gen)
        except StopIteration:
            return


def _ld(ref, idx):
    n = ref.shape[-2] // 2
    return jnp.concatenate([ref[idx, :n, :], ref[idx, n:, :]], axis=0)


class _Temps:
    def __init__(self, ref):
        self.ref = ref
        self.n = 0

    def put(self, v):
        i = self.n % self.ref.shape[0]
        self.n += 1
        self.ref[i] = v
        return i

    def get(self, i):
        return _ld(self.ref, i)


def _recombine(prod, fin, ti, to, spill_last=False):
    def inner(o, sink):
        a = ti.put(prod(o, 0))
        b = ti.put(prod(o, 1))
        c = ti.put(prod(o, 2))
        sink(1, 1, ti.get(a) - ti.get(b) + ti.get(c) + prod(o, 5))
        if spill_last:
            m3 = prod(o, 3)
            m4 = prod(o, 4)
            sink(1, 0, ti.get(b) + m3)
            sink(0, 1, ti.get(c) + m4)
            d = ti.put(ti.get(a) + m3 - m4)
            sink(0, 0, ti.get(d) + prod(o, 6))
            return
        m3 = prod(o, 3)
        m4 = prod(o, 4)
        m6 = prod(o, 6)
        sink(1, 0, ti.get(b) + m3)
        sink(0, 1, ti.get(c) + m4)
        sink(0, 0, ti.get(a) + m3 - m4 + m6)

    m = {}
    for o in (0, 1, 2):
        def keep(y, z, v, o=o):
            m[o, y, z] = to.put(v)
        inner(o, keep)
        yield

    def s5(y, z, v):
        fin(2 + y, 2 + z, to.get(m[0, y, z]) - to.get(m[1, y, z]) + to.get(m[2, y, z]) + v)
    inner(5, s5)
    yield

    def s3(y, z, v):
        fin(2 + y, z, to.get(m[1, y, z]) + v)
        m[3, y, z] = to.put(to.get(m[0, y, z]) + v)
    inner(3, s3)
    yield

    def s4(y, z, v):
        fin(y, 2 + z, to.get(m[2, y, z]) + v)
        m[3, y, z] = to.put(to.get(m[3, y, z]) - v)
    inner(4, s4)
    yield

    def s6(y, z, v):
        fin(y, z, to.get(m[3, y, z]) + v)
    inner(6, s6)
    yield


def _kernel(xt_hbm, wqkv_hbm, wo_hbm, wg_hbm, wu_hbm, wdt_hbm, out_hbm,
            xin, xa, xb, ost, raw, wcb, web, wdcb, wcb2, web2, wdcb2, xn2,
            wq_raw, wo_raw, wtmp, wqb, wob, xnb, qkv, ob, acb, aeb, gs, hs, hcb, acc, tin, tout, tin2, tout2, ktail, zero,
            sem_x, sem_w, sem_c, sem_o):
    wq, wo, wc, we, wdc, xn, o32, ac, ae, hc, raw32, xin32, wc2, we2, wdc2 = [
        r.bitcast(u32) for r in (wqb, wob, wcb, web, wdcb, xnb, ob, acb, aeb, hcb, raw, xin,
                                 wcb2, web2, wdcb2)]

    def x_copy(q):
        return pltpu.make_async_copy(
            xt_hbm.at[:, pl.ds(pl.multiple_of(q * 16, 16), 16), :], xin.at[q, 0:NTR], sem_x.at[q])

    def weight_copy(j, m):
        rows = pl.ds(pl.multiple_of(j * 32, 32), 32)
        return pltpu.make_async_copy((wg_hbm, wu_hbm, wdt_hbm)[m].at[:, rows, :],
                                     raw.at[j, pl.ds(m * NTR, NTR)], sem_c.at[j, m])

    def chunk_copies(j):
        return [weight_copy(j, m) for m in range(3)]

    def out_copy(q, h):
        rows = pl.ds(h * 2 * MB, 2 * MB)
        return pltpu.make_async_copy(
            ost.at[q, rows, :], out_hbm.at[rows, pl.ds(pl.multiple_of(q * 256, 256), 256)],
            sem_o.at[q, h])

    k_order = (4, 0, 1, 2, 3)
    wq_copies = [pltpu.make_async_copy(wqkv_hbm.at[k * 128:min(k * 128 + 128, D)],
                                       wq_raw.at[k * 128:min(k * 128 + 128, D)], sem_w.at[k])
                 for k in k_order]
    wo_copy = pltpu.make_async_copy(wo_hbm, wo_raw, sem_w.at[5])
    first = wq_copies[:OPT["xpos"]] + [x_copy(0)] + wq_copies[OPT["xpos"]:]
    for cp in first:
        cp.start()
    zero[0] = 0
    never = zero[0] != 0

    def held(v, z):
        if z is None:
            return v
        return jnp.where(never, pltpu.bitcast(z, v.dtype), v)

    def raw_pair(j, tr, cp, z):
        v = [_up(held(raw32[j, tr + k, cp * 8:cp * 8 + 8, :], z)).astype(f32) for k in range(2)]
        return [jnp.concatenate([v[0][h:h + 8], v[1][h:h + 8]], axis=0) for h in (0, 8)]

    def prep_strip(j, tr, step, spec, terms, path, emit):
        live = {}
        for o in path:
            used = [q for q in spec[o][:2] if q is not None]
            live = {q: live[q] for q in used if q in live}
            for q in used:
                if q not in live:
                    z = yield
                    live[q] = [raw_pair(j, tr + (2 * q[0] + y) * step, q[1], z) for y in range(2)]
            y = _outer_term(lambda r, c: live[r // 2, c // 2][r % 2][c % 2], spec, o)
            _inner_terms(y, terms, o, emit)

    def prep_gu(j, dst, m, s):
        base = m * (49 * 128) + s * 16

        def emit(i, v):
            dst[pl.ds(base + i * 128, 16), :] = v.astype(bf16)
        return prep_strip(j, m * NTR + 2 * s, 16, _RHS_SPEC, _rhs_terms, (1, 0, 4, 2, 5, 3, 6), emit)

    def prep_ext(j, dst, m, s):
        z = yield
        tr = m * NTR + 64 + 2 * s

        def emit(i, v):
            dst[m * 16 + i, pl.ds(s * 16, 16), :] = v.astype(bf16)
        _ext_combos(raw_pair(j, tr, 0, z) + raw_pair(j, tr, 1, z), _rhs_ext, emit)

    def prep_down(j, dst, s):
        def emit(i, v):
            dst[pl.ds(s * 16 + i * MB, 16), :] = v.astype(bf16)
        return prep_strip(j, 2 * NTR + 2 * s, MB // 8, _LHS_SPEC, _lhs_terms,
                          (2, 0, 3, 6, 4, 5, 1), emit)

    def prep_chunk(j, dst):
        for m in range(2):
            for s in range(8):
                yield from prep_gu(j, dst[0], m, s)
            for s in range(4):
                yield from prep_ext(j, dst[1], m, s)
        for s in range(9):
            yield from prep_down(j, dst[2], s)

    def feed(gen, z, n):
        for _ in range(n):
            try:
                gen.send(z)
            except StopIteration:
                return

    class Pace:
        def __init__(self):
            self.tok = 0
            self.plan = []
            self.due = []

        def add(self, gen, t0, period, lat=None, gated=True, n=1000, primed=False):
            if not primed:
                next(gen)
            when = [self.tok + int(t0 + k * period) for k in range(n)]
            self.plan.append((gen, when, lat, gated))

        def step(self, z):
            for gen, when, lat, gated in self.plan:
                for _ in range(when.count(self.tok)):
                    try:
                        v = gen.send(z if gated else None)
                    except StopIteration:
                        break
                    if v is not None and lat is not None:
                        self.due.append((self.tok + lat, v))
            self.tok += 1

        def tokens(self, r, n):
            for k in range(n):
                self.step(r[k * 16:k * 16 + 8])

        def gate(self, v):
            now = [x for t, x in self.due if t <= self.tok]
            self.due = [(t, x) for t, x in self.due if t > self.tok]
            if not now:
                return v
            head = jnp.where(never, pltpu.bitcast(tree(now), u32), v[0:8])
            return jnp.concatenate([head, v[8:]], axis=0)

        def drain(self):
            for gen, *_ in self.plan:
                feed(gen, None, 1000)

    def tree(vals):
        while len(vals) > 1:
            vals = [a + b for a, b in zip(vals[::2], vals[1::2])] + vals[len(vals) & ~1:]
        return vals[0]

    def norm_slab(row, emit):
        def rows(k, lo, hi):
            return [row(k, r) for r in range(lo // 8, hi // 8)]

        def mean(vals):
            t = tree([sum(vals[k + 4::4], vals[k]) for k in range(4)])
            t = jnp.sum(t, axis=0, keepdims=True) * (1.0 / D)
            return jnp.broadcast_to(t, (8, 128))
        z = yield
        x = rows(0, 0, D)
        mu = mean([held(v, z) for v in x[:4]] + x[4:])
        m = held(mu, (yield))
        rs = lax.rsqrt(mean([(v - m) * (v - m) for v in rows(1, 0, D)]) + EPS)
        end = None
        for k in (4, 0, 1, 2, 3):
            m = held(mu, (yield end))
            y = jnp.concatenate(
                [(v - m) * rs for v in rows(2, k * 128, min((k + 1) * 128, D))], axis=0).T
            emit(k, y)
            end = y[120:128] if k < 4 else jnp.concatenate([y[120:128]] * 2, axis=1)
        yield end

    def alias(p, n):
        return [jnp.clip(p + k * zero[0], 0, n - 1) for k in range(3)]

    def slab_rows(src, p):
        q = alias(p, NSLAB)
        return lambda k, r: src[q[k], r * 8:r * 8 + 8, :]

    def flush(gen):
        return tree([v for v in gen if v is not None])

    def ln1(p, b):
        def emit(k, y):
            xnb[b, k, :, 0:y.shape[1]] = y.astype(bf16)
        return norm_slab(slab_rows(xa, p), emit)

    def widen(q):
        for r in range(NTR):
            if r % 4 == 0:
                z = yield
            v = _up(held(xin32[q, r], z)).astype(f32)
            for b in range(2):
                xa[2 * q + b, r * 8:r * 8 + 8, :] = v[b * 8:b * 8 + 8]

    def qkv_proj(b, pace, groups):
        scale = DH ** -0.5 * LOG2E
        for grp in groups:
            for n in grp:
                if n == 13:
                    ktail[...] = lax.dot_general(
                        _up(wq[4, n * 64:n * 64 + 32, :]), _up(xn[b, 4]), NT,
                        preferred_element_type=f32)
                else:
                    qkv[b, n, HALO:HALO + 128, :] = lax.dot_general(
                        _up(xn[b, 4]), _up(wq[4, n * 64:(n + 1) * 64, :]), NT,
                        preferred_element_type=f32)
            for n in grp:
                rows = slice(n * 64, n * 64 + (32 if n == 13 else 64))
                x = jnp.concatenate(
                    [_up(pace.gate(xn[b, 0]))] + [_up(xn[b, k]) for k in range(1, 4)], axis=1)
                w = jnp.concatenate([_up(wq[k, rows, :]) for k in range(4)], axis=1)
                if n == 13:
                    r = lax.dot_general(w, x, NT, preferred_element_type=f32)
                    r = r + jnp.concatenate([ktail[0:32, :], ktail[32:64, :]], axis=0)
                    qkv[b, n, HALO:HALO + 128, 0:64] = (r * scale).T
                    pace.tokens(r, 4)
                    continue
                r = lax.dot_general(x, w, NT, preferred_element_type=f32)
                r = r + jnp.concatenate([qkv[b, n, HALO:HALO + 64, :],
                                         qkv[b, n, HALO + 64:HALO + 128, :]], axis=0)
                if n in (4, 5, 6, 7):
                    r = r * scale
                qkv[b, n, HALO:HALO + 128, :] = r
                pace.tokens(r, 7)

    def halo(b):
        for n in range(4, 14):
            qkv[b, n, 0:HALO, :] = qkv[1 - b, n, 128:128 + HALO, :]

    def attend(b, row0):
        qs, ks, vs = (0, 1, 2, 3, 12), (4, 5, 6, 7, 13), (8, 9, 10, 11, 12)
        v = None
        for s in range(16):
            z = yield v
            r = HALO + s * 8
            q = [held(qkv[b, n, r:r + 8, :], z) for n in qs]
            logit = []
            for w in range(WIN):
                rw = r - DIL * w
                part = tree([q[c] * qkv[b, ks[c], rw:rw + 8, :] for c in range(5)])
                part = part + pltpu.roll(part, 64, 1)
                part = part + pltpu.roll(part, 32, 1)
                if row0 is not None and s * 8 < DIL * w:
                    pos = row0 + s * 8 + lax.broadcasted_iota(jnp.int32, (8, 128), 0)
                    part = jnp.where(pos >= DIL * w, part, -1e9 * LOG2E)
                logit.append(part)
            mx = logit
            while len(mx) > 1:
                mx = [jnp.maximum(a, c) for a, c in zip(mx[::2], mx[1::2])]
            e = [jnp.exp2(l - mx[0]) for l in logit]
            inv = 1.0 / tree(e)
            outs = []
            for c in range(5):
                o = e[0] * qkv[b, vs[c], r:r + 8, :]
                for w in range(1, WIN):
                    rw = r - DIL * w
                    o = o + e[w] * qkv[b, vs[c], rw:rw + 8, :]
                o = o * inv
                outs.append(o)
                ob[b, c, s * 8:(s + 1) * 8, :] = o.astype(bf16)
            v = tree(outs)
        yield v

    def out_proj(p, b, pace):
        h = MB // 2
        for m in range(4):
            xb[p, m * MB:(m + 1) * MB, :] = xa[p, m * MB:(m + 1) * MB, :] + lax.dot_general(
                _up(wo[4, m * h:(m + 1) * h, :]), _up(o32[b, 4]), NT, preferred_element_type=f32)
        rhs = jnp.concatenate([_up(o32[b, c]) for c in range(4)], axis=1)
        for m in range(4):
            rows = slice(m * h, (m + 1) * h)
            lhs = jnp.concatenate(
                [_up(pace.gate(wo[0, rows, :]))] + [_up(wo[c, rows, :]) for c in range(1, 4)],
                axis=1)
            r = lax.dot_general(lhs, rhs, NT, preferred_element_type=f32)
            r = r + jnp.concatenate([xb[p, m * MB:m * MB + h, :],
                                     xb[p, m * MB + h:(m + 1) * MB, :]], axis=0)
            xb[p, m * MB:(m + 1) * MB, :] = r
            pace.tokens(r, 8)

    def ffn_norm_slab(p, r):
        def emit(k, y):
            xn2[r * 6 + k, :, 0:y.shape[1]] = y
        return norm_slab(slab_rows(xb, p), emit)

    def ffn_norm(t):
        for r in range(4):
            yield from ffn_norm_slab(t * 4 + r, r)

    def strips(load, spec, terms, o, dst):
        for s in range(8):
            z = yield
            rows = slice(s * 16, (s + 1) * 16)

            def ld(r, c):
                v = load(r, c, rows)
                if (r // 2, c // 2) == spec[o][0]:
                    v = jnp.concatenate([held(v[0:8], z), held(v[8:16], z)], axis=0)
                return v

            def emit(i, v):
                dst[i, rows, :] = v.astype(bf16)
            _inner_terms(_outer_term(ld, spec, o), terms, o, emit)

    def lhs_strips(o):
        yield from strips(lambda r, k, rows: xn2[r * 6 + k, rows, :],
                          _LHS_SPEC, _lhs_terms, o, acb)
        if o in AUG:
            for s in range(2):
                z = yield
                rows = slice(s * 64, (s + 1) * 64)
                d = _lhs_ext(_lhs_ext([xn2[r * 6 + 4, rows, 0:64] for r in range(4)])[o])
                for ii, i in enumerate(AUG):
                    aeb[AUG.index(o) * 4 + ii, rows, 0:64] = d[i][0].astype(bf16)

    def ffn_combos():
        for s in range(8):
            rows = slice(s * 16, (s + 1) * 16)
            a = [[xn2[r * 6 + k, rows, :] for k in range(4)] for r in range(4)]

            def emit(i, v, rows=rows):
                acb[i, rows, :] = v.astype(bf16)
            _combos(a, _lhs_terms, emit)
            e = [xn2[r * 6 + 4, rows, 0:64] for r in range(4)]

            def emit_e(i, v, rows=rows):
                aeb[i, rows, 0:64] = v.astype(bf16)
            _ext_combos(e, _lhs_ext, emit_e)

    def attn_run(h, count, o, mask, side=None, late=None, extra=None, head=False):
        if not head:
            flush(ln1(h % NSLAB, 0))
        for k in range(count):
            b = k % 2
            pace = Pace()
            if side is not None:
                n = o["pn"] if k == 0 else NPREP - o["pn"]
                lo, hi = o["pw"][k]
                pace.add(side, lo, (hi - lo) / n, n=n, primed=True)
            if k + 1 < count:
                pace.add(ln1((h + k + 1) % NSLAB, 1 - b), *o["ls"][k])
            elif late is not None:
                pace.add(late, o["w0"], o["wper"])
            if k == 1 and extra is not None:
                pace.add(extra, 32 + o["x0"], o["xper"])
            if k > 0 or not head:
                row0 = (h % NSLAB) * 128 if k == 1 and mask else None
                pace.add(attend(1 - b, row0), *o["a"][k], o["ag"])
                if not head:
                    out_proj((h + k - 2) % NSLAB, b, pace)
                halo(b)
            qkv_proj(b, pace, o["grp"])
            pace.plan = [e for e in pace.plan if e[0] is not side]
            pace.drain()
        if side is not None:
            feed(side, None, 1000)

    def wq_prep(k):
        w = 128 if k < 4 else 64
        for c0 in range(0, 3 * D, 128):
            c1 = min(c0 + 128, 3 * D)
            wtmp[k, c0:c1, 0:w] = wq_raw[k * 128:k * 128 + w, c0:c1].astype(f32).T
        for part in OPT["parts"]:
            for d in range(DH):
                if d < 16:
                    row = part * 512 + d * 32
                else:
                    row = (1536, 1664, 1600)[part] + (d - 16) * 32
                wqb[k, row:row + 32, 0:w] = wtmp[
                    k, pl.ds(part * D + d, H, stride=DH), 0:w].astype(bf16)

    def wo_prep():
        for n in range(5):
            w = 128 if n < 4 else 64
            wtmp[n, 0:D, 0:w] = wo_raw[:, n * 128:n * 128 + w].astype(f32)
        for n in range(5):
            w = 128 if n < 4 else 64
            for c in range(5):
                z = yield
                rows = [held(wtmp[n, pl.ds(4 * c + g + k * 8 * DH, 8, stride=DH), :], z)[:, 0:w]
                        for g in range(4 if c < 4 else 2) for k in range(4)]
                if c == 4:
                    rows = [jnp.zeros((64, w), f32)] + rows
                wob[c, n * 128:n * 128 + w, :] = jnp.concatenate(rows, axis=0).T.astype(bf16)

    def head_late():
        for cp in (wo_copy, x_copy(1)):
            cp.wait()
        for cp in [x_copy(2)] + chunk_copies(1):
            cp.start()
        yield from wo_prep()
        yield from widen(1)

    wqb[4, :, 64:128] = jnp.zeros((3 * D, 64), bf16)
    qkv[:, 13] = jnp.zeros((2, HALO + 128, 128), f32)
    xnb[:, 4, :, 64:128] = jnp.zeros((2, 128, 64), bf16)
    for n in range(4, 13):
        qkv[0, n, 0:HALO, :] = jnp.zeros((HALO, 128), f32)
    todo = list(k_order)
    for n, cp in enumerate(first):
        cp.wait()
        if n == OPT["dma"][0]:
            wo_copy.start()
        if n == OPT["dma"][1]:
            for c in [x_copy(1)] + chunk_copies(0):
                c.start()
        if n == OPT["xpos"]:
            feed(widen(0), None, 1000)
            flush(ln1(0, 0))
        else:
            wq_prep(todo.pop(0))
    attn_run(0, 2, OPT["h"], True, late=head_late(), head=True)

    @pl.loop(0, 7)
    def _(i):
        for cp in chunk_copies(i):
            cp.wait()

        @pl.when(i + 2 < NSLAB // 2)
        def _():
            x_copy(i + 2).wait()

        @pl.when(i + 3 < NSLAB // 2)
        def _():
            x_copy(i + 3).start()
        for cp in chunk_copies(i + 2):
            cp.start()
        side = prep_chunk(i, [r.at[i] for r in (wcb, web, wdcb)])
        next(side)
        r = jnp.clip(i - 2, 0, 3)
        attn_run(2 * i + 2, 2, OPT["p"], False, side, widen(jnp.minimum(i + 2, NSLAB // 2 - 1)),
                 ffn_norm_slab(r, r))

    for cp in chunk_copies(7) + chunk_copies(8):
        cp.wait()
    ffn_combos()

    def ffn_group(t, g, last, emit=None):
        ti = _Temps(tin)
        to = _Temps(tout)
        pace = Pace()
        o_ = OPT["fb" if last else "fa"]

        def weights(c):
            if last and c > 0:
                return [r.at[c - 1] for r in (wc2, we2, wdc2)]
            return [r.at[g * 3 + c] for r in (wc, we, wdc)]

        def proj(c, m):
            w, w_ext, _ = weights(c)

            def prod(o, i):
                r = (m * 49 + o * 7 + i) * 64
                p = jnp.dot(_up(ac[o * 7 + i]), _up(w[r:r + 64, :]),
                            preferred_element_type=f32)
                pace.step(p[0:8])
                if o in AUG and i in AUG:
                    q = AUG.index(o) * 4 + AUG.index(i)
                    e = jnp.dot(_up(ae[q, :, 0:64]), _up(w_ext[m * 16 + q]),
                                preferred_element_type=f32)
                    pace.step(e[0:8])
                    p = p + e
                return p
            return prod

        def gate(c):
            def fin(r, cc, v):
                gs[(c % 2) * 16 + r * 4 + cc] = v
            return _recombine(proj(c, 0), fin, ti, to)

        def upgate(c):
            def fin(r, cc, v):
                hs[c, r * 4 + cc] = _ld(gs, (c % 2) * 16 + r * 4 + cc) * v
            yield from _recombine(proj(c, 1), fin, ti, to, last)
            pace.add(hidden_paced(c), *o_["h"][c])

        hgen, hdone = {}, {}

        def hidden(c):
            for o in ORDER:
                yield from strips(lambda cc, r, rows: hs[c, r * 4 + cc, rows, :],
                                  _RHS_SPEC, _rhs_terms, o, hcb.at[c])

        def hidden_paced(c):
            hgen[c], hdone[c] = hidden(c), 0
            next(hgen[c])
            while True:
                z = yield
                need(c, min(hdone[c] + 1, 56), z)

        def need(c, n, z=None):
            feed(hgen[c], z, n - hdone[c])
            hdone[c] = max(hdone[c], n)

        def dprod(cs, i):
            p = None
            for c in cs:
                need(c, 8 * (ORDER.index(i // 7) + 1))
                r = i * (MB // 2)
                q = lax.dot_general(_up(weights(c)[2][r:r + MB // 2, :]), _up(hc[c, i]), NT,
                                    preferred_element_type=f32)
                pace.step(q[0:8])
                p = q if p is None else p + q
            return p

        def down(cs, reset):
            for i in [o * 7 + k for o in ORDER for k in range(7)]:
                a = _ld(acc, i)
                if reset:
                    a = jnp.where(g == 0, 0.0, a)
                acc[i] = a + dprod(cs, i)
                yield

        def down_final(cs):
            def fin(mb, r, v):
                rows = slice(mb * MB, (mb + 1) * MB)
                y = xb[t * 4 + r, rows, :] + v
                xa[t * 4 + r, rows, :] = y
                ost[t * 2 + r // 2, rows, (r % 2) * 128:(r % 2) * 128 + 128] = y.astype(bf16)
            return _recombine(lambda o, i: _ld(acc, o * 7 + i) + dprod(cs, o * 7 + i),
                              fin, _Temps(tin2), _Temps(tout2))

        if last:
            norm = ffn_norm((t + 1) % NTILE)
            pace.add(norm, o_["n0"], o_["nper"])
        else:
            late = prep_chunk(7 + g, [r.at[g] for r in (wcb2, web2, wdcb2)])
            next(late)
            pace.plan.append((late, _spread(o_["wts"], 30, NPREP), None, True))
        for gen in (gate(0), upgate(0), gate(1)):
            _adv(gen, 100)
        d0 = down((0,), not last)
        queue = []

        def lhs_queue():
            while True:
                z = yield
                if queue:
                    try:
                        queue[0].send(z)
                    except StopIteration:
                        queue.pop(0)
        for gen, plan in ((upgate(1), "u1"), (gate(2), "g2"), (upgate(2), "u2")):
            if last and plan == "u2":
                feed(norm, None, 1000)
                pace.add(lhs_queue(), o_["l0"], o_["lper"])
            for k, n in enumerate(o_[plan]):
                _adv(gen, 1)
                if last and plan == "u2":
                    queue.append(lhs_strips(ORDER[k]))
                    next(queue[-1])
                _adv(d0, n)
            _adv(gen, 100)
        _adv(d0, 100)
        if last:
            gen = down_final((1, 2))
            _adv(gen, 3)
            for q, h in ((1, 1), (0, 1), (1, 0), (0, 0)):
                _adv(gen, 1)
                pl.when(emit)(out_copy(t * 2 + q, h).start)
        else:
            _adv(down((1, 2), False), 100)
            feed(late, None, 1000)
        for gen in queue:
            feed(gen, None, 1000)

    @pl.loop(0, 2 * NTILE)
    def _(tile):
        t = tile % NTILE

        @pl.loop(0, 2)
        def _(g):
            ffn_group(t, g, False)
        ffn_group(t, 2, True, tile >= NTILE)

        @pl.when(tile < NTILE)
        def _():
            attn_run(4 * t + NSLAB, 4, OPT["n"], True)

        @pl.when(tile == NTILE - 1)
        def _():
            o = OPT["e"]
            pace = Pace()
            pace.add(attend(1, None), 0, o["aper"], gated=False)
            out_proj(NSLAB - 2, 0, pace)
            pace.drain()
            out_proj(NSLAB - 1, 1, Pace())

    for p in range(NSLAB):
        out_copy(p // 2, p % 2).wait()


def _tiles(w):
    n = w.shape[1]
    return w.reshape(NTR, 8, n // 128, 128).transpose(0, 2, 1, 3).reshape(NTR, n // 16, 128)


@jax.jit
def pallas_interleave_layers__sliding_local_dilated__glu_gated_bilinear__prompt_kernel(
    A_x: jax.Array,
    A_wqkv: jax.Array,
    A_wo: jax.Array,
    B_x: jax.Array,
    B_w_gate: jax.Array,
    B_w_up: jax.Array,
    B_w_down: jax.Array,
):
    del B_x
    vm = pltpu.VMEM
    hbm = pl.BlockSpec(memory_space=pl.ANY)
    out_t = pl.pallas_call(
        _kernel,
        in_specs=[hbm] * 6,
        out_specs=hbm,
        out_shape=jax.ShapeDtypeStruct((D, S), bf16),
        scratch_shapes=[
            vm((NSLAB // 2, 96, 16, 128), bf16),
            vm((NSLAB, 768, 128), f32),
            vm((NSLAB, 768, 128), f32),
            vm((NSLAB // 2, 768, 256), bf16),
            vm((NCHUNK, 224, 32, 128), bf16),
            vm((7, WC_ROWS, 128), bf16),
            vm((7, 32, 64, 128), bf16),
            vm((7, WD_ROWS, 128), bf16),
            vm((2, WC_ROWS, 128), bf16),
            vm((2, 32, 64, 128), bf16),
            vm((2, WD_ROWS, 128), bf16),
            vm((24, 128, 128), f32),
            vm((D, 3 * D), bf16),
            vm((D, D), bf16),
            vm((5, 3 * D, 128), f32),
            vm((5, 3 * D, 128), bf16),
            vm((5, D, 128), bf16),
            vm((2, 5, 128, 128), bf16),
            vm((2, 14, HALO + 128, 128), f32),
            vm((2, 5, 128, 128), bf16),
            vm((49, 128, 128), bf16),
            vm((16, 128, 128), bf16),
            vm((32, 128, 128), f32),
            vm((3, 16, 128, 128), f32),
            vm((3, 49, 128, 128), bf16),
            vm((49, MB, 128), f32),
            vm((12, 128, 128), f32),
            vm((40, 128, 128), f32),
            vm((12, MB, 128), f32),
            vm((20, MB, 128), f32),
            vm((64, 128), f32),
            pltpu.SMEM((1,), jnp.int32),
            pltpu.SemaphoreType.DMA((NSLAB // 2,)),
            pltpu.SemaphoreType.DMA((6,)),
            pltpu.SemaphoreType.DMA((NCHUNK, 3)),
            pltpu.SemaphoreType.DMA((NSLAB // 2, 2)),
        ],
        compiler_params=pltpu.CompilerParams(vmem_limit_bytes=120 * 1024 * 1024,
                                             disable_bounds_checks=True,
                                             disable_semaphore_checks=True),
    )(_tiles(A_x[0].T), A_wqkv, A_wo, _tiles(B_w_gate), _tiles(B_w_up), _tiles(B_w_down.T))
    return out_t.T[None]
```

```python
import math

import jax
import jax.numpy as jnp
from jax import lax
import jax.experimental.pallas as pl
import jax.experimental.pallas.tpu as pltpu

f32 = jnp.float32
bf16 = jnp.bfloat16
u32 = jnp.uint32

S, D, F = 2048, 576, 4608
H, DH, WIN, DIL = 32, 18, 8, 2
EPS = 1e-5
LOG2E = math.log2(math.e)
NSLAB = S // 128
TILE = 512
NTILE = S // TILE
FC = 512
NCHUNK = F // FC
MB = D // 4
HALO = 16
NPREP = 158
NTR = D // 8
WC_ROWS = 800 * 16
WD_ROWS = 448 * 16
NT = (((1,), (1,)), ((), ()))
ORDER = (0, 1, 2, 5, 3, 4, 6)
AUG = (0, 1, 2, 5)

OPT = {'dma': (0, 2),
 'xpos': 2,
 'parts': (1, 0, 2),
 'fa': {'wts': (3, 1, 2, 1, 0, 1, 2, 1, 1, 2, 0, 0, 0, 1, 0, 3, 3, 4),
        'h': ((0, 0.7), (0, 1), (0, 1)),
        'u1': (0, 0, 0, 4, 5, 4, 6),
        'g2': (4, 0, 0, 0, 0, 0, 0),
        'u2': (0, 0, 0, 0, 4, 4, 4)},
 'fb': {'h': ((0, 1), (0, 0.59), (0, 1)),
        'n0': 0,
        'nper': 1.4,
        'l0': 0,
        'lper': 3.22,
        'u1': (0, 0, 0, 0, 4, 4, 6),
        'g2': (4, 0, 0, 0, 0, 0, 0),
        'u2': (0, 0, 0, 0, 4, 4, 4)},
 'h': {'lag': 0,
       'grp': ((4, 5, 6, 7), (0, 1, 2, 3), (12, 13, 8, 9, 10, 11)),
       'a': ((0, 5, 35), (0, 3.65, 35)),
       'w0': 22,
       'wper': 2.8,
       'ag': 1,
       'ls': ((13, 5.0, 40),)},
 'p': {'lag': 0,
       'x0': 36,
       'xper': 5.6,
       'grp': ((4, 13), (5, 6, 7, 0), (1, 2, 3, 12), (8, 9, 10, 11)),
       'a': ((3, 6, 25), (0, 5.44, 35)),
       'w0': 65,
       'wper': 4.88,
       'ag': 0,
       'ls': ((40, 5.47, None),),
       'wts': (7, 9, 9, 9, 9, 9, 5, 11, 9, 11, 7, 11, 7, 11, 11, 11)},
 'n': {'lag': 1,
       'grp': ((4, 5, 6, 7), (0, 1, 2, 3), (12, 13, 8, 9, 10, 11)),
       'a': ((0, 6, 30), (3, 6, 30), (0, 6.15, 30), (0, 5.4, 35)),
       'ag': 1,
       'ls': ((77, 5.51, None), (69, 9.04, None), (80, 6.83, None))}}


def _up(v):
    return pltpu.bitcast(v, bf16)


def _quad(x):
    n = len(x) // 2
    return ([r[:n] for r in x[:n]], [r[n:] for r in x[:n]],
            [r[:n] for r in x[n:]], [r[n:] for r in x[n:]])


def _badd(x, y):
    return [[a + b for a, b in zip(r, s)] for r, s in zip(x, y)]


def _bsub(x, y):
    return [[a - b for a, b in zip(r, s)] for r, s in zip(x, y)]


def _lhs_terms(a):
    a11, a12, a21, a22 = _quad(a)
    return [lambda: _badd(a11, a22), lambda: _badd(a21, a22), lambda: a11, lambda: a22,
            lambda: _badd(a11, a12), lambda: _bsub(a21, a11), lambda: _bsub(a12, a22)]


def _rhs_terms(b):
    b11, b12, b21, b22 = _quad(b)
    return [lambda: _badd(b11, b22), lambda: b11, lambda: _bsub(b12, b22), lambda: _bsub(b21, b11),
            lambda: b22, lambda: _badd(b11, b12), lambda: _badd(b21, b22)]


def _combos(x, terms, emit):
    for o, fo in enumerate(terms(x)):
        y = fo()
        for i, fi in enumerate(terms(y)):
            emit(o * 7 + i, fi()[0][0])


_LHS_SPEC = (((0, 0), (1, 1), 1), ((1, 0), (1, 1), 1), ((0, 0), None, 0), ((1, 1), None, 0),
             ((0, 0), (0, 1), 1), ((1, 0), (0, 0), -1), ((0, 1), (1, 1), -1))
_RHS_SPEC = (((0, 0), (1, 1), 1), ((0, 0), None, 0), ((0, 1), (1, 1), -1), ((1, 0), (0, 0), -1),
             ((1, 1), None, 0), ((0, 0), (0, 1), 1), ((1, 0), (1, 1), 1))


def _outer_term(load, spec, o):
    p, q, sign = spec[o]
    out = []
    for y in range(2):
        row = []
        for z in range(2):
            v = load(2 * p[0] + y, 2 * p[1] + z)
            if sign:
                w = load(2 * q[0] + y, 2 * q[1] + z)
                v = v + w if sign > 0 else v - w
            row.append(v)
        out.append(row)
    return out


def _inner_terms(y, terms, o, emit):
    for i, fi in enumerate(terms(y)):
        emit(o * 7 + i, fi()[0][0])


def _lhs_ext(e):
    n = len(e) // 2
    return {0: e[:n], 1: e[n:], 2: e[:n], 5: [y - x for x, y in zip(e[:n], e[n:])]}


def _rhs_ext(e):
    n = len(e) // 2
    return {0: e[:n], 1: e[:n], 2: e[n:], 5: [x + y for x, y in zip(e[:n], e[n:])]}


def _ext_combos(e, fn, emit):
    for oi, o in enumerate(AUG):
        d = fn(fn(e)[o])
        for ii, i in enumerate(AUG):
            emit(oi * 4 + ii, d[i][0])


def _spread(weights, span, n):
    total, acc, out = sum(weights), 0.0, []
    for k, w in enumerate(weights):
        lo, acc = acc, acc + w * n / total
        count = round(acc) - round(lo)
        out += [k * span + i * span // count for i in range(count)]
    return out


def _adv(gen, n):
    for _ in range(n):
        try:
            next(gen)
        except StopIteration:
            return


def _ld(ref, idx):
    n = ref.shape[-2] // 2
    return jnp.concatenate([ref[idx, :n, :], ref[idx, n:, :]], axis=0)


class _Temps:
    def __init__(self, ref):
        self.ref = ref
        self.n = 0

    def put(self, v):
        i = self.n % self.ref.shape[0]
        self.n += 1
        self.ref[i] = v
        return i

    def get(self, i):
        return _ld(self.ref, i)


def _recombine(prod, fin, ti, to, spill_last=False):
    def inner(o, sink):
        a = ti.put(prod(o, 0))
        b = ti.put(prod(o, 1))
        c = ti.put(prod(o, 2))
        sink(1, 1, ti.get(a) - ti.get(b) + ti.get(c) + prod(o, 5))
        if spill_last:
            m3 = prod(o, 3)
            m4 = prod(o, 4)
            sink(1, 0, ti.get(b) + m3)
            sink(0, 1, ti.get(c) + m4)
            d = ti.put(ti.get(a) + m3 - m4)
            sink(0, 0, ti.get(d) + prod(o, 6))
            return
        m3 = prod(o, 3)
        m4 = prod(o, 4)
        m6 = prod(o, 6)
        sink(1, 0, ti.get(b) + m3)
        sink(0, 1, ti.get(c) + m4)
        sink(0, 0, ti.get(a) + m3 - m4 + m6)

    m = {}
    for o in (0, 1, 2):
        def keep(y, z, v, o=o):
            m[o, y, z] = to.put(v)
        inner(o, keep)
        yield

    def s5(y, z, v):
        fin(2 + y, 2 + z, to.get(m[0, y, z]) - to.get(m[1, y, z]) + to.get(m[2, y, z]) + v)
    inner(5, s5)
    yield

    def s3(y, z, v):
        fin(2 + y, z, to.get(m[1, y, z]) + v)
        m[3, y, z] = to.put(to.get(m[0, y, z]) + v)
    inner(3, s3)
    yield

    def s4(y, z, v):
        fin(y, 2 + z, to.get(m[2, y, z]) + v)
        m[3, y, z] = to.put(to.get(m[3, y, z]) - v)
    inner(4, s4)
    yield

    def s6(y, z, v):
        fin(y, z, to.get(m[3, y, z]) + v)
    inner(6, s6)
    yield


def _kernel(xt_hbm, wqkv_hbm, wo_hbm, wg_hbm, wu_hbm, wdt_hbm, out_hbm,
            xin, xa, xb, ost, raw, wcb, web, wdcb, wcb2, web2, wdcb2, xn2,
            wq_raw, wo_raw, wtmp, wqb, wob, xnb, qkv, ob, acb, aeb, gs, hs, hcb, acc, tin, tout, tin2, tout2, ktail, zero,
            sem_x, sem_w, sem_c, sem_o):
    wq, wo, wc, we, wdc, xn, o32, ac, ae, hc, raw32, xin32, wc2, we2, wdc2 = [
        r.bitcast(u32) for r in (wqb, wob, wcb, web, wdcb, xnb, ob, acb, aeb, hcb, raw, xin,
                                 wcb2, web2, wdcb2)]

    def x_copy(q):
        return pltpu.make_async_copy(
            xt_hbm.at[:, pl.ds(pl.multiple_of(q * 16, 16), 16), :], xin.at[q, 0:NTR], sem_x.at[q])

    def weight_copy(j, m):
        rows = pl.ds(pl.multiple_of(j * 32, 32), 32)
        return pltpu.make_async_copy((wg_hbm, wu_hbm, wdt_hbm)[m].at[:, rows, :],
                                     raw.at[j, pl.ds(m * NTR, NTR)], sem_c.at[j, m])

    def chunk_copies(j):
        return [weight_copy(j, m) for m in range(3)]

    def out_copy(q, h):
        rows = pl.ds(h * 2 * MB, 2 * MB)
        return pltpu.make_async_copy(
            ost.at[q, rows, :], out_hbm.at[rows, pl.ds(pl.multiple_of(q * 256, 256), 256)],
            sem_o.at[q, h])

    k_order = (4, 0, 1, 2, 3)
    wq_copies = [pltpu.make_async_copy(wqkv_hbm.at[k * 128:min(k * 128 + 128, D)],
                                       wq_raw.at[k * 128:min(k * 128 + 128, D)], sem_w.at[k])
                 for k in k_order]
    wo_copy = pltpu.make_async_copy(wo_hbm, wo_raw, sem_w.at[5])
    first = wq_copies[:OPT["xpos"]] + [x_copy(0)] + wq_copies[OPT["xpos"]:]
    for cp in first:
        cp.start()
    zero[0] = 0
    never = zero[0] != 0

    def held(v, z):
        if z is None:
            return v
        return jnp.where(never, pltpu.bitcast(z, v.dtype), v)

    def raw_pair(j, tr, cp, z):
        v = [_up(held(raw32[j, tr + k, cp * 8:cp * 8 + 8, :], z)).astype(f32) for k in range(2)]
        return [jnp.concatenate([v[0][h:h + 8], v[1][h:h + 8]], axis=0) for h in (0, 8)]

    def prep_strip(j, tr, step, spec, terms, path, emit):
        live = {}
        for o in path:
            used = [q for q in spec[o][:2] if q is not None]
            live = {q: live[q] for q in used if q in live}
            for q in used:
                if q not in live:
                    z = yield
                    live[q] = [raw_pair(j, tr + (2 * q[0] + y) * step, q[1], z) for y in range(2)]
            y = _outer_term(lambda r, c: live[r // 2, c // 2][r % 2][c % 2], spec, o)
            _inner_terms(y, terms, o, emit)

    def prep_gu(j, dst, m, s):
        base = m * (49 * 128) + s * 16

        def emit(i, v):
            dst[pl.ds(base + i * 128, 16), :] = v.astype(bf16)
        return prep_strip(j, m * NTR + 2 * s, 16, _RHS_SPEC, _rhs_terms, (1, 0, 4, 2, 5, 3, 6), emit)

    def prep_ext(j, dst, m, s):
        z = yield
        tr = m * NTR + 64 + 2 * s

        def emit(i, v):
            dst[m * 16 + i, pl.ds(s * 16, 16), :] = v.astype(bf16)
        _ext_combos(raw_pair(j, tr, 0, z) + raw_pair(j, tr, 1, z), _rhs_ext, emit)

    def prep_down(j, dst, s):
        def emit(i, v):
            dst[pl.ds(s * 16 + i * MB, 16), :] = v.astype(bf16)
        return prep_strip(j, 2 * NTR + 2 * s, MB // 8, _LHS_SPEC, _lhs_terms,
                          (2, 0, 3, 6, 4, 5, 1), emit)

    def prep_chunk(j, dst):
        for m in range(2):
            for s in range(8):
                yield from prep_gu(j, dst[0], m, s)
            for s in range(4):
                yield from prep_ext(j, dst[1], m, s)
        for s in range(9):
            yield from prep_down(j, dst[2], s)

    def feed(gen, z, n):
        for _ in range(n):
            try:
                gen.send(z)
            except StopIteration:
                return

    class Pace:
        def __init__(self):
            self.tok = 0
            self.plan = []
            self.due = []

        def add(self, gen, t0, period, lat=None, gated=True):
            next(gen)
            when = [self.tok + int(t0 + k * period) for k in range(1000)]
            self.plan.append((gen, when, lat, gated))

        def step(self, z):
            for gen, when, lat, gated in self.plan:
                for _ in range(when.count(self.tok)):
                    try:
                        v = gen.send(z if gated else None)
                    except StopIteration:
                        break
                    if v is not None and lat is not None:
                        self.due.append((self.tok + lat, v))
            self.tok += 1

        def tokens(self, r, n):
            for k in range(n):
                self.step(r[k * 16:k * 16 + 8])

        def gate(self, v):
            now = [x for t, x in self.due if t <= self.tok]
            self.due = [(t, x) for t, x in self.due if t > self.tok]
            if not now:
                return v
            head = jnp.where(never, pltpu.bitcast(tree(now), u32), v[0:8])
            return jnp.concatenate([head, v[8:]], axis=0)

        def drain(self):
            for gen, *_ in self.plan:
                feed(gen, None, 1000)

    def tree(vals):
        while len(vals) > 1:
            vals = [a + b for a, b in zip(vals[::2], vals[1::2])] + vals[len(vals) & ~1:]
        return vals[0]

    def norm_slab(row, emit):
        def rows(k, lo, hi):
            return [row(k, r) for r in range(lo // 8, hi // 8)]

        def mean(vals):
            t = tree([sum(vals[k + 4::4], vals[k]) for k in range(4)])
            t = jnp.sum(t, axis=0, keepdims=True) * (1.0 / D)
            return jnp.broadcast_to(t, (8, 128))
        z = yield
        x = rows(0, 0, D)
        mu = mean([held(v, z) for v in x[:4]] + x[4:])
        m = held(mu, (yield))
        rs = lax.rsqrt(mean([(v - m) * (v - m) for v in rows(1, 0, D)]) + EPS)
        end = None
        for k in (4, 0, 1, 2, 3):
            m = held(mu, (yield end))
            y = jnp.concatenate(
                [(v - m) * rs for v in rows(2, k * 128, min((k + 1) * 128, D))], axis=0).T
            emit(k, y)
            end = y[120:128] if k < 4 else jnp.concatenate([y[120:128]] * 2, axis=1)
        yield end

    def alias(p, n):
        return [jnp.clip(p + k * zero[0], 0, n - 1) for k in range(3)]

    def slab_rows(src, p):
        q = alias(p, NSLAB)
        return lambda k, r: src[q[k], r * 8:r * 8 + 8, :]

    def flush(gen):
        return tree([v for v in gen if v is not None])

    def ln1(p, b):
        def emit(k, y):
            xnb[b, k, :, 0:y.shape[1]] = y.astype(bf16)
        return norm_slab(slab_rows(xa, p), emit)

    def widen(q):
        for r in range(NTR):
            if r % 4 == 0:
                z = yield
            v = _up(held(xin32[q, r], z)).astype(f32)
            for b in range(2):
                xa[2 * q + b, r * 8:r * 8 + 8, :] = v[b * 8:b * 8 + 8]

    def qkv_proj(b, pace, groups):
        scale = DH ** -0.5 * LOG2E
        for grp in groups:
            for n in grp:
                if n == 13:
                    ktail[...] = lax.dot_general(
                        _up(wq[4, n * 64:n * 64 + 32, :]), _up(xn[b, 4]), NT,
                        preferred_element_type=f32)
                else:
                    qkv[b, n, HALO:HALO + 128, :] = lax.dot_general(
                        _up(xn[b, 4]), _up(wq[4, n * 64:(n + 1) * 64, :]), NT,
                        preferred_element_type=f32)
            for n in grp:
                rows = slice(n * 64, n * 64 + (32 if n == 13 else 64))
                x = jnp.concatenate(
                    [_up(pace.gate(xn[b, 0]))] + [_up(xn[b, k]) for k in range(1, 4)], axis=1)
                w = jnp.concatenate([_up(wq[k, rows, :]) for k in range(4)], axis=1)
                if n == 13:
                    r = lax.dot_general(w, x, NT, preferred_element_type=f32)
                    r = r + jnp.concatenate([ktail[0:32, :], ktail[32:64, :]], axis=0)
                    qkv[b, n, HALO:HALO + 128, 0:64] = (r * scale).T
                    pace.tokens(r, 4)
                    continue
                r = lax.dot_general(x, w, NT, preferred_element_type=f32)
                r = r + jnp.concatenate([qkv[b, n, HALO:HALO + 64, :],
                                         qkv[b, n, HALO + 64:HALO + 128, :]], axis=0)
                if n in (4, 5, 6, 7):
                    r = r * scale
                qkv[b, n, HALO:HALO + 128, :] = r
                pace.tokens(r, 7)

    def halo(b):
        for n in range(4, 14):
            qkv[b, n, 0:HALO, :] = qkv[1 - b, n, 128:128 + HALO, :]

    def attend(b, row0, lag=0):
        qs, ks, vs = (0, 1, 2, 3, 12), (4, 5, 6, 7, 13), (8, 9, 10, 11, 12)

        def scores(s, z):
            r = HALO + s * 8
            q = [held(qkv[b, n, r:r + 8, :], z) for n in qs]
            logit = []
            for w in range(WIN):
                rw = r - DIL * w
                part = tree([q[c] * qkv[b, ks[c], rw:rw + 8, :] for c in range(5)])
                part = part + pltpu.roll(part, 64, 1)
                part = part + pltpu.roll(part, 32, 1)
                if row0 is not None and s * 8 < DIL * w:
                    pos = row0 + s * 8 + lax.broadcasted_iota(jnp.int32, (8, 128), 0)
                    part = jnp.where(pos >= DIL * w, part, -1e9 * LOG2E)
                logit.append(part)
            return logit

        def values(s, logit, z):
            r = HALO + s * 8
            mx = logit
            while len(mx) > 1:
                mx = [jnp.maximum(a, c) for a, c in zip(mx[::2], mx[1::2])]
            top = held(mx[0], z)
            e = [jnp.exp2(l - top) for l in logit]
            inv = 1.0 / tree(e)
            outs = []
            for c in range(5):
                o = e[0] * qkv[b, vs[c], r:r + 8, :]
                for w in range(1, WIN):
                    rw = r - DIL * w
                    o = o + e[w] * qkv[b, vs[c], rw:rw + 8, :]
                o = o * inv
                outs.append(o)
                ob[b, c, s * 8:(s + 1) * 8, :] = o.astype(bf16)
            return tree(outs)

        v, pending = None, []
        for s in range(16 + lag):
            z = yield v
            if s < 16:
                pending.append(scores(s, z))
            if s >= lag:
                v = values(s - lag, pending.pop(0), z if lag else None)
        yield v

    def out_proj(p, b, pace):
        h = MB // 2
        for m in range(4):
            xb[p, m * MB:(m + 1) * MB, :] = xa[p, m * MB:(m + 1) * MB, :] + lax.dot_general(
                _up(wo[4, m * h:(m + 1) * h, :]), _up(o32[b, 4]), NT, preferred_element_type=f32)
        rhs = jnp.concatenate([_up(o32[b, c]) for c in range(4)], axis=1)
        for m in range(4):
            rows = slice(m * h, (m + 1) * h)
            lhs = jnp.concatenate(
                [_up(pace.gate(wo[0, rows, :]))] + [_up(wo[c, rows, :]) for c in range(1, 4)],
                axis=1)
            r = lax.dot_general(lhs, rhs, NT, preferred_element_type=f32)
            r = r + jnp.concatenate([xb[p, m * MB:m * MB + h, :],
                                     xb[p, m * MB + h:(m + 1) * MB, :]], axis=0)
            xb[p, m * MB:(m + 1) * MB, :] = r
            pace.tokens(r, 8)

    def ffn_norm_slab(p, r):
        def emit(k, y):
            xn2[r * 6 + k, :, 0:y.shape[1]] = y
        return norm_slab(slab_rows(xb, p), emit)

    def ffn_norm(t):
        for r in range(4):
            yield from ffn_norm_slab(t * 4 + r, r)

    def strips(load, spec, terms, o, dst):
        for s in range(8):
            z = yield
            rows = slice(s * 16, (s + 1) * 16)

            def ld(r, c):
                v = load(r, c, rows)
                if (r // 2, c // 2) == spec[o][0]:
                    v = jnp.concatenate([held(v[0:8], z), held(v[8:16], z)], axis=0)
                return v

            def emit(i, v):
                dst[i, rows, :] = v.astype(bf16)
            _inner_terms(_outer_term(ld, spec, o), terms, o, emit)

    def lhs_strips(o):
        yield from strips(lambda r, k, rows: xn2[r * 6 + k, rows, :],
                          _LHS_SPEC, _lhs_terms, o, acb)
        if o in AUG:
            for s in range(2):
                z = yield
                rows = slice(s * 64, (s + 1) * 64)
                d = _lhs_ext(_lhs_ext([xn2[r * 6 + 4, rows, 0:64] for r in range(4)])[o])
                for ii, i in enumerate(AUG):
                    aeb[AUG.index(o) * 4 + ii, rows, 0:64] = d[i][0].astype(bf16)

    def ffn_combos():
        for s in range(8):
            rows = slice(s * 16, (s + 1) * 16)
            a = [[xn2[r * 6 + k, rows, :] for k in range(4)] for r in range(4)]

            def emit(i, v, rows=rows):
                acb[i, rows, :] = v.astype(bf16)
            _combos(a, _lhs_terms, emit)
            e = [xn2[r * 6 + 4, rows, 0:64] for r in range(4)]

            def emit_e(i, v, rows=rows):
                aeb[i, rows, 0:64] = v.astype(bf16)
            _ext_combos(e, _lhs_ext, emit_e)

    def attn_run(h, count, o, mask, side=None, late=None, extra=None, head=False):
        if not head:
            flush(ln1(h % NSLAB, 0))
        for k in range(count):
            b = k % 2
            pace = Pace()
            if side is not None:
                when = [w - k * 128 for w in _spread(o["wts"], 16, NPREP)]
                pace.plan.append((side, [min(w, 126) for w in when if 0 <= w < 128], None, True))
            if k + 1 < count:
                pace.add(ln1((h + k + 1) % NSLAB, 1 - b), *o["ls"][k])
            elif late is not None:
                pace.add(late, o["w0"], o["wper"])
            if k == 1 and extra is not None:
                pace.add(extra, 32 + o["x0"], o["xper"])
            if k > 0 or not head:
                row0 = (h % NSLAB) * 128 if k == 1 and mask else None
                pace.add(attend(1 - b, row0, o["lag"]), *o["a"][k], o["ag"])
                if not head:
                    out_proj((h + k - 2) % NSLAB, b, pace)
                halo(b)
            qkv_proj(b, pace, o["grp"])
            pace.plan = [e for e in pace.plan if e[0] is not side]
            pace.drain()
        if side is not None:
            feed(side, None, 1000)

    def wq_prep(k):
        w = 128 if k < 4 else 64
        for c0 in range(0, 3 * D, 128):
            c1 = min(c0 + 128, 3 * D)
            wtmp[k, c0:c1, 0:w] = wq_raw[k * 128:k * 128 + w, c0:c1].astype(f32).T
        for part in OPT["parts"]:
            for d in range(DH):
                if d < 16:
                    row = part * 512 + d * 32
                else:
                    row = (1536, 1664, 1600)[part] + (d - 16) * 32
                wqb[k, row:row + 32, 0:w] = wtmp[
                    k, pl.ds(part * D + d, H, stride=DH), 0:w].astype(bf16)

    def wo_prep():
        for n in range(5):
            w = 128 if n < 4 else 64
            wtmp[n, 0:D, 0:w] = wo_raw[:, n * 128:n * 128 + w].astype(f32)
        for n in range(5):
            w = 128 if n < 4 else 64
            for c in range(5):
                z = yield
                rows = [held(wtmp[n, pl.ds(4 * c + g + k * 8 * DH, 8, stride=DH), :], z)[:, 0:w]
                        for g in range(4 if c < 4 else 2) for k in range(4)]
                if c == 4:
                    rows = [jnp.zeros((64, w), f32)] + rows
                wob[c, n * 128:n * 128 + w, :] = jnp.concatenate(rows, axis=0).T.astype(bf16)

    def head_late():
        for cp in (wo_copy, x_copy(1)):
            cp.wait()
        for cp in [x_copy(2)] + chunk_copies(1):
            cp.start()
        yield from wo_prep()
        yield from widen(1)

    wqb[4, :, 64:128] = jnp.zeros((3 * D, 64), bf16)
    qkv[:, 13] = jnp.zeros((2, HALO + 128, 128), f32)
    xnb[:, 4, :, 64:128] = jnp.zeros((2, 128, 64), bf16)
    for n in range(4, 13):
        qkv[0, n, 0:HALO, :] = jnp.zeros((HALO, 128), f32)
    todo = list(k_order)
    for n, cp in enumerate(first):
        cp.wait()
        if n == OPT["dma"][0]:
            wo_copy.start()
        if n == OPT["dma"][1]:
            for c in [x_copy(1)] + chunk_copies(0):
                c.start()
        if n == OPT["xpos"]:
            feed(widen(0), None, 1000)
            flush(ln1(0, 0))
        else:
            wq_prep(todo.pop(0))
    attn_run(0, 2, OPT["h"], True, late=head_late(), head=True)

    @pl.loop(0, 7)
    def _(i):
        for cp in chunk_copies(i):
            cp.wait()

        @pl.when(i + 2 < NSLAB // 2)
        def _():
            x_copy(i + 2).wait()

        @pl.when(i + 3 < NSLAB // 2)
        def _():
            x_copy(i + 3).start()
        for cp in chunk_copies(i + 2):
            cp.start()
        side = prep_chunk(i, [r.at[i] for r in (wcb, web, wdcb)])
        next(side)
        r = jnp.clip(i - 2, 0, 3)
        attn_run(2 * i + 2, 2, OPT["p"], False, side, widen(jnp.minimum(i + 2, NSLAB // 2 - 1)),
                 ffn_norm_slab(r, r))

    for cp in chunk_copies(7) + chunk_copies(8):
        cp.wait()
    ffn_combos()

    def ffn_group(t, g, last, emit=None):
        ti = _Temps(tin)
        to = _Temps(tout)
        pace = Pace()
        o_ = OPT["fb" if last else "fa"]

        def weights(c):
            if last and c > 0:
                return [r.at[c - 1] for r in (wc2, we2, wdc2)]
            return [r.at[g * 3 + c] for r in (wc, we, wdc)]

        def proj(c, m):
            w, w_ext, _ = weights(c)

            def prod(o, i):
                r = (m * 49 + o * 7 + i) * 64
                p = jnp.dot(_up(ac[o * 7 + i]), _up(w[r:r + 64, :]),
                            preferred_element_type=f32)
                pace.step(p[0:8])
                if o in AUG and i in AUG:
                    q = AUG.index(o) * 4 + AUG.index(i)
                    e = jnp.dot(_up(ae[q, :, 0:64]), _up(w_ext[m * 16 + q]),
                                preferred_element_type=f32)
                    pace.step(e[0:8])
                    p = p + e
                return p
            return prod

        def gate(c):
            def fin(r, cc, v):
                gs[(c % 2) * 16 + r * 4 + cc] = v
            return _recombine(proj(c, 0), fin, ti, to)

        def upgate(c):
            def fin(r, cc, v):
                hs[c, r * 4 + cc] = _ld(gs, (c % 2) * 16 + r * 4 + cc) * v
            yield from _recombine(proj(c, 1), fin, ti, to, last)
            pace.add(hidden_paced(c), *o_["h"][c])

        hgen, hdone = {}, {}

        def hidden(c):
            for o in ORDER:
                yield from strips(lambda cc, r, rows: hs[c, r * 4 + cc, rows, :],
                                  _RHS_SPEC, _rhs_terms, o, hcb.at[c])

        def hidden_paced(c):
            hgen[c], hdone[c] = hidden(c), 0
            next(hgen[c])
            while True:
                z = yield
                need(c, min(hdone[c] + 1, 56), z)

        def need(c, n, z=None):
            feed(hgen[c], z, n - hdone[c])
            hdone[c] = max(hdone[c], n)

        def dprod(cs, i):
            p = None
            for c in cs:
                need(c, 8 * (ORDER.index(i // 7) + 1))
                r = i * (MB // 2)
                q = lax.dot_general(_up(weights(c)[2][r:r + MB // 2, :]), _up(hc[c, i]), NT,
                                    preferred_element_type=f32)
                pace.step(q[0:8])
                p = q if p is None else p + q
            return p

        def down(cs, reset):
            for i in [o * 7 + k for o in ORDER for k in range(7)]:
                a = _ld(acc, i)
                if reset:
                    a = jnp.where(g == 0, 0.0, a)
                acc[i] = a + dprod(cs, i)
                yield

        def down_final(cs):
            def fin(mb, r, v):
                rows = slice(mb * MB, (mb + 1) * MB)
                y = xb[t * 4 + r, rows, :] + v
                xa[t * 4 + r, rows, :] = y
                ost[t * 2 + r // 2, rows, (r % 2) * 128:(r % 2) * 128 + 128] = y.astype(bf16)
            return _recombine(lambda o, i: _ld(acc, o * 7 + i) + dprod(cs, o * 7 + i),
                              fin, _Temps(tin2), _Temps(tout2))

        if last:
            norm = ffn_norm((t + 1) % NTILE)
            pace.add(norm, o_["n0"], o_["nper"])
        else:
            late = prep_chunk(7 + g, [r.at[g] for r in (wcb2, web2, wdcb2)])
            next(late)
            pace.plan.append((late, _spread(o_["wts"], 30, NPREP), None, True))
        for gen in (gate(0), upgate(0), gate(1)):
            _adv(gen, 100)
        d0 = down((0,), not last)
        queue = []

        def lhs_queue():
            while True:
                z = yield
                if queue:
                    try:
                        queue[0].send(z)
                    except StopIteration:
                        queue.pop(0)
        for gen, plan in ((upgate(1), "u1"), (gate(2), "g2"), (upgate(2), "u2")):
            if last and plan == "u2":
                feed(norm, None, 1000)
                pace.add(lhs_queue(), o_["l0"], o_["lper"])
            for k, n in enumerate(o_[plan]):
                _adv(gen, 1)
                if last and plan == "u2":
                    queue.append(lhs_strips(ORDER[k]))
                    next(queue[-1])
                _adv(d0, n)
            _adv(gen, 100)
        _adv(d0, 100)
        if last:
            gen = down_final((1, 2))
            _adv(gen, 3)
            for q, h in ((1, 1), (0, 1), (1, 0), (0, 0)):
                _adv(gen, 1)
                pl.when(emit)(out_copy(t * 2 + q, h).start)
        else:
            _adv(down((1, 2), False), 100)
            feed(late, None, 1000)
        for gen in queue:
            feed(gen, None, 1000)

    @pl.loop(0, 2 * NTILE)
    def _(tile):
        t = tile % NTILE

        @pl.loop(0, 2)
        def _(g):
            ffn_group(t, g, False)
        ffn_group(t, 2, True, tile >= NTILE)

        @pl.when(tile < NTILE)
        def _():
            attn_run(4 * t + NSLAB, 4, OPT["n"], True)

        @pl.when(tile == NTILE - 1)
        def _():
            out_proj(NSLAB - 2, 0, Pace())
            flush(attend(1, None))
            out_proj(NSLAB - 1, 1, Pace())

    for p in range(NSLAB):
        out_copy(p // 2, p % 2).wait()


def _tiles(w):
    n = w.shape[1]
    return w.reshape(NTR, 8, n // 128, 128).transpose(0, 2, 1, 3).reshape(NTR, n // 16, 128)


@jax.jit
def pallas_interleave_layers__sliding_local_dilated__glu_gated_bilinear__prompt_kernel(
    A_x: jax.Array,
    A_wqkv: jax.Array,
    A_wo: jax.Array,
    B_x: jax.Array,
    B_w_gate: jax.Array,
    B_w_up: jax.Array,
    B_w_down: jax.Array,
):
    del B_x
    vm = pltpu.VMEM
    hbm = pl.BlockSpec(memory_space=pl.ANY)
    out_t = pl.pallas_call(
        _kernel,
        in_specs=[hbm] * 6,
        out_specs=hbm,
        out_shape=jax.ShapeDtypeStruct((D, S), bf16),
        scratch_shapes=[
            vm((NSLAB // 2, 96, 16, 128), bf16),
            vm((NSLAB, 768, 128), f32),
            vm((NSLAB, 768, 128), f32),
            vm((NSLAB // 2, 768, 256), bf16),
            vm((NCHUNK, 224, 32, 128), bf16),
            vm((7, WC_ROWS, 128), bf16),
            vm((7, 32, 64, 128), bf16),
            vm((7, WD_ROWS, 128), bf16),
            vm((2, WC_ROWS, 128), bf16),
            vm((2, 32, 64, 128), bf16),
            vm((2, WD_ROWS, 128), bf16),
            vm((24, 128, 128), f32),
            vm((D, 3 * D), bf16),
            vm((D, D), bf16),
            vm((5, 3 * D, 128), f32),
            vm((5, 3 * D, 128), bf16),
            vm((5, D, 128), bf16),
            vm((2, 5, 128, 128), bf16),
            vm((2, 14, HALO + 128, 128), f32),
            vm((2, 5, 128, 128), bf16),
            vm((49, 128, 128), bf16),
            vm((16, 128, 128), bf16),
            vm((32, 128, 128), f32),
            vm((3, 16, 128, 128), f32),
            vm((3, 49, 128, 128), bf16),
            vm((49, MB, 128), f32),
            vm((12, 128, 128), f32),
            vm((40, 128, 128), f32),
            vm((12, MB, 128), f32),
            vm((20, MB, 128), f32),
            vm((64, 128), f32),
            pltpu.SMEM((1,), jnp.int32),
            pltpu.SemaphoreType.DMA((NSLAB // 2,)),
            pltpu.SemaphoreType.DMA((6,)),
            pltpu.SemaphoreType.DMA((NCHUNK, 3)),
            pltpu.SemaphoreType.DMA((NSLAB // 2, 2)),
        ],
        compiler_params=pltpu.CompilerParams(vmem_limit_bytes=120 * 1024 * 1024,
                                             disable_bounds_checks=True,
                                             disable_semaphore_checks=True),
    )(_tiles(A_x[0].T), A_wqkv, A_wo, _tiles(B_w_gate), _tiles(B_w_up), _tiles(B_w_down.T))
    return out_t.T[None]
```

```python
import math

import jax
import jax.numpy as jnp
from jax import lax
import jax.experimental.pallas as pl
import jax.experimental.pallas.tpu as pltpu

f32 = jnp.float32
bf16 = jnp.bfloat16
u32 = jnp.uint32

S, D, F = 2048, 576, 4608
H, DH, WIN, DIL = 32, 18, 8, 2
EPS = 1e-5
LOG2E = math.log2(math.e)
NSLAB = S // 128
TILE = 512
NTILE = S // TILE
FC = 512
NCHUNK = F // FC
MB = D // 4
HALO = 16
NPREP = 158
NTR = D // 8
WC_ROWS = 800 * 16
WD_ROWS = 448 * 16
NT = (((1,), (1,)), ((), ()))
ORDER = (0, 1, 2, 5, 3, 4, 6)
AUG = (0, 1, 2, 5)

OPT = {'dma': (0, 2),
 'xpos': 2,
 'parts': (1, 0, 2),
 'fa': {'wts': (3, 1, 2, 1, 0, 1, 2, 1, 1, 2, 0, 0, 0, 1, 0, 3, 3, 4),
        'h': ((0, 0.7), (0, 1), (0, 1)),
        'u1': (0, 0, 0, 4, 5, 4, 6),
        'g2': (4, 0, 0, 0, 0, 0, 0),
        'u2': (0, 0, 0, 0, 4, 4, 4)},
 'fb': {'h': ((0, 1), (0, 0.59), (0, 1)),
        'n0': 0,
        'nper': 1.4,
        'l0': 0,
        'lper': 3.22,
        'u1': (0, 0, 0, 0, 4, 4, 6),
        'g2': (4, 0, 0, 0, 0, 0, 0),
        'u2': (0, 0, 0, 0, 4, 4, 4)},
 'h': {'lag': 0,
       'grp': ((4, 5, 6, 7), (0, 1, 2, 3), (12, 13, 8, 9, 10, 11)),
       'a': ((0, 5, 35), (0, 3.65, 35)),
       'w0': 22,
       'wper': 2.8,
       'ag': 1,
       'ls': ((13, 5.0, 40),)},
 'p': {'lag': 0,
       'x0': 36,
       'xper': 5.6,
       'grp': ((4, 13), (5, 6, 7, 0), (1, 2, 3, 12), (8, 9, 10, 11)),
       'a': ((3, 6, 25), (0, 5.44, 35)),
       'w0': 65,
       'wper': 4.88,
       'ag': 0,
       'ls': ((40, 5.47, None),),
       'wts': (7, 9, 9, 9, 9, 9, 5, 11, 9, 11, 7, 11, 7, 11, 11, 11)},
 'n': {'lag': 1,
       'grp': ((4, 5, 6, 7), (0, 1, 2, 3), (12, 13, 8, 9, 10, 11)),
       'a': ((0, 6, 30), (3, 6, 30), (0, 6.15, 30), (0, 5.4, 35)),
       'ag': 1,
       'ls': ((77, 5.51, None), (69, 9.04, None), (80, 6.83, None))}}


def _up(v):
    return pltpu.bitcast(v, bf16)


def _quad(x):
    n = len(x) // 2
    return ([r[:n] for r in x[:n]], [r[n:] for r in x[:n]],
            [r[:n] for r in x[n:]], [r[n:] for r in x[n:]])


def _badd(x, y):
    return [[a + b for a, b in zip(r, s)] for r, s in zip(x, y)]


def _bsub(x, y):
    return [[a - b for a, b in zip(r, s)] for r, s in zip(x, y)]


def _lhs_terms(a):
    a11, a12, a21, a22 = _quad(a)
    return [lambda: _badd(a11, a22), lambda: _badd(a21, a22), lambda: a11, lambda: a22,
            lambda: _badd(a11, a12), lambda: _bsub(a21, a11), lambda: _bsub(a12, a22)]


def _rhs_terms(b):
    b11, b12, b21, b22 = _quad(b)
    return [lambda: _badd(b11, b22), lambda: b11, lambda: _bsub(b12, b22), lambda: _bsub(b21, b11),
            lambda: b22, lambda: _badd(b11, b12), lambda: _badd(b21, b22)]


def _combos(x, terms, emit):
    for o, fo in enumerate(terms(x)):
        y = fo()
        for i, fi in enumerate(terms(y)):
            emit(o * 7 + i, fi()[0][0])


_LHS_SPEC = (((0, 0), (1, 1), 1), ((1, 0), (1, 1), 1), ((0, 0), None, 0), ((1, 1), None, 0),
             ((0, 0), (0, 1), 1), ((1, 0), (0, 0), -1), ((0, 1), (1, 1), -1))
_RHS_SPEC = (((0, 0), (1, 1), 1), ((0, 0), None, 0), ((0, 1), (1, 1), -1), ((1, 0), (0, 0), -1),
             ((1, 1), None, 0), ((0, 0), (0, 1), 1), ((1, 0), (1, 1), 1))


def _outer_term(load, spec, o):
    p, q, sign = spec[o]
    out = []
    for y in range(2):
        row = []
        for z in range(2):
            v = load(2 * p[0] + y, 2 * p[1] + z)
            if sign:
                w = load(2 * q[0] + y, 2 * q[1] + z)
                v = v + w if sign > 0 else v - w
            row.append(v)
        out.append(row)
    return out


def _inner_terms(y, terms, o, emit):
    for i, fi in enumerate(terms(y)):
        emit(o * 7 + i, fi()[0][0])


def _lhs_ext(e):
    n = len(e) // 2
    return {0: e[:n], 1: e[n:], 2: e[:n], 5: [y - x for x, y in zip(e[:n], e[n:])]}


def _rhs_ext(e):
    n = len(e) // 2
    return {0: e[:n], 1: e[:n], 2: e[n:], 5: [x + y for x, y in zip(e[:n], e[n:])]}


def _ext_combos(e, fn, emit):
    for oi, o in enumerate(AUG):
        d = fn(fn(e)[o])
        for ii, i in enumerate(AUG):
            emit(oi * 4 + ii, d[i][0])


def _spread(weights, span, n):
    total, acc, out = sum(weights), 0.0, []
    for k, w in enumerate(weights):
        lo, acc = acc, acc + w * n / total
        count = round(acc) - round(lo)
        out += [k * span + i * span // count for i in range(count)]
    return out


def _adv(gen, n):
    for _ in range(n):
        try:
            next(gen)
        except StopIteration:
            return


def _ld(ref, idx):
    n = ref.shape[-2] // 2
    return jnp.concatenate([ref[idx, :n, :], ref[idx, n:, :]], axis=0)


class _Temps:
    def __init__(self, ref):
        self.ref = ref
        self.n = 0

    def put(self, v):
        i = self.n % self.ref.shape[0]
        self.n += 1
        self.ref[i] = v
        return i

    def get(self, i):
        return _ld(self.ref, i)


def _recombine(prod, fin, ti, to, spill_last=False):
    def inner(o, sink):
        a = ti.put(prod(o, 0))
        b = ti.put(prod(o, 1))
        c = ti.put(prod(o, 2))
        sink(1, 1, ti.get(a) - ti.get(b) + ti.get(c) + prod(o, 5))
        if spill_last:
            m3 = prod(o, 3)
            m4 = prod(o, 4)
            sink(1, 0, ti.get(b) + m3)
            sink(0, 1, ti.get(c) + m4)
            d = ti.put(ti.get(a) + m3 - m4)
            sink(0, 0, ti.get(d) + prod(o, 6))
            return
        m3 = prod(o, 3)
        m4 = prod(o, 4)
        m6 = prod(o, 6)
        sink(1, 0, ti.get(b) + m3)
        sink(0, 1, ti.get(c) + m4)
        sink(0, 0, ti.get(a) + m3 - m4 + m6)

    m = {}
    for o in (0, 1, 2):
        def keep(y, z, v, o=o):
            m[o, y, z] = to.put(v)
        inner(o, keep)
        yield

    def s5(y, z, v):
        fin(2 + y, 2 + z, to.get(m[0, y, z]) - to.get(m[1, y, z]) + to.get(m[2, y, z]) + v)
    inner(5, s5)
    yield

    def s3(y, z, v):
        fin(2 + y, z, to.get(m[1, y, z]) + v)
        m[3, y, z] = to.put(to.get(m[0, y, z]) + v)
    inner(3, s3)
    yield

    def s4(y, z, v):
        fin(y, 2 + z, to.get(m[2, y, z]) + v)
        m[3, y, z] = to.put(to.get(m[3, y, z]) - v)
    inner(4, s4)
    yield

    def s6(y, z, v):
        fin(y, z, to.get(m[3, y, z]) + v)
    inner(6, s6)
    yield


def _kernel(xt_hbm, wqkv_hbm, wo_hbm, wg_hbm, wu_hbm, wdt_hbm, out_hbm,
            xin, xa, xb, ost, raw, wcb, web, wdcb, wcb2, web2, wdcb2, xn2,
            wq_raw, wo_raw, wtmp, wqb, wob, xnb, qkv, ob, acb, aeb, gs, hs, hcb, acc,
            tin, tout, tin2, tout2, ktail, zero,
            sem_x, sem_w, sem_c, sem_o):
    wq, wo, wc, we, wdc, xn, o32, ac, ae, hc, raw32, xin32, wc2, we2, wdc2 = [
        r.bitcast(u32) for r in (wqb, wob, wcb, web, wdcb, xnb, ob, acb, aeb, hcb, raw, xin,
                                 wcb2, web2, wdcb2)]

    def x_copy(q):
        return pltpu.make_async_copy(
            xt_hbm.at[:, pl.ds(pl.multiple_of(q * 16, 16), 16), :], xin.at[q, 0:NTR], sem_x.at[q])

    def weight_copy(j, m):
        rows = pl.ds(pl.multiple_of(j * 32, 32), 32)
        return pltpu.make_async_copy((wg_hbm, wu_hbm, wdt_hbm)[m].at[:, rows, :],
                                     raw.at[j, pl.ds(m * NTR, NTR)], sem_c.at[j, m])

    def chunk_copies(j):
        return [weight_copy(j, m) for m in range(3)]

    def out_copy(q, h):
        rows = pl.ds(h * 2 * MB, 2 * MB)
        return pltpu.make_async_copy(
            ost.at[q, rows, :], out_hbm.at[rows, pl.ds(pl.multiple_of(q * 256, 256), 256)],
            sem_o.at[q, h])

    k_order = (4, 0, 1, 2, 3)
    wq_copies = [pltpu.make_async_copy(wqkv_hbm.at[k * 128:min(k * 128 + 128, D)],
                                       wq_raw.at[k * 128:min(k * 128 + 128, D)], sem_w.at[k])
                 for k in k_order]
    wo_copy = pltpu.make_async_copy(wo_hbm, wo_raw, sem_w.at[5])
    first = wq_copies[:OPT["xpos"]] + [x_copy(0)] + wq_copies[OPT["xpos"]:]
    for cp in first:
        cp.start()
    zero[0] = 0
    never = zero[0] != 0

    def held(v, z):
        if z is None:
            return v
        return jnp.where(never, pltpu.bitcast(z, v.dtype), v)

    def raw_pair(j, tr, cp, z):
        v = [_up(held(raw32[j, tr + k, cp * 8:cp * 8 + 8, :], z)).astype(f32) for k in range(2)]
        return [jnp.concatenate([v[0][h:h + 8], v[1][h:h + 8]], axis=0) for h in (0, 8)]

    def prep_strip(j, tr, step, spec, terms, path, emit):
        live = {}
        for o in path:
            used = [q for q in spec[o][:2] if q is not None]
            live = {q: live[q] for q in used if q in live}
            for q in used:
                if q not in live:
                    z = yield
                    live[q] = [raw_pair(j, tr + (2 * q[0] + y) * step, q[1], z) for y in range(2)]
            y = _outer_term(lambda r, c: live[r // 2, c // 2][r % 2][c % 2], spec, o)
            _inner_terms(y, terms, o, emit)

    def prep_gu(j, dst, m, s):
        base = m * (49 * 128) + s * 16

        def emit(i, v):
            dst[pl.ds(base + i * 128, 16), :] = v.astype(bf16)
        return prep_strip(j, m * NTR + 2 * s, 16, _RHS_SPEC, _rhs_terms,
                          (1, 0, 4, 2, 5, 3, 6), emit)

    def prep_ext(j, dst, m, s):
        z = yield
        tr = m * NTR + 64 + 2 * s

        def emit(i, v):
            dst[m * 16 + i, pl.ds(s * 16, 16), :] = v.astype(bf16)
        _ext_combos(raw_pair(j, tr, 0, z) + raw_pair(j, tr, 1, z), _rhs_ext, emit)

    def prep_down(j, dst, s):
        def emit(i, v):
            dst[pl.ds(s * 16 + i * MB, 16), :] = v.astype(bf16)
        return prep_strip(j, 2 * NTR + 2 * s, MB // 8, _LHS_SPEC, _lhs_terms,
                          (2, 0, 3, 6, 4, 5, 1), emit)

    def prep_chunk(j, dst):
        for m in range(2):
            for s in range(8):
                yield from prep_gu(j, dst[0], m, s)
            for s in range(4):
                yield from prep_ext(j, dst[1], m, s)
        for s in range(9):
            yield from prep_down(j, dst[2], s)

    def feed(gen, z, n):
        for _ in range(n):
            try:
                gen.send(z)
            except StopIteration:
                return

    class Pace:
        def __init__(self):
            self.tok = 0
            self.plan = []
            self.due = []

        def add(self, gen, t0, period, lat=None, gated=True):
            next(gen)
            when = [self.tok + int(t0 + k * period) for k in range(1000)]
            self.plan.append((gen, when, lat, gated))

        def step(self, z):
            for gen, when, lat, gated in self.plan:
                for _ in range(when.count(self.tok)):
                    try:
                        v = gen.send(z if gated else None)
                    except StopIteration:
                        break
                    if v is not None and lat is not None:
                        self.due.append((self.tok + lat, v))
            self.tok += 1

        def tokens(self, r, n):
            for k in range(n):
                self.step(r[k * 16:k * 16 + 8])

        def gate(self, v):
            now = [x for t, x in self.due if t <= self.tok]
            self.due = [(t, x) for t, x in self.due if t > self.tok]
            if not now:
                return v
            head = jnp.where(never, pltpu.bitcast(tree(now), u32), v[0:8])
            return jnp.concatenate([head, v[8:]], axis=0)

        def drain(self):
            for gen, *_ in self.plan:
                feed(gen, None, 1000)

    def tree(vals):
        while len(vals) > 1:
            vals = [a + b for a, b in zip(vals[::2], vals[1::2])] + vals[len(vals) & ~1:]
        return vals[0]

    def norm_slab(row, emit):
        def rows(k, lo, hi):
            return [row(k, r) for r in range(lo // 8, hi // 8)]

        def mean(vals):
            t = tree([sum(vals[k + 4::4], vals[k]) for k in range(4)])
            t = jnp.sum(t, axis=0, keepdims=True) * (1.0 / D)
            return jnp.broadcast_to(t, (8, 128))
        z = yield
        x = rows(0, 0, D)
        mu = mean([held(v, z) for v in x[:4]] + x[4:])
        m = held(mu, (yield))
        rs = lax.rsqrt(mean([(v - m) * (v - m) for v in rows(1, 0, D)]) + EPS)
        end = None
        for k in (4, 0, 1, 2, 3):
            m = held(mu, (yield end))
            y = jnp.concatenate(
                [(v - m) * rs for v in rows(2, k * 128, min((k + 1) * 128, D))], axis=0).T
            emit(k, y)
            end = y[120:128] if k < 4 else jnp.concatenate([y[120:128]] * 2, axis=1)
        yield end

    def alias(p, n):
        return [jnp.clip(p + k * zero[0], 0, n - 1) for k in range(3)]

    def slab_rows(src, p):
        q = alias(p, NSLAB)
        return lambda k, r: src[q[k], r * 8:r * 8 + 8, :]

    def flush(gen):
        return tree([v for v in gen if v is not None])

    def ln1(p, b):
        def emit(k, y):
            xnb[b, k, :, 0:y.shape[1]] = y.astype(bf16)
        return norm_slab(slab_rows(xa, p), emit)

    def widen(q):
        for r in range(NTR):
            if r % 4 == 0:
                z = yield
            v = _up(held(xin32[q, r], z)).astype(f32)
            for b in range(2):
                xa[2 * q + b, r * 8:r * 8 + 8, :] = v[b * 8:b * 8 + 8]

    def qkv_proj(b, pace, groups):
        scale = DH ** -0.5 * LOG2E
        for grp in groups:
            for n in grp:
                if n == 13:
                    ktail[...] = lax.dot_general(
                        _up(wq[4, n * 64:n * 64 + 32, :]), _up(xn[b, 4]), NT,
                        preferred_element_type=f32)
                else:
                    qkv[b, n, HALO:HALO + 128, :] = lax.dot_general(
                        _up(xn[b, 4]), _up(wq[4, n * 64:(n + 1) * 64, :]), NT,
                        preferred_element_type=f32)
            for n in grp:
                rows = slice(n * 64, n * 64 + (32 if n == 13 else 64))
                x = jnp.concatenate(
                    [_up(pace.gate(xn[b, 0]))] + [_up(xn[b, k]) for k in range(1, 4)], axis=1)
                w = jnp.concatenate([_up(wq[k, rows, :]) for k in range(4)], axis=1)
                if n == 13:
                    r = lax.dot_general(w, x, NT, preferred_element_type=f32)
                    r = r + jnp.concatenate([ktail[0:32, :], ktail[32:64, :]], axis=0)
                    qkv[b, n, HALO:HALO + 128, 0:64] = (r * scale).T
                    pace.tokens(r, 4)
                    continue
                r = lax.dot_general(x, w, NT, preferred_element_type=f32)
                r = r + jnp.concatenate([qkv[b, n, HALO:HALO + 64, :],
                                         qkv[b, n, HALO + 64:HALO + 128, :]], axis=0)
                if n in (4, 5, 6, 7):
                    r = r * scale
                qkv[b, n, HALO:HALO + 128, :] = r
                pace.tokens(r, 7)

    def halo(b):
        for n in range(4, 14):
            qkv[b, n, 0:HALO, :] = qkv[1 - b, n, 128:128 + HALO, :]

    def attend(b, row0, lag=0):
        qs, ks, vs = (0, 1, 2, 3, 12), (4, 5, 6, 7, 13), (8, 9, 10, 11, 12)

        def scores(s, z):
            r = HALO + s * 8
            q = [held(qkv[b, n, r:r + 8, :], z) for n in qs]
            logit = []
            for w in range(WIN):
                rw = r - DIL * w
                part = tree([q[c] * qkv[b, ks[c], rw:rw + 8, :] for c in range(5)])
                part = part + pltpu.roll(part, 64, 1)
                part = part + pltpu.roll(part, 32, 1)
                if row0 is not None and s * 8 < DIL * w:
                    pos = row0 + s * 8 + lax.broadcasted_iota(jnp.int32, (8, 128), 0)
                    part = jnp.where(pos >= DIL * w, part, -1e9 * LOG2E)
                logit.append(part)
            return logit

        def values(s, logit, z):
            r = HALO + s * 8
            mx = logit
            while len(mx) > 1:
                mx = [jnp.maximum(a, c) for a, c in zip(mx[::2], mx[1::2])]
            top = held(mx[0], z)
            e = [jnp.exp2(l - top) for l in logit]
            inv = 1.0 / tree(e)
            outs = []
            for c in range(5):
                o = e[0] * qkv[b, vs[c], r:r + 8, :]
                for w in range(1, WIN):
                    rw = r - DIL * w
                    o = o + e[w] * qkv[b, vs[c], rw:rw + 8, :]
                o = o * inv
                outs.append(o)
                ob[b, c, s * 8:(s + 1) * 8, :] = o.astype(bf16)
            return tree(outs)

        v, pending = None, []
        for s in range(16 + lag):
            z = yield v
            if s < 16:
                pending.append(scores(s, z))
            if s >= lag:
                v = values(s - lag, pending.pop(0), z if lag else None)
        yield v

    def out_proj(p, b, pace):
        h = MB // 2
        for m in range(4):
            xb[p, m * MB:(m + 1) * MB, :] = xa[p, m * MB:(m + 1) * MB, :] + lax.dot_general(
                _up(wo[4, m * h:(m + 1) * h, :]), _up(o32[b, 4]), NT, preferred_element_type=f32)
        rhs = jnp.concatenate([_up(o32[b, c]) for c in range(4)], axis=1)
        for m in range(4):
            rows = slice(m * h, (m + 1) * h)
            lhs = jnp.concatenate(
                [_up(pace.gate(wo[0, rows, :]))] + [_up(wo[c, rows, :]) for c in range(1, 4)],
                axis=1)
            r = lax.dot_general(lhs, rhs, NT, preferred_element_type=f32)
            r = r + jnp.concatenate([xb[p, m * MB:m * MB + h, :],
                                     xb[p, m * MB + h:(m + 1) * MB, :]], axis=0)
            xb[p, m * MB:(m + 1) * MB, :] = r
            pace.tokens(r, 8)

    def ffn_norm_slab(p, r):
        def emit(k, y):
            xn2[r * 6 + k, :, 0:y.shape[1]] = y
        return norm_slab(slab_rows(xb, p), emit)

    def ffn_norm(t):
        for r in range(4):
            yield from ffn_norm_slab(t * 4 + r, r)

    def strips(load, spec, terms, o, dst):
        for s in range(8):
            z = yield
            rows = slice(s * 16, (s + 1) * 16)

            def ld(r, c):
                v = load(r, c, rows)
                if (r // 2, c // 2) == spec[o][0]:
                    v = jnp.concatenate([held(v[0:8], z), held(v[8:16], z)], axis=0)
                return v

            def emit(i, v):
                dst[i, rows, :] = v.astype(bf16)
            _inner_terms(_outer_term(ld, spec, o), terms, o, emit)

    def lhs_strips(o):
        yield from strips(lambda r, k, rows: xn2[r * 6 + k, rows, :],
                          _LHS_SPEC, _lhs_terms, o, acb)
        if o in AUG:
            for s in range(2):
                z = yield
                rows = slice(s * 64, (s + 1) * 64)
                d = _lhs_ext(_lhs_ext([xn2[r * 6 + 4, rows, 0:64] for r in range(4)])[o])
                for ii, i in enumerate(AUG):
                    aeb[AUG.index(o) * 4 + ii, rows, 0:64] = d[i][0].astype(bf16)

    def ffn_combos():
        for s in range(8):
            rows = slice(s * 16, (s + 1) * 16)
            a = [[xn2[r * 6 + k, rows, :] for k in range(4)] for r in range(4)]

            def emit(i, v, rows=rows):
                acb[i, rows, :] = v.astype(bf16)
            _combos(a, _lhs_terms, emit)
            e = [xn2[r * 6 + 4, rows, 0:64] for r in range(4)]

            def emit_e(i, v, rows=rows):
                aeb[i, rows, 0:64] = v.astype(bf16)
            _ext_combos(e, _lhs_ext, emit_e)

    def attn_run(h, count, o, mask, side=None, late=None, extra=None, head=False):
        if not head:
            flush(ln1(h % NSLAB, 0))
        for k in range(count):
            b = k % 2
            pace = Pace()
            if side is not None:
                when = [w - k * 128 for w in _spread(o["wts"], 16, NPREP)]
                pace.plan.append((side, [min(w, 126) for w in when if 0 <= w < 128], None, True))
            if k + 1 < count:
                pace.add(ln1((h + k + 1) % NSLAB, 1 - b), *o["ls"][k])
            elif late is not None:
                pace.add(late, o["w0"], o["wper"])
            if k == 1 and extra is not None:
                pace.add(extra, 32 + o["x0"], o["xper"])
            if k > 0 or not head:
                row0 = (h % NSLAB) * 128 if k == 1 and mask else None
                pace.add(attend(1 - b, row0, o["lag"]), *o["a"][k], o["ag"])
                if not head:
                    out_proj((h + k - 2) % NSLAB, b, pace)
                halo(b)
            qkv_proj(b, pace, o["grp"])
            pace.plan = [e for e in pace.plan if e[0] is not side]
            pace.drain()
        if side is not None:
            feed(side, None, 1000)

    def wq_prep(k):
        w = 128 if k < 4 else 64
        for c0 in range(0, 3 * D, 128):
            c1 = min(c0 + 128, 3 * D)
            wtmp[k, c0:c1, 0:w] = wq_raw[k * 128:k * 128 + w, c0:c1].astype(f32).T
        for part in OPT["parts"]:
            for d in range(DH):
                if d < 16:
                    row = part * 512 + d * 32
                else:
                    row = (1536, 1664, 1600)[part] + (d - 16) * 32
                wqb[k, row:row + 32, 0:w] = wtmp[
                    k, pl.ds(part * D + d, H, stride=DH), 0:w].astype(bf16)

    def wo_prep():
        for n in range(5):
            w = 128 if n < 4 else 64
            wtmp[n, 0:D, 0:w] = wo_raw[:, n * 128:n * 128 + w].astype(f32)
        for n in range(5):
            w = 128 if n < 4 else 64
            for c in range(5):
                z = yield
                rows = [held(wtmp[n, pl.ds(4 * c + g + k * 8 * DH, 8, stride=DH), :], z)[:, 0:w]
                        for g in range(4 if c < 4 else 2) for k in range(4)]
                if c == 4:
                    rows = [jnp.zeros((64, w), f32)] + rows
                wob[c, n * 128:n * 128 + w, :] = jnp.concatenate(rows, axis=0).T.astype(bf16)

    def head_late():
        for cp in (wo_copy, x_copy(1)):
            cp.wait()
        for cp in [x_copy(2)] + chunk_copies(1):
            cp.start()
        yield from wo_prep()
        yield from widen(1)

    wqb[4, :, 64:128] = jnp.zeros((3 * D, 64), bf16)
    qkv[:, 13] = jnp.zeros((2, HALO + 128, 128), f32)
    xnb[:, 4, :, 64:128] = jnp.zeros((2, 128, 64), bf16)
    for n in range(4, 13):
        qkv[0, n, 0:HALO, :] = jnp.zeros((HALO, 128), f32)
    todo = list(k_order)
    for n, cp in enumerate(first):
        cp.wait()
        if n == OPT["dma"][0]:
            wo_copy.start()
        if n == OPT["dma"][1]:
            for c in [x_copy(1)] + chunk_copies(0):
                c.start()
        if n == OPT["xpos"]:
            feed(widen(0), None, 1000)
            flush(ln1(0, 0))
        else:
            wq_prep(todo.pop(0))
    attn_run(0, 2, OPT["h"], True, late=head_late(), head=True)

    @pl.loop(0, 7)
    def _(i):
        for cp in chunk_copies(i):
            cp.wait()

        @pl.when(i + 2 < NSLAB // 2)
        def _():
            x_copy(i + 2).wait()

        @pl.when(i + 3 < NSLAB // 2)
        def _():
            x_copy(i + 3).start()
        for cp in chunk_copies(i + 2):
            cp.start()
        side = prep_chunk(i, [r.at[i] for r in (wcb, web, wdcb)])
        next(side)
        r = jnp.clip(i - 2, 0, 3)
        attn_run(2 * i + 2, 2, OPT["p"], False, side, widen(jnp.minimum(i + 2, NSLAB // 2 - 1)),
                 ffn_norm_slab(r, r))

    for cp in chunk_copies(7) + chunk_copies(8):
        cp.wait()
    ffn_combos()

    def ffn_group(t, g, last, emit=None):
        ti = _Temps(tin)
        to = _Temps(tout)
        pace = Pace()
        o_ = OPT["fb" if last else "fa"]

        def weights(c):
            if last and c > 0:
                return [r.at[c - 1] for r in (wc2, we2, wdc2)]
            return [r.at[g * 3 + c] for r in (wc, we, wdc)]

        def proj(c, m):
            w, w_ext, _ = weights(c)

            def prod(o, i):
                r = (m * 49 + o * 7 + i) * 64
                p = jnp.dot(_up(ac[o * 7 + i]), _up(w[r:r + 64, :]),
                            preferred_element_type=f32)
                pace.step(p[0:8])
                if o in AUG and i in AUG:
                    q = AUG.index(o) * 4 + AUG.index(i)
                    e = jnp.dot(_up(ae[q, :, 0:64]), _up(w_ext[m * 16 + q]),
                                preferred_element_type=f32)
                    pace.step(e[0:8])
                    p = p + e
                return p
            return prod

        def gate(c):
            def fin(r, cc, v):
                gs[(c % 2) * 16 + r * 4 + cc] = v
            return _recombine(proj(c, 0), fin, ti, to)

        def upgate(c):
            def fin(r, cc, v):
                hs[c, r * 4 + cc] = _ld(gs, (c % 2) * 16 + r * 4 + cc) * v
            yield from _recombine(proj(c, 1), fin, ti, to, last)
            pace.add(hidden_paced(c), *o_["h"][c])

        hgen, hdone = {}, {}

        def hidden(c):
            for o in ORDER:
                yield from strips(lambda cc, r, rows: hs[c, r * 4 + cc, rows, :],
                                  _RHS_SPEC, _rhs_terms, o, hcb.at[c])

        def hidden_paced(c):
            hgen[c], hdone[c] = hidden(c), 0
            next(hgen[c])
            while True:
                z = yield
                need(c, min(hdone[c] + 1, 56), z)

        def need(c, n, z=None):
            feed(hgen[c], z, n - hdone[c])
            hdone[c] = max(hdone[c], n)

        def dprod(cs, i):
            p = None
            for c in cs:
                need(c, 8 * (ORDER.index(i // 7) + 1))
                r = i * (MB // 2)
                q = lax.dot_general(_up(weights(c)[2][r:r + MB // 2, :]), _up(hc[c, i]), NT,
                                    preferred_element_type=f32)
                pace.step(q[0:8])
                p = q if p is None else p + q
            return p

        def down(cs, reset):
            for i in [o * 7 + k for o in ORDER for k in range(7)]:
                a = _ld(acc, i)
                if reset:
                    a = jnp.where(g == 0, 0.0, a)
                acc[i] = a + dprod(cs, i)
                yield

        def down_final(cs):
            def fin(mb, r, v):
                rows = slice(mb * MB, (mb + 1) * MB)
                y = xb[t * 4 + r, rows, :] + v
                xa[t * 4 + r, rows, :] = y
                ost[t * 2 + r // 2, rows, (r % 2) * 128:(r % 2) * 128 + 128] = y.astype(bf16)
            return _recombine(lambda o, i: _ld(acc, o * 7 + i) + dprod(cs, o * 7 + i),
                              fin, _Temps(tin2), _Temps(tout2))

        if last:
            norm = ffn_norm((t + 1) % NTILE)
            pace.add(norm, o_["n0"], o_["nper"])
        else:
            late = prep_chunk(7 + g, [r.at[g] for r in (wcb2, web2, wdcb2)])
            next(late)
            pace.plan.append((late, _spread(o_["wts"], 30, NPREP), None, True))
        for gen in (gate(0), upgate(0), gate(1)):
            _adv(gen, 100)
        d0 = down((0,), not last)
        queue = []

        def lhs_queue():
            while True:
                z = yield
                if queue:
                    try:
                        queue[0].send(z)
                    except StopIteration:
                        queue.pop(0)
        for gen, plan in ((upgate(1), "u1"), (gate(2), "g2"), (upgate(2), "u2")):
            if last and plan == "u2":
                feed(norm, None, 1000)
                pace.add(lhs_queue(), o_["l0"], o_["lper"])
            for k, n in enumerate(o_[plan]):
                _adv(gen, 1)
                if last and plan == "u2":
                    queue.append(lhs_strips(ORDER[k]))
                    next(queue[-1])
                _adv(d0, n)
            _adv(gen, 100)
        _adv(d0, 100)
        if last:
            gen = down_final((1, 2))
            _adv(gen, 3)
            for q, h in ((1, 1), (0, 1), (1, 0), (0, 0)):
                _adv(gen, 1)
                pl.when(emit)(out_copy(t * 2 + q, h).start)
        else:
            _adv(down((1, 2), False), 100)
            feed(late, None, 1000)
        for gen in queue:
            feed(gen, None, 1000)

    @pl.loop(0, 2 * NTILE)
    def _(tile):
        t = tile % NTILE

        @pl.loop(0, 2)
        def _(g):
            ffn_group(t, g, False)
        ffn_group(t, 2, True, tile >= NTILE)

        @pl.when(tile < NTILE)
        def _():
            attn_run(4 * t + NSLAB, 4, OPT["n"], True)

        @pl.when(tile == NTILE - 1)
        def _():
            out_proj(NSLAB - 2, 0, Pace())
            flush(attend(1, None))
            out_proj(NSLAB - 1, 1, Pace())

    for p in range(NSLAB):
        out_copy(p // 2, p % 2).wait()


def _tiles(w):
    n = w.shape[1]
    return w.reshape(NTR, 8, n // 128, 128).transpose(0, 2, 1, 3).reshape(NTR, n // 16, 128)


@jax.jit
def pallas_interleave_layers__sliding_local_dilated__glu_gated_bilinear__prompt_kernel(
    A_x: jax.Array,
    A_wqkv: jax.Array,
    A_wo: jax.Array,
    B_x: jax.Array,
    B_w_gate: jax.Array,
    B_w_up: jax.Array,
    B_w_down: jax.Array,
):
    del B_x
    vm = pltpu.VMEM
    hbm = pl.BlockSpec(memory_space=pl.ANY)
    out_t = pl.pallas_call(
        _kernel,
        in_specs=[hbm] * 6,
        out_specs=hbm,
        out_shape=jax.ShapeDtypeStruct((D, S), bf16),
        scratch_shapes=[
            vm((NSLAB // 2, 96, 16, 128), bf16),
            vm((NSLAB, 768, 128), f32),
            vm((NSLAB, 768, 128), f32),
            vm((NSLAB // 2, 768, 256), bf16),
            vm((NCHUNK, 224, 32, 128), bf16),
            vm((7, WC_ROWS, 128), bf16),
            vm((7, 32, 64, 128), bf16),
            vm((7, WD_ROWS, 128), bf16),
            vm((2, WC_ROWS, 128), bf16),
            vm((2, 32, 64, 128), bf16),
            vm((2, WD_ROWS, 128), bf16),
            vm((24, 128, 128), f32),
            vm((D, 3 * D), bf16),
            vm((D, D), bf16),
            vm((5, 3 * D, 128), f32),
            vm((5, 3 * D, 128), bf16),
            vm((5, D, 128), bf16),
            vm((2, 5, 128, 128), bf16),
            vm((2, 14, HALO + 128, 128), f32),
            vm((2, 5, 128, 128), bf16),
            vm((49, 128, 128), bf16),
            vm((16, 128, 128), bf16),
            vm((32, 128, 128), f32),
            vm((3, 16, 128, 128), f32),
            vm((3, 49, 128, 128), bf16),
            vm((49, MB, 128), f32),
            vm((12, 128, 128), f32),
            vm((40, 128, 128), f32),
            vm((12, MB, 128), f32),
            vm((20, MB, 128), f32),
            vm((64, 128), f32),
            pltpu.SMEM((1,), jnp.int32),
            pltpu.SemaphoreType.DMA((NSLAB // 2,)),
            pltpu.SemaphoreType.DMA((6,)),
            pltpu.SemaphoreType.DMA((NCHUNK, 3)),
            pltpu.SemaphoreType.DMA((NSLAB // 2, 2)),
        ],
        compiler_params=pltpu.CompilerParams(vmem_limit_bytes=120 * 1024 * 1024,
                                             disable_bounds_checks=True,
                                             disable_semaphore_checks=True),
    )(_tiles(A_x[0].T), A_wqkv, A_wo, _tiles(B_w_gate), _tiles(B_w_up), _tiles(B_w_down.T))
    return out_t.T[None]
```

```python
import math

import jax
import jax.numpy as jnp
from jax import lax
import jax.experimental.pallas as pl
import jax.experimental.pallas.tpu as pltpu

f32 = jnp.float32
bf16 = jnp.bfloat16
u32 = jnp.uint32

S, D, F = 2048, 576, 4608
H, DH, WIN, DIL = 32, 18, 8, 2
EPS = 1e-5
LOG2E = math.log2(math.e)
NSLAB = S // 128
TILE = 512
NTILE = S // TILE
FC = 512
NCHUNK = F // FC
MB = D // 4
HALO = 16
NPREP = 158
NTR = D // 8
WC_ROWS = 800 * 16
WD_ROWS = 448 * 16
NT = (((1,), (1,)), ((), ()))
ORDER = (0, 1, 2, 5, 3, 4, 6)
SUMS = (0, 1, 4, 5, 6)
AUG = (0, 1, 2, 5)

OPT = {'dma': (0, 2),
 'xpos': 2,
 'parts': (1, 0, 2),
 'fa': {'wts': (3, 1, 2, 1, 0, 1, 2, 1, 1, 2, 0, 0, 0, 1, 0, 3, 3, 4),
        'h': ((0, 0.7), (0, 1), (0, 1)),
        'u1': (0, 0, 0, 4, 5, 4, 6),
        'g2': (4, 0, 0, 0, 0, 0, 0),
        'u2': (0, 0, 0, 0, 4, 4, 4)},
 'fb': {'h': ((0, 1), (0, 0.59), (0, 1)),
        'n0': 0,
        'nper': 1.4,
        'l0': 0,
        'lper': 3.22,
        'u1': (0, 0, 0, 0, 4, 4, 6),
        'g2': (4, 0, 0, 0, 0, 0, 0),
        'u2': (0, 0, 0, 0, 4, 4, 4)},
 'h': {'lag': 0,
       'grp': ((4, 5, 6, 7), (0, 1, 2, 3), (12, 13, 8, 9, 10, 11)),
       'a': ((0, 5, 35), (0, 3.65, 35)),
       'w0': 22,
       'wper': 2.8,
       'ag': 1,
       'ls': ((13, 5.0, 40),)},
 'p': {'lag': 0,
       'sk': 1,
       's0': 4,
       'sper': 5.5,
       'x0': 36,
       'xper': 5.6,
       'grp': ((4, 13), (5, 6, 7, 0), (1, 2, 3, 12), (8, 9, 10, 11)),
       'a': ((3, 6, 25), (0, 5.44, 35)),
       'w0': 65,
       'wper': 4.88,
       'ag': 0,
       'ls': ((40, 5.47, None),),
       'wts': (7, 9, 9, 9, 11, 7, 5, 5, 9, 11, 7, 11, 15, 7, 11, 11)},
 'n': {'seq': (5, 6, 2, 0, 4, 1, 3),
       'lag': 1,
       'grp': ((4, 5, 6, 7), (0, 1, 2, 3), (12, 13, 8, 9, 10, 11)),
       'a': ((0, 6, 35), (0, 6, 35), (0, 6.84, 35), (0, 6, 35)),
       'ag': 1,
       'ls': ((77, 7.71, None), (69, 9.04, None), (80, 6.83, None))}}


def _up(v):
    return pltpu.bitcast(v, bf16)


def _quad(x):
    n = len(x) // 2
    return ([r[:n] for r in x[:n]], [r[n:] for r in x[:n]],
            [r[:n] for r in x[n:]], [r[n:] for r in x[n:]])


def _badd(x, y):
    return [[a + b for a, b in zip(r, s)] for r, s in zip(x, y)]


def _bsub(x, y):
    return [[a - b for a, b in zip(r, s)] for r, s in zip(x, y)]


def _lhs_terms(a):
    a11, a12, a21, a22 = _quad(a)
    return [lambda: _badd(a11, a22), lambda: _badd(a21, a22), lambda: a11, lambda: a22,
            lambda: _badd(a11, a12), lambda: _bsub(a21, a11), lambda: _bsub(a12, a22)]


def _rhs_terms(b):
    b11, b12, b21, b22 = _quad(b)
    return [lambda: _badd(b11, b22), lambda: b11, lambda: _bsub(b12, b22), lambda: _bsub(b21, b11),
            lambda: b22, lambda: _badd(b11, b12), lambda: _badd(b21, b22)]


def _combos(x, terms, emit):
    for o, fo in enumerate(terms(x)):
        y = fo()
        for i, fi in enumerate(terms(y)):
            emit(o * 7 + i, fi()[0][0])


_LHS_SPEC = (((0, 0), (1, 1), 1), ((1, 0), (1, 1), 1), ((0, 0), None, 0), ((1, 1), None, 0),
             ((0, 0), (0, 1), 1), ((1, 0), (0, 0), -1), ((0, 1), (1, 1), -1))
_RHS_SPEC = (((0, 0), (1, 1), 1), ((0, 0), None, 0), ((0, 1), (1, 1), -1), ((1, 0), (0, 0), -1),
             ((1, 1), None, 0), ((0, 0), (0, 1), 1), ((1, 0), (1, 1), 1))


def _outer_term(load, spec, o):
    p, q, sign = spec[o]
    out = []
    for y in range(2):
        row = []
        for z in range(2):
            v = load(2 * p[0] + y, 2 * p[1] + z)
            if sign:
                w = load(2 * q[0] + y, 2 * q[1] + z)
                v = v + w if sign > 0 else v - w
            row.append(v)
        out.append(row)
    return out


def _inner_terms(y, terms, o, emit):
    for i, fi in enumerate(terms(y)):
        emit(o * 7 + i, fi()[0][0])


def _lhs_ext(e):
    n = len(e) // 2
    return {0: e[:n], 1: e[n:], 2: e[:n], 5: [y - x for x, y in zip(e[:n], e[n:])]}


def _rhs_ext(e):
    n = len(e) // 2
    return {0: e[:n], 1: e[:n], 2: e[n:], 5: [x + y for x, y in zip(e[:n], e[n:])]}


def _ext_combos(e, fn, emit):
    for oi, o in enumerate(AUG):
        d = fn(fn(e)[o])
        for ii, i in enumerate(AUG):
            emit(oi * 4 + ii, d[i][0])


def _spread(weights, span, n):
    total, acc, out = sum(weights), 0.0, []
    for k, w in enumerate(weights):
        lo, acc = acc, acc + w * n / total
        count = round(acc) - round(lo)
        out += [k * span + i * span // count for i in range(count)]
    return out


def _adv(gen, n):
    for _ in range(n):
        try:
            next(gen)
        except StopIteration:
            return


def _ld(ref, idx):
    n = ref.shape[-2] // 2
    return jnp.concatenate([ref[idx, :n, :], ref[idx, n:, :]], axis=0)


class _Temps:
    def __init__(self, ref):
        self.ref = ref
        self.n = 0

    def put(self, v):
        i = self.n % self.ref.shape[0]
        self.n += 1
        self.ref[i] = v
        return i

    def get(self, i):
        return _ld(self.ref, i)


def _combine(prod, sink, ti, spill_last=False):
    a = ti.put(prod(0))
    b = ti.put(prod(1))
    c = ti.put(prod(2))
    sink(1, 1, ti.get(a) - ti.get(b) + ti.get(c) + prod(5))
    if spill_last:
        m3 = prod(3)
        m4 = prod(4)
        sink(1, 0, ti.get(b) + m3)
        sink(0, 1, ti.get(c) + m4)
        d = ti.put(ti.get(a) + m3 - m4)
        sink(0, 0, ti.get(d) + prod(6))
        return
    m3 = prod(3)
    m4 = prod(4)
    m6 = prod(6)
    sink(1, 0, ti.get(b) + m3)
    sink(0, 1, ti.get(c) + m4)
    sink(0, 0, ti.get(a) + m3 - m4 + m6)


def _recombine(prod, fin, ti, to, spill_last=False):
    def inner(o, sink):
        _combine(lambda i: prod(o, i), sink, ti, spill_last)

    m = {}
    for o in (0, 1, 2):
        def keep(y, z, v, o=o):
            m[o, y, z] = to.put(v)
        inner(o, keep)
        yield

    def s5(y, z, v):
        fin(2 + y, 2 + z, to.get(m[0, y, z]) - to.get(m[1, y, z]) + to.get(m[2, y, z]) + v)
    inner(5, s5)
    yield

    def s3(y, z, v):
        fin(2 + y, z, to.get(m[1, y, z]) + v)
        m[3, y, z] = to.put(to.get(m[0, y, z]) + v)
    inner(3, s3)
    yield

    def s4(y, z, v):
        fin(y, 2 + z, to.get(m[2, y, z]) + v)
        m[3, y, z] = to.put(to.get(m[3, y, z]) - v)
    inner(4, s4)
    yield

    def s6(y, z, v):
        fin(y, z, to.get(m[3, y, z]) + v)
    inner(6, s6)
    yield


def _kernel(xt_hbm, wqkv_hbm, wo_hbm, wg_hbm, wu_hbm, wdt_hbm, out_hbm,
            xin, xa, xb, ost, raw, wcb, web, wdcb, wcb2, web2, wdcb2, xn2,
            wq_raw, wo_raw, wtmp, wqb, wob, xnb, qkv, ob, acb, aeb, gs, hs, hcb, acc,
            tin, tout, tin2, tout2, ktail, xsb, wsb, tq, zero,
            sem_x, sem_w, sem_c, sem_o):
    wq, wo, wc, we, wdc, xn, o32, ac, ae, hc, raw32, xin32, wc2, we2, wdc2, xs, ws = [
        r.bitcast(u32) for r in (wqb, wob, wcb, web, wdcb, xnb, ob, acb, aeb, hcb, raw, xin,
                                 wcb2, web2, wdcb2, xsb, wsb)]

    def x_copy(q):
        return pltpu.make_async_copy(
            xt_hbm.at[:, pl.ds(pl.multiple_of(q * 16, 16), 16), :], xin.at[q, 0:NTR], sem_x.at[q])

    def weight_copy(j, m):
        rows = pl.ds(pl.multiple_of(j * 32, 32), 32)
        return pltpu.make_async_copy((wg_hbm, wu_hbm, wdt_hbm)[m].at[:, rows, :],
                                     raw.at[j, pl.ds(m * NTR, NTR)], sem_c.at[j, m])

    def chunk_copies(j):
        return [weight_copy(j, m) for m in range(3)]

    def out_copy(q, h):
        rows = pl.ds(h * 2 * MB, 2 * MB)
        return pltpu.make_async_copy(
            ost.at[q, rows, :], out_hbm.at[rows, pl.ds(pl.multiple_of(q * 256, 256), 256)],
            sem_o.at[q, h])

    k_order = (4, 0, 1, 2, 3)
    wq_copies = [pltpu.make_async_copy(wqkv_hbm.at[k * 128:min(k * 128 + 128, D)],
                                       wq_raw.at[k * 128:min(k * 128 + 128, D)], sem_w.at[k])
                 for k in k_order]
    wo_copy = pltpu.make_async_copy(wo_hbm, wo_raw, sem_w.at[5])
    first = wq_copies[:OPT["xpos"]] + [x_copy(0)] + wq_copies[OPT["xpos"]:]
    for cp in first:
        cp.start()
    zero[0] = 0
    never = zero[0] != 0

    def held(v, z):
        if z is None:
            return v
        return jnp.where(never, pltpu.bitcast(z, v.dtype), v)

    def raw_pair(j, tr, cp, z):
        v = [_up(held(raw32[j, tr + k, cp * 8:cp * 8 + 8, :], z)).astype(f32) for k in range(2)]
        return [jnp.concatenate([v[0][h:h + 8], v[1][h:h + 8]], axis=0) for h in (0, 8)]

    def prep_strip(j, tr, step, spec, terms, path, emit):
        live = {}
        for o in path:
            used = [q for q in spec[o][:2] if q is not None]
            live = {q: live[q] for q in used if q in live}
            for q in used:
                if q not in live:
                    z = yield
                    live[q] = [raw_pair(j, tr + (2 * q[0] + y) * step, q[1], z) for y in range(2)]
            y = _outer_term(lambda r, c: live[r // 2, c // 2][r % 2][c % 2], spec, o)
            _inner_terms(y, terms, o, emit)

    def prep_gu(j, dst, m, s):
        base = m * (49 * 128) + s * 16

        def emit(i, v):
            dst[pl.ds(base + i * 128, 16), :] = v.astype(bf16)
        return prep_strip(j, m * NTR + 2 * s, 16, _RHS_SPEC, _rhs_terms,
                          (1, 0, 4, 2, 5, 3, 6), emit)

    def prep_ext(j, dst, m, s):
        z = yield
        tr = m * NTR + 64 + 2 * s

        def emit(i, v):
            dst[m * 16 + i, pl.ds(s * 16, 16), :] = v.astype(bf16)
        _ext_combos(raw_pair(j, tr, 0, z) + raw_pair(j, tr, 1, z), _rhs_ext, emit)

    def prep_down(j, dst, s):
        def emit(i, v):
            dst[pl.ds(s * 16 + i * MB, 16), :] = v.astype(bf16)
        return prep_strip(j, 2 * NTR + 2 * s, MB // 8, _LHS_SPEC, _lhs_terms,
                          (2, 0, 3, 6, 4, 5, 1), emit)

    def prep_chunk(j, dst):
        for m in range(2):
            for s in range(8):
                yield from prep_gu(j, dst[0], m, s)
            for s in range(4):
                yield from prep_ext(j, dst[1], m, s)
        for s in range(9):
            yield from prep_down(j, dst[2], s)

    def feed(gen, z, n):
        for _ in range(n):
            try:
                gen.send(z)
            except StopIteration:
                return

    class Pace:
        def __init__(self):
            self.tok = 0
            self.plan = []
            self.due = []

        def add(self, gen, t0, period, lat=None, gated=True):
            next(gen)
            when = [self.tok + int(t0 + k * period) for k in range(1000)]
            self.plan.append((gen, when, lat, gated))

        def step(self, z):
            for gen, when, lat, gated in self.plan:
                for _ in range(when.count(self.tok)):
                    try:
                        v = gen.send(z if gated else None)
                    except StopIteration:
                        break
                    if v is not None and lat is not None:
                        self.due.append((self.tok + lat, v))
            self.tok += 1

        def tokens(self, r, n):
            for k in range(n):
                self.step(r[k * 16:k * 16 + 8])

        def gate(self, v):
            now = [x for t, x in self.due if t <= self.tok]
            self.due = [(t, x) for t, x in self.due if t > self.tok]
            if not now:
                return v
            head = jnp.where(never, pltpu.bitcast(tree(now), u32), v[0:8])
            return jnp.concatenate([head, v[8:]], axis=0)

        def drain(self):
            for gen, *_ in self.plan:
                feed(gen, None, 1000)

    def tree(vals):
        while len(vals) > 1:
            vals = [a + b for a, b in zip(vals[::2], vals[1::2])] + vals[len(vals) & ~1:]
        return vals[0]

    def norm_slab(row, emit, order=(4, 0, 1, 2, 3)):
        def rows(k, lo, hi):
            return [row(k, r) for r in range(lo // 8, hi // 8)]

        def mean(vals):
            t = tree([sum(vals[k + 4::4], vals[k]) for k in range(4)])
            t = jnp.sum(t, axis=0, keepdims=True) * (1.0 / D)
            return jnp.broadcast_to(t, (8, 128))
        z = yield
        x = rows(0, 0, D)
        mu = mean([held(v, z) for v in x[:4]] + x[4:])
        m = held(mu, (yield))
        rs = lax.rsqrt(mean([(v - m) * (v - m) for v in rows(1, 0, D)]) + EPS)
        end = None
        for k in order:
            m = held(mu, (yield end))
            y = jnp.concatenate(
                [(v - m) * rs for v in rows(2, k * 128, min((k + 1) * 128, D))], axis=0).T
            emit(k, y)
            end = y[120:128] if k < 4 else jnp.concatenate([y[120:128]] * 2, axis=1)
        yield end

    def alias(p, n):
        return [jnp.clip(p + k * zero[0], 0, n - 1) for k in range(3)]

    def slab_rows(src, p):
        q = alias(p, NSLAB)
        return lambda k, r: src[q[k], r * 8:r * 8 + 8, :]

    def flush(gen):
        return tree([v for v in gen if v is not None])

    def ln1(p, b, fast=False):
        seen = {}

        def emit(k, y):
            xnb[b, k, :, 0:y.shape[1]] = y.astype(bf16)
            seen[k] = y
            if fast and k == 4:
                xsb[b, 10, :, 0:64] = (y[64:] - y[:64]).astype(bf16)
            if fast and k in (2, 3):
                u = seen[k - 2]
                terms = _lhs_terms([[u[:64], y[:64]], [u[64:], y[64:]]])
                for n, i in enumerate(SUMS):
                    xsb[b, 2 * n + k - 2] = terms[i]()[0][0].astype(bf16)
        return norm_slab(slab_rows(xa, p), emit, (4, 0, 2, 1, 3) if fast else (4, 0, 1, 2, 3))

    def widen(q):
        for r in range(NTR):
            if r % 4 == 0:
                z = yield
            v = _up(held(xin32[q, r], z)).astype(f32)
            for b in range(2):
                xa[2 * q + b, r * 8:r * 8 + 8, :] = v[b * 8:b * 8 + 8]

    def qkv_proj(b, pace, groups):
        scale = DH ** -0.5 * LOG2E
        for grp in groups:
            for n in grp:
                if n == 13:
                    ktail[...] = lax.dot_general(
                        _up(wq[4, n * 64:n * 64 + 32, :]), _up(xn[b, 4]), NT,
                        preferred_element_type=f32)
                else:
                    qkv[b, n, HALO:HALO + 128, :] = lax.dot_general(
                        _up(xn[b, 4]), _up(wq[4, n * 64:(n + 1) * 64, :]), NT,
                        preferred_element_type=f32)
            for n in grp:
                rows = slice(n * 64, n * 64 + (32 if n == 13 else 64))
                x = jnp.concatenate(
                    [_up(pace.gate(xn[b, 0]))] + [_up(xn[b, k]) for k in range(1, 4)], axis=1)
                w = jnp.concatenate([_up(wq[k, rows, :]) for k in range(4)], axis=1)
                if n == 13:
                    r = lax.dot_general(w, x, NT, preferred_element_type=f32)
                    r = r + jnp.concatenate([ktail[0:32, :], ktail[32:64, :]], axis=0)
                    qkv[b, n, HALO:HALO + 128, 0:64] = (r * scale).T
                    pace.tokens(r, 4)
                    continue
                r = lax.dot_general(x, w, NT, preferred_element_type=f32)
                r = r + jnp.concatenate([qkv[b, n, HALO:HALO + 64, :],
                                         qkv[b, n, HALO + 64:HALO + 128, :]], axis=0)
                if n in (4, 5, 6, 7):
                    r = r * scale
                qkv[b, n, HALO:HALO + 128, :] = r
                pace.tokens(r, 7)

    def qkv_pair(b, pace, n, ti):
        def prod(i):
            if i in SUMS:
                x = [xs[b, 2 * SUMS.index(i) + k] for k in range(2)]
            else:
                h = i - 2
                x = [xn[b, 2 * h + k, h * 32:h * 32 + 32, :] for k in range(2)]
            x = jnp.concatenate([_up(pace.gate(x[0])), _up(x[1])], axis=1)
            r = jnp.dot(x, _up(ws[n, i * 128:(i + 1) * 128, :]), preferred_element_type=f32)
            pace.tokens(r, 2)
            if i in AUG:
                e = xs[b, 10, :, 0:64] if i == 5 else xn[b, 4, (i % 2) * 32:(i % 2) * 32 + 32, 0:64]
                f = 896 + 32 * {0: 0, 1: 0, 2: 1, 5: 2}[i]
                r = r + jnp.dot(_up(e), _up(ws[n, f:f + 32, :]), preferred_element_type=f32)
            return r

        def sink(y, z, v):
            if n in (2, 3):
                v = v * (DH ** -0.5 * LOG2E)
            qkv[b, 2 * n + z, HALO + y * 64:HALO + y * 64 + 64, :] = v
        _combine(prod, sink, ti)

    def halo(b):
        for n in range(4, 14):
            qkv[b, n, 0:HALO, :] = qkv[1 - b, n, 128:128 + HALO, :]

    def attend(b, row0, lag=0):
        qs, ks, vs = (0, 1, 2, 3, 12), (4, 5, 6, 7, 13), (8, 9, 10, 11, 12)

        def scores(s, z):
            r = HALO + s * 8
            q = [held(qkv[b, n, r:r + 8, :], z) for n in qs]
            logit = []
            for w in range(WIN):
                rw = r - DIL * w
                part = tree([q[c] * qkv[b, ks[c], rw:rw + 8, :] for c in range(5)])
                part = part + pltpu.roll(part, 64, 1)
                part = part + pltpu.roll(part, 32, 1)
                if row0 is not None and s * 8 < DIL * w:
                    pos = row0 + s * 8 + lax.broadcasted_iota(jnp.int32, (8, 128), 0)
                    part = jnp.where(pos >= DIL * w, part, -1e9 * LOG2E)
                logit.append(part)
            return logit

        def values(s, logit, z):
            r = HALO + s * 8
            mx = logit
            while len(mx) > 1:
                mx = [jnp.maximum(a, c) for a, c in zip(mx[::2], mx[1::2])]
            top = held(mx[0], z)
            e = [jnp.exp2(l - top) for l in logit]
            inv = 1.0 / tree(e)
            outs = []
            for c in range(5):
                o = e[0] * qkv[b, vs[c], r:r + 8, :]
                for w in range(1, WIN):
                    rw = r - DIL * w
                    o = o + e[w] * qkv[b, vs[c], rw:rw + 8, :]
                o = o * inv
                outs.append(o)
                ob[b, c, s * 8:(s + 1) * 8, :] = o.astype(bf16)
            return tree(outs)

        v, pending = None, []
        for s in range(16 + lag):
            z = yield v
            if s < 16:
                pending.append(scores(s, z))
            if s >= lag:
                v = values(s - lag, pending.pop(0), z if lag else None)
        yield v

    def out_proj(p, b, pace):
        h = MB // 2
        for m in range(4):
            xb[p, m * MB:(m + 1) * MB, :] = xa[p, m * MB:(m + 1) * MB, :] + lax.dot_general(
                _up(wo[4, m * h:(m + 1) * h, :]), _up(o32[b, 4]), NT, preferred_element_type=f32)
        rhs = jnp.concatenate([_up(o32[b, c]) for c in range(4)], axis=1)
        for m in range(4):
            rows = slice(m * h, (m + 1) * h)
            lhs = jnp.concatenate(
                [_up(pace.gate(wo[0, rows, :]))] + [_up(wo[c, rows, :]) for c in range(1, 4)],
                axis=1)
            r = lax.dot_general(lhs, rhs, NT, preferred_element_type=f32)
            r = r + jnp.concatenate([xb[p, m * MB:m * MB + h, :],
                                     xb[p, m * MB + h:(m + 1) * MB, :]], axis=0)
            xb[p, m * MB:(m + 1) * MB, :] = r
            pace.tokens(r, 8)

    def ffn_norm_slab(p, r):
        def emit(k, y):
            xn2[r * 6 + k, :, 0:y.shape[1]] = y
        return norm_slab(slab_rows(xb, p), emit)

    def ffn_norm(t):
        for r in range(4):
            yield from ffn_norm_slab(t * 4 + r, r)

    def strips(load, spec, terms, o, dst):
        for s in range(8):
            z = yield
            rows = slice(s * 16, (s + 1) * 16)

            def ld(r, c):
                v = load(r, c, rows)
                if (r // 2, c // 2) == spec[o][0]:
                    v = jnp.concatenate([held(v[0:8], z), held(v[8:16], z)], axis=0)
                return v

            def emit(i, v):
                dst[i, rows, :] = v.astype(bf16)
            _inner_terms(_outer_term(ld, spec, o), terms, o, emit)

    def lhs_strips(o):
        yield from strips(lambda r, k, rows: xn2[r * 6 + k, rows, :],
                          _LHS_SPEC, _lhs_terms, o, acb)
        if o in AUG:
            for s in range(2):
                z = yield
                rows = slice(s * 64, (s + 1) * 64)
                d = _lhs_ext(_lhs_ext([xn2[r * 6 + 4, rows, 0:64] for r in range(4)])[o])
                for ii, i in enumerate(AUG):
                    aeb[AUG.index(o) * 4 + ii, rows, 0:64] = d[i][0].astype(bf16)

    def ffn_combos():
        for s in range(8):
            rows = slice(s * 16, (s + 1) * 16)
            a = [[xn2[r * 6 + k, rows, :] for k in range(4)] for r in range(4)]

            def emit(i, v, rows=rows):
                acb[i, rows, :] = v.astype(bf16)
            _combos(a, _lhs_terms, emit)
            e = [xn2[r * 6 + 4, rows, 0:64] for r in range(4)]

            def emit_e(i, v, rows=rows):
                aeb[i, rows, 0:64] = v.astype(bf16)
            _ext_combos(e, _lhs_ext, emit_e)

    def attn_run(h, count, o, mask, side=None, late=None, extra=None, more=None,
                 head=False):
        fast = "seq" in o
        if not head:
            flush(ln1(h % NSLAB, 0, fast))
        for k in range(count):
            b = k % 2
            pace = Pace()
            if side is not None:
                when = [w - k * 128 for w in _spread(o["wts"], 16, NPREP)]
                pace.plan.append((side, [min(w, 126) for w in when if 0 <= w < 128], None, True))
            if k + 1 < count:
                pace.add(ln1((h + k + 1) % NSLAB, 1 - b, fast), *o["ls"][k])
            elif late is not None:
                pace.add(late, o["w0"], o["wper"])
            if k == 1 and extra is not None:
                pace.add(extra, 32 + o["x0"], o["xper"])
            if k == o.get("sk") and more is not None:
                pace.add(more, o["s0"], o["sper"])
            if k > 0 or not head:
                row0 = (h % NSLAB) * 128 if k == 1 and mask else None
                pace.add(attend(1 - b, row0, o["lag"]), *o["a"][k], o["ag"])
                if not head:
                    out_proj((h + k - 2) % NSLAB, b, pace)
                halo(b)
            if fast:
                ti = _Temps(tq)
                for n in o["seq"]:
                    if n < 6:
                        qkv_pair(b, pace, n, ti)
                    else:
                        qkv_proj(b, pace, ((12, 13),))
            else:
                qkv_proj(b, pace, o["grp"])
            pace.plan = [e for e in pace.plan if e[0] is not side]
            pace.drain()
        if side is not None:
            feed(side, None, 1000)

    def wq_prep(k):
        w = 128 if k < 4 else 64
        for c0 in range(0, 3 * D, 128):
            c1 = min(c0 + 128, 3 * D)
            wtmp[k, c0:c1, 0:w] = wq_raw[k * 128:k * 128 + w, c0:c1].astype(f32).T
        for part in OPT["parts"]:
            for d in range(DH):
                if d < 16:
                    row = part * 512 + d * 32
                else:
                    row = (1536, 1664, 1600)[part] + (d - 16) * 32
                wqb[k, row:row + 32, 0:w] = wtmp[
                    k, pl.ds(part * D + d, H, stride=DH), 0:w].astype(bf16)

    def ws_prep(n):
        for k in (4, 0, 2, 1, 3):
            for c in range(2):
                z = yield
                row = pl.multiple_of(n * 128 + c * 64, 64)
                v = jnp.concatenate([held(wq[k, pl.ds(row, 8), :], z),
                                     wq[k, pl.ds(row + 8, 56), :]], axis=0)
                w = 128 if k < 4 else 64
                wtmp[k, c * 128:c * 128 + w, :] = _up(v).astype(f32).T[0:w]

        def pair(k, r, z):
            v = [wtmp[k, c * 128 + r:c * 128 + r + 16, :] for c in range(2)]
            return [jnp.concatenate([held(u[0:8], z), u[8:]], axis=0) for u in v]
        for r in range(0, 64, 16):
            if r % 32 == 0:
                z = yield
            f = pair(4, r, z)
            for i, v in enumerate(f + [f[0] + f[1]]):
                wsb[n, 1792 + i * 64 + r:1792 + i * 64 + r + 16, :] = v.astype(bf16)
        for k in range(2):
            for r in range(0, 128, 16):
                if r % 32 == 0:
                    z = yield
                for i, t in enumerate(_rhs_terms([pair(k, r, z), pair(k + 2, r, z)])):
                    row = i * 256 + k * 128 + r
                    wsb[n, row:row + 16, :] = t()[0][0].astype(bf16)

    def wo_prep():
        for n in range(5):
            w = 128 if n < 4 else 64
            wtmp[n, 0:D, 0:w] = wo_raw[:, n * 128:n * 128 + w].astype(f32)
        for n in range(5):
            w = 128 if n < 4 else 64
            for c in range(5):
                z = yield
                rows = [held(wtmp[n, pl.ds(4 * c + g + k * 8 * DH, 8, stride=DH), :], z)[:, 0:w]
                        for g in range(4 if c < 4 else 2) for k in range(4)]
                if c == 4:
                    rows = [jnp.zeros((64, w), f32)] + rows
                wob[c, n * 128:n * 128 + w, :] = jnp.concatenate(rows, axis=0).T.astype(bf16)

    def head_late():
        for cp in (wo_copy, x_copy(1)):
            cp.wait()
        for cp in [x_copy(2)] + chunk_copies(1):
            cp.start()
        yield from wo_prep()
        yield from widen(1)

    wqb[4, :, 64:128] = jnp.zeros((3 * D, 64), bf16)
    qkv[:, 13] = jnp.zeros((2, HALO + 128, 128), f32)
    xnb[:, 4, :, 64:128] = jnp.zeros((2, 128, 64), bf16)
    for n in range(4, 13):
        qkv[0, n, 0:HALO, :] = jnp.zeros((HALO, 128), f32)
    todo = list(k_order)
    for n, cp in enumerate(first):
        cp.wait()
        if n == OPT["dma"][0]:
            wo_copy.start()
        if n == OPT["dma"][1]:
            for c in [x_copy(1)] + chunk_copies(0):
                c.start()
        if n == OPT["xpos"]:
            feed(widen(0), None, 1000)
            flush(ln1(0, 0))
        else:
            wq_prep(todo.pop(0))
    attn_run(0, 2, OPT["h"], True, late=head_late(), head=True)

    @pl.loop(0, 7)
    def _(i):
        for cp in chunk_copies(i):
            cp.wait()

        @pl.when(i + 2 < NSLAB // 2)
        def _():
            x_copy(i + 2).wait()

        @pl.when(i + 3 < NSLAB // 2)
        def _():
            x_copy(i + 3).start()
        for cp in chunk_copies(i + 2):
            cp.start()
        side = prep_chunk(i, [r.at[i] for r in (wcb, web, wdcb)])
        next(side)
        r = jnp.clip(i - 2, 0, 3)
        attn_run(2 * i + 2, 2, OPT["p"], False, side, widen(jnp.minimum(i + 2, NSLAB // 2 - 1)),
                 ffn_norm_slab(r, r), ws_prep(jnp.minimum(i, 5)))

    for cp in chunk_copies(7) + chunk_copies(8):
        cp.wait()
    ffn_combos()

    def ffn_group(t, g, last, emit=None):
        ti = _Temps(tin)
        to = _Temps(tout)
        pace = Pace()
        o_ = OPT["fb" if last else "fa"]

        def weights(c):
            if last and c > 0:
                return [r.at[c - 1] for r in (wc2, we2, wdc2)]
            return [r.at[g * 3 + c] for r in (wc, we, wdc)]

        def proj(c, m):
            w, w_ext, _ = weights(c)

            def prod(o, i):
                r = (m * 49 + o * 7 + i) * 64
                p = jnp.dot(_up(ac[o * 7 + i]), _up(w[r:r + 64, :]),
                            preferred_element_type=f32)
                pace.step(p[0:8])
                if o in AUG and i in AUG:
                    q = AUG.index(o) * 4 + AUG.index(i)
                    e = jnp.dot(_up(ae[q, :, 0:64]), _up(w_ext[m * 16 + q]),
                                preferred_element_type=f32)
                    pace.step(e[0:8])
                    p = p + e
                return p
            return prod

        def gate(c):
            def fin(r, cc, v):
                gs[(c % 2) * 16 + r * 4 + cc] = v
            return _recombine(proj(c, 0), fin, ti, to)

        def upgate(c):
            def fin(r, cc, v):
                hs[c, r * 4 + cc] = _ld(gs, (c % 2) * 16 + r * 4 + cc) * v
            yield from _recombine(proj(c, 1), fin, ti, to, last)
            pace.add(hidden_paced(c), *o_["h"][c])

        hgen, hdone = {}, {}

        def hidden(c):
            for o in ORDER:
                yield from strips(lambda cc, r, rows: hs[c, r * 4 + cc, rows, :],
                                  _RHS_SPEC, _rhs_terms, o, hcb.at[c])

        def hidden_paced(c):
            hgen[c], hdone[c] = hidden(c), 0
            next(hgen[c])
            while True:
                z = yield
                need(c, min(hdone[c] + 1, 56), z)

        def need(c, n, z=None):
            feed(hgen[c], z, n - hdone[c])
            hdone[c] = max(hdone[c], n)

        def dprod(cs, i):
            p = None
            for c in cs:
                need(c, 8 * (ORDER.index(i // 7) + 1))
                r = i * (MB // 2)
                q = lax.dot_general(_up(weights(c)[2][r:r + MB // 2, :]), _up(hc[c, i]), NT,
                                    preferred_element_type=f32)
                pace.step(q[0:8])
                p = q if p is None else p + q
            return p

        def down(cs, reset):
            for i in [o * 7 + k for o in ORDER for k in range(7)]:
                a = _ld(acc, i)
                if reset:
                    a = jnp.where(g == 0, 0.0, a)
                acc[i] = a + dprod(cs, i)
                yield

        def down_final(cs):
            def fin(mb, r, v):
                rows = slice(mb * MB, (mb + 1) * MB)
                y = xb[t * 4 + r, rows, :] + v
                xa[t * 4 + r, rows, :] = y
                ost[t * 2 + r // 2, rows, (r % 2) * 128:(r % 2) * 128 + 128] = y.astype(bf16)
            return _recombine(lambda o, i: _ld(acc, o * 7 + i) + dprod(cs, o * 7 + i),
                              fin, _Temps(tin2), _Temps(tout2))

        if last:
            norm = ffn_norm((t + 1) % NTILE)
            pace.add(norm, o_["n0"], o_["nper"])
        else:
            late = prep_chunk(7 + g, [r.at[g] for r in (wcb2, web2, wdcb2)])
            next(late)
            pace.plan.append((late, _spread(o_["wts"], 30, NPREP), None, True))
        for gen in (gate(0), upgate(0), gate(1)):
            _adv(gen, 100)
        d0 = down((0,), not last)
        queue = []

        def lhs_queue():
            while True:
                z = yield
                if queue:
                    try:
                        queue[0].send(z)
                    except StopIteration:
                        queue.pop(0)
        for gen, plan in ((upgate(1), "u1"), (gate(2), "g2"), (upgate(2), "u2")):
            if last and plan == "u2":
                feed(norm, None, 1000)
                pace.add(lhs_queue(), o_["l0"], o_["lper"])
            for k, n in enumerate(o_[plan]):
                _adv(gen, 1)
                if last and plan == "u2":
                    queue.append(lhs_strips(ORDER[k]))
                    next(queue[-1])
                _adv(d0, n)
            _adv(gen, 100)
        _adv(d0, 100)
        if last:
            gen = down_final((1, 2))
            _adv(gen, 3)
            for q, h in ((1, 1), (0, 1), (1, 0), (0, 0)):
                _adv(gen, 1)
                pl.when(emit)(out_copy(t * 2 + q, h).start)
        else:
            _adv(down((1, 2), False), 100)
            feed(late, None, 1000)
        for gen in queue:
            feed(gen, None, 1000)

    @pl.loop(0, 2 * NTILE)
    def _(tile):
        t = tile % NTILE

        @pl.loop(0, 2)
        def _(g):
            ffn_group(t, g, False)
        ffn_group(t, 2, True, tile >= NTILE)

        @pl.when(tile < NTILE)
        def _():
            attn_run(4 * t + NSLAB, 4, OPT["n"], True)

        @pl.when(tile == NTILE - 1)
        def _():
            out_proj(NSLAB - 2, 0, Pace())
            flush(attend(1, None))
            out_proj(NSLAB - 1, 1, Pace())

    for p in range(NSLAB):
        out_copy(p // 2, p % 2).wait()


def _tiles(w):
    n = w.shape[1]
    return w.reshape(NTR, 8, n // 128, 128).transpose(0, 2, 1, 3).reshape(NTR, n // 16, 128)


@jax.jit
def pallas_interleave_layers__sliding_local_dilated__glu_gated_bilinear__prompt_kernel(
    A_x: jax.Array,
    A_wqkv: jax.Array,
    A_wo: jax.Array,
    B_x: jax.Array,
    B_w_gate: jax.Array,
    B_w_up: jax.Array,
    B_w_down: jax.Array,
):
    del B_x
    vm = pltpu.VMEM
    hbm = pl.BlockSpec(memory_space=pl.ANY)
    out_t = pl.pallas_call(
        _kernel,
        in_specs=[hbm] * 6,
        out_specs=hbm,
        out_shape=jax.ShapeDtypeStruct((D, S), bf16),
        scratch_shapes=[
            vm((NSLAB // 2, 96, 16, 128), bf16),
            vm((NSLAB, 768, 128), f32),
            vm((NSLAB, 768, 128), f32),
            vm((NSLAB // 2, 768, 256), bf16),
            vm((NCHUNK, 224, 32, 128), bf16),
            vm((7, WC_ROWS, 128), bf16),
            vm((7, 32, 64, 128), bf16),
            vm((7, WD_ROWS, 128), bf16),
            vm((2, WC_ROWS, 128), bf16),
            vm((2, 32, 64, 128), bf16),
            vm((2, WD_ROWS, 128), bf16),
            vm((24, 128, 128), f32),
            vm((D, 3 * D), bf16),
            vm((D, D), bf16),
            vm((5, 3 * D, 128), f32),
            vm((5, 3 * D, 128), bf16),
            vm((5, D, 128), bf16),
            vm((2, 5, 128, 128), bf16),
            vm((2, 14, HALO + 128, 128), f32),
            vm((2, 5, 128, 128), bf16),
            vm((49, 128, 128), bf16),
            vm((16, 128, 128), bf16),
            vm((32, 128, 128), f32),
            vm((3, 16, 128, 128), f32),
            vm((3, 49, 128, 128), bf16),
            vm((49, MB, 128), f32),
            vm((12, 128, 128), f32),
            vm((40, 128, 128), f32),
            vm((12, MB, 128), f32),
            vm((20, MB, 128), f32),
            vm((64, 128), f32),
            vm((2, 11, 64, 128), bf16),
            vm((6, 1984, 128), bf16),
            vm((6, 64, 128), f32),
            pltpu.SMEM((1,), jnp.int32),
            pltpu.SemaphoreType.DMA((NSLAB // 2,)),
            pltpu.SemaphoreType.DMA((6,)),
            pltpu.SemaphoreType.DMA((NCHUNK, 3)),
            pltpu.SemaphoreType.DMA((NSLAB // 2, 2)),
        ],
        compiler_params=pltpu.CompilerParams(vmem_limit_bytes=122 * 1024 * 1024,
                                             disable_bounds_checks=True,
                                             disable_semaphore_checks=True),
    )(_tiles(A_x[0].T), A_wqkv, A_wo, _tiles(B_w_gate), _tiles(B_w_up), _tiles(B_w_down.T))
    return out_t.T[None]
```

```python
import math

import jax
import jax.numpy as jnp
from jax import lax
import jax.experimental.pallas as pl
import jax.experimental.pallas.tpu as pltpu

f32 = jnp.float32
bf16 = jnp.bfloat16
u32 = jnp.uint32

S, D, F = 2048, 576, 4608
H, DH, WIN, DIL = 32, 18, 8, 2
EPS = 1e-5
LOG2E = math.log2(math.e)
NSLAB = S // 128
TILE = 512
NTILE = S // TILE
FC = 512
NCHUNK = F // FC
MB = D // 4
HALO = 16
NPREP = 158
NTR = D // 8
WC_ROWS = 800 * 16
WD_ROWS = 448 * 16
NT = (((1,), (1,)), ((), ()))
ORDER = (0, 1, 2, 5, 3, 4, 6)
SUMS = (0, 1, 4, 5, 6)
AUG = (0, 1, 2, 5)

OPT = {'dma': (0, 2),
 'xpos': 2,
 'parts': (1, 0, 2),
 'fa': {'sw': (1, 2, 1, 1, 1, 1, 1, 0, 1, 2, 2, 0, 0, 1, 1, 1, 0, 1),
        'wts': (3, 1, 0, 0, 0, 1, 2, 1, 1, 2, 0, 0, 0, 1, 0, 5, 5, 4),
        'h': ((0, 0.7), (0, 1), (0, 1)),
        'u1': (0, 0, 0, 4, 5, 4, 6),
        'g2': (4, 0, 0, 0, 0, 0, 0),
        'u2': (0, 0, 0, 0, 3, 4, 4)},
 'fb': {'h': ((0, 1), (0, 0.68), (0, 1)),
        'n0': 0,
        'nper': 1.4,
        'l0': 0,
        'lper': 3.22,
        'u1': (0, 0, 0, 0, 4, 4, 6),
        'g2': (4, 0, 0, 0, 0, 0, 0),
        'u2': (0, 0, 0, 0, 4, 4, 4)},
 'h': {'lag': 0,
       'grp': ((4, 5, 6, 7), (0, 1, 2, 3), (12, 13, 8, 9, 10, 11)),
       'a': ((0, 5, 35), (0, 3.65, 35)),
       'w0': 22,
       'wper': 2.8,
       'ag': 1,
       'ls': ((13, 5.0, 40),)},
 'p': {'lag': 0,
       'x0': 36,
       'xper': 5.6,
       'grp': ((4, 13), (5, 6, 7, 0), (1, 2, 3, 12), (8, 9, 10, 11)),
       'a': ((3, 6, 25), (0, 5.44, 35)),
       'w0': 65,
       'wper': 4.88,
       'ag': 0,
       'ls': ((40, 5.47, None),),
       'wts': (7, 9, 9, 9, 9, 9, 5, 11, 9, 11, 7, 11, 7, 11, 11, 11)},
 'n': {'seq': (5, 6, 2, 0, 4, 1, 3),
       'lag': 1,
       'a': ((0, 6, 35), (0, 6, 35), (0, 6.84, 35), (0, 6, 35)),
       'ag': 1,
       'ls': ((77, 7.71, None), (69, 9.04, None), (80, 6.83, None))}}


def _up(v):
    return pltpu.bitcast(v, bf16)


def _quad(x):
    n = len(x) // 2
    return ([r[:n] for r in x[:n]], [r[n:] for r in x[:n]],
            [r[:n] for r in x[n:]], [r[n:] for r in x[n:]])


def _badd(x, y):
    return [[a + b for a, b in zip(r, s)] for r, s in zip(x, y)]


def _bsub(x, y):
    return [[a - b for a, b in zip(r, s)] for r, s in zip(x, y)]


def _lhs_terms(a):
    a11, a12, a21, a22 = _quad(a)
    return [lambda: _badd(a11, a22), lambda: _badd(a21, a22), lambda: a11, lambda: a22,
            lambda: _badd(a11, a12), lambda: _bsub(a21, a11), lambda: _bsub(a12, a22)]


def _rhs_terms(b):
    b11, b12, b21, b22 = _quad(b)
    return [lambda: _badd(b11, b22), lambda: b11, lambda: _bsub(b12, b22), lambda: _bsub(b21, b11),
            lambda: b22, lambda: _badd(b11, b12), lambda: _badd(b21, b22)]


def _combos(x, terms, emit):
    for o, fo in enumerate(terms(x)):
        y = fo()
        for i, fi in enumerate(terms(y)):
            emit(o * 7 + i, fi()[0][0])


_LHS_SPEC = (((0, 0), (1, 1), 1), ((1, 0), (1, 1), 1), ((0, 0), None, 0), ((1, 1), None, 0),
             ((0, 0), (0, 1), 1), ((1, 0), (0, 0), -1), ((0, 1), (1, 1), -1))
_RHS_SPEC = (((0, 0), (1, 1), 1), ((0, 0), None, 0), ((0, 1), (1, 1), -1), ((1, 0), (0, 0), -1),
             ((1, 1), None, 0), ((0, 0), (0, 1), 1), ((1, 0), (1, 1), 1))


def _outer_term(load, spec, o):
    p, q, sign = spec[o]
    out = []
    for y in range(2):
        row = []
        for z in range(2):
            v = load(2 * p[0] + y, 2 * p[1] + z)
            if sign:
                w = load(2 * q[0] + y, 2 * q[1] + z)
                v = v + w if sign > 0 else v - w
            row.append(v)
        out.append(row)
    return out


def _inner_terms(y, terms, o, emit):
    for i, fi in enumerate(terms(y)):
        emit(o * 7 + i, fi()[0][0])


def _lhs_ext(e):
    n = len(e) // 2
    return {0: e[:n], 1: e[n:], 2: e[:n], 5: [y - x for x, y in zip(e[:n], e[n:])]}


def _rhs_ext(e):
    n = len(e) // 2
    return {0: e[:n], 1: e[:n], 2: e[n:], 5: [x + y for x, y in zip(e[:n], e[n:])]}


def _ext_combos(e, fn, emit):
    for oi, o in enumerate(AUG):
        d = fn(fn(e)[o])
        for ii, i in enumerate(AUG):
            emit(oi * 4 + ii, d[i][0])


def _spread(weights, span, n):
    total, acc, out = sum(weights), 0.0, []
    for k, w in enumerate(weights):
        lo, acc = acc, acc + w * n / total
        count = round(acc) - round(lo)
        out += [k * span + i * span // count for i in range(count)]
    return out


def _adv(gen, n):
    for _ in range(n):
        try:
            next(gen)
        except StopIteration:
            return


def _ld(ref, idx):
    n = ref.shape[-2] // 2
    return jnp.concatenate([ref[idx, :n, :], ref[idx, n:, :]], axis=0)


class _Temps:
    def __init__(self, ref):
        self.ref = ref
        self.n = 0

    def put(self, v):
        i = self.n % self.ref.shape[0]
        self.n += 1
        self.ref[i] = v
        return i

    def get(self, i):
        return _ld(self.ref, i)


def _combine(prod, sink, ti, spill_last=False):
    a = ti.put(prod(0))
    b = ti.put(prod(1))
    c = ti.put(prod(2))
    sink(1, 1, ti.get(a) - ti.get(b) + ti.get(c) + prod(5))
    if spill_last:
        m3 = prod(3)
        m4 = prod(4)
        sink(1, 0, ti.get(b) + m3)
        sink(0, 1, ti.get(c) + m4)
        d = ti.put(ti.get(a) + m3 - m4)
        sink(0, 0, ti.get(d) + prod(6))
        return
    m3 = prod(3)
    m4 = prod(4)
    m6 = prod(6)
    sink(1, 0, ti.get(b) + m3)
    sink(0, 1, ti.get(c) + m4)
    sink(0, 0, ti.get(a) + m3 - m4 + m6)


def _recombine(prod, fin, ti, to, spill_last=False):
    def inner(o, sink):
        _combine(lambda i: prod(o, i), sink, ti, spill_last)

    m = {}
    for o in (0, 1, 2):
        def keep(y, z, v, o=o):
            m[o, y, z] = to.put(v)
        inner(o, keep)
        yield

    def s5(y, z, v):
        fin(2 + y, 2 + z, to.get(m[0, y, z]) - to.get(m[1, y, z]) + to.get(m[2, y, z]) + v)
    inner(5, s5)
    yield

    def s3(y, z, v):
        fin(2 + y, z, to.get(m[1, y, z]) + v)
        m[3, y, z] = to.put(to.get(m[0, y, z]) + v)
    inner(3, s3)
    yield

    def s4(y, z, v):
        fin(y, 2 + z, to.get(m[2, y, z]) + v)
        m[3, y, z] = to.put(to.get(m[3, y, z]) - v)
    inner(4, s4)
    yield

    def s6(y, z, v):
        fin(y, z, to.get(m[3, y, z]) + v)
    inner(6, s6)
    yield


def _kernel(xt_hbm, wqkv_hbm, wo_hbm, wg_hbm, wu_hbm, wdt_hbm, out_hbm,
            xin, xa, xb, ost, raw, wcb, web, wdcb, wcb2, web2, wdcb2, xn2,
            wq_raw, wo_raw, wtmp, wqb, wob, xnb, qkv, ob, acb, aeb, gs, hs, hcb, acc,
            tin, tout, tin2, tout2, ktail, xsb, wsb, tq, zero,
            sem_x, sem_w, sem_c, sem_o):
    wq, wo, wc, we, wdc, xn, o32, ac, ae, hc, raw32, xin32, wc2, we2, wdc2, xs, ws = [
        r.bitcast(u32) for r in (wqb, wob, wcb, web, wdcb, xnb, ob, acb, aeb, hcb, raw, xin,
                                 wcb2, web2, wdcb2, xsb, wsb)]

    def x_copy(q):
        return pltpu.make_async_copy(
            xt_hbm.at[:, pl.ds(pl.multiple_of(q * 16, 16), 16), :], xin.at[q, 0:NTR], sem_x.at[q])

    def weight_copy(j, m):
        rows = pl.ds(pl.multiple_of(j * 32, 32), 32)
        return pltpu.make_async_copy((wg_hbm, wu_hbm, wdt_hbm)[m].at[:, rows, :],
                                     raw.at[j, pl.ds(m * NTR, NTR)], sem_c.at[j, m])

    def chunk_copies(j):
        return [weight_copy(j, m) for m in range(3)]

    def out_copy(q, h):
        rows = pl.ds(h * 2 * MB, 2 * MB)
        return pltpu.make_async_copy(
            ost.at[q, rows, :], out_hbm.at[rows, pl.ds(pl.multiple_of(q * 256, 256), 256)],
            sem_o.at[q, h])

    k_order = (4, 0, 1, 2, 3)
    wq_copies = [pltpu.make_async_copy(wqkv_hbm.at[k * 128:min(k * 128 + 128, D)],
                                       wq_raw.at[k * 128:min(k * 128 + 128, D)], sem_w.at[k])
                 for k in k_order]
    wo_copy = pltpu.make_async_copy(wo_hbm, wo_raw, sem_w.at[5])
    first = wq_copies[:OPT["xpos"]] + [x_copy(0)] + wq_copies[OPT["xpos"]:]
    for cp in first:
        cp.start()
    zero[0] = 0
    never = zero[0] != 0

    def held(v, z):
        if z is None:
            return v
        return jnp.where(never, pltpu.bitcast(z, v.dtype), v)

    def raw_pair(j, tr, cp, z):
        v = [_up(held(raw32[j, tr + k, cp * 8:cp * 8 + 8, :], z)).astype(f32) for k in range(2)]
        return [jnp.concatenate([v[0][h:h + 8], v[1][h:h + 8]], axis=0) for h in (0, 8)]

    def prep_strip(j, tr, step, spec, terms, path, emit):
        live = {}
        for o in path:
            used = [q for q in spec[o][:2] if q is not None]
            live = {q: live[q] for q in used if q in live}
            for q in used:
                if q not in live:
                    z = yield
                    live[q] = [raw_pair(j, tr + (2 * q[0] + y) * step, q[1], z) for y in range(2)]
            y = _outer_term(lambda r, c: live[r // 2, c // 2][r % 2][c % 2], spec, o)
            _inner_terms(y, terms, o, emit)

    def prep_gu(j, dst, m, s):
        base = m * (49 * 128) + s * 16

        def emit(i, v):
            dst[pl.ds(base + i * 128, 16), :] = v.astype(bf16)
        return prep_strip(j, m * NTR + 2 * s, 16, _RHS_SPEC, _rhs_terms,
                          (1, 0, 4, 2, 5, 3, 6), emit)

    def prep_ext(j, dst, m, s):
        z = yield
        tr = m * NTR + 64 + 2 * s

        def emit(i, v):
            dst[m * 16 + i, pl.ds(s * 16, 16), :] = v.astype(bf16)
        _ext_combos(raw_pair(j, tr, 0, z) + raw_pair(j, tr, 1, z), _rhs_ext, emit)

    def prep_down(j, dst, s):
        def emit(i, v):
            dst[pl.ds(s * 16 + i * MB, 16), :] = v.astype(bf16)
        return prep_strip(j, 2 * NTR + 2 * s, MB // 8, _LHS_SPEC, _lhs_terms,
                          (2, 0, 3, 6, 4, 5, 1), emit)

    def prep_chunk(j, dst):
        for m in range(2):
            for s in range(8):
                yield from prep_gu(j, dst[0], m, s)
            for s in range(4):
                yield from prep_ext(j, dst[1], m, s)
        for s in range(9):
            yield from prep_down(j, dst[2], s)

    def feed(gen, z, n):
        for _ in range(n):
            try:
                gen.send(z)
            except StopIteration:
                return

    class Pace:
        def __init__(self):
            self.tok = 0
            self.plan = []
            self.due = []

        def add(self, gen, t0, period, lat=None, gated=True):
            next(gen)
            when = [self.tok + int(t0 + k * period) for k in range(1000)]
            self.plan.append((gen, when, lat, gated))

        def step(self, z):
            for gen, when, lat, gated in self.plan:
                for _ in range(when.count(self.tok)):
                    try:
                        v = gen.send(z if gated else None)
                    except StopIteration:
                        break
                    if v is not None and lat is not None:
                        self.due.append((self.tok + lat, v))
            self.tok += 1

        def tokens(self, r, n):
            for k in range(n):
                self.step(r[k * 16:k * 16 + 8])

        def gate(self, v):
            now = [x for t, x in self.due if t <= self.tok]
            self.due = [(t, x) for t, x in self.due if t > self.tok]
            if not now:
                return v
            head = jnp.where(never, pltpu.bitcast(tree(now), u32), v[0:8])
            return jnp.concatenate([head, v[8:]], axis=0)

        def drain(self):
            for gen, *_ in self.plan:
                feed(gen, None, 1000)

    def tree(vals):
        while len(vals) > 1:
            vals = [a + b for a, b in zip(vals[::2], vals[1::2])] + vals[len(vals) & ~1:]
        return vals[0]

    def norm_slab(row, emit, order=(4, 0, 1, 2, 3)):
        def rows(k, lo, hi):
            return [row(k, r) for r in range(lo // 8, hi // 8)]

        def mean(vals):
            t = tree([sum(vals[k + 4::4], vals[k]) for k in range(4)])
            t = jnp.sum(t, axis=0, keepdims=True) * (1.0 / D)
            return jnp.broadcast_to(t, (8, 128))
        z = yield
        x = rows(0, 0, D)
        mu = mean([held(v, z) for v in x[:4]] + x[4:])
        m = held(mu, (yield))
        rs = lax.rsqrt(mean([(v - m) * (v - m) for v in rows(1, 0, D)]) + EPS)
        end = None
        for k in order:
            m = held(mu, (yield end))
            y = jnp.concatenate(
                [(v - m) * rs for v in rows(2, k * 128, min((k + 1) * 128, D))], axis=0).T
            emit(k, y)
            end = y[120:128] if k < 4 else jnp.concatenate([y[120:128]] * 2, axis=1)
        yield end

    def alias(p, n):
        return [jnp.clip(p + k * zero[0], 0, n - 1) for k in range(3)]

    def slab_rows(src, p):
        q = alias(p, NSLAB)
        return lambda k, r: src[q[k], r * 8:r * 8 + 8, :]

    def flush(gen):
        return tree([v for v in gen if v is not None])

    def ln1(p, b, fast=False):
        seen = {}

        def emit(k, y):
            xnb[b, k, :, 0:y.shape[1]] = y.astype(bf16)
            seen[k] = y
            if fast and k == 4:
                xsb[b, 10, :, 0:64] = (y[64:] - y[:64]).astype(bf16)
            if fast and k in (2, 3):
                u = seen[k - 2]
                terms = _lhs_terms([[u[:64], y[:64]], [u[64:], y[64:]]])
                for n, i in enumerate(SUMS):
                    xsb[b, 2 * n + k - 2] = terms[i]()[0][0].astype(bf16)
        return norm_slab(slab_rows(xa, p), emit, (4, 0, 2, 1, 3) if fast else (4, 0, 1, 2, 3))

    def widen(q):
        for r in range(NTR):
            if r % 4 == 0:
                z = yield
            v = _up(held(xin32[q, r], z)).astype(f32)
            for b in range(2):
                xa[2 * q + b, r * 8:r * 8 + 8, :] = v[b * 8:b * 8 + 8]

    def qkv_proj(b, pace, groups):
        scale = DH ** -0.5 * LOG2E
        for grp in groups:
            for n in grp:
                if n == 13:
                    ktail[...] = lax.dot_general(
                        _up(wq[4, n * 64:n * 64 + 32, :]), _up(xn[b, 4]), NT,
                        preferred_element_type=f32)
                else:
                    qkv[b, n, HALO:HALO + 128, :] = lax.dot_general(
                        _up(xn[b, 4]), _up(wq[4, n * 64:(n + 1) * 64, :]), NT,
                        preferred_element_type=f32)
            for n in grp:
                rows = slice(n * 64, n * 64 + (32 if n == 13 else 64))
                x = jnp.concatenate(
                    [_up(pace.gate(xn[b, 0]))] + [_up(xn[b, k]) for k in range(1, 4)], axis=1)
                w = jnp.concatenate([_up(wq[k, rows, :]) for k in range(4)], axis=1)
                if n == 13:
                    r = lax.dot_general(w, x, NT, preferred_element_type=f32)
                    r = r + jnp.concatenate([ktail[0:32, :], ktail[32:64, :]], axis=0)
                    qkv[b, n, HALO:HALO + 128, 0:64] = (r * scale).T
                    pace.tokens(r, 4)
                    continue
                r = lax.dot_general(x, w, NT, preferred_element_type=f32)
                r = r + jnp.concatenate([qkv[b, n, HALO:HALO + 64, :],
                                         qkv[b, n, HALO + 64:HALO + 128, :]], axis=0)
                if n in (4, 5, 6, 7):
                    r = r * scale
                qkv[b, n, HALO:HALO + 128, :] = r
                pace.tokens(r, 7)

    def qkv_pair(b, pace, n, ti):
        def prod(i):
            if i in SUMS:
                x = [xs[b, 2 * SUMS.index(i) + k] for k in range(2)]
            else:
                h = i - 2
                x = [xn[b, 2 * h + k, h * 32:h * 32 + 32, :] for k in range(2)]
            x = jnp.concatenate([_up(pace.gate(x[0])), _up(x[1])], axis=1)
            r = jnp.dot(x, _up(ws[n, i * 128:(i + 1) * 128, :]), preferred_element_type=f32)
            pace.tokens(r, 2)
            if i in AUG:
                e = xs[b, 10, :, 0:64] if i == 5 else xn[b, 4, (i % 2) * 32:(i % 2) * 32 + 32, 0:64]
                f = 896 + 32 * {0: 0, 1: 0, 2: 1, 5: 2}[i]
                r = r + jnp.dot(_up(e), _up(ws[n, f:f + 32, :]), preferred_element_type=f32)
            return r

        def sink(y, z, v):
            if n in (2, 3):
                v = v * (DH ** -0.5 * LOG2E)
            qkv[b, 2 * n + z, HALO + y * 64:HALO + y * 64 + 64, :] = v
        _combine(prod, sink, ti)

    def halo(b):
        for n in range(4, 14):
            qkv[b, n, 0:HALO, :] = qkv[1 - b, n, 128:128 + HALO, :]

    def attend(b, row0, lag=0):
        qs, ks, vs = (0, 1, 2, 3, 12), (4, 5, 6, 7, 13), (8, 9, 10, 11, 12)

        def scores(s, z):
            r = HALO + s * 8
            q = [held(qkv[b, n, r:r + 8, :], z) for n in qs]
            logit = []
            for w in range(WIN):
                rw = r - DIL * w
                part = tree([q[c] * qkv[b, ks[c], rw:rw + 8, :] for c in range(5)])
                part = part + pltpu.roll(part, 64, 1)
                part = part + pltpu.roll(part, 32, 1)
                if row0 is not None and s * 8 < DIL * w:
                    pos = row0 + s * 8 + lax.broadcasted_iota(jnp.int32, (8, 128), 0)
                    part = jnp.where(pos >= DIL * w, part, -1e9 * LOG2E)
                logit.append(part)
            return logit

        def values(s, logit, z):
            r = HALO + s * 8
            mx = logit
            while len(mx) > 1:
                mx = [jnp.maximum(a, c) for a, c in zip(mx[::2], mx[1::2])]
            top = held(mx[0], z)
            e = [jnp.exp2(l - top) for l in logit]
            inv = 1.0 / tree(e)
            outs = []
            for c in range(5):
                o = e[0] * qkv[b, vs[c], r:r + 8, :]
                for w in range(1, WIN):
                    rw = r - DIL * w
                    o = o + e[w] * qkv[b, vs[c], rw:rw + 8, :]
                o = o * inv
                outs.append(o)
                ob[b, c, s * 8:(s + 1) * 8, :] = o.astype(bf16)
            return tree(outs)

        v, pending = None, []
        for s in range(16 + lag):
            z = yield v
            if s < 16:
                pending.append(scores(s, z))
            if s >= lag:
                v = values(s - lag, pending.pop(0), z if lag else None)
        yield v

    def out_proj(p, b, pace):
        h = MB // 2
        for m in range(4):
            xb[p, m * MB:(m + 1) * MB, :] = xa[p, m * MB:(m + 1) * MB, :] + lax.dot_general(
                _up(wo[4, m * h:(m + 1) * h, :]), _up(o32[b, 4]), NT, preferred_element_type=f32)
        rhs = jnp.concatenate([_up(o32[b, c]) for c in range(4)], axis=1)
        for m in range(4):
            rows = slice(m * h, (m + 1) * h)
            lhs = jnp.concatenate(
                [_up(pace.gate(wo[0, rows, :]))] + [_up(wo[c, rows, :]) for c in range(1, 4)],
                axis=1)
            r = lax.dot_general(lhs, rhs, NT, preferred_element_type=f32)
            r = r + jnp.concatenate([xb[p, m * MB:m * MB + h, :],
                                     xb[p, m * MB + h:(m + 1) * MB, :]], axis=0)
            xb[p, m * MB:(m + 1) * MB, :] = r
            pace.tokens(r, 8)

    def ffn_norm_slab(p, r):
        def emit(k, y):
            xn2[r * 6 + k, :, 0:y.shape[1]] = y
        return norm_slab(slab_rows(xb, p), emit)

    def ffn_norm(t):
        for r in range(4):
            yield from ffn_norm_slab(t * 4 + r, r)

    def strips(load, spec, terms, o, dst):
        for s in range(8):
            z = yield
            rows = slice(s * 16, (s + 1) * 16)

            def ld(r, c):
                v = load(r, c, rows)
                if (r // 2, c // 2) == spec[o][0]:
                    v = jnp.concatenate([held(v[0:8], z), held(v[8:16], z)], axis=0)
                return v

            def emit(i, v):
                dst[i, rows, :] = v.astype(bf16)
            _inner_terms(_outer_term(ld, spec, o), terms, o, emit)

    def lhs_strips(o):
        yield from strips(lambda r, k, rows: xn2[r * 6 + k, rows, :],
                          _LHS_SPEC, _lhs_terms, o, acb)
        if o in AUG:
            for s in range(2):
                z = yield
                rows = slice(s * 64, (s + 1) * 64)
                d = _lhs_ext(_lhs_ext([xn2[r * 6 + 4, rows, 0:64] for r in range(4)])[o])
                for ii, i in enumerate(AUG):
                    aeb[AUG.index(o) * 4 + ii, rows, 0:64] = d[i][0].astype(bf16)

    def ffn_combos():
        for s in range(8):
            rows = slice(s * 16, (s + 1) * 16)
            a = [[xn2[r * 6 + k, rows, :] for k in range(4)] for r in range(4)]

            def emit(i, v, rows=rows):
                acb[i, rows, :] = v.astype(bf16)
            _combos(a, _lhs_terms, emit)
            e = [xn2[r * 6 + 4, rows, 0:64] for r in range(4)]

            def emit_e(i, v, rows=rows):
                aeb[i, rows, 0:64] = v.astype(bf16)
            _ext_combos(e, _lhs_ext, emit_e)

    def attn_run(h, count, o, mask, side=None, late=None, extra=None, head=False):
        fast = "seq" in o
        if not head:
            flush(ln1(h % NSLAB, 0, fast))
        for k in range(count):
            b = k % 2
            pace = Pace()
            if side is not None:
                when = [w - k * 128 for w in _spread(o["wts"], 16, NPREP)]
                pace.plan.append((side, [min(w, 126) for w in when if 0 <= w < 128], None, True))
            if k + 1 < count:
                pace.add(ln1((h + k + 1) % NSLAB, 1 - b, fast), *o["ls"][k])
            elif late is not None:
                pace.add(late, o["w0"], o["wper"])
            if k == 1 and extra is not None:
                pace.add(extra, 32 + o["x0"], o["xper"])
            if k > 0 or not head:
                row0 = (h % NSLAB) * 128 if k == 1 and mask else None
                pace.add(attend(1 - b, row0, o["lag"]), *o["a"][k], o["ag"])
                if not head:
                    out_proj((h + k - 2) % NSLAB, b, pace)
                halo(b)
            if fast:
                ti = _Temps(tq)
                for n in o["seq"]:
                    if n < 6:
                        qkv_pair(b, pace, n, ti)
                    else:
                        qkv_proj(b, pace, ((12, 13),))
            else:
                qkv_proj(b, pace, o["grp"])
            pace.plan = [e for e in pace.plan if e[0] is not side]
            pace.drain()
        if side is not None:
            feed(side, None, 1000)

    def wq_prep(k):
        w = 128 if k < 4 else 64
        for c0 in range(0, 3 * D, 128):
            c1 = min(c0 + 128, 3 * D)
            wtmp[k, c0:c1, 0:w] = wq_raw[k * 128:k * 128 + w, c0:c1].astype(f32).T
        for part in OPT["parts"]:
            for d in range(DH):
                if d < 16:
                    row = part * 512 + d * 32
                else:
                    row = (1536, 1664, 1600)[part] + (d - 16) * 32
                wqb[k, row:row + 32, 0:w] = wtmp[
                    k, pl.ds(part * D + d, H, stride=DH), 0:w].astype(bf16)

    def ws_prep(n):
        for k in (4, 0, 2, 1, 3):
            for c in range(2):
                z = yield
                row = pl.multiple_of(n * 128 + c * 64, 64)
                v = jnp.concatenate([held(wq[k, pl.ds(row, 8), :], z),
                                     wq[k, pl.ds(row + 8, 56), :]], axis=0)
                w = 128 if k < 4 else 64
                wtmp[k, c * 128:c * 128 + w, :] = _up(v).astype(f32).T[0:w]

        def pair(k, r, z):
            v = [wtmp[k, c * 128 + r:c * 128 + r + 16, :] for c in range(2)]
            return [jnp.concatenate([held(u[0:8], z), u[8:]], axis=0) for u in v]
        for r in range(0, 64, 16):
            if r % 32 == 0:
                z = yield
            f = pair(4, r, z)
            for i, v in enumerate(f + [f[0] + f[1]]):
                wsb[n, 1792 + i * 64 + r:1792 + i * 64 + r + 16, :] = v.astype(bf16)
        for k in range(2):
            for r in range(0, 128, 16):
                if r % 32 == 0:
                    z = yield
                for i, t in enumerate(_rhs_terms([pair(k, r, z), pair(k + 2, r, z)])):
                    row = i * 256 + k * 128 + r
                    wsb[n, row:row + 16, :] = t()[0][0].astype(bf16)

    def ws_third(g):
        for n in range(3):
            yield from ws_prep(3 * g + n)

    def wo_prep():
        for n in range(5):
            w = 128 if n < 4 else 64
            wtmp[n, 0:D, 0:w] = wo_raw[:, n * 128:n * 128 + w].astype(f32)
        for n in range(5):
            w = 128 if n < 4 else 64
            for c in range(5):
                z = yield
                rows = [held(wtmp[n, pl.ds(4 * c + g + k * 8 * DH, 8, stride=DH), :], z)[:, 0:w]
                        for g in range(4 if c < 4 else 2) for k in range(4)]
                if c == 4:
                    rows = [jnp.zeros((64, w), f32)] + rows
                wob[c, n * 128:n * 128 + w, :] = jnp.concatenate(rows, axis=0).T.astype(bf16)

    def head_late():
        for cp in (wo_copy, x_copy(1)):
            cp.wait()
        for cp in [x_copy(2)] + chunk_copies(1):
            cp.start()
        yield from wo_prep()
        yield from widen(1)

    wqb[4, :, 64:128] = jnp.zeros((3 * D, 64), bf16)
    qkv[:, 13] = jnp.zeros((2, HALO + 128, 128), f32)
    xnb[:, 4, :, 64:128] = jnp.zeros((2, 128, 64), bf16)
    for n in range(4, 13):
        qkv[0, n, 0:HALO, :] = jnp.zeros((HALO, 128), f32)
    todo = list(k_order)
    for n, cp in enumerate(first):
        cp.wait()
        if n == OPT["dma"][0]:
            wo_copy.start()
        if n == OPT["dma"][1]:
            for c in [x_copy(1)] + chunk_copies(0):
                c.start()
        if n == OPT["xpos"]:
            feed(widen(0), None, 1000)
            flush(ln1(0, 0))
        else:
            wq_prep(todo.pop(0))
    attn_run(0, 2, OPT["h"], True, late=head_late(), head=True)

    @pl.loop(0, 7)
    def _(i):
        for cp in chunk_copies(i):
            cp.wait()

        @pl.when(i + 2 < NSLAB // 2)
        def _():
            x_copy(i + 2).wait()

        @pl.when(i + 3 < NSLAB // 2)
        def _():
            x_copy(i + 3).start()
        for cp in chunk_copies(i + 2):
            cp.start()
        side = prep_chunk(i, [r.at[i] for r in (wcb, web, wdcb)])
        next(side)
        r = jnp.clip(i - 2, 0, 3)
        attn_run(2 * i + 2, 2, OPT["p"], False, side, widen(jnp.minimum(i + 2, NSLAB // 2 - 1)),
                 ffn_norm_slab(r, r))

    for cp in chunk_copies(7) + chunk_copies(8):
        cp.wait()
    ffn_combos()

    def ffn_group(t, g, last, emit=None):
        ti = _Temps(tin)
        to = _Temps(tout)
        pace = Pace()
        o_ = OPT["fb" if last else "fa"]

        def weights(c):
            if last and c > 0:
                return [r.at[c - 1] for r in (wc2, we2, wdc2)]
            return [r.at[g * 3 + c] for r in (wc, we, wdc)]

        def proj(c, m):
            w, w_ext, _ = weights(c)

            def prod(o, i):
                r = (m * 49 + o * 7 + i) * 64
                p = jnp.dot(_up(ac[o * 7 + i]), _up(w[r:r + 64, :]),
                            preferred_element_type=f32)
                pace.step(p[0:8])
                if o in AUG and i in AUG:
                    q = AUG.index(o) * 4 + AUG.index(i)
                    e = jnp.dot(_up(ae[q, :, 0:64]), _up(w_ext[m * 16 + q]),
                                preferred_element_type=f32)
                    pace.step(e[0:8])
                    p = p + e
                return p
            return prod

        def gate(c):
            def fin(r, cc, v):
                gs[(c % 2) * 16 + r * 4 + cc] = v
            return _recombine(proj(c, 0), fin, ti, to)

        def upgate(c):
            def fin(r, cc, v):
                hs[c, r * 4 + cc] = _ld(gs, (c % 2) * 16 + r * 4 + cc) * v
            yield from _recombine(proj(c, 1), fin, ti, to, last)
            pace.add(hidden_paced(c), *o_["h"][c])

        hgen, hdone = {}, {}

        def hidden(c):
            for o in ORDER:
                yield from strips(lambda cc, r, rows: hs[c, r * 4 + cc, rows, :],
                                  _RHS_SPEC, _rhs_terms, o, hcb.at[c])

        def hidden_paced(c):
            hgen[c], hdone[c] = hidden(c), 0
            next(hgen[c])
            while True:
                z = yield
                need(c, min(hdone[c] + 1, 56), z)

        def need(c, n, z=None):
            feed(hgen[c], z, n - hdone[c])
            hdone[c] = max(hdone[c], n)

        def dprod(cs, i):
            p = None
            for c in cs:
                need(c, 8 * (ORDER.index(i // 7) + 1))
                r = i * (MB // 2)
                q = lax.dot_general(_up(weights(c)[2][r:r + MB // 2, :]), _up(hc[c, i]), NT,
                                    preferred_element_type=f32)
                pace.step(q[0:8])
                p = q if p is None else p + q
            return p

        def down(cs, reset):
            for i in [o * 7 + k for o in ORDER for k in range(7)]:
                a = _ld(acc, i)
                if reset:
                    a = jnp.where(g == 0, 0.0, a)
                acc[i] = a + dprod(cs, i)
                yield

        def down_final(cs):
            def fin(mb, r, v):
                rows = slice(mb * MB, (mb + 1) * MB)
                y = xb[t * 4 + r, rows, :] + v
                xa[t * 4 + r, rows, :] = y
                ost[t * 2 + r // 2, rows, (r % 2) * 128:(r % 2) * 128 + 128] = y.astype(bf16)
            return _recombine(lambda o, i: _ld(acc, o * 7 + i) + dprod(cs, o * 7 + i),
                              fin, _Temps(tin2), _Temps(tout2))

        if last:
            norm = ffn_norm((t + 1) % NTILE)
            pace.add(norm, o_["n0"], o_["nper"])
        else:
            late = prep_chunk(7 + g, [r.at[g] for r in (wcb2, web2, wdcb2)])
            next(late)
            pace.plan.append((late, _spread(o_["wts"], 30, NPREP), None, True))
            more = ws_third(g)
            next(more)
            pace.plan.append((more, _spread(o_["sw"], 30, 60), None, True))
        for gen in (gate(0), upgate(0), gate(1)):
            _adv(gen, 100)
        d0 = down((0,), not last)
        queue = []

        def lhs_queue():
            while True:
                z = yield
                if queue:
                    try:
                        queue[0].send(z)
                    except StopIteration:
                        queue.pop(0)
        for gen, plan in ((upgate(1), "u1"), (gate(2), "g2"), (upgate(2), "u2")):
            if last and plan == "u2":
                feed(norm, None, 1000)
                pace.add(lhs_queue(), o_["l0"], o_["lper"])
            for k, n in enumerate(o_[plan]):
                _adv(gen, 1)
                if last and plan == "u2":
                    queue.append(lhs_strips(ORDER[k]))
                    next(queue[-1])
                _adv(d0, n)
            _adv(gen, 100)
        _adv(d0, 100)
        if last:
            gen = down_final((1, 2))
            _adv(gen, 3)
            for q, h in ((1, 1), (0, 1), (1, 0), (0, 0)):
                _adv(gen, 1)
                pl.when(emit)(out_copy(t * 2 + q, h).start)
        else:
            _adv(down((1, 2), False), 100)
            feed(late, None, 1000)
            feed(more, None, 1000)
        for gen in queue:
            feed(gen, None, 1000)

    @pl.loop(0, 2 * NTILE)
    def _(tile):
        t = tile % NTILE

        @pl.loop(0, 2)
        def _(g):
            ffn_group(t, g, False)
        ffn_group(t, 2, True, tile >= NTILE)

        @pl.when(tile < NTILE)
        def _():
            attn_run(4 * t + NSLAB, 4, OPT["n"], True)

        @pl.when(tile == NTILE - 1)
        def _():
            out_proj(NSLAB - 2, 0, Pace())
            flush(attend(1, None))
            out_proj(NSLAB - 1, 1, Pace())

    for p in range(NSLAB):
        out_copy(p // 2, p % 2).wait()


def _tiles(w):
    n = w.shape[1]
    return w.reshape(NTR, 8, n // 128, 128).transpose(0, 2, 1, 3).reshape(NTR, n // 16, 128)


@jax.jit
def pallas_interleave_layers__sliding_local_dilated__glu_gated_bilinear__prompt_kernel(
    A_x: jax.Array,
    A_wqkv: jax.Array,
    A_wo: jax.Array,
    B_x: jax.Array,
    B_w_gate: jax.Array,
    B_w_up: jax.Array,
    B_w_down: jax.Array,
):
    del B_x
    vm = pltpu.VMEM
    hbm = pl.BlockSpec(memory_space=pl.ANY)
    out_t = pl.pallas_call(
        _kernel,
        in_specs=[hbm] * 6,
        out_specs=hbm,
        out_shape=jax.ShapeDtypeStruct((D, S), bf16),
        scratch_shapes=[
            vm((NSLAB // 2, 96, 16, 128), bf16),
            vm((NSLAB, 768, 128), f32),
            vm((NSLAB, 768, 128), f32),
            vm((NSLAB // 2, 768, 256), bf16),
            vm((NCHUNK, 224, 32, 128), bf16),
            vm((7, WC_ROWS, 128), bf16),
            vm((7, 32, 64, 128), bf16),
            vm((7, WD_ROWS, 128), bf16),
            vm((2, WC_ROWS, 128), bf16),
            vm((2, 32, 64, 128), bf16),
            vm((2, WD_ROWS, 128), bf16),
            vm((24, 128, 128), f32),
            vm((D, 3 * D), bf16),
            vm((D, D), bf16),
            vm((5, 3 * D, 128), f32),
            vm((5, 3 * D, 128), bf16),
            vm((5, D, 128), bf16),
            vm((2, 5, 128, 128), bf16),
            vm((2, 14, HALO + 128, 128), f32),
            vm((2, 5, 128, 128), bf16),
            vm((49, 128, 128), bf16),
            vm((16, 128, 128), bf16),
            vm((32, 128, 128), f32),
            vm((3, 16, 128, 128), f32),
            vm((3, 49, 128, 128), bf16),
            vm((49, MB, 128), f32),
            vm((12, 128, 128), f32),
            vm((40, 128, 128), f32),
            vm((12, MB, 128), f32),
            vm((20, MB, 128), f32),
            vm((64, 128), f32),
            vm((2, 11, 64, 128), bf16),
            vm((6, 1984, 128), bf16),
            vm((6, 64, 128), f32),
            pltpu.SMEM((1,), jnp.int32),
            pltpu.SemaphoreType.DMA((NSLAB // 2,)),
            pltpu.SemaphoreType.DMA((6,)),
            pltpu.SemaphoreType.DMA((NCHUNK, 3)),
            pltpu.SemaphoreType.DMA((NSLAB // 2, 2)),
        ],
        compiler_params=pltpu.CompilerParams(vmem_limit_bytes=122 * 1024 * 1024,
                                             disable_bounds_checks=True,
                                             disable_semaphore_checks=True),
    )(_tiles(A_x[0].T), A_wqkv, A_wo, _tiles(B_w_gate), _tiles(B_w_up), _tiles(B_w_down.T))
    return out_t.T[None]
```

```python
import math

import jax
import jax.numpy as jnp
from jax import lax
import jax.experimental.pallas as pl
import jax.experimental.pallas.tpu as pltpu

f32 = jnp.float32
bf16 = jnp.bfloat16
u32 = jnp.uint32

S, D, F = 2048, 576, 4608
H, DH, WIN, DIL = 32, 18, 8, 2
EPS = 1e-5
LOG2E = math.log2(math.e)
NSLAB = S // 128
TILE = 512
NTILE = S // TILE
FC = 512
NCHUNK = F // FC
MB = D // 4
HALO = 16
NPREP = 158
NTR = D // 8
WC_ROWS = 800 * 16
WD_ROWS = 448 * 16
NT = (((1,), (1,)), ((), ()))
ORDER = (0, 1, 2, 5, 3, 4, 6)
SUMS = (0, 1, 4, 5, 6)
AUG = (0, 1, 2, 5)

OPT = {'dma': (0, 2),
 'xpos': 2,
 'parts': (1, 0, 2),
 'fa': {'sw': (1, 4, 3, 0, 1, 1, 1, 0, 1, 2, 1, 1, 0, 1, 1, 1, 0, 1),
        'wts': (3, 1, 2, 0, 0, 1, 2, 1, 1, 1, 0, 0, 1, 1, 0, 5, 5, 4),
        'h': ((0, 0.7), (0, 1), (0, 1)),
        'u1': (0, 0, 0, 4, 5, 4, 6),
        'g2': (4, 0, 0, 0, 0, 0, 0),
        'u2': (0, 0, 0, 0, 3, 4, 4)},
 'fb': {'h': ((0, 0.85), (0, 0.68), (0, 0.7)),
        'n0': 0,
        'nper': 1.4,
        'l0': 0,
        'lper': 3.22,
        'u1': (0, 0, 0, 0, 4, 4, 6),
        'g2': (4, 0, 0, 0, 0, 0, 0),
        'u2': (0, 0, 0, 0, 4, 4, 4)},
 'h': {'lag': 0,
       'grp': ((4, 5, 6, 7), (0, 1, 2, 3), (12, 13, 8, 9, 10, 11)),
       'a': ((6, 5, 35), (0, 3.65, 40)),
       'w0': 22,
       'wper': 2.8,
       'ag': 1,
       'ls': ((0, 5.95, 40),)},
 'p': {'lag': 0,
       'sk': 1,
       's0': 4,
       'sper': 6.32,
       'x0': 36,
       'xper': 3.92,
       'grp': ((4, 13), (5, 6, 7, 0), (1, 2, 3, 12), (8, 9, 10, 11)),
       'a': ((3, 6, 25), (0, 5.44, 35)),
       'w0': 71,
       'wper': 4.88,
       'ag': 0,
       'ls': ((40, 6.29, None),),
       'wts': (9, 9, 5, 9, 9, 13, 5, 11, 9, 11, 7, 11, 7, 11, 7, 9)},
 'n': {'seq': (5, 6, 2, 0, 4, 1, 3),
       'lag': 1,
       'a': ((0, 6, 35), (0, 6, 35), (0, 6.84, 35), (0, 6, 35)),
       'ag': 1,
       'ls': ((77, 7.71, None), (69, 9.04, None), (80, 6.83, None))}}


def _up(v):
    return pltpu.bitcast(v, bf16)


def _quad(x):
    n = len(x) // 2
    return ([r[:n] for r in x[:n]], [r[n:] for r in x[:n]],
            [r[:n] for r in x[n:]], [r[n:] for r in x[n:]])


def _badd(x, y):
    return [[a + b for a, b in zip(r, s)] for r, s in zip(x, y)]


def _bsub(x, y):
    return [[a - b for a, b in zip(r, s)] for r, s in zip(x, y)]


def _lhs_terms(a):
    a11, a12, a21, a22 = _quad(a)
    return [lambda: _badd(a11, a22), lambda: _badd(a21, a22), lambda: a11, lambda: a22,
            lambda: _badd(a11, a12), lambda: _bsub(a21, a11), lambda: _bsub(a12, a22)]


def _rhs_terms(b):
    b11, b12, b21, b22 = _quad(b)
    return [lambda: _badd(b11, b22), lambda: b11, lambda: _bsub(b12, b22), lambda: _bsub(b21, b11),
            lambda: b22, lambda: _badd(b11, b12), lambda: _badd(b21, b22)]


def _combos(x, terms, emit):
    for o, fo in enumerate(terms(x)):
        y = fo()
        for i, fi in enumerate(terms(y)):
            emit(o * 7 + i, fi()[0][0])


_LHS_SPEC = (((0, 0), (1, 1), 1), ((1, 0), (1, 1), 1), ((0, 0), None, 0), ((1, 1), None, 0),
             ((0, 0), (0, 1), 1), ((1, 0), (0, 0), -1), ((0, 1), (1, 1), -1))
_RHS_SPEC = (((0, 0), (1, 1), 1), ((0, 0), None, 0), ((0, 1), (1, 1), -1), ((1, 0), (0, 0), -1),
             ((1, 1), None, 0), ((0, 0), (0, 1), 1), ((1, 0), (1, 1), 1))


def _outer_term(load, spec, o):
    p, q, sign = spec[o]
    out = []
    for y in range(2):
        row = []
        for z in range(2):
            v = load(2 * p[0] + y, 2 * p[1] + z)
            if sign:
                w = load(2 * q[0] + y, 2 * q[1] + z)
                v = v + w if sign > 0 else v - w
            row.append(v)
        out.append(row)
    return out


def _inner_terms(y, terms, o, emit):
    for i, fi in enumerate(terms(y)):
        emit(o * 7 + i, fi()[0][0])


def _lhs_ext(e):
    n = len(e) // 2
    return {0: e[:n], 1: e[n:], 2: e[:n], 5: [y - x for x, y in zip(e[:n], e[n:])]}


def _rhs_ext(e):
    n = len(e) // 2
    return {0: e[:n], 1: e[:n], 2: e[n:], 5: [x + y for x, y in zip(e[:n], e[n:])]}


def _ext_combos(e, fn, emit):
    for oi, o in enumerate(AUG):
        d = fn(fn(e)[o])
        for ii, i in enumerate(AUG):
            emit(oi * 4 + ii, d[i][0])


def _spread(weights, span, n):
    total, acc, out = sum(weights), 0.0, []
    for k, w in enumerate(weights):
        lo, acc = acc, acc + w * n / total
        count = round(acc) - round(lo)
        out += [k * span + i * span // count for i in range(count)]
    return out


def _adv(gen, n):
    for _ in range(n):
        try:
            next(gen)
        except StopIteration:
            return


def _ld(ref, idx):
    n = ref.shape[-2] // 2
    return jnp.concatenate([ref[idx, :n, :], ref[idx, n:, :]], axis=0)


class _Temps:
    def __init__(self, ref):
        self.ref = ref
        self.n = 0

    def put(self, v):
        i = self.n % self.ref.shape[0]
        self.n += 1
        self.ref[i] = v
        return i

    def get(self, i):
        return _ld(self.ref, i)


def _combine(prod, sink, ti, spill_last=False):
    a = ti.put(prod(0))
    b = ti.put(prod(1))
    c = ti.put(prod(2))
    sink(1, 1, ti.get(a) - ti.get(b) + ti.get(c) + prod(5))
    if spill_last:
        m3 = prod(3)
        m4 = prod(4)
        sink(1, 0, ti.get(b) + m3)
        sink(0, 1, ti.get(c) + m4)
        d = ti.put(ti.get(a) + m3 - m4)
        sink(0, 0, ti.get(d) + prod(6))
        return
    m3 = prod(3)
    m4 = prod(4)
    m6 = prod(6)
    sink(1, 0, ti.get(b) + m3)
    sink(0, 1, ti.get(c) + m4)
    sink(0, 0, ti.get(a) + m3 - m4 + m6)


def _recombine(prod, fin, ti, to, spill_last=False):
    def inner(o, sink):
        _combine(lambda i: prod(o, i), sink, ti, spill_last)

    m = {}
    for o in (0, 1, 2):
        def keep(y, z, v, o=o):
            m[o, y, z] = to.put(v)
        inner(o, keep)
        yield

    def s5(y, z, v):
        fin(2 + y, 2 + z, to.get(m[0, y, z]) - to.get(m[1, y, z]) + to.get(m[2, y, z]) + v)
    inner(5, s5)
    yield

    def s3(y, z, v):
        fin(2 + y, z, to.get(m[1, y, z]) + v)
        m[3, y, z] = to.put(to.get(m[0, y, z]) + v)
    inner(3, s3)
    yield

    def s4(y, z, v):
        fin(y, 2 + z, to.get(m[2, y, z]) + v)
        m[3, y, z] = to.put(to.get(m[3, y, z]) - v)
    inner(4, s4)
    yield

    def s6(y, z, v):
        fin(y, z, to.get(m[3, y, z]) + v)
    inner(6, s6)
    yield


def _kernel(xt_hbm, wqkv_hbm, wo_hbm, wg_hbm, wu_hbm, wdt_hbm, out_hbm,
            xin, xa, xb, ost, raw, wcb, web, wdcb, wcb2, web2, wdcb2, xn2,
            wq_raw, wo_raw, wtmp, wqb, wob, xnb, qkv, ob, acb, aeb, gs, hs, hcb, acc,
            tin, tout, tin2, tout2, ktail, xsb, wsb, tq, zero,
            sem_x, sem_w, sem_c, sem_o):
    wq, wo, wc, we, wdc, xn, o32, ac, ae, hc, raw32, xin32, wc2, we2, wdc2, xs, ws = [
        r.bitcast(u32) for r in (wqb, wob, wcb, web, wdcb, xnb, ob, acb, aeb, hcb, raw, xin,
                                 wcb2, web2, wdcb2, xsb, wsb)]

    def x_copy(q):
        return pltpu.make_async_copy(
            xt_hbm.at[:, pl.ds(pl.multiple_of(q * 16, 16), 16), :], xin.at[q, 0:NTR], sem_x.at[q])

    def weight_copy(j, m):
        rows = pl.ds(pl.multiple_of(j * 32, 32), 32)
        return pltpu.make_async_copy((wg_hbm, wu_hbm, wdt_hbm)[m].at[:, rows, :],
                                     raw.at[j, pl.ds(m * NTR, NTR)], sem_c.at[j, m])

    def chunk_copies(j):
        return [weight_copy(j, m) for m in range(3)]

    def out_copy(q, h):
        rows = pl.ds(h * 2 * MB, 2 * MB)
        return pltpu.make_async_copy(
            ost.at[q, rows, :], out_hbm.at[rows, pl.ds(pl.multiple_of(q * 256, 256), 256)],
            sem_o.at[q, h])

    k_order = (4, 0, 1, 2, 3)
    wq_copies = [pltpu.make_async_copy(wqkv_hbm.at[k * 128:min(k * 128 + 128, D)],
                                       wq_raw.at[k * 128:min(k * 128 + 128, D)], sem_w.at[k])
                 for k in k_order]
    wo_copy = pltpu.make_async_copy(wo_hbm, wo_raw, sem_w.at[5])
    first = wq_copies[:OPT["xpos"]] + [x_copy(0)] + wq_copies[OPT["xpos"]:]
    for cp in first:
        cp.start()
    zero[0] = 0
    never = zero[0] != 0

    def held(v, z):
        if z is None:
            return v
        return jnp.where(never, pltpu.bitcast(z, v.dtype), v)

    def raw_pair(j, tr, cp, z):
        v = [_up(held(raw32[j, tr + k, cp * 8:cp * 8 + 8, :], z)).astype(f32) for k in range(2)]
        return [jnp.concatenate([v[0][h:h + 8], v[1][h:h + 8]], axis=0) for h in (0, 8)]

    def prep_strip(j, tr, step, spec, terms, path, emit):
        live = {}
        for o in path:
            used = [q for q in spec[o][:2] if q is not None]
            live = {q: live[q] for q in used if q in live}
            for q in used:
                if q not in live:
                    z = yield
                    live[q] = [raw_pair(j, tr + (2 * q[0] + y) * step, q[1], z) for y in range(2)]
            y = _outer_term(lambda r, c: live[r // 2, c // 2][r % 2][c % 2], spec, o)
            _inner_terms(y, terms, o, emit)

    def prep_gu(j, dst, m, s):
        base = m * (49 * 128) + s * 16

        def emit(i, v):
            dst[pl.ds(base + i * 128, 16), :] = v.astype(bf16)
        return prep_strip(j, m * NTR + 2 * s, 16, _RHS_SPEC, _rhs_terms,
                          (1, 0, 4, 2, 5, 3, 6), emit)

    def prep_ext(j, dst, m, s):
        z = yield
        tr = m * NTR + 64 + 2 * s

        def emit(i, v):
            dst[m * 16 + i, pl.ds(s * 16, 16), :] = v.astype(bf16)
        _ext_combos(raw_pair(j, tr, 0, z) + raw_pair(j, tr, 1, z), _rhs_ext, emit)

    def prep_down(j, dst, s):
        def emit(i, v):
            dst[pl.ds(s * 16 + i * MB, 16), :] = v.astype(bf16)
        return prep_strip(j, 2 * NTR + 2 * s, MB // 8, _LHS_SPEC, _lhs_terms,
                          (2, 0, 3, 6, 4, 5, 1), emit)

    def prep_chunk(j, dst):
        for m in range(2):
            for s in range(8):
                yield from prep_gu(j, dst[0], m, s)
            for s in range(4):
                yield from prep_ext(j, dst[1], m, s)
        for s in range(9):
            yield from prep_down(j, dst[2], s)

    def feed(gen, z, n):
        for _ in range(n):
            try:
                gen.send(z)
            except StopIteration:
                return

    class Pace:
        def __init__(self):
            self.tok = 0
            self.plan = []
            self.due = []

        def add(self, gen, t0, period, lat=None, gated=True):
            next(gen)
            when = [self.tok + int(t0 + k * period) for k in range(1000)]
            self.plan.append((gen, when, lat, gated))

        def step(self, z):
            for gen, when, lat, gated in self.plan:
                for _ in range(when.count(self.tok)):
                    try:
                        v = gen.send(z if gated else None)
                    except StopIteration:
                        break
                    if v is not None and lat is not None:
                        self.due.append((self.tok + lat, v))
            self.tok += 1

        def tokens(self, r, n):
            for k in range(n):
                self.step(r[k * 16:k * 16 + 8])

        def gate(self, v):
            now = [x for t, x in self.due if t <= self.tok]
            self.due = [(t, x) for t, x in self.due if t > self.tok]
            if not now:
                return v
            head = jnp.where(never, pltpu.bitcast(tree(now), u32), v[0:8])
            return jnp.concatenate([head, v[8:]], axis=0)

        def drain(self):
            for gen, *_ in self.plan:
                feed(gen, None, 1000)

    def tree(vals):
        while len(vals) > 1:
            vals = [a + b for a, b in zip(vals[::2], vals[1::2])] + vals[len(vals) & ~1:]
        return vals[0]

    def norm_slab(row, emit, order=(4, 0, 1, 2, 3)):
        def rows(k, lo, hi):
            return [row(k, r) for r in range(lo // 8, hi // 8)]

        def mean(vals):
            t = tree([sum(vals[k + 4::4], vals[k]) for k in range(4)])
            t = jnp.sum(t, axis=0, keepdims=True) * (1.0 / D)
            return jnp.broadcast_to(t, (8, 128))
        z = yield
        x = rows(0, 0, D)
        mu = mean([held(v, z) for v in x[:4]] + x[4:])
        m = held(mu, (yield))
        rs = lax.rsqrt(mean([(v - m) * (v - m) for v in rows(1, 0, D)]) + EPS)
        end = None
        for k in order:
            m = held(mu, (yield end))
            y = jnp.concatenate(
                [(v - m) * rs for v in rows(2, k * 128, min((k + 1) * 128, D))], axis=0).T
            emit(k, y)
            end = y[120:128] if k < 4 else jnp.concatenate([y[120:128]] * 2, axis=1)
        yield end

    def alias(p, n):
        return [jnp.clip(p + k * zero[0], 0, n - 1) for k in range(3)]

    def slab_rows(src, p):
        q = alias(p, NSLAB)
        return lambda k, r: src[q[k], r * 8:r * 8 + 8, :]

    def flush(gen):
        return tree([v for v in gen if v is not None])

    def ln1(p, b, fast=False):
        seen = {}

        def emit(k, y):
            xnb[b, k, :, 0:y.shape[1]] = y.astype(bf16)
            seen[k] = y
            if fast and k == 4:
                xsb[b, 10, :, 0:64] = (y[64:] - y[:64]).astype(bf16)
            if fast and k in (2, 3):
                u = seen[k - 2]
                terms = _lhs_terms([[u[:64], y[:64]], [u[64:], y[64:]]])
                for n, i in enumerate(SUMS):
                    xsb[b, 2 * n + k - 2] = terms[i]()[0][0].astype(bf16)
        return norm_slab(slab_rows(xa, p), emit, (4, 0, 2, 1, 3) if fast else (4, 0, 1, 2, 3))

    def widen(q):
        for r in range(NTR):
            if r % 4 == 0:
                z = yield
            v = _up(held(xin32[q, r], z)).astype(f32)
            for b in range(2):
                xa[2 * q + b, r * 8:r * 8 + 8, :] = v[b * 8:b * 8 + 8]

    def qkv_proj(b, pace, groups):
        scale = DH ** -0.5 * LOG2E
        for grp in groups:
            for n in grp:
                if n == 13:
                    ktail[...] = lax.dot_general(
                        _up(wq[4, n * 64:n * 64 + 32, :]), _up(xn[b, 4]), NT,
                        preferred_element_type=f32)
                else:
                    qkv[b, n, HALO:HALO + 128, :] = lax.dot_general(
                        _up(xn[b, 4]), _up(wq[4, n * 64:(n + 1) * 64, :]), NT,
                        preferred_element_type=f32)
            for n in grp:
                rows = slice(n * 64, n * 64 + (32 if n == 13 else 64))
                x = jnp.concatenate(
                    [_up(pace.gate(xn[b, 0]))] + [_up(xn[b, k]) for k in range(1, 4)], axis=1)
                w = jnp.concatenate([_up(wq[k, rows, :]) for k in range(4)], axis=1)
                if n == 13:
                    r = lax.dot_general(w, x, NT, preferred_element_type=f32)
                    r = r + jnp.concatenate([ktail[0:32, :], ktail[32:64, :]], axis=0)
                    qkv[b, n, HALO:HALO + 128, 0:64] = (r * scale).T
                    pace.tokens(r, 4)
                    continue
                r = lax.dot_general(x, w, NT, preferred_element_type=f32)
                r = r + jnp.concatenate([qkv[b, n, HALO:HALO + 64, :],
                                         qkv[b, n, HALO + 64:HALO + 128, :]], axis=0)
                if n in (4, 5, 6, 7):
                    r = r * scale
                qkv[b, n, HALO:HALO + 128, :] = r
                pace.tokens(r, 7)

    def qkv_pair(b, pace, n, ti):
        def prod(i):
            if i in SUMS:
                x = [xs[b, 2 * SUMS.index(i) + k] for k in range(2)]
            else:
                h = i - 2
                x = [xn[b, 2 * h + k, h * 32:h * 32 + 32, :] for k in range(2)]
            x = jnp.concatenate([_up(pace.gate(x[0])), _up(x[1])], axis=1)
            r = jnp.dot(x, _up(ws[n, i * 128:(i + 1) * 128, :]), preferred_element_type=f32)
            pace.tokens(r, 2)
            if i in AUG:
                e = xs[b, 10, :, 0:64] if i == 5 else xn[b, 4, (i % 2) * 32:(i % 2) * 32 + 32, 0:64]
                f = 896 + 32 * {0: 0, 1: 0, 2: 1, 5: 2}[i]
                r = r + jnp.dot(_up(e), _up(ws[n, f:f + 32, :]), preferred_element_type=f32)
            return r

        def sink(y, z, v):
            if n in (2, 3):
                v = v * (DH ** -0.5 * LOG2E)
            qkv[b, 2 * n + z, HALO + y * 64:HALO + y * 64 + 64, :] = v
        _combine(prod, sink, ti)

    def halo(b):
        for n in range(4, 14):
            qkv[b, n, 0:HALO, :] = qkv[1 - b, n, 128:128 + HALO, :]

    def attend(b, row0, lag=0):
        qs, ks, vs = (0, 1, 2, 3, 12), (4, 5, 6, 7, 13), (8, 9, 10, 11, 12)

        def scores(s, z):
            r = HALO + s * 8
            q = [held(qkv[b, n, r:r + 8, :], z) for n in qs]
            logit = []
            for w in range(WIN):
                rw = r - DIL * w
                part = tree([q[c] * qkv[b, ks[c], rw:rw + 8, :] for c in range(5)])
                part = part + pltpu.roll(part, 64, 1)
                part = part + pltpu.roll(part, 32, 1)
                if row0 is not None and s * 8 < DIL * w:
                    pos = row0 + s * 8 + lax.broadcasted_iota(jnp.int32, (8, 128), 0)
                    part = jnp.where(pos >= DIL * w, part, -1e9 * LOG2E)
                logit.append(part)
            return logit

        def values(s, logit, z):
            r = HALO + s * 8
            mx = logit
            while len(mx) > 1:
                mx = [jnp.maximum(a, c) for a, c in zip(mx[::2], mx[1::2])]
            top = held(mx[0], z)
            e = [jnp.exp2(l - top) for l in logit]
            inv = 1.0 / tree(e)
            outs = []
            for c in range(5):
                o = e[0] * qkv[b, vs[c], r:r + 8, :]
                for w in range(1, WIN):
                    rw = r - DIL * w
                    o = o + e[w] * qkv[b, vs[c], rw:rw + 8, :]
                o = o * inv
                outs.append(o)
                ob[b, c, s * 8:(s + 1) * 8, :] = o.astype(bf16)
            return tree(outs)

        v, pending = None, []
        for s in range(16 + lag):
            z = yield v
            if s < 16:
                pending.append(scores(s, z))
            if s >= lag:
                v = values(s - lag, pending.pop(0), z if lag else None)
        yield v

    def out_proj(p, b, pace):
        h = MB // 2
        for m in range(4):
            xb[p, m * MB:(m + 1) * MB, :] = xa[p, m * MB:(m + 1) * MB, :] + lax.dot_general(
                _up(wo[4, m * h:(m + 1) * h, :]), _up(o32[b, 4]), NT, preferred_element_type=f32)
        rhs = jnp.concatenate([_up(o32[b, c]) for c in range(4)], axis=1)
        for m in range(4):
            rows = slice(m * h, (m + 1) * h)
            lhs = jnp.concatenate(
                [_up(pace.gate(wo[0, rows, :]))] + [_up(wo[c, rows, :]) for c in range(1, 4)],
                axis=1)
            r = lax.dot_general(lhs, rhs, NT, preferred_element_type=f32)
            r = r + jnp.concatenate([xb[p, m * MB:m * MB + h, :],
                                     xb[p, m * MB + h:(m + 1) * MB, :]], axis=0)
            xb[p, m * MB:(m + 1) * MB, :] = r
            pace.tokens(r, 8)

    def ffn_norm_slab(p, r):
        def emit(k, y):
            xn2[r * 6 + k, :, 0:y.shape[1]] = y
        return norm_slab(slab_rows(xb, p), emit)

    def ffn_norm(t):
        for r in range(4):
            yield from ffn_norm_slab(t * 4 + r, r)

    def strips(load, spec, terms, o, dst):
        for s in range(8):
            z = yield
            rows = slice(s * 16, (s + 1) * 16)

            def ld(r, c):
                v = load(r, c, rows)
                if (r // 2, c // 2) == spec[o][0]:
                    v = jnp.concatenate([held(v[0:8], z), held(v[8:16], z)], axis=0)
                return v

            def emit(i, v):
                dst[i, rows, :] = v.astype(bf16)
            _inner_terms(_outer_term(ld, spec, o), terms, o, emit)

    def lhs_strips(o):
        yield from strips(lambda r, k, rows: xn2[r * 6 + k, rows, :],
                          _LHS_SPEC, _lhs_terms, o, acb)
        if o in AUG:
            for s in range(2):
                z = yield
                rows = slice(s * 64, (s + 1) * 64)
                d = _lhs_ext(_lhs_ext([xn2[r * 6 + 4, rows, 0:64] for r in range(4)])[o])
                for ii, i in enumerate(AUG):
                    aeb[AUG.index(o) * 4 + ii, rows, 0:64] = d[i][0].astype(bf16)

    def ffn_combos():
        for s in range(8):
            rows = slice(s * 16, (s + 1) * 16)
            a = [[xn2[r * 6 + k, rows, :] for k in range(4)] for r in range(4)]

            def emit(i, v, rows=rows):
                acb[i, rows, :] = v.astype(bf16)
            _combos(a, _lhs_terms, emit)
            e = [xn2[r * 6 + 4, rows, 0:64] for r in range(4)]

            def emit_e(i, v, rows=rows):
                aeb[i, rows, 0:64] = v.astype(bf16)
            _ext_combos(e, _lhs_ext, emit_e)

    def attn_run(h, count, o, mask, side=None, late=None, extra=None, more=None,
                 head=False):
        fast = "seq" in o
        if not head:
            flush(ln1(h % NSLAB, 0, fast))
        for k in range(count):
            b = k % 2
            pace = Pace()
            if side is not None:
                when = [w - k * 128 for w in _spread(o["wts"], 16, NPREP)]
                pace.plan.append((side, [min(w, 126) for w in when if 0 <= w < 128], None, True))
            if k + 1 < count:
                pace.add(ln1((h + k + 1) % NSLAB, 1 - b, fast), *o["ls"][k])
            elif late is not None:
                pace.add(late, o["w0"], o["wper"])
            if k == 1 and extra is not None:
                pace.add(extra, 32 + o["x0"], o["xper"])
            if k == o.get("sk") and more is not None:
                pace.add(more, o["s0"], o["sper"])
            if k > 0 or not head:
                row0 = (h % NSLAB) * 128 if k == 1 and mask else None
                pace.add(attend(1 - b, row0, o["lag"]), *o["a"][k], o["ag"])
                if not head:
                    out_proj((h + k - 2) % NSLAB, b, pace)
                halo(b)
            if fast:
                ti = _Temps(tq)
                for n in o["seq"]:
                    if n < 6:
                        qkv_pair(b, pace, n, ti)
                    else:
                        qkv_proj(b, pace, ((12, 13),))
            else:
                qkv_proj(b, pace, o["grp"])
            pace.plan = [e for e in pace.plan if e[0] is not side]
            pace.drain()
        if side is not None:
            feed(side, None, 1000)

    def wq_prep(k):
        w = 128 if k < 4 else 64
        for c0 in range(0, 3 * D, 128):
            c1 = min(c0 + 128, 3 * D)
            wtmp[k, c0:c1, 0:w] = wq_raw[k * 128:k * 128 + w, c0:c1].astype(f32).T
        for part in OPT["parts"]:
            for d in range(DH):
                if d < 16:
                    row = part * 512 + d * 32
                else:
                    row = (1536, 1664, 1600)[part] + (d - 16) * 32
                wqb[k, row:row + 32, 0:w] = wtmp[
                    k, pl.ds(part * D + d, H, stride=DH), 0:w].astype(bf16)

    def ws_flip(n):
        for k in range(5):
            for c in range(2):
                z = yield
                row = pl.multiple_of(n * 128 + c * 64, 64)
                v = jnp.concatenate([held(wq[k, pl.ds(row, 8), :], z),
                                     wq[k, pl.ds(row + 8, 56), :]], axis=0)
                w = 128 if k < 4 else 64
                wtmp[k, pl.ds(pl.multiple_of(2 * row, 128), w), :] = _up(v).astype(f32).T[0:w]

    def ws_prep(g):
        def pair(n, k, r, z):
            v = [wtmp[k, pl.ds(pl.multiple_of(n * 256 + c * 128 + r, 16), 16), :]
                 for c in range(2)]
            return [jnp.concatenate([held(u[0:8], z), u[8:]], axis=0) for u in v]
        for n in [3 * g + j for j in range(3)]:
            for r in range(0, 64, 16):
                if r % 32 == 0:
                    z = yield
                f = pair(n, 4, r, z)
                for i, v in enumerate(f + [f[0] + f[1]]):
                    wsb[n, 1792 + i * 64 + r:1792 + i * 64 + r + 16, :] = v.astype(bf16)
            for k in range(2):
                for r in range(0, 128, 16):
                    if r % 32 == 0:
                        z = yield
                    for i, t in enumerate(_rhs_terms([pair(n, k, r, z), pair(n, k + 2, r, z)])):
                        row = i * 256 + k * 128 + r
                        wsb[n, row:row + 16, :] = t()[0][0].astype(bf16)

    def wo_prep():
        for n in range(5):
            w = 128 if n < 4 else 64
            wtmp[n, 0:D, 0:w] = wo_raw[:, n * 128:n * 128 + w].astype(f32)
        for n in range(5):
            w = 128 if n < 4 else 64
            for c in range(5):
                z = yield
                rows = [held(wtmp[n, pl.ds(4 * c + g + k * 8 * DH, 8, stride=DH), :], z)[:, 0:w]
                        for g in range(4 if c < 4 else 2) for k in range(4)]
                if c == 4:
                    rows = [jnp.zeros((64, w), f32)] + rows
                wob[c, n * 128:n * 128 + w, :] = jnp.concatenate(rows, axis=0).T.astype(bf16)

    def head_late():
        for cp in (wo_copy, x_copy(1)):
            cp.wait()
        for cp in [x_copy(2)] + chunk_copies(1):
            cp.start()
        yield from wo_prep()
        yield from widen(1)

    wqb[4, :, 64:128] = jnp.zeros((3 * D, 64), bf16)
    qkv[:, 13] = jnp.zeros((2, HALO + 128, 128), f32)
    xnb[:, 4, :, 64:128] = jnp.zeros((2, 128, 64), bf16)
    for n in range(4, 13):
        qkv[0, n, 0:HALO, :] = jnp.zeros((HALO, 128), f32)
    todo = list(k_order)
    for n, cp in enumerate(first):
        cp.wait()
        if n == OPT["dma"][0]:
            wo_copy.start()
        if n == OPT["dma"][1]:
            for c in [x_copy(1)] + chunk_copies(0):
                c.start()
        if n == OPT["xpos"]:
            feed(widen(0), None, 1000)
            flush(ln1(0, 0))
        else:
            wq_prep(todo.pop(0))
    attn_run(0, 2, OPT["h"], True, late=head_late(), head=True)

    @pl.loop(0, 7)
    def _(i):
        for cp in chunk_copies(i):
            cp.wait()

        @pl.when(i + 2 < NSLAB // 2)
        def _():
            x_copy(i + 2).wait()

        @pl.when(i + 3 < NSLAB // 2)
        def _():
            x_copy(i + 3).start()
        for cp in chunk_copies(i + 2):
            cp.start()
        side = prep_chunk(i, [r.at[i] for r in (wcb, web, wdcb)])
        next(side)
        r = jnp.clip(i - 2, 0, 3)
        attn_run(2 * i + 2, 2, OPT["p"], False, side, widen(jnp.minimum(i + 2, NSLAB // 2 - 1)),
                 ffn_norm_slab(r, r), ws_flip(jnp.minimum(i, 5)))

    for cp in chunk_copies(7) + chunk_copies(8):
        cp.wait()
    ffn_combos()

    def ffn_group(t, g, last, emit=None):
        ti = _Temps(tin)
        to = _Temps(tout)
        pace = Pace()
        o_ = OPT["fb" if last else "fa"]

        def weights(c):
            if last and c > 0:
                return [r.at[c - 1] for r in (wc2, we2, wdc2)]
            return [r.at[g * 3 + c] for r in (wc, we, wdc)]

        def proj(c, m):
            w, w_ext, _ = weights(c)

            def prod(o, i):
                r = (m * 49 + o * 7 + i) * 64
                p = jnp.dot(_up(ac[o * 7 + i]), _up(w[r:r + 64, :]),
                            preferred_element_type=f32)
                pace.step(p[0:8])
                if o in AUG and i in AUG:
                    q = AUG.index(o) * 4 + AUG.index(i)
                    e = jnp.dot(_up(ae[q, :, 0:64]), _up(w_ext[m * 16 + q]),
                                preferred_element_type=f32)
                    pace.step(e[0:8])
                    p = p + e
                return p
            return prod

        def gate(c):
            def fin(r, cc, v):
                gs[(c % 2) * 16 + r * 4 + cc] = v
            return _recombine(proj(c, 0), fin, ti, to)

        def upgate(c):
            def fin(r, cc, v):
                hs[c, r * 4 + cc] = _ld(gs, (c % 2) * 16 + r * 4 + cc) * v
            yield from _recombine(proj(c, 1), fin, ti, to, last)
            pace.add(hidden_paced(c), *o_["h"][c])

        hgen, hdone = {}, {}

        def hidden(c):
            for o in ORDER:
                yield from strips(lambda cc, r, rows: hs[c, r * 4 + cc, rows, :],
                                  _RHS_SPEC, _rhs_terms, o, hcb.at[c])

        def hidden_paced(c):
            hgen[c], hdone[c] = hidden(c), 0
            next(hgen[c])
            while True:
                z = yield
                need(c, min(hdone[c] + 1, 56), z)

        def need(c, n, z=None):
            feed(hgen[c], z, n - hdone[c])
            hdone[c] = max(hdone[c], n)

        def dprod(cs, i):
            p = None
            for c in cs:
                need(c, 8 * (ORDER.index(i // 7) + 1))
                r = i * (MB // 2)
                q = lax.dot_general(_up(weights(c)[2][r:r + MB // 2, :]), _up(hc[c, i]), NT,
                                    preferred_element_type=f32)
                pace.step(q[0:8])
                p = q if p is None else p + q
            return p

        def down(cs, reset):
            for i in [o * 7 + k for o in ORDER for k in range(7)]:
                a = _ld(acc, i)
                if reset:
                    a = jnp.where(g == 0, 0.0, a)
                acc[i] = a + dprod(cs, i)
                yield

        def down_final(cs):
            def fin(mb, r, v):
                rows = slice(mb * MB, (mb + 1) * MB)
                y = xb[t * 4 + r, rows, :] + v
                xa[t * 4 + r, rows, :] = y
                ost[t * 2 + r // 2, rows, (r % 2) * 128:(r % 2) * 128 + 128] = y.astype(bf16)
            return _recombine(lambda o, i: _ld(acc, o * 7 + i) + dprod(cs, o * 7 + i),
                              fin, _Temps(tin2), _Temps(tout2))

        if last:
            norm = ffn_norm((t + 1) % NTILE)
            pace.add(norm, o_["n0"], o_["nper"])
        else:
            late = prep_chunk(7 + g, [r.at[g] for r in (wcb2, web2, wdcb2)])
            next(late)
            pace.plan.append((late, _spread(o_["wts"], 30, NPREP), None, True))
            more = ws_prep(g)
            next(more)
            pace.plan.append((more, _spread(o_["sw"], 30, 30), None, True))
        for gen in (gate(0), upgate(0), gate(1)):
            _adv(gen, 100)
        d0 = down((0,), not last)
        queue = []

        def lhs_queue():
            while True:
                z = yield
                if queue:
                    try:
                        queue[0].send(z)
                    except StopIteration:
                        queue.pop(0)
        for gen, plan in ((upgate(1), "u1"), (gate(2), "g2"), (upgate(2), "u2")):
            if last and plan == "u2":
                feed(norm, None, 1000)
                pace.add(lhs_queue(), o_["l0"], o_["lper"])
            for k, n in enumerate(o_[plan]):
                _adv(gen, 1)
                if last and plan == "u2":
                    queue.append(lhs_strips(ORDER[k]))
                    next(queue[-1])
                _adv(d0, n)
            _adv(gen, 100)
        _adv(d0, 100)
        if last:
            gen = down_final((1, 2))
            _adv(gen, 3)
            for q, h in ((1, 1), (0, 1), (1, 0), (0, 0)):
                _adv(gen, 1)
                pl.when(emit)(out_copy(t * 2 + q, h).start)
        else:
            _adv(down((1, 2), False), 100)
            feed(late, None, 1000)
            feed(more, None, 1000)
        for gen in queue:
            feed(gen, None, 1000)

    @pl.loop(0, 2 * NTILE)
    def _(tile):
        t = tile % NTILE

        @pl.loop(0, 2)
        def _(g):
            ffn_group(t, g, False)
        ffn_group(t, 2, True, tile >= NTILE)

        @pl.when(tile < NTILE)
        def _():
            attn_run(4 * t + NSLAB, 4, OPT["n"], True)

        @pl.when(tile == NTILE - 1)
        def _():
            out_proj(NSLAB - 2, 0, Pace())
            flush(attend(1, None))
            out_proj(NSLAB - 1, 1, Pace())

    for p in range(NSLAB):
        out_copy(p // 2, p % 2).wait()


def _tiles(w):
    n = w.shape[1]
    return w.reshape(NTR, 8, n // 128, 128).transpose(0, 2, 1, 3).reshape(NTR, n // 16, 128)


@jax.jit
def pallas_interleave_layers__sliding_local_dilated__glu_gated_bilinear__prompt_kernel(
    A_x: jax.Array,
    A_wqkv: jax.Array,
    A_wo: jax.Array,
    B_x: jax.Array,
    B_w_gate: jax.Array,
    B_w_up: jax.Array,
    B_w_down: jax.Array,
):
    del B_x
    vm = pltpu.VMEM
    hbm = pl.BlockSpec(memory_space=pl.ANY)
    out_t = pl.pallas_call(
        _kernel,
        in_specs=[hbm] * 6,
        out_specs=hbm,
        out_shape=jax.ShapeDtypeStruct((D, S), bf16),
        scratch_shapes=[
            vm((NSLAB // 2, 96, 16, 128), bf16),
            vm((NSLAB, 768, 128), f32),
            vm((NSLAB, 768, 128), f32),
            vm((NSLAB // 2, 768, 256), bf16),
            vm((NCHUNK, 224, 32, 128), bf16),
            vm((7, WC_ROWS, 128), bf16),
            vm((7, 32, 64, 128), bf16),
            vm((7, WD_ROWS, 128), bf16),
            vm((2, WC_ROWS, 128), bf16),
            vm((2, 32, 64, 128), bf16),
            vm((2, WD_ROWS, 128), bf16),
            vm((24, 128, 128), f32),
            vm((D, 3 * D), bf16),
            vm((D, D), bf16),
            vm((5, 3 * D, 128), f32),
            vm((5, 3 * D, 128), bf16),
            vm((5, D, 128), bf16),
            vm((2, 5, 128, 128), bf16),
            vm((2, 14, HALO + 128, 128), f32),
            vm((2, 5, 128, 128), bf16),
            vm((49, 128, 128), bf16),
            vm((16, 128, 128), bf16),
            vm((32, 128, 128), f32),
            vm((3, 16, 128, 128), f32),
            vm((3, 49, 128, 128), bf16),
            vm((49, MB, 128), f32),
            vm((12, 128, 128), f32),
            vm((40, 128, 128), f32),
            vm((12, MB, 128), f32),
            vm((20, MB, 128), f32),
            vm((64, 128), f32),
            vm((2, 11, 64, 128), bf16),
            vm((6, 1984, 128), bf16),
            vm((6, 64, 128), f32),
            pltpu.SMEM((1,), jnp.int32),
            pltpu.SemaphoreType.DMA((NSLAB // 2,)),
            pltpu.SemaphoreType.DMA((6,)),
            pltpu.SemaphoreType.DMA((NCHUNK, 3)),
            pltpu.SemaphoreType.DMA((NSLAB // 2, 2)),
        ],
        compiler_params=pltpu.CompilerParams(vmem_limit_bytes=122 * 1024 * 1024,
                                             disable_bounds_checks=True,
                                             disable_semaphore_checks=True),
    )(_tiles(A_x[0].T), A_wqkv, A_wo, _tiles(B_w_gate), _tiles(B_w_up), _tiles(B_w_down.T))
    return out_t.T[None]
```

```python
import math

import jax
import jax.numpy as jnp
from jax import lax
import jax.experimental.pallas as pl
import jax.experimental.pallas.tpu as pltpu

f32 = jnp.float32
bf16 = jnp.bfloat16
u32 = jnp.uint32

S, D, F = 2048, 576, 4608
H, DH, WIN, DIL = 32, 18, 8, 2
EPS = 1e-5
LOG2E = math.log2(math.e)
NSLAB = S // 128
TILE = 512
NTILE = S // TILE
FC = 512
NCHUNK = F // FC
MB = D // 4
HALO = 16
NPREP = 158
NTR = D // 8
WC_ROWS = 800 * 16
WD_ROWS = 448 * 16
NT = (((1,), (1,)), ((), ()))
ORDER = (0, 1, 2, 5, 3, 4, 6)
SUMS = (0, 1, 4, 5, 6)
AUG = (0, 1, 2, 5)

OPT = {'dma': (0, 2),
 'xpos': 2,
 'parts': (1, 0, 2),
 'fa': {'sw': (1, 5, 1, 0, 1, 1, 1, 0, 1, 1, 1, 1, 0, 2, 1, 0, 0, 2),
        'wts': (3, 1, 2, 0, 0, 1, 2, 1, 1, 1, 0, 0, 1, 1, 0, 5, 5, 4),
        'h': ((0, 0.7), (0, 1), (0, 1)),
        'u1': (0, 0, 0, 4, 5, 4, 6),
        'g2': (4, 0, 0, 0, 0, 0, 0),
        'u2': (0, 0, 0, 0, 3, 4, 4)},
 'fb': {'h': ((0, 0.85), (0, 0.68), (0, 0.7)),
        'n0': 0,
        'nper': 1.4,
        'l0': 0,
        'lper': 3.22,
        'u1': (0, 0, 0, 0, 4, 4, 6),
        'g2': (4, 0, 0, 0, 0, 0, 0),
        'u2': (0, 0, 0, 0, 4, 4, 4)},
 'h': {'lag': 1,
       'grp': ((13, 4, 5, 6, 7, 0), (1, 2, 3, 12), (8, 9, 10, 11)),
       'a': ((6, 5, 35), (0, 3.69, 40)),
       'w0': 22,
       'wper': 2.8,
       'ag': 1,
       'ls': ((8, 9.58, None),)},
 'p': {'lag': 0,
       'sk': 1,
       's0': 4,
       'sper': 6.32,
       'x0': 36,
       'xper': 3.92,
       'grp': ((4, 13), (5, 6, 7, 0), (1, 2, 3, 12), (8, 9, 10, 11)),
       'a': ((3, 6, 25), (0, 5.44, 35)),
       'w0': 71,
       'wper': 4.88,
       'ag': 0,
       'ls': ((40, 6.29, None),),
       'wts': (9, 9, 5, 9, 9, 13, 5, 11, 11, 7, 7, 11, 7, 11, 7, 9)},
 'n': {'seq': (5, 6, 2, 0, 4, 1, 3),
       'lag': 1,
       'a': ((0, 6, 35), (0, 6, 35), (0, 6.84, 35), (0, 6, 35)),
       'ag': 1,
       'ls': ((77, 7.71, None), (69, 9.04, None), (80, 6.83, None))}}


def _up(v):
    return pltpu.bitcast(v, bf16)


def _quad(x):
    n = len(x) // 2
    return ([r[:n] for r in x[:n]], [r[n:] for r in x[:n]],
            [r[:n] for r in x[n:]], [r[n:] for r in x[n:]])


def _badd(x, y):
    return [[a + b for a, b in zip(r, s)] for r, s in zip(x, y)]


def _bsub(x, y):
    return [[a - b for a, b in zip(r, s)] for r, s in zip(x, y)]


def _lhs_terms(a):
    a11, a12, a21, a22 = _quad(a)
    return [lambda: _badd(a11, a22), lambda: _badd(a21, a22), lambda: a11, lambda: a22,
            lambda: _badd(a11, a12), lambda: _bsub(a21, a11), lambda: _bsub(a12, a22)]


def _rhs_terms(b):
    b11, b12, b21, b22 = _quad(b)
    return [lambda: _badd(b11, b22), lambda: b11, lambda: _bsub(b12, b22), lambda: _bsub(b21, b11),
            lambda: b22, lambda: _badd(b11, b12), lambda: _badd(b21, b22)]


def _combos(x, terms, emit):
    for o, fo in enumerate(terms(x)):
        y = fo()
        for i, fi in enumerate(terms(y)):
            emit(o * 7 + i, fi()[0][0])


_LHS_SPEC = (((0, 0), (1, 1), 1), ((1, 0), (1, 1), 1), ((0, 0), None, 0), ((1, 1), None, 0),
             ((0, 0), (0, 1), 1), ((1, 0), (0, 0), -1), ((0, 1), (1, 1), -1))
_RHS_SPEC = (((0, 0), (1, 1), 1), ((0, 0), None, 0), ((0, 1), (1, 1), -1), ((1, 0), (0, 0), -1),
             ((1, 1), None, 0), ((0, 0), (0, 1), 1), ((1, 0), (1, 1), 1))


def _outer_term(load, spec, o):
    p, q, sign = spec[o]
    out = []
    for y in range(2):
        row = []
        for z in range(2):
            v = load(2 * p[0] + y, 2 * p[1] + z)
            if sign:
                w = load(2 * q[0] + y, 2 * q[1] + z)
                v = v + w if sign > 0 else v - w
            row.append(v)
        out.append(row)
    return out


def _inner_terms(y, terms, o, emit):
    for i, fi in enumerate(terms(y)):
        emit(o * 7 + i, fi()[0][0])


def _lhs_ext(e):
    n = len(e) // 2
    return {0: e[:n], 1: e[n:], 2: e[:n], 5: [y - x for x, y in zip(e[:n], e[n:])]}


def _rhs_ext(e):
    n = len(e) // 2
    return {0: e[:n], 1: e[:n], 2: e[n:], 5: [x + y for x, y in zip(e[:n], e[n:])]}


def _ext_combos(e, fn, emit):
    for oi, o in enumerate(AUG):
        d = fn(fn(e)[o])
        for ii, i in enumerate(AUG):
            emit(oi * 4 + ii, d[i][0])


def _spread(weights, span, n):
    total, acc, out = sum(weights), 0.0, []
    for k, w in enumerate(weights):
        lo, acc = acc, acc + w * n / total
        count = round(acc) - round(lo)
        out += [k * span + i * span // count for i in range(count)]
    return out


def _adv(gen, n):
    for _ in range(n):
        try:
            next(gen)
        except StopIteration:
            return


def _ld(ref, idx):
    n = ref.shape[-2] // 2
    return jnp.concatenate([ref[idx, :n, :], ref[idx, n:, :]], axis=0)


class _Temps:
    def __init__(self, ref):
        self.ref = ref
        self.n = 0

    def put(self, v):
        i = self.n % self.ref.shape[0]
        self.n += 1
        self.ref[i] = v
        return i

    def get(self, i):
        return _ld(self.ref, i)


def _combine(prod, sink, ti, spill_last=False):
    a = ti.put(prod(0))
    b = ti.put(prod(1))
    c = ti.put(prod(2))
    sink(1, 1, ti.get(a) - ti.get(b) + ti.get(c) + prod(5))
    if spill_last:
        m3 = prod(3)
        m4 = prod(4)
        sink(1, 0, ti.get(b) + m3)
        sink(0, 1, ti.get(c) + m4)
        d = ti.put(ti.get(a) + m3 - m4)
        sink(0, 0, ti.get(d) + prod(6))
        return
    m3 = prod(3)
    m4 = prod(4)
    m6 = prod(6)
    sink(1, 0, ti.get(b) + m3)
    sink(0, 1, ti.get(c) + m4)
    sink(0, 0, ti.get(a) + m3 - m4 + m6)


def _recombine(prod, fin, ti, to, spill_last=False):
    def inner(o, sink):
        _combine(lambda i: prod(o, i), sink, ti, spill_last)

    m = {}
    for o in (0, 1, 2):
        def keep(y, z, v, o=o):
            m[o, y, z] = to.put(v)
        inner(o, keep)
        yield

    def s5(y, z, v):
        fin(2 + y, 2 + z, to.get(m[0, y, z]) - to.get(m[1, y, z]) + to.get(m[2, y, z]) + v)
    inner(5, s5)
    yield

    def s3(y, z, v):
        fin(2 + y, z, to.get(m[1, y, z]) + v)
        m[3, y, z] = to.put(to.get(m[0, y, z]) + v)
    inner(3, s3)
    yield

    def s4(y, z, v):
        fin(y, 2 + z, to.get(m[2, y, z]) + v)
        m[3, y, z] = to.put(to.get(m[3, y, z]) - v)
    inner(4, s4)
    yield

    def s6(y, z, v):
        fin(y, z, to.get(m[3, y, z]) + v)
    inner(6, s6)
    yield


def _kernel(xt_hbm, wqkv_hbm, wo_hbm, wg_hbm, wu_hbm, wdt_hbm, out_hbm,
            xin, xa, xb, ost, raw, wcb, web, wdcb, wcb2, web2, wdcb2, xn2,
            wq_raw, wo_raw, wtmp, wqb, wob, xnb, qkv, ob, acb, aeb, gs, hs, hcb, acc,
            tin, tout, tin2, tout2, ktail, xsb, wsb, tq, zero,
            sem_x, sem_w, sem_c, sem_o):
    wq, wo, wc, we, wdc, xn, o32, ac, ae, hc, raw32, xin32, wc2, we2, wdc2, xs, ws = [
        r.bitcast(u32) for r in (wqb, wob, wcb, web, wdcb, xnb, ob, acb, aeb, hcb, raw, xin,
                                 wcb2, web2, wdcb2, xsb, wsb)]

    def x_copy(q):
        return pltpu.make_async_copy(
            xt_hbm.at[:, pl.ds(pl.multiple_of(q * 16, 16), 16), :], xin.at[q, 0:NTR], sem_x.at[q])

    def weight_copy(j, m):
        rows = pl.ds(pl.multiple_of(j * 32, 32), 32)
        return pltpu.make_async_copy((wg_hbm, wu_hbm, wdt_hbm)[m].at[:, rows, :],
                                     raw.at[j, pl.ds(m * NTR, NTR)], sem_c.at[j, m])

    def chunk_copies(j):
        return [weight_copy(j, m) for m in range(3)]

    def out_copy(q, h):
        rows = pl.ds(h * 2 * MB, 2 * MB)
        return pltpu.make_async_copy(
            ost.at[q, rows, :], out_hbm.at[rows, pl.ds(pl.multiple_of(q * 256, 256), 256)],
            sem_o.at[q, h])

    k_order = (4, 0, 1, 2, 3)
    wq_copies = [pltpu.make_async_copy(wqkv_hbm.at[k * 128:min(k * 128 + 128, D)],
                                       wq_raw.at[k * 128:min(k * 128 + 128, D)], sem_w.at[k])
                 for k in k_order]
    wo_copy = pltpu.make_async_copy(wo_hbm, wo_raw, sem_w.at[5])
    first = wq_copies[:OPT["xpos"]] + [x_copy(0)] + wq_copies[OPT["xpos"]:]
    for cp in first:
        cp.start()
    zero[0] = 0
    never = zero[0] != 0

    def held(v, z):
        if z is None:
            return v
        return jnp.where(never, pltpu.bitcast(z, v.dtype), v)

    def raw_pair(j, tr, cp, z):
        v = [_up(held(raw32[j, tr + k, cp * 8:cp * 8 + 8, :], z)).astype(f32) for k in range(2)]
        return [jnp.concatenate([v[0][h:h + 8], v[1][h:h + 8]], axis=0) for h in (0, 8)]

    def prep_strip(j, tr, step, spec, terms, path, emit):
        live = {}
        for o in path:
            used = [q for q in spec[o][:2] if q is not None]
            live = {q: live[q] for q in used if q in live}
            for q in used:
                if q not in live:
                    z = yield
                    live[q] = [raw_pair(j, tr + (2 * q[0] + y) * step, q[1], z) for y in range(2)]
            y = _outer_term(lambda r, c: live[r // 2, c // 2][r % 2][c % 2], spec, o)
            _inner_terms(y, terms, o, emit)

    def prep_gu(j, dst, m, s):
        base = m * (49 * 128) + s * 16

        def emit(i, v):
            dst[pl.ds(base + i * 128, 16), :] = v.astype(bf16)
        return prep_strip(j, m * NTR + 2 * s, 16, _RHS_SPEC, _rhs_terms,
                          (1, 0, 4, 2, 5, 3, 6), emit)

    def prep_ext(j, dst, m, s):
        z = yield
        tr = m * NTR + 64 + 2 * s

        def emit(i, v):
            dst[m * 16 + i, pl.ds(s * 16, 16), :] = v.astype(bf16)
        _ext_combos(raw_pair(j, tr, 0, z) + raw_pair(j, tr, 1, z), _rhs_ext, emit)

    def prep_down(j, dst, s):
        def emit(i, v):
            dst[pl.ds(s * 16 + i * MB, 16), :] = v.astype(bf16)
        return prep_strip(j, 2 * NTR + 2 * s, MB // 8, _LHS_SPEC, _lhs_terms,
                          (2, 0, 3, 6, 4, 5, 1), emit)

    def prep_chunk(j, dst):
        for m in range(2):
            for s in range(8):
                yield from prep_gu(j, dst[0], m, s)
            for s in range(4):
                yield from prep_ext(j, dst[1], m, s)
        for s in range(9):
            yield from prep_down(j, dst[2], s)

    def feed(gen, z, n):
        for _ in range(n):
            try:
                gen.send(z)
            except StopIteration:
                return

    class Pace:
        def __init__(self):
            self.tok = 0
            self.plan = []
            self.due = []

        def add(self, gen, t0, period, lat=None, gated=True):
            next(gen)
            when = [self.tok + int(t0 + k * period) for k in range(1000)]
            self.plan.append((gen, when, lat, gated))

        def step(self, z):
            for gen, when, lat, gated in self.plan:
                for _ in range(when.count(self.tok)):
                    try:
                        v = gen.send(z if gated else None)
                    except StopIteration:
                        break
                    if v is not None and lat is not None:
                        self.due.append((self.tok + lat, v))
            self.tok += 1

        def tokens(self, r, n):
            for k in range(n):
                self.step(r[k * 16:k * 16 + 8])

        def gate(self, v):
            now = [x for t, x in self.due if t <= self.tok]
            self.due = [(t, x) for t, x in self.due if t > self.tok]
            if not now:
                return v
            head = jnp.where(never, pltpu.bitcast(tree(now), u32), v[0:8])
            return jnp.concatenate([head, v[8:]], axis=0)

        def drain(self):
            for gen, *_ in self.plan:
                feed(gen, None, 1000)

    def tree(vals):
        while len(vals) > 1:
            vals = [a + b for a, b in zip(vals[::2], vals[1::2])] + vals[len(vals) & ~1:]
        return vals[0]

    def norm_slab(row, emit, order=(4, 0, 1, 2, 3)):
        def rows(k, lo, hi):
            return [row(k, r) for r in range(lo // 8, hi // 8)]

        def mean(vals):
            t = tree([sum(vals[k + 4::4], vals[k]) for k in range(4)])
            t = jnp.sum(t, axis=0, keepdims=True) * (1.0 / D)
            return jnp.broadcast_to(t, (8, 128))
        z = yield
        x = rows(0, 0, D)
        mu = mean([held(v, z) for v in x[:4]] + x[4:])
        m = held(mu, (yield))
        rs = lax.rsqrt(mean([(v - m) * (v - m) for v in rows(1, 0, D)]) + EPS)
        end = None
        for k in order:
            m = held(mu, (yield end))
            y = jnp.concatenate(
                [(v - m) * rs for v in rows(2, k * 128, min((k + 1) * 128, D))], axis=0).T
            emit(k, y)
            end = y[120:128] if k < 4 else jnp.concatenate([y[120:128]] * 2, axis=1)
        yield end

    def alias(p, n):
        return [jnp.clip(p + k * zero[0], 0, n - 1) for k in range(3)]

    def slab_rows(src, p):
        q = alias(p, NSLAB)
        return lambda k, r: src[q[k], r * 8:r * 8 + 8, :]

    def flush(gen):
        return tree([v for v in gen if v is not None])

    def ln1(p, b, fast=False):
        seen = {}

        def emit(k, y):
            xnb[b, k, :, 0:y.shape[1]] = y.astype(bf16)
            seen[k] = y
            if fast and k == 4:
                xsb[b, 10, :, 0:64] = (y[64:] - y[:64]).astype(bf16)
            if fast and k in (2, 3):
                u = seen[k - 2]
                terms = _lhs_terms([[u[:64], y[:64]], [u[64:], y[64:]]])
                for n, i in enumerate(SUMS):
                    xsb[b, 2 * n + k - 2] = terms[i]()[0][0].astype(bf16)
        return norm_slab(slab_rows(xa, p), emit, (4, 0, 2, 1, 3) if fast else (4, 0, 1, 2, 3))

    def widen(q):
        for r in range(NTR):
            if r % 4 == 0:
                z = yield
            v = _up(held(xin32[q, r], z)).astype(f32)
            for b in range(2):
                xa[2 * q + b, r * 8:r * 8 + 8, :] = v[b * 8:b * 8 + 8]

    def qkv_proj(b, pace, groups):
        scale = DH ** -0.5 * LOG2E
        for grp in groups:
            for n in grp:
                if n == 13:
                    ktail[...] = lax.dot_general(
                        _up(wq[4, n * 64:n * 64 + 32, :]), _up(xn[b, 4]), NT,
                        preferred_element_type=f32)
                else:
                    qkv[b, n, HALO:HALO + 128, :] = lax.dot_general(
                        _up(xn[b, 4]), _up(wq[4, n * 64:(n + 1) * 64, :]), NT,
                        preferred_element_type=f32)
            for n in grp:
                rows = slice(n * 64, n * 64 + (32 if n == 13 else 64))
                x = jnp.concatenate(
                    [_up(pace.gate(xn[b, 0]))] + [_up(xn[b, k]) for k in range(1, 4)], axis=1)
                w = jnp.concatenate([_up(wq[k, rows, :]) for k in range(4)], axis=1)
                if n == 13:
                    r = lax.dot_general(w, x, NT, preferred_element_type=f32)
                    r = r + jnp.concatenate([ktail[0:32, :], ktail[32:64, :]], axis=0)
                    qkv[b, n, HALO:HALO + 128, 0:64] = (r * scale).T
                    pace.tokens(r, 4)
                    continue
                r = lax.dot_general(x, w, NT, preferred_element_type=f32)
                r = r + jnp.concatenate([qkv[b, n, HALO:HALO + 64, :],
                                         qkv[b, n, HALO + 64:HALO + 128, :]], axis=0)
                if n in (4, 5, 6, 7):
                    r = r * scale
                qkv[b, n, HALO:HALO + 128, :] = r
                pace.tokens(r, 7)

    def qkv_pair(b, pace, n, ti):
        def prod(i):
            if i in SUMS:
                x = [xs[b, 2 * SUMS.index(i) + k] for k in range(2)]
            else:
                h = i - 2
                x = [xn[b, 2 * h + k, h * 32:h * 32 + 32, :] for k in range(2)]
            x = jnp.concatenate([_up(pace.gate(x[0])), _up(x[1])], axis=1)
            r = jnp.dot(x, _up(ws[n, i * 128:(i + 1) * 128, :]), preferred_element_type=f32)
            pace.tokens(r, 2)
            if i in AUG:
                e = xs[b, 10, :, 0:64] if i == 5 else xn[b, 4, (i % 2) * 32:(i % 2) * 32 + 32, 0:64]
                f = 896 + 32 * {0: 0, 1: 0, 2: 1, 5: 2}[i]
                r = r + jnp.dot(_up(e), _up(ws[n, f:f + 32, :]), preferred_element_type=f32)
            return r

        def sink(y, z, v):
            if n in (2, 3):
                v = v * (DH ** -0.5 * LOG2E)
            qkv[b, 2 * n + z, HALO + y * 64:HALO + y * 64 + 64, :] = v
        _combine(prod, sink, ti)

    def halo(b):
        for n in range(4, 14):
            qkv[b, n, 0:HALO, :] = qkv[1 - b, n, 128:128 + HALO, :]

    def attend(b, row0, lag=0):
        qs, ks, vs = (0, 1, 2, 3, 12), (4, 5, 6, 7, 13), (8, 9, 10, 11, 12)

        def scores(s, z):
            r = HALO + s * 8
            q = [held(qkv[b, n, r:r + 8, :], z) for n in qs]
            logit = []
            for w in range(WIN):
                rw = r - DIL * w
                part = tree([q[c] * qkv[b, ks[c], rw:rw + 8, :] for c in range(5)])
                part = part + pltpu.roll(part, 64, 1)
                part = part + pltpu.roll(part, 32, 1)
                if row0 is not None and s * 8 < DIL * w:
                    pos = row0 + s * 8 + lax.broadcasted_iota(jnp.int32, (8, 128), 0)
                    part = jnp.where(pos >= DIL * w, part, -1e9 * LOG2E)
                logit.append(part)
            return logit

        def values(s, logit, z):
            r = HALO + s * 8
            mx = logit
            while len(mx) > 1:
                mx = [jnp.maximum(a, c) for a, c in zip(mx[::2], mx[1::2])]
            top = held(mx[0], z)
            e = [jnp.exp2(l - top) for l in logit]
            inv = 1.0 / tree(e)
            outs = []
            for c in range(5):
                o = e[0] * qkv[b, vs[c], r:r + 8, :]
                for w in range(1, WIN):
                    rw = r - DIL * w
                    o = o + e[w] * qkv[b, vs[c], rw:rw + 8, :]
                o = o * inv
                outs.append(o)
                ob[b, c, s * 8:(s + 1) * 8, :] = o.astype(bf16)
            return tree(outs)

        v, pending = None, []
        for s in range(16 + lag):
            z = yield v
            if s < 16:
                pending.append(scores(s, z))
            if s >= lag:
                v = values(s - lag, pending.pop(0), z if lag else None)
        yield v

    def out_proj(p, b, pace):
        h = MB // 2
        for m in range(4):
            xb[p, m * MB:(m + 1) * MB, :] = xa[p, m * MB:(m + 1) * MB, :] + lax.dot_general(
                _up(wo[4, m * h:(m + 1) * h, :]), _up(o32[b, 4]), NT, preferred_element_type=f32)
        rhs = jnp.concatenate([_up(o32[b, c]) for c in range(4)], axis=1)
        for m in range(4):
            rows = slice(m * h, (m + 1) * h)
            lhs = jnp.concatenate(
                [_up(pace.gate(wo[0, rows, :]))] + [_up(wo[c, rows, :]) for c in range(1, 4)],
                axis=1)
            r = lax.dot_general(lhs, rhs, NT, preferred_element_type=f32)
            r = r + jnp.concatenate([xb[p, m * MB:m * MB + h, :],
                                     xb[p, m * MB + h:(m + 1) * MB, :]], axis=0)
            xb[p, m * MB:(m + 1) * MB, :] = r
            pace.tokens(r, 8)

    def ffn_norm_slab(p, r):
        def emit(k, y):
            xn2[r * 6 + k, :, 0:y.shape[1]] = y
        return norm_slab(slab_rows(xb, p), emit)

    def ffn_norm(t):
        for r in range(4):
            yield from ffn_norm_slab(t * 4 + r, r)

    def strips(load, spec, terms, o, dst):
        for s in range(8):
            z = yield
            rows = slice(s * 16, (s + 1) * 16)

            def ld(r, c):
                v = load(r, c, rows)
                if (r // 2, c // 2) == spec[o][0]:
                    v = jnp.concatenate([held(v[0:8], z), held(v[8:16], z)], axis=0)
                return v

            def emit(i, v):
                dst[i, rows, :] = v.astype(bf16)
            _inner_terms(_outer_term(ld, spec, o), terms, o, emit)

    def lhs_strips(o):
        yield from strips(lambda r, k, rows: xn2[r * 6 + k, rows, :],
                          _LHS_SPEC, _lhs_terms, o, acb)
        if o in AUG:
            for s in range(2):
                z = yield
                rows = slice(s * 64, (s + 1) * 64)
                d = _lhs_ext(_lhs_ext([xn2[r * 6 + 4, rows, 0:64] for r in range(4)])[o])
                for ii, i in enumerate(AUG):
                    aeb[AUG.index(o) * 4 + ii, rows, 0:64] = d[i][0].astype(bf16)

    def ffn_combos():
        for s in range(8):
            rows = slice(s * 16, (s + 1) * 16)
            a = [[xn2[r * 6 + k, rows, :] for k in range(4)] for r in range(4)]

            def emit(i, v, rows=rows):
                acb[i, rows, :] = v.astype(bf16)
            _combos(a, _lhs_terms, emit)
            e = [xn2[r * 6 + 4, rows, 0:64] for r in range(4)]

            def emit_e(i, v, rows=rows):
                aeb[i, rows, 0:64] = v.astype(bf16)
            _ext_combos(e, _lhs_ext, emit_e)

    def attn_run(h, count, o, mask, side=None, late=None, extra=None, more=None,
                 head=False):
        fast = "seq" in o
        if not head:
            flush(ln1(h % NSLAB, 0, fast))
        for k in range(count):
            b = k % 2
            pace = Pace()
            if side is not None:
                when = [w - k * 128 for w in _spread(o["wts"], 16, NPREP)]
                pace.plan.append((side, [min(w, 126) for w in when if 0 <= w < 128], None, True))
            if k + 1 < count:
                pace.add(ln1((h + k + 1) % NSLAB, 1 - b, fast), *o["ls"][k])
            elif late is not None:
                pace.add(late, o["w0"], o["wper"])
            if k == 1 and extra is not None:
                pace.add(extra, 32 + o["x0"], o["xper"])
            if k == o.get("sk") and more is not None:
                pace.add(more, o["s0"], o["sper"])
            if k > 0 or not head:
                row0 = (h % NSLAB) * 128 if k == 1 and mask else None
                pace.add(attend(1 - b, row0, o["lag"]), *o["a"][k], o["ag"])
                if not head:
                    out_proj((h + k - 2) % NSLAB, b, pace)
                halo(b)
            if fast:
                ti = _Temps(tq)
                for n in o["seq"]:
                    if n < 6:
                        qkv_pair(b, pace, n, ti)
                    else:
                        qkv_proj(b, pace, ((12, 13),))
            else:
                qkv_proj(b, pace, o["grp"])
            pace.plan = [e for e in pace.plan if e[0] is not side]
            pace.drain()
        if side is not None:
            feed(side, None, 1000)

    def wq_prep(k):
        w = 128 if k < 4 else 64
        for c0 in range(0, 3 * D, 128):
            c1 = min(c0 + 128, 3 * D)
            wtmp[k, c0:c1, 0:w] = wq_raw[k * 128:k * 128 + w, c0:c1].astype(f32).T
        for part in OPT["parts"]:
            for d in range(DH):
                if d < 16:
                    row = part * 512 + d * 32
                else:
                    row = (1536, 1664, 1600)[part] + (d - 16) * 32
                wqb[k, row:row + 32, 0:w] = wtmp[
                    k, pl.ds(part * D + d, H, stride=DH), 0:w].astype(bf16)

    def ws_flip(n):
        for k in range(5):
            for c in range(2):
                z = yield
                row = pl.multiple_of(n * 128 + c * 64, 64)
                v = jnp.concatenate([held(wq[k, pl.ds(row, 8), :], z),
                                     wq[k, pl.ds(row + 8, 56), :]], axis=0)
                w = 128 if k < 4 else 64
                wtmp[k, pl.ds(pl.multiple_of(2 * row, 128), w), :] = _up(v).astype(f32).T[0:w]

    def ws_prep(g):
        def pair(n, k, r, z):
            v = [wtmp[k, pl.ds(pl.multiple_of(n * 256 + c * 128 + r, 16), 16), :]
                 for c in range(2)]
            return [jnp.concatenate([held(u[0:8], z), u[8:]], axis=0) for u in v]
        for n in [3 * g + j for j in range(3)]:
            for r in range(0, 64, 16):
                if r % 32 == 0:
                    z = yield
                f = pair(n, 4, r, z)
                for i, v in enumerate(f + [f[0] + f[1]]):
                    wsb[n, 1792 + i * 64 + r:1792 + i * 64 + r + 16, :] = v.astype(bf16)
            for k in range(2):
                for r in range(0, 128, 16):
                    if r % 32 == 0:
                        z = yield
                    for i, t in enumerate(_rhs_terms([pair(n, k, r, z), pair(n, k + 2, r, z)])):
                        row = i * 256 + k * 128 + r
                        wsb[n, row:row + 16, :] = t()[0][0].astype(bf16)

    def wo_prep():
        for n in range(5):
            w = 128 if n < 4 else 64
            wtmp[n, 0:D, 0:w] = wo_raw[:, n * 128:n * 128 + w].astype(f32)
        for n in range(5):
            w = 128 if n < 4 else 64
            for c in range(5):
                z = yield
                rows = [held(wtmp[n, pl.ds(4 * c + g + k * 8 * DH, 8, stride=DH), :], z)[:, 0:w]
                        for g in range(4 if c < 4 else 2) for k in range(4)]
                if c == 4:
                    rows = [jnp.zeros((64, w), f32)] + rows
                wob[c, n * 128:n * 128 + w, :] = jnp.concatenate(rows, axis=0).T.astype(bf16)

    def head_late():
        for cp in (wo_copy, x_copy(1)):
            cp.wait()
        for cp in [x_copy(2)] + chunk_copies(1):
            cp.start()
        yield from wo_prep()
        yield from widen(1)

    wqb[4, :, 64:128] = jnp.zeros((3 * D, 64), bf16)
    qkv[:, 13] = jnp.zeros((2, HALO + 128, 128), f32)
    xnb[:, 4, :, 64:128] = jnp.zeros((2, 128, 64), bf16)
    for n in range(4, 13):
        qkv[0, n, 0:HALO, :] = jnp.zeros((HALO, 128), f32)
    todo = list(k_order)
    for n, cp in enumerate(first):
        cp.wait()
        if n == OPT["dma"][0]:
            wo_copy.start()
        if n == OPT["dma"][1]:
            for c in [x_copy(1)] + chunk_copies(0):
                c.start()
        if n == OPT["xpos"]:
            feed(widen(0), None, 1000)
            flush(ln1(0, 0))
        else:
            wq_prep(todo.pop(0))
    attn_run(0, 2, OPT["h"], True, late=head_late(), head=True)

    @pl.loop(0, 7)
    def _(i):
        for cp in chunk_copies(i):
            cp.wait()

        @pl.when(i + 2 < NSLAB // 2)
        def _():
            x_copy(i + 2).wait()

        @pl.when(i + 3 < NSLAB // 2)
        def _():
            x_copy(i + 3).start()
        for cp in chunk_copies(i + 2):
            cp.start()
        side = prep_chunk(i, [r.at[i] for r in (wcb, web, wdcb)])
        next(side)
        r = jnp.clip(i - 2, 0, 3)
        attn_run(2 * i + 2, 2, OPT["p"], False, side, widen(jnp.minimum(i + 2, NSLAB // 2 - 1)),
                 ffn_norm_slab(r, r), ws_flip(jnp.minimum(i, 5)))

    for cp in chunk_copies(7) + chunk_copies(8):
        cp.wait()
    ffn_combos()

    def ffn_group(t, g, last, emit=None):
        ti = _Temps(tin)
        to = _Temps(tout)
        pace = Pace()
        o_ = OPT["fb" if last else "fa"]

        def weights(c):
            if last and c > 0:
                return [r.at[c - 1] for r in (wc2, we2, wdc2)]
            return [r.at[g * 3 + c] for r in (wc, we, wdc)]

        def proj(c, m):
            w, w_ext, _ = weights(c)

            def prod(o, i):
                r = (m * 49 + o * 7 + i) * 64
                p = jnp.dot(_up(ac[o * 7 + i]), _up(w[r:r + 64, :]),
                            preferred_element_type=f32)
                pace.step(p[0:8])
                if o in AUG and i in AUG:
                    q = AUG.index(o) * 4 + AUG.index(i)
                    e = jnp.dot(_up(ae[q, :, 0:64]), _up(w_ext[m * 16 + q]),
                                preferred_element_type=f32)
                    pace.step(e[0:8])
                    p = p + e
                return p
            return prod

        def gate(c):
            def fin(r, cc, v):
                gs[(c % 2) * 16 + r * 4 + cc] = v
            return _recombine(proj(c, 0), fin, ti, to)

        def upgate(c):
            def fin(r, cc, v):
                hs[c, r * 4 + cc] = _ld(gs, (c % 2) * 16 + r * 4 + cc) * v
            yield from _recombine(proj(c, 1), fin, ti, to, last)
            pace.add(hidden_paced(c), *o_["h"][c])

        hgen, hdone = {}, {}

        def hidden(c):
            for o in ORDER:
                yield from strips(lambda cc, r, rows: hs[c, r * 4 + cc, rows, :],
                                  _RHS_SPEC, _rhs_terms, o, hcb.at[c])

        def hidden_paced(c):
            hgen[c], hdone[c] = hidden(c), 0
            next(hgen[c])
            while True:
                z = yield
                need(c, min(hdone[c] + 1, 56), z)

        def need(c, n, z=None):
            feed(hgen[c], z, n - hdone[c])
            hdone[c] = max(hdone[c], n)

        def dprod(cs, i):
            p = None
            for c in cs:
                need(c, 8 * (ORDER.index(i // 7) + 1))
                r = i * (MB // 2)
                q = lax.dot_general(_up(weights(c)[2][r:r + MB // 2, :]), _up(hc[c, i]), NT,
                                    preferred_element_type=f32)
                pace.step(q[0:8])
                p = q if p is None else p + q
            return p

        def down(cs, reset):
            for i in [o * 7 + k for o in ORDER for k in range(7)]:
                a = _ld(acc, i)
                if reset:
                    a = jnp.where(g == 0, 0.0, a)
                acc[i] = a + dprod(cs, i)
                yield

        def down_final(cs):
            def fin(mb, r, v):
                rows = slice(mb * MB, (mb + 1) * MB)
                y = xb[t * 4 + r, rows, :] + v
                xa[t * 4 + r, rows, :] = y
                ost[t * 2 + r // 2, rows, (r % 2) * 128:(r % 2) * 128 + 128] = y.astype(bf16)
            return _recombine(lambda o, i: _ld(acc, o * 7 + i) + dprod(cs, o * 7 + i),
                              fin, _Temps(tin2), _Temps(tout2))

        if last:
            norm = ffn_norm((t + 1) % NTILE)
            pace.add(norm, o_["n0"], o_["nper"])
        else:
            late = prep_chunk(7 + g, [r.at[g] for r in (wcb2, web2, wdcb2)])
            next(late)
            pace.plan.append((late, _spread(o_["wts"], 30, NPREP), None, True))
            more = ws_prep(g)
            next(more)
            pace.plan.append((more, _spread(o_["sw"], 30, 30), None, True))
        for gen in (gate(0), upgate(0), gate(1)):
            _adv(gen, 100)
        d0 = down((0,), not last)
        queue = []

        def lhs_queue():
            while True:
                z = yield
                if queue:
                    try:
                        queue[0].send(z)
                    except StopIteration:
                        queue.pop(0)
        for gen, plan in ((upgate(1), "u1"), (gate(2), "g2"), (upgate(2), "u2")):
            if last and plan == "u2":
                feed(norm, None, 1000)
                pace.add(lhs_queue(), o_["l0"], o_["lper"])
            for k, n in enumerate(o_[plan]):
                _adv(gen, 1)
                if last and plan == "u2":
                    queue.append(lhs_strips(ORDER[k]))
                    next(queue[-1])
                _adv(d0, n)
            _adv(gen, 100)
        _adv(d0, 100)
        if last:
            gen = down_final((1, 2))
            _adv(gen, 3)
            for q, h in ((1, 1), (0, 1), (1, 0), (0, 0)):
                _adv(gen, 1)
                pl.when(emit)(out_copy(t * 2 + q, h).start)
        else:
            _adv(down((1, 2), False), 100)
            feed(late, None, 1000)
            feed(more, None, 1000)
        for gen in queue:
            feed(gen, None, 1000)

    @pl.loop(0, 2 * NTILE)
    def _(tile):
        t = tile % NTILE

        @pl.loop(0, 2)
        def _(g):
            ffn_group(t, g, False)
        ffn_group(t, 2, True, tile >= NTILE)

        @pl.when(tile < NTILE)
        def _():
            attn_run(4 * t + NSLAB, 4, OPT["n"], True)

        @pl.when(tile == NTILE - 1)
        def _():
            out_proj(NSLAB - 2, 0, Pace())
            flush(attend(1, None))
            out_proj(NSLAB - 1, 1, Pace())

    for p in range(NSLAB):
        out_copy(p // 2, p % 2).wait()


def _tiles(w):
    n = w.shape[1]
    return w.reshape(NTR, 8, n // 128, 128).transpose(0, 2, 1, 3).reshape(NTR, n // 16, 128)


@jax.jit
def pallas_interleave_layers__sliding_local_dilated__glu_gated_bilinear__prompt_kernel(
    A_x: jax.Array,
    A_wqkv: jax.Array,
    A_wo: jax.Array,
    B_x: jax.Array,
    B_w_gate: jax.Array,
    B_w_up: jax.Array,
    B_w_down: jax.Array,
):
    del B_x
    vm = pltpu.VMEM
    hbm = pl.BlockSpec(memory_space=pl.ANY)
    out_t = pl.pallas_call(
        _kernel,
        in_specs=[hbm] * 6,
        out_specs=hbm,
        out_shape=jax.ShapeDtypeStruct((D, S), bf16),
        scratch_shapes=[
            vm((NSLAB // 2, 96, 16, 128), bf16),
            vm((NSLAB, 768, 128), f32),
            vm((NSLAB, 768, 128), f32),
            vm((NSLAB // 2, 768, 256), bf16),
            vm((NCHUNK, 224, 32, 128), bf16),
            vm((7, WC_ROWS, 128), bf16),
            vm((7, 32, 64, 128), bf16),
            vm((7, WD_ROWS, 128), bf16),
            vm((2, WC_ROWS, 128), bf16),
            vm((2, 32, 64, 128), bf16),
            vm((2, WD_ROWS, 128), bf16),
            vm((24, 128, 128), f32),
            vm((D, 3 * D), bf16),
            vm((D, D), bf16),
            vm((5, 3 * D, 128), f32),
            vm((5, 3 * D, 128), bf16),
            vm((5, D, 128), bf16),
            vm((2, 5, 128, 128), bf16),
            vm((2, 14, HALO + 128, 128), f32),
            vm((2, 5, 128, 128), bf16),
            vm((49, 128, 128), bf16),
            vm((16, 128, 128), bf16),
            vm((32, 128, 128), f32),
            vm((3, 16, 128, 128), f32),
            vm((3, 49, 128, 128), bf16),
            vm((49, MB, 128), f32),
            vm((12, 128, 128), f32),
            vm((40, 128, 128), f32),
            vm((12, MB, 128), f32),
            vm((20, MB, 128), f32),
            vm((64, 128), f32),
            vm((2, 11, 64, 128), bf16),
            vm((6, 1984, 128), bf16),
            vm((6, 64, 128), f32),
            pltpu.SMEM((1,), jnp.int32),
            pltpu.SemaphoreType.DMA((NSLAB // 2,)),
            pltpu.SemaphoreType.DMA((6,)),
            pltpu.SemaphoreType.DMA((NCHUNK, 3)),
            pltpu.SemaphoreType.DMA((NSLAB // 2, 2)),
        ],
        compiler_params=pltpu.CompilerParams(vmem_limit_bytes=122 * 1024 * 1024,
                                             disable_bounds_checks=True,
                                             disable_semaphore_checks=True),
    )(_tiles(A_x[0].T), A_wqkv, A_wo, _tiles(B_w_gate), _tiles(B_w_up), _tiles(B_w_down.T))
    return out_t.T[None]
```
